```python
import jax
import jax.numpy as jnp

def _softmax(x, axis=-1):
    return jax.nn.softmax(x, axis=axis)

def _gelu(x):
    return jax.nn.gelu(x, approximate=True)

def _silu(x):
    return jax.nn.silu(x)

def _sigmoid(x):
    return jax.nn.sigmoid(x)

def _layernorm(x, axis=-1, eps=1e-05):
    m = jnp.mean(x, axis=axis, keepdims=True)
    v = jnp.var(x, axis=axis, keepdims=True)
    return (x - m) / jnp.sqrt(v + eps)

def _scatter_add(tgt, idx, src, axis=0):
    return tgt.at[idx].add(src)

def _segment_sum(src, seg, n):
    return jax.ops.segment_sum(src, seg, n)

class _Rng:

    def __init__(self, key):
        self._k = key

    def _next(self):
        self._k, sub = jax.random.split(self._k)
        return sub

    def normal(self, shape):
        return jax.random.normal(self._next(), shape, dtype=jnp.bfloat16)

    def randint(self, lo, hi, shape):
        return jax.random.randint(self._next(), shape, lo, hi, dtype=jnp.int32)

    def uniform(self, shape, lo=0.0, hi=1.0):
        return jax.random.uniform(self._next(), shape, jnp.bfloat16, lo, hi)

    def permutation(self, n):
        return jax.random.permutation(self._next(), n)
kernel_name = 'interleave_layers__memory_aug_infini_attn__sliding_local_dilated__prompt'

def setup_inputs():
    _rng = _Rng(jax.random.key(int.from_bytes(__import__("os").urandom(4), "little")))
    _w = lambda a: (lambda t: t.astype(jnp.bfloat16) if jnp.issubdtype(t.dtype, jnp.floating) else t)(jnp.asarray(a))

    def _A_setup():
        B, S, D, H = (1, 2048, 1024, 32)
        N = 4
        L = max(1, S // N)
        sc = D ** (-0.5)
        return {'x': _w((lambda *s: _rng.normal(s) * 0.05)(B, N * L, D)), 'wq': _w((lambda *s: _rng.normal(s) * 0.05)(D, D) * sc), 'wk': _w((lambda *s: _rng.normal(s) * 0.05)(D, D) * sc), 'wv': _w((lambda *s: _rng.normal(s) * 0.05)(D, D) * sc), 'wo': _w((lambda *s: _rng.normal(s) * 0.05)(D, D) * sc), 'beta': _w((lambda *s: _rng.normal(s) * 0.05)(H))}
    _A_in = _A_setup()

    def _B_setup():
        B, S, D = (1, 2048, 1024)
        return {'x': _w((lambda *s: _rng.normal(s) * 0.05)(B, S, D)), 'wqkv': _w((lambda *s: _rng.normal(s) * 0.05)(D, 3 * D)), 'wo': _w((lambda *s: _rng.normal(s) * 0.05)(D, D))}
    _B_in = _B_setup()
    return {'A_x': _A_in['x'], 'A_wq': _A_in['wq'], 'A_wk': _A_in['wk'], 'A_wv': _A_in['wv'], 'A_wo': _A_in['wo'], 'A_beta': _A_in['beta'], 'B_x': _B_in['x'], 'B_wqkv': _B_in['wqkv'], 'B_wo': _B_in['wo']}

def reference(A_x, A_wq, A_wk, A_wv, A_wo, A_beta, B_x, B_wqkv, B_wo):

    def _A_ref(x, wq, wk, wv, wo, beta):
        B, S, D = x.shape
        H = 32
        Dh = D // H
        N = 4
        L = S // N
        q = (lambda x, *d: x.transpose(*d))((x @ wq).reshape(B, S, H, Dh), 0, 2, 1, 3).reshape(B, H, N, L, Dh)
        k = (lambda x, *d: x.transpose(*d))((x @ wk).reshape(B, S, H, Dh), 0, 2, 1, 3).reshape(B, H, N, L, Dh)
        v = (lambda x, *d: x.transpose(*d))((x @ wv).reshape(B, S, H, Dh), 0, 2, 1, 3).reshape(B, H, N, L, Dh)
        phi = lambda t: jnp.where(t > 0, t + 1.0, jnp.exp(t))
        scale = Dh ** (-0.5)
        ar = jnp.arange(L)
        mask = (lambda x, dt: x.astype(dt))(ar[:, None] < ar[None, :], x.dtype) * -1000000000.0
        g = _sigmoid(beta).reshape(1, H, 1, 1)
        M = jnp.einsum('bhd,bhe->bhde', q[:, :, 0, 0, :] * 0.0, q[:, :, 0, 0, :] * 0.0)
        z = q[:, :, 0, 0, :] * 0.0
        outs = []
        for s in range(N):
            qs, ks, vs = (q[:, :, s].copy(), k[:, :, s].copy(), v[:, :, s].copy())
            logits = jnp.einsum('bhqd,bhkd->bhqk', qs, ks) * scale + mask
            p = _softmax(logits, axis=-1)
            a_dot = jnp.einsum('bhqk,bhkd->bhqd', p, vs)
            pq = phi(qs)
            num = jnp.einsum('bhld,bhde->bhle', pq, M)
            den = jnp.einsum('bhld,bhd->bhl', pq, z)[..., None] + 1e-06
            a_mem = num / den
            o = g * a_mem + (1.0 - g) * a_dot
            outs.append(o)
            pk = phi(ks)
            M = M + jnp.einsum('bhld,bhle->bhde', pk, vs)
            z = z + jnp.einsum('bhld->bhd', pk)
        o = (lambda x, *d: x.transpose(*d))(jnp.stack(outs, 2).reshape(B, H, S, Dh), 0, 2, 1, 3).reshape(B, S, D)
        return o @ wo

    def _B_ref(x, wqkv, wo):
        B, S, D = x.shape
        H = 32
        Dh = D // H
        W, dil = (8, 2)
        qkv = (lambda x, *d: x.transpose(*d))((x @ wqkv).reshape(B, S, 3, H, Dh), 2, 0, 3, 1, 4)
        q, k, v = (qkv[0], qkv[1], qkv[2])
        scale = Dh ** (-0.5)
        pos = jnp.arange(S)
        off = jnp.arange(W) * dil
        idx = pos[:, None] - off[None, :]
        mask = idx >= 0
        idx_c = jnp.where(mask, idx, 0).reshape(-1)
        kg = k[:, :, idx_c, :].reshape(B, H, S, W, Dh)
        vg = v[:, :, idx_c, :].reshape(B, H, S, W, Dh)
        logits = jnp.einsum('bhsd,bhswd->bhsw', q, kg) * scale
        logits = jnp.where(mask[None, None, :, :], logits, -1000000000.0)
        attn = _softmax(logits, axis=-1)
        o = jnp.einsum('bhsw,bhswd->bhsd', attn, vg)
        return (lambda x, *d: x.transpose(*d))(o, 0, 2, 1, 3).reshape(B, S, D) @ wo
    x = A_x
    x = x + _A_ref(_layernorm(x, axis=-1), A_wq, A_wk, A_wv, A_wo, A_beta)
    x = x + _B_ref(_layernorm(x, axis=-1), B_wqkv, B_wo)
    x = x + _A_ref(_layernorm(x, axis=-1), A_wq, A_wk, A_wv, A_wo, A_beta)
    x = x + _B_ref(_layernorm(x, axis=-1), B_wqkv, B_wo)
    return x
```

```python
import math

import jax
import jax.numpy as jnp
from jax import lax
import jax.experimental.pallas as pl
import jax.experimental.pallas.tpu as pltpu

S, D, H, DH = 2048, 1024, 32, 32
L, NSEG, G = 512, 4, 8
W, DIL = 8, 2
HALO = 16
BF, F32 = jnp.bfloat16, jnp.float32
QSCALE = (DH ** -0.5) * math.log2(math.e)
NEG = -1e30
NT = (((1,), (1,)), ((), ()))
OFF = (0, 128, 384, 768)
PITCH = 33


def _dot(a, b):
    return jnp.dot(a, b, preferred_element_type=F32)


def _dot_nt(a, b):
    return lax.dot_general(a, b, NT, preferred_element_type=F32)


def _rows(x, n):
    return slice(x, x + n) if isinstance(x, int) else pl.ds(pl.multiple_of(x, n), n)


def _phi(t):
    return jnp.where(t > 0, t + 1.0, jnp.exp(t))


def _layernorm(x_ref, xn_ref, chunk=32):
    for r0 in range(0, L, chunk):
        x = x_ref[r0:r0 + chunk, :]
        d = x - jnp.mean(x, axis=-1, keepdims=True)
        v = jnp.mean(d * d, axis=-1, keepdims=True)
        xn_ref[r0:r0 + chunk, :] = (d * lax.rsqrt(v + 1e-5)).astype(BF)


def _shuffle_rows(tf, tmp, store):
    for h in range(H):
        tmp[h * PITCH:h * PITCH + DH, :] = tf[h * DH:(h + 1) * DH]
    for d in range(DH):
        for th in range(2):
            rows = tmp[pl.ds(th * 16 * PITCH + d, 16, stride=PITCH), :]
            store(d * H + th * 16, rows.astype(BF))


def _qk_stage(g, q_ref, k_ref, s_ref, m_ref):
    lane = lax.broadcasted_iota(jnp.int32, (64, 128), 1)
    key = lax.broadcasted_iota(jnp.int32, (128, 512), 0)
    qry = lax.broadcasted_iota(jnp.int32, (128, 512), 1) & 127
    causal = key <= qry
    for j in range(4):
        nk = 128 * (j + 1)
        qt = pltpu.bitcast(q_ref[g, j * 128:(j + 1) * 128, :], jnp.uint32)
        wq = jnp.concatenate(
            [jnp.where((lane >> 5) == h, qt, jnp.uint32(0)) for h in range(4)], axis=0)
        wq = pltpu.bitcast(wq, BF)
        st = _dot_nt(k_ref[g, 0:nk, :], wq)
        diag = jnp.where(causal, st[j * 128:], NEG)
        s_ref[OFF[j] + j * 128:OFF[j] + nk, :] = diag
        m = jnp.max(diag.reshape(16, 8, 512), axis=0)
        if j > 0:
            s_ref[OFF[j]:OFF[j] + j * 128, :] = st[:j * 128]
            m = jnp.maximum(m, jnp.max(st[:j * 128].reshape(16 * j, 8, 512), axis=0))
        m_ref[j] = jnp.broadcast_to(jnp.max(m, axis=0, keepdims=True), (8, 512))


def _sm_stage(s_ref, m_ref, p_ref, l_ref, sub=16):
    for j in range(4):
        nk = 128 * (j + 1)
        for h in range(4):
            m = m_ref[j, :, h * 128:(h + 1) * 128]
            l = None
            for r in range(0, nk, sub):
                s = s_ref[OFF[j] + r:OFF[j] + r + sub, h * 128:(h + 1) * 128]
                p = jnp.exp2(s.reshape(sub // 8, 8, 128) - m[None])
                ls = jnp.sum(p, axis=0)
                l = ls if l is None else l + ls
                p_ref[h, OFF[j] + r:OFF[j] + r + sub, :] = p.reshape(sub, 128).astype(BF)
            l_ref[j, :, h * 128:(h + 1) * 128] = l


def _pv_stage(g, p_ref, l_ref, vt_ref, ot_ref, pq_ref, pk_ref, mt_ref, gate_ref):
    nd = _dot_nt(mt_ref[g].astype(BF), pq_ref[g])
    for h in range(4):
        r0 = (g * 4 + h) * DH
        gate = gate_ref[pl.ds(g * 4 + h, 1), :]
        for j in range(4):
            acc = None
            for t in range(j + 1):
                o = _dot(vt_ref[t, _rows(r0, DH), :],
                         p_ref[h, OFF[j] + t * 128:OFF[j] + (t + 1) * 128, :])
                acc = o if acc is None else acc + o
            l = jnp.sum(l_ref[j, :, h * 128:(h + 1) * 128], axis=0, keepdims=True)
            den = nd[128 + h:129 + h, j * 128:(j + 1) * 128] + 1e-6
            num = nd[h * DH:(h + 1) * DH, j * 128:(j + 1) * 128]
            res = num * (gate / den) + acc * ((1.0 - gate) / l)
            ot_ref[j, _rows(r0, DH), :] = res.astype(BF)
    row = lax.broadcasted_iota(jnp.int32, (144, 128), 0)
    lane = lax.broadcasted_iota(jnp.int32, (144, 128), 1)
    keep = jnp.where(row < 128, row >> 5, row - 128) == (lane >> 5)
    row16 = lax.broadcasted_iota(jnp.int32, (16, 128), 0)
    ones = jnp.where(row16 < 4, 1.0, 0.0).astype(BF)
    upd = None
    for t in range(4):
        lhs = jnp.concatenate([vt_ref[t, _rows(g * 128, 128), :], ones], axis=0)
        u = _dot(lhs, pk_ref[g, t * 128:(t + 1) * 128, :])
        upd = u if upd is None else upd + u
    mt_ref[g] = mt_ref[g] + jnp.where(keep, upd, 0.0)


def _band_attention(seg, q_ref, k_ref, v_ref, o_ref, chunk=8):
    for r0 in range(0, L, chunk):
        q = [q_ref[b, r0:r0 + chunk, :] for b in range(G)]
        logit = []
        for w in range(W):
            base = HALO + r0 - DIL * w
            acc = q[0] * k_ref[0, base:base + chunk, :]
            for b in range(1, G):
                acc = acc + q[b] * k_ref[b, base:base + chunk, :]
            acc = acc + pltpu.roll(acc, 64, 1)
            acc = acc + pltpu.roll(acc, 32, 1)
            if r0 - DIL * w < 0:
                pos = seg * L + r0 - DIL * w + lax.broadcasted_iota(jnp.int32, (chunk, 128), 0)
                acc = jnp.where(pos >= 0, acc, NEG)
            logit.append(acc)
        m = logit[0]
        for w in range(1, W):
            m = jnp.maximum(m, logit[w])
        e = [jnp.exp2(lg - m) for lg in logit]
        l = e[0]
        for w in range(1, W):
            l = l + e[w]
        inv = 1.0 / l
        for b in range(G):
            acc = e[0] * v_ref[b, HALO + r0:HALO + r0 + chunk, :]
            for w in range(1, W):
                base = HALO + r0 - DIL * w
                acc = acc + e[w] * v_ref[b, base:base + chunk, :]
            o_ref[r0:r0 + chunk, b * 128:(b + 1) * 128] = (acc * inv).astype(o_ref.dtype)


def _kernel(x_in, wq_hbm, wk_hbm, wv_hbm, woa_hbm, beta_ref, wqkv_hbm, wob_hbm, out_ref,
            x_f, xn, wq, wk, woa, wstage, wstage3, wvt, wbt, wob, tmp_a, tmp_b,
            q_ref, pq_ref, k_ref, pk_ref, vt_ref, ot_ref, o_nat,
            s_a, s_b, m_a, m_b, p_a, p_b, l_a, l_b, mt_ref, gate_ref,
            qb, kb, vb, halo, ob, sems):
    t = pl.program_id(0)
    seg = t // 2
    layer = t % 2

    copies = [
        pltpu.make_async_copy(wq_hbm, wq, sems.at[0]),
        pltpu.make_async_copy(wk_hbm, wk, sems.at[1]),
        pltpu.make_async_copy(wv_hbm, wstage, sems.at[2]),
        pltpu.make_async_copy(woa_hbm, woa, sems.at[3]),
        pltpu.make_async_copy(wqkv_hbm, wstage3, sems.at[4]),
        pltpu.make_async_copy(wob_hbm, wob, sems.at[5]),
    ]

    @pl.when(t == 0)
    def _():
        for c in copies:
            c.start()
        b = beta_ref[...].astype(F32).reshape(1, H)
        gt = jax.nn.sigmoid(b)
        row = lax.broadcasted_iota(jnp.int32, (H, H), 0)
        lane = lax.broadcasted_iota(jnp.int32, (H, H), 1)
        col = jnp.sum(jnp.where(row == lane, jnp.broadcast_to(gt, (H, H)), 0.0), axis=1, keepdims=True)
        gate_ref[...] = jnp.broadcast_to(col, (H, 128))

    @pl.when(layer == 0)
    def _():
        x_f[...] = x_in[...].astype(F32)

    @pl.when(seg == 0)
    def _():
        mt_ref[layer] = jnp.zeros((G, 144, 128), F32)
        halo[layer] = jnp.zeros((2, G, HALO, 128), F32)

    _layernorm(x_f, xn)

    @pl.when(t == 0)
    def _():
        copies[0].wait()
        copies[1].wait()
        copies[2].wait()
        for kbk in range(8):
            wvt[:, kbk * 128:(kbk + 1) * 128] = wstage[kbk * 128:(kbk + 1) * 128, :].T

    for c in range(4):
        y = _dot(xn[...], wq[:, c * 256:(c + 1) * 256])
        for gg in range(2):
            yq = y[:, gg * 128:(gg + 1) * 128]
            q_ref[2 * c + gg] = (yq * QSCALE).astype(BF)
            pq_ref[2 * c + gg] = _phi(yq).astype(BF)
    for c in range(4):
        y = _dot(xn[...], wk[:, c * 256:(c + 1) * 256])
        for gg in range(2):
            yk = y[:, gg * 128:(gg + 1) * 128]
            k_ref[2 * c + gg] = yk.astype(BF)
            pk_ref[2 * c + gg] = _phi(yk).astype(BF)
    for c in range(2):
        y = _dot_nt(wvt[...], xn[c * 256:(c + 1) * 256, :])
        vt_ref[2 * c] = y[:, :128].astype(BF)
        vt_ref[2 * c + 1] = y[:, 128:].astype(BF)

    mt = mt_ref.at[layer]
    pv = lambda g, p, l: _pv_stage(g, p, l, vt_ref, ot_ref, pq_ref, pk_ref, mt, gate_ref)
    _qk_stage(0, q_ref, k_ref, s_a, m_a)
    _qk_stage(1, q_ref, k_ref, s_b, m_b)
    _sm_stage(s_a, m_a, p_a, l_a)

    def pair(u, c):
        g = 2 * u + 1
        _qk_stage(g + 1, q_ref, k_ref, s_a, m_a)
        _sm_stage(s_b, m_b, p_b, l_b)
        pv(g - 1, p_a, l_a)
        _qk_stage(g + 2, q_ref, k_ref, s_b, m_b)
        _sm_stage(s_a, m_a, p_a, l_a)
        pv(g, p_b, l_b)
        return c

    lax.fori_loop(0, 3, pair, 0)
    _sm_stage(s_b, m_b, p_b, l_b)
    pv(6, p_a, l_a)
    pv(7, p_b, l_b)

    @pl.when(t == 0)
    def _():
        copies[3].wait()

    for j in range(4):
        o_nat[j * 128:(j + 1) * 128, :] = ot_ref[j].T
    for c in range(4):
        x_f[:, c * 256:(c + 1) * 256] += _dot(o_nat[...], woa[:, c * 256:(c + 1) * 256])

    @pl.when(t == 0)
    def _():
        copies[4].wait()
        copies[5].wait()
        n = 0
        for part in range(3):
            for kbk in range(8):
                tf = wstage3[kbk * 128:(kbk + 1) * 128, part * D:(part + 1) * D].T.astype(F32)

                def store(r, val, part=part, kbk=kbk):
                    wbt[part * D + r:part * D + r + 16, kbk * 128:(kbk + 1) * 128] = val

                _shuffle_rows(tf, tmp_a if n % 2 == 0 else tmp_b, store)
                n += 1
        for cb in range(8):
            tf = wob[:, cb * 128:(cb + 1) * 128].astype(F32)

            def store(r, val, cb=cb):
                wstage[r:r + 16, cb * 128:(cb + 1) * 128] = val

            _shuffle_rows(tf, tmp_a if n % 2 == 0 else tmp_b, store)
            n += 1

    _layernorm(x_f, xn)
    kb[:, 0:HALO, :] = halo[layer, 0]
    vb[:, 0:HALO, :] = halo[layer, 1]
    for c in range(4):
        y = _dot_nt(xn[...], wbt[c * 256:(c + 1) * 256, :]) * QSCALE
        qb[2 * c] = y[:, :128]
        qb[2 * c + 1] = y[:, 128:]
    for part, dst in ((1, kb), (2, vb)):
        for c in range(4):
            y = _dot_nt(xn[...], wbt[part * D + c * 256:part * D + (c + 1) * 256, :])
            dst[2 * c, HALO:, :] = y[:, :128]
            dst[2 * c + 1, HALO:, :] = y[:, 128:]
    halo[layer, 0] = kb[:, L:L + HALO, :]
    halo[layer, 1] = vb[:, L:L + HALO, :]
    _band_attention(seg, qb, kb, vb, ob)
    for c in range(4):
        x_f[:, c * 256:(c + 1) * 256] += _dot(ob[...], wstage[:, c * 256:(c + 1) * 256])

    @pl.when(layer == 1)
    def _():
        out_ref[...] = x_f[...].astype(out_ref.dtype)


@jax.jit
def pallas_interleave_layers__memory_aug_infini_attn__sliding_local_dilated__prompt_kernel(
    A_x: jax.Array,
    A_wq: jax.Array,
    A_wk: jax.Array,
    A_wv: jax.Array,
    A_wo: jax.Array,
    A_beta: jax.Array,
    B_x: jax.Array,
    B_wqkv: jax.Array,
    B_wo: jax.Array,
):
    del B_x
    x = A_x.reshape(S, D)
    any_spec = pl.BlockSpec(memory_space=pl.ANY)
    scratch = [
        pltpu.VMEM((L, D), F32),
        pltpu.VMEM((L, D), BF),
        pltpu.VMEM((D, D), BF),
        pltpu.VMEM((D, D), BF),
        pltpu.VMEM((D, D), BF),
        pltpu.VMEM((D, D), BF),
        pltpu.VMEM((D, 3 * D), BF),
        pltpu.VMEM((D, D), BF),
        pltpu.VMEM((3 * D, D), BF),
        pltpu.VMEM((D, D), BF),
        pltpu.VMEM((H * PITCH, 128), F32),
        pltpu.VMEM((H * PITCH, 128), F32),
        pltpu.VMEM((G, L, 128), BF),
        pltpu.VMEM((G, L, 128), BF),
        pltpu.VMEM((G, L, 128), BF),
        pltpu.VMEM((G, L, 128), BF),
        pltpu.VMEM((4, D, 128), BF),
        pltpu.VMEM((4, D, 128), BF),
        pltpu.VMEM((L, D), BF),
        pltpu.VMEM((1280, 512), F32),
        pltpu.VMEM((1280, 512), F32),
        pltpu.VMEM((4, 8, 512), F32),
        pltpu.VMEM((4, 8, 512), F32),
        pltpu.VMEM((4, 1280, 128), BF),
        pltpu.VMEM((4, 1280, 128), BF),
        pltpu.VMEM((4, 8, 512), F32),
        pltpu.VMEM((4, 8, 512), F32),
        pltpu.VMEM((2, G, 144, 128), F32),
        pltpu.VMEM((H, 128), F32),
        pltpu.VMEM((G, L, 128), F32),
        pltpu.VMEM((G, L + HALO, 128), F32),
        pltpu.VMEM((G, L + HALO, 128), F32),
        pltpu.VMEM((2, 2, G, HALO, 128), F32),
        pltpu.VMEM((L, D), BF),
        pltpu.SemaphoreType.DMA((6,)),
    ]
    out = pl.pallas_call(
        _kernel,
        grid=(2 * NSEG,),
        in_specs=[
            pl.BlockSpec((L, D), lambda t: (t // 2, 0)),
            any_spec, any_spec, any_spec, any_spec,
            pl.BlockSpec((H,), lambda t: (0,)),
            any_spec, any_spec,
        ],
        out_specs=pl.BlockSpec((L, D), lambda t: (t // 2, 0)),
        out_shape=jax.ShapeDtypeStruct((S, D), BF),
        scratch_shapes=scratch,
        compiler_params=pltpu.CompilerParams(
            dimension_semantics=("arbitrary",),
            vmem_limit_bytes=100 * 1024 * 1024,
        ),
    )(x, A_wq, A_wk, A_wv, A_wo, A_beta, B_wqkv, B_wo)
    return out.reshape(1, S, D)
```

```python
import math

import jax
import jax.numpy as jnp
from jax import lax
import jax.experimental.pallas as pl
import jax.experimental.pallas.tpu as pltpu

S, D, H, DH = 2048, 1024, 32, 32
L, NSEG, G = 512, 4, 8
W, DIL = 8, 2
HALO = 16
BF, F32 = jnp.bfloat16, jnp.float32
QSCALE = (DH ** -0.5) * math.log2(math.e)
NEG = -1e30
NT = (((1,), (1,)), ((), ()))
OFF = (0, 128, 384, 768)
SCOPES = False
PITCH = 33


class _scope:
    def __init__(self, name):
        self.cm = jax.named_scope(name) if SCOPES else None

    def __enter__(self):
        if self.cm is not None:
            self.cm.__enter__()

    def __exit__(self, *a):
        if self.cm is not None:
            self.cm.__exit__(*a)


def _dot(a, b):
    return jnp.dot(a, b, preferred_element_type=F32)


def _dot_nt(a, b):
    return lax.dot_general(a, b, NT, preferred_element_type=F32)


def _rows(x, n):
    return slice(x, x + n) if isinstance(x, int) else pl.ds(pl.multiple_of(x, n), n)


def _phi(t):
    return jnp.where(t > 0, t + 1.0, jnp.exp(t))


def _ln_items(x_ref, xn_ref, row0, nrows, chunk=16, dst0=None):
    shift = 0 if dst0 is None else dst0 - row0

    def item(r0):
        def run():
            x = x_ref[r0:r0 + chunk, :]
            d = x - jnp.mean(x, axis=-1, keepdims=True)
            v = jnp.mean(d * d, axis=-1, keepdims=True)
            xn_ref[r0 + shift:r0 + shift + chunk, :] = (d * lax.rsqrt(v + 1e-5)).astype(BF)
        return run
    return [item(r0) for r0 in range(row0, row0 + nrows, chunk)]


def _interleave(main, side):
    done = 0
    for i, it in enumerate(main):
        it()
        upto = (len(side) * (i + 1)) // len(main)
        for s_it in side[done:upto]:
            s_it()
        done = upto


def _run(items):
    for it in items:
        it()


def _shuffle_rows(tf, tmp, store):
    for h in range(H):
        tmp[h * PITCH:h * PITCH + DH, :] = tf[h * DH:(h + 1) * DH]
    for d in range(DH):
        for th in range(2):
            rows = tmp[pl.ds(th * 16 * PITCH + d, 16, stride=PITCH), :]
            store(d * H + th * 16, rows.astype(BF))


def _qk_stage(g, q_ref, k_ref, s_ref, m_ref):
    lane = lax.broadcasted_iota(jnp.int32, (64, 128), 1)
    key = lax.broadcasted_iota(jnp.int32, (128, 512), 0)
    qry = lax.broadcasted_iota(jnp.int32, (128, 512), 1) & 127
    causal = key <= qry
    for j in range(4):
        nk = 128 * (j + 1)
        qt = pltpu.bitcast(q_ref[g, j * 128:(j + 1) * 128, :], jnp.uint32)
        wq = jnp.concatenate(
            [jnp.where((lane >> 5) == h, qt, jnp.uint32(0)) for h in range(4)], axis=0)
        wq = pltpu.bitcast(wq, BF)
        st = _dot_nt(k_ref[g, 0:nk, :], wq)
        diag = jnp.where(causal, st[j * 128:], NEG)
        s_ref[OFF[j] + j * 128:OFF[j] + nk, :] = diag
        m = jnp.max(diag.reshape(16, 8, 512), axis=0)
        if j > 0:
            s_ref[OFF[j]:OFF[j] + j * 128, :] = st[:j * 128]
            m = jnp.maximum(m, jnp.max(st[:j * 128].reshape(16 * j, 8, 512), axis=0))
        m_ref[j] = jnp.broadcast_to(jnp.max(m, axis=0, keepdims=True), (8, 512))


def _sm_stage(s_ref, m_ref, p_ref, l_ref, sub=16):
    for j in range(4):
        nk = 128 * (j + 1)
        for h in range(4):
            m = m_ref[j, :, h * 128:(h + 1) * 128]
            l = None
            for r in range(0, nk, sub):
                s = s_ref[OFF[j] + r:OFF[j] + r + sub, h * 128:(h + 1) * 128]
                p = jnp.exp2(s.reshape(sub // 8, 8, 128) - m[None])
                ls = jnp.sum(p, axis=0)
                l = ls if l is None else l + ls
                p_ref[h, OFF[j] + r:OFF[j] + r + sub, :] = p.reshape(sub, 128).astype(BF)
            l_ref[j, :, h * 128:(h + 1) * 128] = l


def _pv_stage(g, p_ref, l_ref, vt_ref, ot_ref, pq_ref, pk_ref, mt_ref, gate_ref):
    nd = _dot_nt(mt_ref[g].astype(BF), pq_ref[g])
    for h in range(4):
        r0 = (g * 4 + h) * DH
        gate = gate_ref[pl.ds(g * 4 + h, 1), :]
        for j in range(4):
            acc = None
            for t in range(j + 1):
                o = _dot(vt_ref[t, _rows(r0, DH), :],
                         p_ref[h, OFF[j] + t * 128:OFF[j] + (t + 1) * 128, :])
                acc = o if acc is None else acc + o
            l = jnp.sum(l_ref[j, :, h * 128:(h + 1) * 128], axis=0, keepdims=True)
            den = nd[128 + h:129 + h, j * 128:(j + 1) * 128] + 1e-6
            num = nd[h * DH:(h + 1) * DH, j * 128:(j + 1) * 128]
            res = num * (gate / den) + acc * ((1.0 - gate) / l)
            ot_ref[j, _rows(r0, DH), :] = res.astype(BF)
    row = lax.broadcasted_iota(jnp.int32, (144, 128), 0)
    lane = lax.broadcasted_iota(jnp.int32, (144, 128), 1)
    keep = jnp.where(row < 128, row >> 5, row - 128) == (lane >> 5)
    row16 = lax.broadcasted_iota(jnp.int32, (16, 128), 0)
    ones = jnp.where(row16 < 4, 1.0, 0.0).astype(BF)
    upd = None
    for t in range(4):
        lhs = jnp.concatenate([vt_ref[t, _rows(g * 128, 128), :], ones], axis=0)
        u = _dot(lhs, pk_ref[g, t * 128:(t + 1) * 128, :])
        upd = u if upd is None else upd + u
    mt_ref[g] = mt_ref[g] + jnp.where(keep, upd, 0.0)


def _band_items(seg, blk0, nblk, q_ref, k_ref, v_ref, a_ref, e_ref, o_ref):
    def logits(r0):
        def run():
            q = [q_ref[b, r0:r0 + 8, :] for b in range(G)]
            for w in range(W):
                base = HALO + r0 - DIL * w
                acc = q[0] * k_ref[0, base:base + 8, :]
                for b in range(1, G):
                    acc = acc + q[b] * k_ref[b, base:base + 8, :]
                a_ref[w, r0:r0 + 8, :] = acc
        return run

    def softmax(r0):
        def run():
            lg = []
            for w in range(W):
                t = a_ref[w, r0:r0 + 128, :].T
                t = (t[0:32] + t[32:64]) + (t[64:96] + t[96:128])
                if r0 == 0 and w > 0:
                    pos = seg * L - DIL * w + lax.broadcasted_iota(jnp.int32, (H, 128), 1)
                    t = jnp.where(pos >= 0, t, NEG)
                lg.append(t)
            m = lg[0]
            for w in range(1, W):
                m = jnp.maximum(m, lg[w])
            e = [jnp.exp2(x - m) for x in lg]
            l = e[0]
            for w in range(1, W):
                l = l + e[w]
            inv = 1.0 / l
            for w in range(W):
                p = e[w] * inv
                e_ref[w, r0:r0 + 128, :] = jnp.concatenate([p, p, p, p], axis=0).T
        return run

    def pv(r0, n=8):
        def run():
            e = [e_ref[w, r0:r0 + n, :] for w in range(W)]
            outs = []
            for b in range(G):
                acc = e[0] * v_ref[b, HALO + r0:HALO + r0 + n, :]
                for w in range(1, W):
                    base = HALO + r0 - DIL * w
                    acc = acc + e[w] * v_ref[b, base:base + n, :]
                outs.append(acc)
            return outs
        return run

    def pv16(r0):
        def run():
            lo = pv(r0)()
            hi = pv(r0 + 8)()
            for b in range(G):
                o_ref[r0:r0 + 16, b * 128:(b + 1) * 128] = jnp.concatenate([lo[b], hi[b]], axis=0).astype(BF)
        return run

    items = []
    for blk in range(blk0, blk0 + nblk):
        r0 = blk * 128
        items += [logits(r) for r in range(r0, r0 + 128, 8)]
        items.append(softmax(r0))
        items += [pv16(r) for r in range(r0, r0 + 128, 16)]
    return items


def _kernel(x_in, wq_hbm, wk_hbm, wv_hbm, woa_hbm, beta_ref, wqkv_hbm, wob_hbm, out_ref,
            x_f, xn, xc, xnx, wq, wk, woa, wstage, wstage3, wvt, wbt, wob, wobp, tmp_a,
            q_ref, pq_ref, k_ref, pk_ref, vt_ref, ot_ref, o_nat,
            s_a, s_b, m_a, m_b, p_a, p_b, l_a, l_b, mt_ref, gate_ref,
            qb, kb, vb, halo, ab, eb, ob, sems):
    t = pl.program_id(0)
    seg = t // 2
    layer = t % 2

    copies = [
        pltpu.make_async_copy(wq_hbm, wq, sems.at[0]),
        pltpu.make_async_copy(wk_hbm, wk, sems.at[1]),
        pltpu.make_async_copy(wv_hbm, wstage, sems.at[2]),
        pltpu.make_async_copy(woa_hbm, woa, sems.at[3]),
        pltpu.make_async_copy(wqkv_hbm, wstage3, sems.at[4]),
        pltpu.make_async_copy(wob_hbm, wob, sems.at[5]),
    ]

    @pl.when(t == 0)
    def _():
        for c in copies:
            c.start()
        b = beta_ref[...].astype(F32).reshape(1, H)
        gt = jax.nn.sigmoid(b)
        row = lax.broadcasted_iota(jnp.int32, (H, H), 0)
        lane = lax.broadcasted_iota(jnp.int32, (H, H), 1)
        col = jnp.sum(jnp.where(row == lane, jnp.broadcast_to(gt, (H, H)), 0.0), axis=1, keepdims=True)
        gate_ref[...] = jnp.broadcast_to(col, (H, 128))

    @pl.when(layer == 0)
    def _():
        x_f[...] = x_in[...].astype(F32)

    @pl.when(seg == 0)
    def _():
        mt_ref[layer] = jnp.zeros((G, 144, 128), F32)
        halo[layer] = jnp.zeros((2, G, HALO, 128), F32)

    @pl.when(t == 0)
    def _():
        with _scope("prepA"):
            copies[0].wait()
            copies[1].wait()
            copies[2].wait()

            def tr(kbk, c):
                wvt[kbk] = wstage[pl.ds(pl.multiple_of(kbk * 128, 128), 128), :].T
                return c
            lax.fori_loop(0, 8, tr, 0)

    HL = L // 2

    def a_proj_items(hf):
        rows = pl.ds(pl.multiple_of(hf * HL, HL), HL)
        items = []

        def q_item(c):
            def run():
                y = _dot(xc[...], wq[:, c * 256:(c + 1) * 256])
                for gg in range(2):
                    yq = y[:, gg * 128:(gg + 1) * 128]
                    q_ref[2 * c + gg, rows, :] = (yq * QSCALE).astype(BF)
                    pq_ref[2 * c + gg, rows, :] = _phi(yq).astype(BF)
            return run

        def k_item(c):
            def run():
                y = _dot(xc[...], wk[:, c * 256:(c + 1) * 256])
                for gg in range(2):
                    yk = y[:, gg * 128:(gg + 1) * 128]
                    k_ref[2 * c + gg, rows, :] = yk.astype(BF)
                    pk_ref[2 * c + gg, rows, :] = _phi(yk).astype(BF)
            return run

        def v_item(c):
            def run():
                y = None
                for kbk in range(8):
                    u = _dot_nt(wvt[kbk, c * 512:(c + 1) * 512, :], xc[:, kbk * 128:(kbk + 1) * 128])
                    y = u if y is None else y + u
                vt_ref[2 * hf, c * 512:(c + 1) * 512, :] = y[:, :128].astype(BF)
                vt_ref[2 * hf + 1, c * 512:(c + 1) * 512, :] = y[:, 128:].astype(BF)
            return run

        return [q_item(c) for c in range(4)] + [k_item(c) for c in range(4)] + [v_item(c) for c in range(2)]

    with _scope("A_proj"):
        _run(_ln_items(x_f, xc, 0, HL))

        def a_half(hf, c):
            _interleave(a_proj_items(hf), _ln_items(x_f, xnx, HL, HL, dst0=0))
            xc[...] = xnx[...]
            return c

        lax.fori_loop(0, 2, a_half, 0)

    mt = mt_ref.at[layer]
    pv = lambda g, p, l: _pv_stage(g, p, l, vt_ref, ot_ref, pq_ref, pk_ref, mt, gate_ref)
    with _scope("A_attn_pro"):
        _qk_stage(0, q_ref, k_ref, s_a, m_a)
        _qk_stage(1, q_ref, k_ref, s_b, m_b)
        _sm_stage(s_a, m_a, p_a, l_a)

    @pl.when(t == 0)
    def _():
        with _scope("prepB"):
            copies[3].wait()
            copies[4].wait()
            copies[5].wait()

            def shuf_qkv(i, c):
                part = i // 8
                kbk = i % 8
                src = wstage3[pl.ds(pl.multiple_of(kbk * 128, 128), 128), pl.ds(pl.multiple_of(part * D, D), D)]
                tf = src.T.astype(F32)

                def store(r, val):
                    wbt[kbk, pl.ds(pl.multiple_of(part * D + r, 16), 16), :] = val

                _shuffle_rows(tf, tmp_a, store)
                return c
            lax.fori_loop(0, 24, shuf_qkv, 0)

            def shuf_wo(cb, c):
                tf = wob[:, pl.ds(pl.multiple_of(cb * 128, 128), 128)].astype(F32)

                def store(r, val):
                    wobp[cb, r:r + 16, :] = val

                _shuffle_rows(tf, tmp_a, store)
                return c
            lax.fori_loop(0, 8, shuf_wo, 0)

    def pair(u, c):
        g = 2 * u + 1
        _qk_stage(g + 1, q_ref, k_ref, s_a, m_a)
        _sm_stage(s_b, m_b, p_b, l_b)
        pv(g - 1, p_a, l_a)
        _qk_stage(g + 2, q_ref, k_ref, s_b, m_b)
        _sm_stage(s_a, m_a, p_a, l_a)
        pv(g, p_b, l_b)
        return c

    with _scope("A_attn_loop"):
        lax.fori_loop(0, 3, pair, 0)

    def out_items(src, w_ref, hf, blocked=False):
        rows = slice(hf * HL, (hf + 1) * HL)

        def item(c):
            def run():
                if blocked:
                    for cc in range(2):
                        cb = 2 * c + cc
                        x_f[rows, cb * 128:(cb + 1) * 128] += _dot(src[rows, :], w_ref[cb])
                else:
                    x_f[rows, c * 256:(c + 1) * 256] += _dot(src[rows, :], w_ref[:, c * 256:(c + 1) * 256])
            return run
        return [item(c) for c in range(4)]

    def b_proj_items(hf):
        rows = slice(hf * HL, (hf + 1) * HL)
        hrows = slice(HALO + hf * HL, HALO + (hf + 1) * HL)

        def item(part, c):
            def run():
                y = None
                for kbk in range(8):
                    u = _dot_nt(xn[rows, kbk * 128:(kbk + 1) * 128],
                                wbt[kbk, part * D + c * 256:part * D + (c + 1) * 256, :])
                    y = u if y is None else y + u
                if part == 0:
                    y = y * QSCALE
                    qb[2 * c, rows, :] = y[:, :128]
                    qb[2 * c + 1, rows, :] = y[:, 128:]
                else:
                    dst = kb if part == 1 else vb
                    dst[2 * c, hrows, :] = y[:, :128]
                    dst[2 * c + 1, hrows, :] = y[:, 128:]
            return run
        return [item(part, c) for part in range(3) for c in range(4)]

    with _scope("tail"):
        _sm_stage(s_b, m_b, p_b, l_b)
        pv(6, p_a, l_a)
        pv(7, p_b, l_b)
        for j in range(4):
            o_nat[j * 128:(j + 1) * 128, :] = ot_ref[j].T
        kb[:, 0:HALO, :] = halo[layer, 0]
        vb[:, 0:HALO, :] = halo[layer, 1]
        _run(out_items(o_nat, woa, 0))
        _interleave(out_items(o_nat, woa, 1), _ln_items(x_f, xn, 0, HL))
        _interleave(b_proj_items(0), _ln_items(x_f, xn, HL, HL))
        _interleave(b_proj_items(1), _band_items(seg, 0, 2, qb, kb, vb, ab, eb, ob))
        halo[layer, 0] = kb[:, L:L + HALO, :]
        halo[layer, 1] = vb[:, L:L + HALO, :]
        _interleave(out_items(ob, wobp, 0, True), _band_items(seg, 2, 2, qb, kb, vb, ab, eb, ob))
        _run(out_items(ob, wobp, 1, True))

    @pl.when(layer == 1)
    def _():
        out_ref[...] = x_f[...].astype(out_ref.dtype)


@jax.jit
def pallas_interleave_layers__memory_aug_infini_attn__sliding_local_dilated__prompt_kernel(
    A_x: jax.Array,
    A_wq: jax.Array,
    A_wk: jax.Array,
    A_wv: jax.Array,
    A_wo: jax.Array,
    A_beta: jax.Array,
    B_x: jax.Array,
    B_wqkv: jax.Array,
    B_wo: jax.Array,
):
    del B_x
    x = A_x.reshape(S, D)
    any_spec = pl.BlockSpec(memory_space=pl.ANY)
    scratch = [
        pltpu.VMEM((L, D), F32),
        pltpu.VMEM((L, D), BF),
        pltpu.VMEM((L // 2, D), BF),
        pltpu.VMEM((L // 2, D), BF),
        pltpu.VMEM((D, D), BF),
        pltpu.VMEM((D, D), BF),
        pltpu.VMEM((D, D), BF),
        pltpu.VMEM((D, D), BF),
        pltpu.VMEM((D, 3 * D), BF),
        pltpu.VMEM((8, D, 128), BF),
        pltpu.VMEM((8, 3 * D, 128), BF),
        pltpu.VMEM((D, D), BF),
        pltpu.VMEM((8, D, 128), BF),
        pltpu.VMEM((H * PITCH, 128), F32),
        pltpu.VMEM((G, L, 128), BF),
        pltpu.VMEM((G, L, 128), BF),
        pltpu.VMEM((G, L, 128), BF),
        pltpu.VMEM((G, L, 128), BF),
        pltpu.VMEM((4, D, 128), BF),
        pltpu.VMEM((4, D, 128), BF),
        pltpu.VMEM((L, D), BF),
        pltpu.VMEM((1280, 512), F32),
        pltpu.VMEM((1280, 512), F32),
        pltpu.VMEM((4, 8, 512), F32),
        pltpu.VMEM((4, 8, 512), F32),
        pltpu.VMEM((4, 1280, 128), BF),
        pltpu.VMEM((4, 1280, 128), BF),
        pltpu.VMEM((4, 8, 512), F32),
        pltpu.VMEM((4, 8, 512), F32),
        pltpu.VMEM((2, G, 144, 128), F32),
        pltpu.VMEM((H, 128), F32),
        pltpu.VMEM((G, L, 128), F32),
        pltpu.VMEM((G, L + HALO, 128), F32),
        pltpu.VMEM((G, L + HALO, 128), F32),
        pltpu.VMEM((2, 2, G, HALO, 128), F32),
        pltpu.VMEM((W, L, 128), F32),
        pltpu.VMEM((W, L, 128), F32),
        pltpu.VMEM((L, D), BF),
        pltpu.SemaphoreType.DMA((6,)),
    ]
    out = pl.pallas_call(
        _kernel,
        grid=(2 * NSEG,),
        in_specs=[
            pl.BlockSpec((L, D), lambda t: (t // 2, 0)),
            any_spec, any_spec, any_spec, any_spec,
            pl.BlockSpec((H,), lambda t: (0,)),
            any_spec, any_spec,
        ],
        out_specs=pl.BlockSpec((L, D), lambda t: (t // 2, 0)),
        out_shape=jax.ShapeDtypeStruct((S, D), BF),
        scratch_shapes=scratch,
        compiler_params=pltpu.CompilerParams(
            dimension_semantics=("arbitrary",),
            vmem_limit_bytes=100 * 1024 * 1024,
        ),
    )(x, A_wq, A_wk, A_wv, A_wo, A_beta, B_wqkv, B_wo)
    return out.reshape(1, S, D)
```

```python
import math

import jax
import jax.numpy as jnp
from jax import lax
import jax.experimental.pallas as pl
import jax.experimental.pallas.tpu as pltpu

S, D, H, DH = 2048, 1024, 32, 32
L, NSEG, G = 512, 4, 8
HL = L // 2
W, DIL = 8, 2
HALO = 16
BF, F32, U32 = jnp.bfloat16, jnp.float32, jnp.uint32
QSCALE = (DH ** -0.5) * math.log2(math.e)
NEG = -1e30
NT = (((1,), (1,)), ((), ()))
OFF = (0, 128, 384, 768)
SCOPES = False
PITCH = 33


class _scope:
    def __init__(self, name):
        self.cm = jax.named_scope(name) if SCOPES else None

    def __enter__(self):
        if self.cm is not None:
            self.cm.__enter__()

    def __exit__(self, *a):
        if self.cm is not None:
            self.cm.__exit__(*a)


def _dot(a, b):
    return jnp.dot(a, b, preferred_element_type=F32)


def _dot_nt(a, b):
    return lax.dot_general(a, b, NT, preferred_element_type=F32)


def _prow(r0, n):
    if isinstance(r0, int):
        return slice(r0 // 2, (r0 + n) // 2)
    return pl.ds(pl.multiple_of(r0 // 2, 8), n // 2)


def _ld(ref, b, r0, n, tok=None):
    u = ref[b, _prow(r0, n), :]
    if tok is not None:
        u = jnp.concatenate([u[0:8] | tok, u[8:]], axis=0) if n > 16 else u | tok
    return pltpu.bitcast(u, BF)


def _st(ref, b, r0, val):
    ref[b, _prow(r0, val.shape[0]), :] = pltpu.bitcast(val, U32)


def _wide(ref, r0, n, tok=None):
    tok = [None] * G if tok is None else tok
    return jnp.concatenate([_ld(ref, b, r0, n, tok[b]) for b in range(G)], axis=1)


def _token(v):
    u = pltpu.bitcast(v[0:8, 0:128], U32)
    return lax.shift_right_logical(lax.shift_right_logical(u, jnp.uint32(31)), jnp.uint32(1))


def _phi(t):
    return jnp.where(t > 0, t + 1.0, jnp.exp(t))


def _ln(x):
    d = x - jnp.mean(x, axis=-1, keepdims=True)
    v = jnp.mean(d * d, axis=-1, keepdims=True)
    return d * lax.rsqrt(v + 1e-5)


def _ln_items(x_ref, xn_ref, row0, nrows, dst0, chunk=16):
    def item(r0):
        def run():
            yf = _ln(x_ref[r0:r0 + chunk, :])
            y = yf.astype(BF)
            for b in range(G):
                _st(xn_ref, b, r0 - row0 + dst0, y[:, b * 128:(b + 1) * 128])
            return _token(yf)
        return run
    return [item(r0) for r0 in range(row0, row0 + nrows, chunk)]


def _interleave(main, side, span=None, tokens=True):
    span = len(main) if span is None else span
    done = 0
    toks = None
    for i, it in enumerate(main):
        it(toks if tokens else None)
        upto = len(side) if i + 1 >= span else (len(side) * (i + 1)) // span
        group = side[done:upto]
        toks = [None] * G
        for m, s_it in enumerate(group):
            tk = s_it()
            if tk is not None:
                kbk = (m * G) // len(group)
                toks[kbk] = tk if toks[kbk] is None else toks[kbk] | tk
        done = max(done, upto)


def _run(items):
    for it in items:
        it()


def _shuffle_rows(tf, tmp, store):
    for h in range(H):
        tmp[h * PITCH:h * PITCH + DH, :] = tf[h * DH:(h + 1) * DH]
    for d in range(DH):
        for th in range(2):
            rows = tmp[pl.ds(th * 16 * PITCH + d, 16, stride=PITCH), :]
            store(d * H + th * 16, rows.astype(BF))


def _qk_stage(g, q_ref, k_ref, s_ref, m_ref):
    lane = lax.broadcasted_iota(jnp.int32, (64, 128), 1)
    key = lax.broadcasted_iota(jnp.int32, (128, 512), 0)
    qry = lax.broadcasted_iota(jnp.int32, (128, 512), 1) & 127
    causal = key <= qry
    for j in range(4):
        nk = 128 * (j + 1)
        qt = q_ref[g, j * 64:(j + 1) * 64, :]
        wq = jnp.concatenate([jnp.where((lane >> 5) == h, qt, jnp.uint32(0)) for h in range(4)], axis=0)
        st = _dot_nt(_ld(k_ref, g, 0, nk), pltpu.bitcast(wq, BF))
        diag = jnp.where(causal, st[j * 128:], NEG)
        s_ref[OFF[j] + j * 128:OFF[j] + nk, :] = diag
        m = jnp.max(diag.reshape(16, 8, 512), axis=0)
        if j > 0:
            s_ref[OFF[j]:OFF[j] + j * 128, :] = st[:j * 128]
            m = jnp.maximum(m, jnp.max(st[:j * 128].reshape(16 * j, 8, 512), axis=0))
        m_ref[j] = jnp.broadcast_to(jnp.max(m, axis=0, keepdims=True), (8, 512))


def _sm_stage(s_ref, m_ref, p_ref, l_ref, sub=16):
    for j in range(4):
        nk = 128 * (j + 1)
        for h in range(4):
            m = m_ref[j, :, h * 128:(h + 1) * 128]
            l = None
            for r in range(0, nk, sub):
                s = s_ref[OFF[j] + r:OFF[j] + r + sub, h * 128:(h + 1) * 128]
                p = jnp.exp2(s.reshape(sub // 8, 8, 128) - m[None])
                ls = jnp.sum(p, axis=0)
                l = ls if l is None else l + ls
                _st(p_ref, h, OFF[j] + r, p.reshape(sub, 128).astype(BF))
            l_ref[j, :, h * 128:(h + 1) * 128] = l


def _pv_stage(g, p_ref, l_ref, vt_ref, ot_ref, pq_ref, pk_ref, mt_ref, gate_ref):
    mem = mt_ref[g].astype(BF)
    for j in range(4):
        nd = _dot_nt(mem, _ld(pq_ref, g, j * 128, 128))
        for h in range(4):
            r0 = (g * 4 + h) * DH
            gate = gate_ref[pl.ds(g * 4 + h, 1), :]
            acc = None
            for t in range(j + 1):
                o = _dot(_ld(vt_ref, t, r0, DH), _ld(p_ref, h, OFF[j] + t * 128, 128))
                acc = o if acc is None else acc + o
            l = jnp.sum(l_ref[j, :, h * 128:(h + 1) * 128], axis=0, keepdims=True)
            den = nd[128 + h:129 + h] + 1e-6
            res = nd[h * DH:(h + 1) * DH] * (gate / den) + acc * ((1.0 - gate) / l)
            _st(ot_ref, j, r0, res.astype(BF))
    row = lax.broadcasted_iota(jnp.int32, (144, 128), 0)
    lane = lax.broadcasted_iota(jnp.int32, (144, 128), 1)
    keep = jnp.where(row < 128, row >> 5, row - 128) == (lane >> 5)
    row16 = lax.broadcasted_iota(jnp.int32, (16, 128), 0)
    ones = jnp.where(row16 < 4, 1.0, 0.0).astype(BF)
    upd = None
    for t in range(4):
        lhs = jnp.concatenate([_ld(vt_ref, t, g * 128, 128), ones], axis=0)
        u = _dot(lhs, _ld(pk_ref, g, t * 128, 128))
        upd = u if upd is None else upd + u
    mt_ref[g] = mt_ref[g] + jnp.where(keep, upd, 0.0)


def _band_items(pos0, row0, q_ref, k_ref, v_ref, a_ref, e_ref, o_ref, nrows=HL):
    def logits(r0):
        def run():
            q = [q_ref[b, r0:r0 + 8, :] for b in range(G)]
            for w in range(W):
                base = HALO + r0 - DIL * w
                acc = q[0] * k_ref[0, base:base + 8, :]
                for b in range(1, G):
                    acc = acc + q[b] * k_ref[b, base:base + 8, :]
                a_ref[w, r0 - row0:r0 - row0 + 8, :] = acc
            return _token(acc)
        return run

    def softmax(r0):
        def run():
            lg = []
            for w in range(W):
                t = a_ref[w, r0 - row0:r0 - row0 + 128, :].T
                t = (t[0:32] + t[32:64]) + (t[64:96] + t[96:128])
                if r0 == 0 and w > 0:
                    pos = pos0 - DIL * w + lax.broadcasted_iota(jnp.int32, (H, 128), 1)
                    t = jnp.where(pos >= 0, t, NEG)
                lg.append(t)
            m = lg[0]
            for w in range(1, W):
                m = jnp.maximum(m, lg[w])
            e = [jnp.exp2(x - m) for x in lg]
            l = e[0]
            for w in range(1, W):
                l = l + e[w]
            inv = 1.0 / l
            for w in range(W):
                p = e[w] * inv
                pt = jnp.concatenate([p, p, p, p], axis=0).T
                e_ref[w, r0 - row0:r0 - row0 + 128, :] = pt
            return _token(pt)
        return run

    def pv(r0):
        e = [e_ref[w, r0 - row0:r0 - row0 + 8, :] for w in range(W)]
        outs = []
        for b in range(G):
            acc = e[0] * v_ref[b, HALO + r0:HALO + r0 + 8, :]
            for w in range(1, W):
                base = HALO + r0 - DIL * w
                acc = acc + e[w] * v_ref[b, base:base + 8, :]
            outs.append(acc)
        return outs

    def pv16(r0):
        def run():
            lo = pv(r0)
            hi = pv(r0 + 8)
            for b in range(G):
                _st(o_ref, b, r0, jnp.concatenate([lo[b], hi[b]], axis=0).astype(BF))
            return _token(hi[G - 1])
        return run

    items = []
    for r0 in range(row0, row0 + nrows, 128):
        items += [logits(r) for r in range(r0, r0 + 128, 8)]
        items.append(softmax(r0))
        items += [pv16(r) for r in range(r0, r0 + 128, 16)]
    return items


def _kernel(x_hbm, wq_hbm, wk_hbm, wv_hbm, woa_hbm, beta_ref, wqkv_hbm, wob_hbm, out_hbm,
            xin, obuf, x_f, xn, xc, xnx, wq, wk, woa, wv, wqkv, wvt, wbt, wob, wobp, tmp_a, tmp_b, tmp_c, tmp_d,
            q_ref, pq_ref, k_ref, pk_ref, vt_ref, ot_ref, o_nat,
            s_a, s_b, m_a, m_b, p_a, p_b, l_a, l_b, mt_ref, gate_ref,
            qb, kb, vb, halo, ab, eb, ob, sems):

    def col_copies(src, dst, sem, c0=0, n=G):
        return [pltpu.make_async_copy(src.at[:, (c0 + i) * 128:(c0 + i + 1) * 128], dst.at[c0 + i], sem)
                for i in range(n)]

    cp_wq = [col_copies(wq_hbm, wq, sems.at[c], 2 * c, 2) for c in range(4)]
    cp_wk = col_copies(wk_hbm, wk, sems.at[4])
    cp_wv = [pltpu.make_async_copy(wv_hbm, wv, sems.at[5])]
    cp_wqkv = [[pltpu.make_async_copy(wqkv_hbm.at[:, part * D:(part + 1) * D], wqkv.at[part], sems.at[6 + part])]
               for part in range(3)]
    cp_wob = col_copies(wob_hbm, wob, sems.at[9])
    cp_woa = col_copies(woa_hbm, woa, sems.at[10])
    cp_x0 = [pltpu.make_async_copy(x_hbm.at[0:L], xin.at[0:L], sems.at[11])]
    cp_xr = [pltpu.make_async_copy(x_hbm.at[L:S], xin.at[L:S], sems.at[12])]

    def cp_out(seg):
        return pltpu.make_async_copy(obuf, out_hbm.at[pl.ds(pl.multiple_of(seg * L, L), L)], sems.at[13])

    def wait(cps):
        for c in cps:
            c.wait()

    def wcols(w_ref, c0):
        return jnp.concatenate([w_ref[c0], w_ref[c0 + 1]], axis=1)

    def q_item(src, n, d0, c):
        def run(tok=None):
            y = _dot(_wide(src, 0, n, tok), wcols(wq, 2 * c))
            for gg in range(2):
                yq = y[:, gg * 128:(gg + 1) * 128]
                _st(q_ref, 2 * c + gg, d0, (yq * QSCALE).astype(BF))
                _st(pq_ref, 2 * c + gg, d0, _phi(yq).astype(BF))
        return run

    def k_item(src, n, d0, c):
        def run(tok=None):
            y = _dot(_wide(src, 0, n, tok), wcols(wk, 2 * c))
            for gg in range(2):
                yk = y[:, gg * 128:(gg + 1) * 128]
                _st(k_ref, 2 * c + gg, d0, yk.astype(BF))
                _st(pk_ref, 2 * c + gg, d0, _phi(yk).astype(BF))
        return run

    def v_item(src, r0, tile0, f0):
        def run(tok=None):
            y = _dot_nt(_wide(wvt, f0, 512), _wide(src, r0, HL, tok))
            _st(vt_ref, tile0, f0, y[:, :128].astype(BF))
            _st(vt_ref, tile0 + 1, f0, y[:, 128:].astype(BF))
        return run

    def blk(i):
        return pl.ds(pl.multiple_of(i * 128, 128), 128)

    def qkv_shuffle(part, kbk, tmp):
        tf = wqkv[part, blk(kbk), :].T.astype(F32)
        _shuffle_rows(tf, tmp, lambda r, val: _st(wbt, kbk, part * D + r, val))

    with _scope("first_proj"):
        for cps in [cp_x0] + cp_wq + [cp_wv, cp_wk] + cp_wqkv + [cp_wob, cp_woa, cp_xr]:
            for c in cps:
                c.start()
        b = beta_ref[...].astype(F32).reshape(1, H)
        gt = jax.nn.sigmoid(b)
        row = lax.broadcasted_iota(jnp.int32, (H, H), 0)
        lane = lax.broadcasted_iota(jnp.int32, (H, H), 1)
        col = jnp.sum(jnp.where(row == lane, jnp.broadcast_to(gt, (H, H)), 0.0), axis=1, keepdims=True)
        gate_ref[...] = jnp.broadcast_to(col, (H, 128))
        halo[...] = jnp.zeros(halo.shape, F32)

        def zero_mem(i, c):
            mt_ref[i // G, i % G] = jnp.zeros((144, 128), F32)
            return c
        lax.fori_loop(0, 2 * G, zero_mem, 0)
        with _scope("p_wait_x"):
            wait(cp_x0)

        def ln0(i, c):
            for u in range(8):
                r0 = pl.multiple_of(i * 128 + u * 16, 16)
                x = xin[pl.ds(r0, 16), :].astype(F32)
                x_f[pl.ds(r0, 16), :] = x
                y = _ln(x).astype(BF)
                for b in range(G):
                    _st(xn, b, r0, y[:, b * 128:(b + 1) * 128])
            return c
        with _scope("p_ln"):
            lax.fori_loop(0, L // 128, ln0, 0)

        def q0(c, carry):
            for i in range(2):
                pltpu.make_async_copy(wq_hbm.at[:, 0:128], wq.at[0], sems.at[c]).wait()
            q_item(xn, L, 0, c)()
            return carry
        with _scope("p_q"):
            lax.fori_loop(0, 4, q0, 0)
        wait(cp_wv)

        def tr0(i, carry):
            for u in range(4):
                _st(wvt, 4 * i + u, 0, wv[blk(4 * i + u), :].T)
            return carry
        with _scope("p_tr"):
            lax.fori_loop(0, 2, tr0, 0)

        def v0(i, carry):
            hf = i // 2
            v_item(xn, hf * HL, 2 * hf, (i % 2) * 512)()
            return carry
        with _scope("p_v"):
            lax.fori_loop(0, 4, v0, 0)
        wait(cp_wk)
        wait(cp_wqkv[0])
        wait(cp_wqkv[1])
        tmps = (tmp_a, tmp_b, tmp_c, tmp_d)

        def k0(c, carry):
            k_item(xn, L, 0, c)()
            for u in range(4):
                qkv_shuffle(c // 2, 4 * (c % 2) + u, tmps[u])
            return carry
        with _scope("p_k"):
            lax.fori_loop(0, 4, k0, 0)
        wait(cp_wqkv[2])

        def sh0(i, carry):
            for u in range(4):
                qkv_shuffle(2, 4 * i + u, tmps[u])
            return carry
        with _scope("p_sh0"):
            lax.fori_loop(0, 2, sh0, 0)
        wait(cp_wob)

        def sh1(i, carry):
            for u in range(4):
                cb = 4 * i + u
                _shuffle_rows(wob[cb].astype(F32), tmps[u], lambda r, val, cb=cb: _st(wobp, cb, r, val))
            return carry
        with _scope("p_sh1"):
            lax.fori_loop(0, 2, sh1, 0)
        wait(cp_woa)

    def out_item(src, r0, wcol, c):
        def run(tok=None):
            rows = slice(r0, r0 + HL) if isinstance(r0, int) else pl.ds(pl.multiple_of(r0, HL), HL)
            x_f[rows, c * 256:(c + 1) * 256] += _dot(_wide(src, r0, HL, tok), wcol(c))
        return run

    woa_cols = lambda c: wcols(woa, 2 * c)
    wob_cols = lambda c: jnp.concatenate([_ld(wobp, 2 * c, 0, D), _ld(wobp, 2 * c + 1, 0, D)], axis=1)

    def b_proj_items(hf):
        rows = slice(hf * HL, (hf + 1) * HL)
        hrows = slice(HALO + hf * HL, HALO + (hf + 1) * HL)

        def item(part, c):
            def run(tok=None):
                y = _dot_nt(_wide(xn, hf * HL, HL, tok), _wide(wbt, part * D + c * 256, 256))
                if part == 0:
                    y = y * QSCALE
                    qb[2 * c, rows, :] = y[:, :128]
                    qb[2 * c + 1, rows, :] = y[:, 128:]
                else:
                    dst = kb if part == 1 else vb
                    dst[2 * c, hrows, :] = y[:, :128]
                    dst[2 * c + 1, hrows, :] = y[:, 128:]
            return run
        return [item(part, c) for part in range(3) for c in range(4)]

    def step(t, carry):
        seg = t // 2
        layer = t % 2
        mt = mt_ref.at[layer]
        pv = lambda g, p, l: _pv_stage(g, p, l, vt_ref, ot_ref, pq_ref, pk_ref, mt, gate_ref)

        @pl.when(t > 0)
        def _():
            with _scope("A_proj"):
                _run(_ln_items(x_f, xc, 0, HL, 0))

                def a_half(hf, c):
                    d0 = hf * HL
                    items = ([q_item(xc, HL, d0, c) for c in range(4)]
                             + [k_item(xc, HL, d0, c) for c in range(4)]
                             + [v_item(xc, 0, 2 * hf, f0) for f0 in (0, 512)])
                    _interleave(items, _ln_items(x_f, xnx, HL, HL, 0), span=8)
                    xc[...] = xnx[...]
                    return c

                lax.fori_loop(0, 2, a_half, 0)

        with _scope("A_attn_pro"):
            _qk_stage(0, q_ref, k_ref, s_a, m_a)
            _qk_stage(1, q_ref, k_ref, s_b, m_b)
            _sm_stage(s_a, m_a, p_a, l_a)

        def pair(u, c):
            g = 2 * u + 1
            _qk_stage(g + 1, q_ref, k_ref, s_a, m_a)
            _sm_stage(s_b, m_b, p_b, l_b)
            pv(g - 1, p_a, l_a)
            _qk_stage(g + 2, q_ref, k_ref, s_b, m_b)
            _sm_stage(s_a, m_a, p_a, l_a)
            pv(g, p_b, l_b)
            return c

        with _scope("A_attn_loop"):
            lax.fori_loop(0, 3, pair, 0)

        with _scope("A_attn_epi"):
            _sm_stage(s_b, m_b, p_b, l_b)
            pv(6, p_a, l_a)
            pv(7, p_b, l_b)
            for j in range(4):
                ot = _ld(ot_ref, j, 0, D).T
                for b in range(G):
                    _st(o_nat, b, j * 128, ot[:, b * 128:(b + 1) * 128])
            kb[:, 0:HALO, :] = halo[layer, 0]
            vb[:, 0:HALO, :] = halo[layer, 1]

        def out_half(hf, c):
            _run([out_item(o_nat, hf * HL, woa_cols, c) for c in range(4)])
            return c

        with _scope("A_out"):
            lax.fori_loop(0, 2, out_half, 0)

        with _scope("B"):
            _run(_ln_items(x_f, xn, 0, HL, 0))
            _interleave(b_proj_items(0), _ln_items(x_f, xn, HL, HL, HL), tokens=False)
            _interleave(b_proj_items(1), _band_items(seg * L, 0, qb, kb, vb, ab, eb, ob), tokens=False)
            halo[layer, 0] = kb[:, L:L + HALO, :]
            halo[layer, 1] = vb[:, L:L + HALO, :]
            _interleave([out_item(ob, 0, wob_cols, c) for c in range(4)],
                        _band_items(seg * L, HL, qb, kb, vb, ab, eb, ob), tokens=False)
            _run([out_item(ob, HL, wob_cols, c) for c in range(4)])

        @pl.when(layer == 1)
        def _():
            @pl.when(seg > 0)
            def _():
                cp_out(seg - 1).wait()

            obuf[...] = x_f[...].astype(BF)
            cp_out(seg).start()

            @pl.when(seg == 0)
            def _():
                wait(cp_xr)

            @pl.when(seg < NSEG - 1)
            def _():
                x_f[...] = xin[pl.ds(pl.multiple_of((seg + 1) * L, L), L), :].astype(F32)

        return carry

    lax.fori_loop(0, 2 * NSEG, step, 0)
    cp_out(NSEG - 1).wait()


@jax.jit
def pallas_interleave_layers__memory_aug_infini_attn__sliding_local_dilated__prompt_kernel(
    A_x: jax.Array,
    A_wq: jax.Array,
    A_wk: jax.Array,
    A_wv: jax.Array,
    A_wo: jax.Array,
    A_beta: jax.Array,
    B_x: jax.Array,
    B_wqkv: jax.Array,
    B_wo: jax.Array,
):
    del B_x
    x = A_x.reshape(S, D)
    any_spec = pl.BlockSpec(memory_space=pl.ANY)
    blk = lambda rows, dt: pltpu.VMEM((G, rows, 128), dt)
    packed = lambda rows, n=G: pltpu.VMEM((n, rows // 2, 128), U32)
    scratch = [
        pltpu.VMEM((S, D), BF),
        pltpu.VMEM((L, D), BF),
        pltpu.VMEM((L, D), F32),
        packed(L),
        packed(HL),
        packed(HL),
        blk(D, BF),
        blk(D, BF),
        blk(D, BF),
        pltpu.VMEM((D, D), BF),
        pltpu.VMEM((3, D, D), BF),
        packed(D),
        packed(3 * D),
        blk(D, BF),
        packed(D),
        pltpu.VMEM((H * PITCH, 128), F32),
        pltpu.VMEM((H * PITCH, 128), F32),
        pltpu.VMEM((H * PITCH, 128), F32),
        pltpu.VMEM((H * PITCH, 128), F32),
        packed(L),
        packed(L),
        packed(L),
        packed(L),
        packed(D, 4),
        packed(D, 4),
        packed(L),
        pltpu.VMEM((1280, 512), F32),
        pltpu.VMEM((1280, 512), F32),
        pltpu.VMEM((4, 8, 512), F32),
        pltpu.VMEM((4, 8, 512), F32),
        packed(1280, 4),
        packed(1280, 4),
        pltpu.VMEM((4, 8, 512), F32),
        pltpu.VMEM((4, 8, 512), F32),
        pltpu.VMEM((2, G, 144, 128), F32),
        pltpu.VMEM((H, 128), F32),
        blk(L, F32),
        blk(L + HALO, F32),
        blk(L + HALO, F32),
        pltpu.VMEM((2, 2, G, HALO, 128), F32),
        pltpu.VMEM((W, HL, 128), F32),
        pltpu.VMEM((W, HL, 128), F32),
        packed(L),
        pltpu.SemaphoreType.DMA((14,)),
    ]
    out = pl.pallas_call(
        _kernel,
        in_specs=[any_spec, any_spec, any_spec, any_spec, any_spec,
                  pl.BlockSpec(memory_space=pltpu.VMEM), any_spec, any_spec],
        out_specs=any_spec,
        out_shape=jax.ShapeDtypeStruct((S, D), BF),
        scratch_shapes=scratch,
        compiler_params=pltpu.CompilerParams(vmem_limit_bytes=100 * 1024 * 1024),
    )(x, A_wq, A_wk, A_wv, A_wo, A_beta, B_wqkv, B_wo)
    return out.reshape(1, S, D)
```

```python
import math

import jax
import jax.numpy as jnp
from jax import lax
import jax.experimental.pallas as pl
import jax.experimental.pallas.tpu as pltpu

S, D, H, DH = 2048, 1024, 32, 32
L, NSEG, G = 512, 4, 8
HL = L // 2
W, DIL = 8, 2
HALO = 16
BF, F32, U32 = jnp.bfloat16, jnp.float32, jnp.uint32
QSCALE = (DH ** -0.5) * math.log2(math.e)
NEG = -1e30
NT = (((1,), (1,)), ((), ()))
OFF = (0, 128, 384, 768)
SCOPES = False
PITCH = 33


class _scope:
    def __init__(self, name):
        self.cm = jax.named_scope(name) if SCOPES else None

    def __enter__(self):
        if self.cm is not None:
            self.cm.__enter__()

    def __exit__(self, *a):
        if self.cm is not None:
            self.cm.__exit__(*a)


def _dot(a, b):
    return jnp.dot(a, b, preferred_element_type=F32)


def _dot_nt(a, b):
    return lax.dot_general(a, b, NT, preferred_element_type=F32)


def _rows(r0, n, align=16):
    return slice(r0, r0 + n) if isinstance(r0, int) else pl.ds(pl.multiple_of(r0, align), n)


def _ldu(ref, b, r0, n):
    idx = slice(r0 // 2, (r0 + n) // 2) if isinstance(r0, int) else pl.ds(pl.multiple_of(r0 // 2, 8), n // 2)
    return ref.bitcast(U32)[b, idx, :]


def _ld(ref, b, r0, n, tok=None):
    u = _ldu(ref, b, r0, n)
    if tok is not None:
        u = jnp.concatenate([u[0:8] | tok, u[8:]], axis=0) if n > 16 else u | tok
    return pltpu.bitcast(u, BF)


def _st(ref, b, r0, val):
    ref[b, _rows(r0, val.shape[0]), :] = val


def _wide(ref, r0, n, tok=None):
    tok = [None] * G if tok is None else tok
    return jnp.concatenate([_ld(ref, b, r0, n, tok[b]) for b in range(G)], axis=1)


def _token(v):
    u = pltpu.bitcast(v[0:8, 0:128], U32)
    return lax.shift_right_logical(lax.shift_right_logical(u, jnp.uint32(31)), jnp.uint32(1))


def _phi(t):
    return jnp.where(t > 0, t + 1.0, jnp.exp(t))


def _ln(x):
    d = x - jnp.mean(x, axis=-1, keepdims=True)
    v = jnp.mean(d * d, axis=-1, keepdims=True)
    return d * lax.rsqrt(v + 1e-5)


def _ln_items(x_ref, xn_ref, row0, nrows, dst0, chunk=16):
    def item(r0):
        def run():
            yf = _ln(x_ref[r0:r0 + chunk, :])
            y = yf.astype(BF)
            for b in range(G):
                _st(xn_ref, b, r0 - row0 + dst0, y[:, b * 128:(b + 1) * 128])
            return _token(yf)
        return run
    return [item(r0) for r0 in range(row0, row0 + nrows, chunk)]


def _interleave(main, side, span=None, tokens=True):
    span = len(main) if span is None else span
    done = 0
    toks = None
    for i, it in enumerate(main):
        it(toks if tokens else None)
        upto = len(side) if i + 1 >= span else (len(side) * (i + 1)) // span
        group = side[done:upto]
        toks = [None] * G
        for m, s_it in enumerate(group):
            tk = s_it()
            if tk is not None:
                kbk = (m * G) // len(group)
                toks[kbk] = tk if toks[kbk] is None else toks[kbk] | tk
        done = max(done, upto)


def _run(items):
    for it in items:
        it()


def _shuffle_rows(tf, tmp, store):
    for h in range(H):
        tmp[h * PITCH:h * PITCH + DH, :] = tf[h * DH:(h + 1) * DH]
    for d in range(DH):
        for th in range(2):
            rows = tmp[pl.ds(th * 16 * PITCH + d, 16, stride=PITCH), :]
            store(d * H + th * 16, rows.astype(BF))


def _qk_stage(g, q_ref, k_ref, s_ref, m_ref):
    lane = lax.broadcasted_iota(jnp.int32, (64, 128), 1)
    key = lax.broadcasted_iota(jnp.int32, (128, 512), 0)
    qry = lax.broadcasted_iota(jnp.int32, (128, 512), 1) & 127
    causal = key <= qry
    for j in range(4):
        nk = 128 * (j + 1)
        qt = _ldu(q_ref, g, j * 128, 128)
        wq = jnp.concatenate([jnp.where((lane >> 5) == h, qt, jnp.uint32(0)) for h in range(4)], axis=0)
        st = _dot_nt(_ld(k_ref, g, 0, nk), pltpu.bitcast(wq, BF))
        diag = jnp.where(causal, st[j * 128:], NEG)
        s_ref[OFF[j] + j * 128:OFF[j] + nk, :] = diag
        m = jnp.max(diag.reshape(16, 8, 512), axis=0)
        if j > 0:
            s_ref[OFF[j]:OFF[j] + j * 128, :] = st[:j * 128]
            m = jnp.maximum(m, jnp.max(st[:j * 128].reshape(16 * j, 8, 512), axis=0))
        m_ref[j] = jnp.broadcast_to(jnp.max(m, axis=0, keepdims=True), (8, 512))


def _sm_stage(s_ref, m_ref, p_ref, l_ref, sub=16):
    for j in range(4):
        nk = 128 * (j + 1)
        for h in range(4):
            m = m_ref[j, :, h * 128:(h + 1) * 128]
            l = None
            for r in range(0, nk, sub):
                s = s_ref[OFF[j] + r:OFF[j] + r + sub, h * 128:(h + 1) * 128]
                p = jnp.exp2(s.reshape(sub // 8, 8, 128) - m[None])
                ls = jnp.sum(p, axis=0)
                l = ls if l is None else l + ls
                _st(p_ref, h, OFF[j] + r, p.reshape(sub, 128).astype(BF))
            l_ref[j, :, h * 128:(h + 1) * 128] = l


def _pv_stage(g, p_ref, l_ref, vt_ref, ot_ref, pq_ref, pk_ref, mt_ref, gate_ref):
    mem = mt_ref[g].astype(BF)
    for j in range(4):
        nd = _dot_nt(mem, _ld(pq_ref, g, j * 128, 128))
        for h in range(4):
            r0 = (g * 4 + h) * DH
            gate = gate_ref[pl.ds(g * 4 + h, 1), :]
            acc = None
            for t in range(j + 1):
                o = _dot(_ld(vt_ref, t, r0, DH), _ld(p_ref, h, OFF[j] + t * 128, 128))
                acc = o if acc is None else acc + o
            l = jnp.sum(l_ref[j, :, h * 128:(h + 1) * 128], axis=0, keepdims=True)
            den = nd[128 + h:129 + h] + 1e-6
            res = nd[h * DH:(h + 1) * DH] * (gate / den) + acc * ((1.0 - gate) / l)
            _st(ot_ref, j, r0, res.astype(BF))
    row = lax.broadcasted_iota(jnp.int32, (144, 128), 0)
    lane = lax.broadcasted_iota(jnp.int32, (144, 128), 1)
    keep = jnp.where(row < 128, row >> 5, row - 128) == (lane >> 5)
    row16 = lax.broadcasted_iota(jnp.int32, (16, 128), 0)
    ones = jnp.where(row16 < 4, 1.0, 0.0).astype(BF)
    upd = None
    for t in range(4):
        lhs = jnp.concatenate([_ld(vt_ref, t, g * 128, 128), ones], axis=0)
        u = _dot(lhs, _ld(pk_ref, g, t * 128, 128))
        upd = u if upd is None else upd + u
    mt_ref[g] = mt_ref[g] + jnp.where(keep, upd, 0.0)


def _band_items(pos0, row0, q_ref, k_ref, v_ref, a_ref, e_ref, o_ref, nrows=HL):
    def logits(r0):
        def run():
            q = [q_ref[b, r0:r0 + 8, :] for b in range(G)]
            for w in range(W):
                base = HALO + r0 - DIL * w
                acc = q[0] * k_ref[0, base:base + 8, :]
                for b in range(1, G):
                    acc = acc + q[b] * k_ref[b, base:base + 8, :]
                a_ref[w, r0 - row0:r0 - row0 + 8, :] = acc
            return _token(acc)
        return run

    def softmax(r0):
        def run():
            lg = []
            for w in range(W):
                t = a_ref[w, r0 - row0:r0 - row0 + 128, :].T
                t = ((t[0:32] + t[32:64]) + (t[64:96] + t[96:128])) * QSCALE
                if r0 == 0 and w > 0:
                    pos = pos0 - DIL * w + lax.broadcasted_iota(jnp.int32, (H, 128), 1)
                    t = jnp.where(pos >= 0, t, NEG)
                lg.append(t)
            m = lg[0]
            for w in range(1, W):
                m = jnp.maximum(m, lg[w])
            e = [jnp.exp2(x - m) for x in lg]
            l = e[0]
            for w in range(1, W):
                l = l + e[w]
            inv = 1.0 / l
            for w in range(W):
                p = e[w] * inv
                pt = jnp.concatenate([p, p, p, p], axis=0).T
                e_ref[w, r0 - row0:r0 - row0 + 128, :] = pt
            return _token(pt)
        return run

    def pv(r0):
        e = [e_ref[w, r0 - row0:r0 - row0 + 8, :] for w in range(W)]
        outs = []
        for b in range(G):
            acc = e[0] * v_ref[b, HALO + r0:HALO + r0 + 8, :]
            for w in range(1, W):
                base = HALO + r0 - DIL * w
                acc = acc + e[w] * v_ref[b, base:base + 8, :]
            outs.append(acc)
        return outs

    def pv16(r0):
        def run():
            lo = pv(r0)
            hi = pv(r0 + 8)
            for b in range(G):
                _st(o_ref, b, r0, jnp.concatenate([lo[b], hi[b]], axis=0).astype(BF))
            return _token(hi[G - 1])
        return run

    items = []
    for r0 in range(row0, row0 + nrows, 128):
        items += [logits(r) for r in range(r0, r0 + 128, 8)]
        items.append(softmax(r0))
        items += [pv16(r) for r in range(r0, r0 + 128, 16)]
    return items


def _kernel(x_hbm, wq_hbm, wk_hbm, wv_hbm, woa_hbm, beta_ref, wqkv_hbm, wob_hbm, out_hbm,
            xin, obuf, x_f, xn, xc, xnx, wq, wk, woa, wv, wqkv, wvt, wbt, wob, wobp, tmp_a, tmp_b, tmp_c, tmp_d,
            q_ref, pq_ref, k_ref, pk_ref, vt_ref, ot_ref, o_nat,
            s_a, s_b, m_a, m_b, p_a, p_b, l_a, l_b, mt_ref, gate_ref,
            qb, kb, vb, halo, ab, eb, ob, sems):

    def col_copies(src, dst, sem, c0=0, n=G):
        return [pltpu.make_async_copy(src.at[:, (c0 + i) * 128:(c0 + i + 1) * 128], dst.at[c0 + i], sem)
                for i in range(n)]

    cp_wq = [col_copies(wq_hbm, wq, sems.at[c], 2 * c, 2) for c in range(4)]
    cp_wk = col_copies(wk_hbm, wk, sems.at[4])
    cp_wv = [pltpu.make_async_copy(wv_hbm, wv, sems.at[5])]
    cp_wqkv = [[pltpu.make_async_copy(wqkv_hbm.at[:, part * D:(part + 1) * D], wqkv.at[part], sems.at[6 + part])]
               for part in range(3)]
    cp_wob = col_copies(wob_hbm, wob, sems.at[9])
    cp_woa = col_copies(woa_hbm, woa, sems.at[10])
    cp_x0 = [pltpu.make_async_copy(x_hbm.at[0:L], xin.at[0:L], sems.at[11])]
    cp_xr = [pltpu.make_async_copy(x_hbm.at[L:S], xin.at[L:S], sems.at[12])]

    def cp_out(seg):
        return pltpu.make_async_copy(obuf, out_hbm.at[pl.ds(pl.multiple_of(seg * L, L), L)], sems.at[13])

    def wait(cps):
        for c in cps:
            c.wait()

    def wcols(w_ref, c0):
        return jnp.concatenate([_ld(w_ref, c0, 0, D), _ld(w_ref, c0 + 1, 0, D)], axis=1)

    def q_item(src, n, d0, c):
        def run(tok=None):
            y = _dot(_wide(src, 0, n, tok), wcols(wq, 2 * c))
            for gg in range(2):
                yq = y[:, gg * 128:(gg + 1) * 128]
                _st(q_ref, 2 * c + gg, d0, (yq * QSCALE).astype(BF))
                _st(pq_ref, 2 * c + gg, d0, _phi(yq).astype(BF))
        return run

    def k_item(src, n, d0, c):
        def run(tok=None):
            y = _dot(_wide(src, 0, n, tok), wcols(wk, 2 * c))
            for gg in range(2):
                yk = y[:, gg * 128:(gg + 1) * 128]
                _st(k_ref, 2 * c + gg, d0, yk.astype(BF))
                _st(pk_ref, 2 * c + gg, d0, _phi(yk).astype(BF))
        return run

    def v_item(src, r0, tile0, f0):
        def run(tok=None):
            y = _dot_nt(_wide(wvt, f0, 512), _wide(src, r0, HL, tok))
            _st(vt_ref, tile0, f0, y[:, :128].astype(BF))
            _st(vt_ref, tile0 + 1, f0, y[:, 128:].astype(BF))
        return run

    def blk(i):
        return pl.ds(pl.multiple_of(i * 128, 128), 128)

    def qkv_shuffle(part, kbk, tmp):
        tf = wqkv[part, blk(kbk), :].T.astype(F32)
        _shuffle_rows(tf, tmp, lambda r, val: _st(wbt, kbk, part * D + r, val))

    with _scope("first_proj"):
        for cps in [cp_x0] + cp_wq + [cp_wv, cp_wk] + cp_wqkv + [cp_wob, cp_woa, cp_xr]:
            for c in cps:
                c.start()
        b = beta_ref[...].astype(F32).reshape(1, H)
        gt = jax.nn.sigmoid(b)
        row = lax.broadcasted_iota(jnp.int32, (H, H), 0)
        lane = lax.broadcasted_iota(jnp.int32, (H, H), 1)
        col = jnp.sum(jnp.where(row == lane, jnp.broadcast_to(gt, (H, H)), 0.0), axis=1, keepdims=True)
        gate_ref[...] = jnp.broadcast_to(col, (H, 128))
        halo[...] = jnp.zeros(halo.shape, F32)

        def zero_mem(i, c):
            mt_ref[i // G, i % G] = jnp.zeros((144, 128), F32)
            return c
        lax.fori_loop(0, 2 * G, zero_mem, 0)
        with _scope("p_wait_x"):
            wait(cp_x0)

        def ln0(i, c):
            for u in range(8):
                r0 = pl.multiple_of(i * 128 + u * 16, 16)
                x = xin[pl.ds(r0, 16), :].astype(F32)
                x_f[pl.ds(r0, 16), :] = x
                y = _ln(x).astype(BF)
                for b in range(G):
                    _st(xn, b, r0, y[:, b * 128:(b + 1) * 128])
            return c
        with _scope("p_ln"):
            lax.fori_loop(0, L // 128, ln0, 0)

        def q0(c, carry):
            for i in range(2):
                pltpu.make_async_copy(wq_hbm.at[:, 0:128], wq.at[0], sems.at[c]).wait()
            q_item(xn, L, 0, c)()
            return carry
        with _scope("p_q"):
            lax.fori_loop(0, 4, q0, 0)
        wait(cp_wv)

        def tr0(i, carry):
            for u in range(4):
                _st(wvt, 4 * i + u, 0, wv[blk(4 * i + u), :].T)
            return carry
        with _scope("p_tr"):
            lax.fori_loop(0, 2, tr0, 0)

        def v0(i, carry):
            hf = i // 2
            v_item(xn, hf * HL, 2 * hf, (i % 2) * 512)()
            return carry
        with _scope("p_v"):
            lax.fori_loop(0, 4, v0, 0)
        wait(cp_wk)
        wait(cp_wqkv[0])
        wait(cp_wqkv[1])
        tmps = (tmp_a, tmp_b, tmp_c, tmp_d)

        def k0(c, carry):
            k_item(xn, L, 0, c)()
            for u in range(4):
                qkv_shuffle(c // 2, 4 * (c % 2) + u, tmps[u])
            return carry
        with _scope("p_k"):
            lax.fori_loop(0, 4, k0, 0)
        wait(cp_wqkv[2])

        def sh0(i, carry):
            for u in range(4):
                qkv_shuffle(2, 4 * i + u, tmps[u])
            return carry
        with _scope("p_sh0"):
            lax.fori_loop(0, 2, sh0, 0)
        wait(cp_wob)

        def sh1(i, carry):
            for u in range(4):
                cb = 4 * i + u
                _shuffle_rows(wob[cb].astype(F32), tmps[u], lambda r, val, cb=cb: _st(wobp, cb, r, val))
            return carry
        with _scope("p_sh1"):
            lax.fori_loop(0, 2, sh1, 0)
        wait(cp_woa)

    def out_item(src, r0, wcol, c):
        def run(tok=None):
            rows = slice(r0, r0 + HL) if isinstance(r0, int) else pl.ds(pl.multiple_of(r0, HL), HL)
            x_f[rows, c * 256:(c + 1) * 256] += _dot(_wide(src, r0, HL, tok), wcol(c))
        return run

    woa_cols = lambda c: wcols(woa, 2 * c)
    wob_cols = lambda c: wcols(wobp, 2 * c)

    def b_proj_items(hf):
        rows = slice(hf * HL, (hf + 1) * HL)
        hrows = slice(HALO + hf * HL, HALO + (hf + 1) * HL)

        def item(part, c):
            def run(tok=None):
                y = _dot_nt(_wide(xn, hf * HL, HL, tok), _wide(wbt, part * D + c * 256, 256))
                if part == 0:
                    qb[2 * c, rows, :] = y[:, :128]
                    qb[2 * c + 1, rows, :] = y[:, 128:]
                else:
                    dst = kb if part == 1 else vb
                    dst[2 * c, hrows, :] = y[:, :128]
                    dst[2 * c + 1, hrows, :] = y[:, 128:]
            return run
        return [item(part, c) for part in range(3) for c in range(4)]

    def next_x_items(seg, layer, chunk=16):
        nxt = jnp.minimum(seg + 1, NSEG - 1) * L

        def item(r0):
            def run():
                cur = x_f[r0:r0 + chunk, :]
                obuf[r0:r0 + chunk, :] = cur.astype(BF)
                new = xin[pl.ds(pl.multiple_of(nxt + r0, chunk), chunk), :].astype(F32)
                x = jnp.where(layer == 1, new, cur)
                x_f[r0:r0 + chunk, :] = x
                yf = _ln(x)
                y = yf.astype(BF)
                for b in range(G):
                    _st(xc, b, r0, y[:, b * 128:(b + 1) * 128])
                return _token(yf)
            return run
        return [item(r0) for r0 in range(0, HL, chunk)]

    def step(t, carry):
        seg = t // 2
        layer = t % 2
        mt = mt_ref.at[layer]
        pv = lambda g, p, l: _pv_stage(g, p, l, vt_ref, ot_ref, pq_ref, pk_ref, mt, gate_ref)

        @pl.when(t > 0)
        def _():
            with _scope("A_proj"):
                def a_half(hf, c):
                    d0 = hf * HL
                    items = ([q_item(xc, HL, d0, c) for c in range(4)]
                             + [k_item(xc, HL, d0, c) for c in range(4)]
                             + [v_item(xc, 0, 2 * hf, f0) for f0 in (0, 512)])
                    _interleave(items, _ln_items(x_f, xnx, HL, HL, 0), span=8)
                    xc.bitcast(U32)[...] = xnx.bitcast(U32)[...]
                    return c

                lax.fori_loop(0, 2, a_half, 0)

        with _scope("A_attn_pro"):
            _qk_stage(0, q_ref, k_ref, s_a, m_a)
            _qk_stage(1, q_ref, k_ref, s_b, m_b)
            _sm_stage(s_a, m_a, p_a, l_a)

        def pair(u, c):
            g = 2 * u + 1
            _qk_stage(g + 1, q_ref, k_ref, s_a, m_a)
            _sm_stage(s_b, m_b, p_b, l_b)
            pv(g - 1, p_a, l_a)
            _qk_stage(g + 2, q_ref, k_ref, s_b, m_b)
            _sm_stage(s_a, m_a, p_a, l_a)
            pv(g, p_b, l_b)
            return c

        with _scope("A_attn_loop"):
            lax.fori_loop(0, 3, pair, 0)

        @pl.when(t == 0)
        def _():
            wait(cp_xr)

        @pl.when(jnp.logical_and(layer == 0, seg > 0))
        def _():
            cp_out(seg - 1).wait()

        with _scope("A_attn_epi"):
            _sm_stage(s_b, m_b, p_b, l_b)
            pv(6, p_a, l_a)
            pv(7, p_b, l_b)
            for j in range(4):
                ot = _ld(ot_ref, j, 0, D).T
                for b in range(G):
                    _st(o_nat, b, j * 128, ot[:, b * 128:(b + 1) * 128])
            kb[:, 0:HALO, :] = halo[layer, 0]
            vb[:, 0:HALO, :] = halo[layer, 1]

        def out_half(hf, c):
            toks = [it() for it in _ln_items(x_f, xn, 0, HL, 0)]
            tk = [toks[2 * i] | toks[2 * i + 1] for i in range(G)]
            items = [out_item(o_nat, hf * HL, woa_cols, c) for c in range(4)]
            items[0]()
            items[1]()
            items[2](tk)
            items[3]()
            return c

        with _scope("A_out"):
            lax.fori_loop(0, 2, out_half, 0)

        with _scope("B"):
            _interleave(b_proj_items(0), _ln_items(x_f, xn, HL, HL, HL), tokens=False)
            _interleave(b_proj_items(1), _band_items(seg * L, 0, qb, kb, vb, ab, eb, ob), tokens=False)
            halo[layer, 0] = kb[:, L:L + HALO, :]
            halo[layer, 1] = vb[:, L:L + HALO, :]
            _interleave([out_item(ob, 0, wob_cols, c) for c in range(4)],
                        _band_items(seg * L, HL, qb, kb, vb, ab, eb, ob), tokens=False)
            toks = [it() for it in next_x_items(seg, layer)]
            tk = [toks[2 * i] | toks[2 * i + 1] for i in range(G)]
            items = [out_item(ob, HL, wob_cols, c) for c in range(4)]
            items[0]()
            items[1]()
            items[2](tk)
            items[3]()

        @pl.when(layer == 1)
        def _():
            obuf[HL:L, :] = x_f[HL:L, :].astype(BF)
            cp_out(seg).start()
            x_f[HL:L, :] = xin[pl.ds(pl.multiple_of(jnp.minimum(seg + 1, NSEG - 1) * L + HL, HL), HL), :].astype(F32)

        return carry

    lax.fori_loop(0, 2 * NSEG, step, 0)
    cp_out(NSEG - 1).wait()


@jax.jit
def pallas_interleave_layers__memory_aug_infini_attn__sliding_local_dilated__prompt_kernel(
    A_x: jax.Array,
    A_wq: jax.Array,
    A_wk: jax.Array,
    A_wv: jax.Array,
    A_wo: jax.Array,
    A_beta: jax.Array,
    B_x: jax.Array,
    B_wqkv: jax.Array,
    B_wo: jax.Array,
):
    del B_x
    x = A_x.reshape(S, D)
    any_spec = pl.BlockSpec(memory_space=pl.ANY)
    blk = lambda rows, dt: pltpu.VMEM((G, rows, 128), dt)
    packed = lambda rows, n=G: pltpu.VMEM((n, rows, 128), BF)
    scratch = [
        pltpu.VMEM((S, D), BF),
        pltpu.VMEM((L, D), BF),
        pltpu.VMEM((L, D), F32),
        packed(L),
        packed(HL),
        packed(HL),
        blk(D, BF),
        blk(D, BF),
        blk(D, BF),
        pltpu.VMEM((D, D), BF),
        pltpu.VMEM((3, D, D), BF),
        packed(D),
        packed(3 * D),
        blk(D, BF),
        packed(D),
        pltpu.VMEM((H * PITCH, 128), F32),
        pltpu.VMEM((H * PITCH, 128), F32),
        pltpu.VMEM((H * PITCH, 128), F32),
        pltpu.VMEM((H * PITCH, 128), F32),
        packed(L),
        packed(L),
        packed(L),
        packed(L),
        packed(D, 4),
        packed(D, 4),
        packed(L),
        pltpu.VMEM((1280, 512), F32),
        pltpu.VMEM((1280, 512), F32),
        pltpu.VMEM((4, 8, 512), F32),
        pltpu.VMEM((4, 8, 512), F32),
        packed(1280, 4),
        packed(1280, 4),
        pltpu.VMEM((4, 8, 512), F32),
        pltpu.VMEM((4, 8, 512), F32),
        pltpu.VMEM((2, G, 144, 128), F32),
        pltpu.VMEM((H, 128), F32),
        blk(L, F32),
        blk(L + HALO, F32),
        blk(L + HALO, F32),
        pltpu.VMEM((2, 2, G, HALO, 128), F32),
        pltpu.VMEM((W, HL, 128), F32),
        pltpu.VMEM((W, HL, 128), F32),
        packed(L),
        pltpu.SemaphoreType.DMA((14,)),
    ]
    out = pl.pallas_call(
        _kernel,
        in_specs=[any_spec, any_spec, any_spec, any_spec, any_spec,
                  pl.BlockSpec(memory_space=pltpu.VMEM), any_spec, any_spec],
        out_specs=any_spec,
        out_shape=jax.ShapeDtypeStruct((S, D), BF),
        scratch_shapes=scratch,
        compiler_params=pltpu.CompilerParams(vmem_limit_bytes=100 * 1024 * 1024),
    )(x, A_wq, A_wk, A_wv, A_wo, A_beta, B_wqkv, B_wo)
    return out.reshape(1, S, D)
```

```python
import math

import jax
import jax.numpy as jnp
from jax import lax
import jax.experimental.pallas as pl
import jax.experimental.pallas.tpu as pltpu

S, D, H, DH = 2048, 1024, 32, 32
L, NSEG, G = 512, 4, 8
HL = L // 2
W, DIL = 8, 2
HALO = 16
BF, F32, U32 = jnp.bfloat16, jnp.float32, jnp.uint32
QSCALE = (DH ** -0.5) * math.log2(math.e)
NEG = -1e30
NT = (((1,), (1,)), ((), ()))
OFF = (0, 128, 384, 768)
SCOPES = False
NCH_B1 = 3
PITCH = 33


class _scope:
    def __init__(self, name):
        self.cm = jax.named_scope(name) if SCOPES else None

    def __enter__(self):
        if self.cm is not None:
            self.cm.__enter__()

    def __exit__(self, *a):
        if self.cm is not None:
            self.cm.__exit__(*a)


def _dot(a, b):
    return jnp.dot(a, b, preferred_element_type=F32)


def _dot_nt(a, b):
    return lax.dot_general(a, b, NT, preferred_element_type=F32)


def _rows(r0, n, align=16):
    return slice(r0, r0 + n) if isinstance(r0, int) else pl.ds(pl.multiple_of(r0, align), n)


def _ldu(ref, b, r0, n):
    idx = slice(r0 // 2, (r0 + n) // 2) if isinstance(r0, int) else pl.ds(pl.multiple_of(r0 // 2, 8), n // 2)
    return ref.bitcast(U32)[b, idx, :]


def _ld(ref, b, r0, n):
    return pltpu.bitcast(_ldu(ref, b, r0, n), BF)


def _st(ref, b, r0, val):
    ref[b, _rows(r0, val.shape[0]), :] = val


def _wide(ref, r0, n):
    return jnp.concatenate([_ld(ref, b, r0, n) for b in range(G)], axis=1)


class _Chain:
    def __init__(self, never, n=1):
        self.never, self.n, self.hist = never, n, []

    def link(self, x):
        if self.never is None or len(self.hist) < self.n:
            return x
        return jnp.where(self.never, self.hist[-self.n], x)

    def link_first(self, x):
        head = self.link(x[0:8, 0:128])
        if x.shape[1] > 128:
            head = jnp.concatenate([head, x[0:8, 128:]], axis=1)
        return head if x.shape[0] == 8 else jnp.concatenate([head, x[8:]], axis=0)

    def done(self, v):
        self.hist.append(v[v.shape[0] - 8:, v.shape[1] - 128:])


def _phi(t):
    return jnp.where(t > 0, t + 1.0, jnp.exp(t))


def _ln(x):
    d = x - jnp.mean(x, axis=-1, keepdims=True)
    v = jnp.mean(d * d, axis=-1, keepdims=True)
    return d * lax.rsqrt(v + 1e-5)


def _ln_items(x_ref, xn_ref, row0, nrows, dst0, ch, chunk=16):
    def item(r0):
        def run():
            yf = _ln(ch.link_first(x_ref[r0:r0 + chunk, :]))
            y = yf.astype(BF)
            for b in range(G):
                _st(xn_ref, b, r0 - row0 + dst0, y[:, b * 128:(b + 1) * 128])
            ch.done(yf)
        return run
    return [item(r0) for r0 in range(row0, row0 + nrows, chunk)]


def _interleave(main, side, span=None):
    span = len(main) if span is None else span
    done = 0
    for i, it in enumerate(main):
        upto = len(side) if i + 1 >= span else (len(side) * (i + 1)) // span
        for s_it in side[done:upto]:
            s_it()
        done = max(done, upto)
        it()


def _run(items):
    for it in items:
        it()


def _shuffle_rows(tf, tmp, store):
    for h in range(H):
        tmp[h * PITCH:h * PITCH + DH, :] = tf[h * DH:(h + 1) * DH]
    for d in range(DH):
        for th in range(2):
            rows = tmp[pl.ds(th * 16 * PITCH + d, 16, stride=PITCH), :]
            store(d * H + th * 16, rows.astype(BF))


def _qk_stage(g, q_ref, k_ref, s_ref, m_ref):
    lane = lax.broadcasted_iota(jnp.int32, (64, 128), 1)
    key = lax.broadcasted_iota(jnp.int32, (128, 512), 0)
    qry = lax.broadcasted_iota(jnp.int32, (128, 512), 1) & 127
    causal = key <= qry
    for j in range(4):
        nk = 128 * (j + 1)
        qt = _ldu(q_ref, g, j * 128, 128)
        wq = jnp.concatenate([jnp.where((lane >> 5) == h, qt, jnp.uint32(0)) for h in range(4)], axis=0)
        st = _dot_nt(_ld(k_ref, g, 0, nk), pltpu.bitcast(wq, BF))
        diag = jnp.where(causal, st[j * 128:], NEG)
        s_ref[OFF[j] + j * 128:OFF[j] + nk, :] = diag
        m = jnp.max(diag.reshape(16, 8, 512), axis=0)
        if j > 0:
            s_ref[OFF[j]:OFF[j] + j * 128, :] = st[:j * 128]
            m = jnp.maximum(m, jnp.max(st[:j * 128].reshape(16 * j, 8, 512), axis=0))
        m_ref[j] = jnp.broadcast_to(jnp.max(m, axis=0, keepdims=True), (8, 512))


def _sm_stage(s_ref, m_ref, p_ref, l_ref, sub=16):
    for j in range(4):
        nk = 128 * (j + 1)
        for h in range(4):
            m = m_ref[j, :, h * 128:(h + 1) * 128]
            l = None
            for r in range(0, nk, sub):
                s = s_ref[OFF[j] + r:OFF[j] + r + sub, h * 128:(h + 1) * 128]
                p = jnp.exp2(s.reshape(sub // 8, 8, 128) - m[None])
                ls = jnp.sum(p, axis=0)
                l = ls if l is None else l + ls
                _st(p_ref, h, OFF[j] + r, p.reshape(sub, 128).astype(BF))
            l_ref[j, :, h * 128:(h + 1) * 128] = l


def _pv_stage(g, p_ref, l_ref, vt_ref, ot_ref, pq_ref, pk_ref, mt_ref, gate_ref):
    mem = mt_ref[g].astype(BF)
    for j in range(4):
        nd = _dot_nt(mem, _ld(pq_ref, g, j * 128, 128))
        for h in range(4):
            r0 = (g * 4 + h) * DH
            gate = gate_ref[pl.ds(g * 4 + h, 1), :]
            acc = None
            for t in range(j + 1):
                o = _dot(_ld(vt_ref, t, r0, DH), _ld(p_ref, h, OFF[j] + t * 128, 128))
                acc = o if acc is None else acc + o
            l = jnp.sum(l_ref[j, :, h * 128:(h + 1) * 128], axis=0, keepdims=True)
            den = nd[128 + h:129 + h] + 1e-6
            res = nd[h * DH:(h + 1) * DH] * (gate / den) + acc * ((1.0 - gate) / l)
            _st(ot_ref, j, r0, res.astype(BF))
    row = lax.broadcasted_iota(jnp.int32, (144, 128), 0)
    lane = lax.broadcasted_iota(jnp.int32, (144, 128), 1)
    keep = jnp.where(row < 128, row >> 5, row - 128) == (lane >> 5)
    row16 = lax.broadcasted_iota(jnp.int32, (16, 128), 0)
    ones = jnp.where(row16 < 4, 1.0, 0.0).astype(BF)
    upd = None
    for t in range(4):
        lhs = jnp.concatenate([_ld(vt_ref, t, g * 128, 128), ones], axis=0)
        u = _dot(lhs, _ld(pk_ref, g, t * 128, 128))
        upd = u if upd is None else upd + u
    mt_ref[g] = mt_ref[g] + jnp.where(keep, upd, 0.0)


def _band_items(pos0, row0, q_ref, k_ref, v_ref, a_ref, e_ref, o_ref, ch, nrows=HL):
    def logits(r0):
        def run():
            q = [q_ref[b, r0:r0 + 8, :] for b in range(G)]
            for w in range(W):
                base = HALO + r0 - DIL * w
                acc = ch.link(q[0] * k_ref[0, base:base + 8, :])
                for b in range(1, G):
                    acc = acc + q[b] * k_ref[b, base:base + 8, :]
                a_ref[w, r0 - row0:r0 - row0 + 8, :] = acc
                ch.done(acc)
        return run

    def softmax(r0):
        def run():
            lg = []
            for w in range(W):
                t = a_ref[w, r0 - row0:r0 - row0 + 128, :].T
                t = ((t[0:32] + t[32:64]) + (t[64:96] + t[96:128])) * QSCALE
                if r0 == 0 and w > 0:
                    pos = pos0 - DIL * w + lax.broadcasted_iota(jnp.int32, (H, 128), 1)
                    t = jnp.where(pos >= 0, t, NEG)
                lg.append(t)
            m = lg[0]
            for w in range(1, W):
                m = jnp.maximum(m, lg[w])
            e = [jnp.exp2(x - m) for x in lg]
            l = e[0]
            for w in range(1, W):
                l = l + e[w]
            inv = 1.0 / l
            for w in range(W):
                p = e[w] * inv
                pt = jnp.concatenate([p, p, p, p], axis=0).T
                e_ref[w, r0 - row0:r0 - row0 + 128, :] = pt
        return run

    def pv(r0):
        e = [e_ref[w, r0 - row0:r0 - row0 + 8, :] for w in range(W)]
        outs = []
        for b in range(G):
            acc = ch.link(e[0] * v_ref[b, HALO + r0:HALO + r0 + 8, :])
            for w in range(1, W):
                base = HALO + r0 - DIL * w
                acc = acc + e[w] * v_ref[b, base:base + 8, :]
            outs.append(acc)
            ch.done(acc)
        return outs

    def pv16(r0):
        def run():
            lo = pv(r0)
            hi = pv(r0 + 8)
            for b in range(G):
                _st(o_ref, b, r0, jnp.concatenate([lo[b], hi[b]], axis=0).astype(BF))
        return run

    items = []
    for r0 in range(row0, row0 + nrows, 128):
        items += [logits(r) for r in range(r0, r0 + 128, 8)]
        items.append(softmax(r0))
        items += [pv16(r) for r in range(r0, r0 + 128, 16)]
    return items


def _kernel(x_hbm, wq_hbm, wk_hbm, wv_hbm, woa_hbm, beta_ref, wqkv_hbm, wob_hbm, out_hbm,
            xin, obuf, x_f, xn, xc, xnx, wq, wk, woa, wv, wqkv, wvt, wbt, wob, wobp, tmp_a, tmp_b, tmp_c, tmp_d,
            q_ref, pq_ref, k_ref, pk_ref, vt_ref, ot_ref, o_nat,
            s_a, s_b, m_a, m_b, p_a, p_b, l_a, l_b, mt_ref, gate_ref,
            qb, kb, vb, halo, ab, eb, ob, sems):

    def col_copies(src, dst, sem, c0=0, n=G):
        return [pltpu.make_async_copy(src.at[:, (c0 + i) * 128:(c0 + i + 1) * 128], dst.at[c0 + i], sem)
                for i in range(n)]

    cp_wq = [col_copies(wq_hbm, wq, sems.at[c], 2 * c, 2) for c in range(4)]
    cp_wk = col_copies(wk_hbm, wk, sems.at[4])
    cp_wv = [pltpu.make_async_copy(wv_hbm, wv, sems.at[5])]
    cp_wqkv = [[pltpu.make_async_copy(wqkv_hbm.at[:, part * D:(part + 1) * D], wqkv.at[part], sems.at[6 + part])]
               for part in range(3)]
    cp_wob = col_copies(wob_hbm, wob, sems.at[9])
    cp_woa = col_copies(woa_hbm, woa, sems.at[10])
    cp_x0 = [pltpu.make_async_copy(x_hbm.at[0:L], xin.at[0:L], sems.at[11])]
    cp_xr = [pltpu.make_async_copy(x_hbm.at[L:S], xin.at[L:S], sems.at[12])]

    def cp_out(seg):
        return pltpu.make_async_copy(obuf, out_hbm.at[pl.ds(pl.multiple_of(seg * L, L), L)], sems.at[13])

    def wait(cps):
        for c in cps:
            c.wait()

    def wcols(w_ref, c0):
        return jnp.concatenate([_ld(w_ref, c0, 0, D), _ld(w_ref, c0 + 1, 0, D)], axis=1)

    def q_item(src, n, d0, c):
        def run():
            y = _dot(_wide(src, 0, n), wcols(wq, 2 * c))
            for gg in range(2):
                yq = y[:, gg * 128:(gg + 1) * 128]
                _st(q_ref, 2 * c + gg, d0, (yq * QSCALE).astype(BF))
                _st(pq_ref, 2 * c + gg, d0, _phi(yq).astype(BF))
        return run

    def k_item(src, n, d0, c):
        def run():
            y = _dot(_wide(src, 0, n), wcols(wk, 2 * c))
            for gg in range(2):
                yk = y[:, gg * 128:(gg + 1) * 128]
                _st(k_ref, 2 * c + gg, d0, yk.astype(BF))
                _st(pk_ref, 2 * c + gg, d0, _phi(yk).astype(BF))
        return run

    def v_item(src, r0, tile0, f0):
        def run():
            y = _dot_nt(_wide(wvt, f0, 512), _wide(src, r0, HL))
            _st(vt_ref, tile0, f0, y[:, :128].astype(BF))
            _st(vt_ref, tile0 + 1, f0, y[:, 128:].astype(BF))
        return run

    def blk(i):
        return pl.ds(pl.multiple_of(i * 128, 128), 128)

    def qkv_shuffle(part, kbk, tmp):
        tf = wqkv[part, blk(kbk), :].T.astype(F32)
        _shuffle_rows(tf, tmp, lambda r, val: _st(wbt, kbk, part * D + r, val))

    with _scope("first_proj"):
        for cps in [cp_x0] + cp_wq + [cp_wv, cp_wk] + cp_wqkv + [cp_wob, cp_woa, cp_xr]:
            for c in cps:
                c.start()
        b = beta_ref[...].astype(F32).reshape(1, H)
        gt = jax.nn.sigmoid(b)
        row = lax.broadcasted_iota(jnp.int32, (H, H), 0)
        lane = lax.broadcasted_iota(jnp.int32, (H, H), 1)
        col = jnp.sum(jnp.where(row == lane, jnp.broadcast_to(gt, (H, H)), 0.0), axis=1, keepdims=True)
        gate_ref[...] = jnp.broadcast_to(col, (H, 128))
        halo[...] = jnp.zeros(halo.shape, F32)

        def zero_mem(i, c):
            mt_ref[i // G, i % G] = jnp.zeros((144, 128), F32)
            return c
        lax.fori_loop(0, 2 * G, zero_mem, 0)
        with _scope("p_wait_x"):
            wait(cp_x0)

        def ln0(i, c):
            for u in range(8):
                r0 = pl.multiple_of(i * 128 + u * 16, 16)
                x = xin[pl.ds(r0, 16), :].astype(F32)
                x_f[pl.ds(r0, 16), :] = x
                y = _ln(x).astype(BF)
                for b in range(G):
                    _st(xn, b, r0, y[:, b * 128:(b + 1) * 128])
            return c
        with _scope("p_ln"):
            lax.fori_loop(0, L // 128, ln0, 0)

        def q0(c, carry):
            for i in range(2):
                pltpu.make_async_copy(wq_hbm.at[:, 0:128], wq.at[0], sems.at[c]).wait()
            q_item(xn, L, 0, c)()
            return carry
        with _scope("p_q"):
            lax.fori_loop(0, 4, q0, 0)
        wait(cp_wv)

        def tr0(i, carry):
            for u in range(4):
                _st(wvt, 4 * i + u, 0, wv[blk(4 * i + u), :].T)
            return carry
        with _scope("p_tr"):
            lax.fori_loop(0, 2, tr0, 0)

        def v0(i, carry):
            hf = i // 2
            v_item(xn, hf * HL, 2 * hf, (i % 2) * 512)()
            return carry
        with _scope("p_v"):
            lax.fori_loop(0, 4, v0, 0)
        wait(cp_wk)
        wait(cp_wqkv[0])
        wait(cp_wqkv[1])
        tmps = (tmp_a, tmp_b, tmp_c, tmp_d)

        def k0(c, carry):
            k_item(xn, L, 0, c)()
            for u in range(4):
                qkv_shuffle(c // 2, 4 * (c % 2) + u, tmps[u])
            return carry
        with _scope("p_k"):
            lax.fori_loop(0, 4, k0, 0)
        wait(cp_wqkv[2])

        def sh0(i, carry):
            for u in range(4):
                qkv_shuffle(2, 4 * i + u, tmps[u])
            return carry
        with _scope("p_sh0"):
            lax.fori_loop(0, 2, sh0, 0)
        wait(cp_wob)

        def sh1(i, carry):
            for u in range(4):
                cb = 4 * i + u
                _shuffle_rows(wob[cb].astype(F32), tmps[u], lambda r, val, cb=cb: _st(wobp, cb, r, val))
            return carry
        with _scope("p_sh1"):
            lax.fori_loop(0, 2, sh1, 0)
        wait(cp_woa)

    def out_item(src, r0, wcol, c):
        def run():
            rows = slice(r0, r0 + HL) if isinstance(r0, int) else pl.ds(pl.multiple_of(r0, HL), HL)
            x_f[rows, c * 256:(c + 1) * 256] += _dot(_wide(src, r0, HL), wcol(c))
        return run

    woa_cols = lambda c: wcols(woa, 2 * c)
    wob_cols = lambda c: wcols(wobp, 2 * c)

    def b_proj_items(hf):
        rows = slice(hf * HL, (hf + 1) * HL)
        hrows = slice(HALO + hf * HL, HALO + (hf + 1) * HL)

        def item(part, c):
            def run():
                y = _dot_nt(_wide(xn, hf * HL, HL), _wide(wbt, part * D + c * 256, 256))
                if part == 0:
                    qb[2 * c, rows, :] = y[:, :128]
                    qb[2 * c + 1, rows, :] = y[:, 128:]
                else:
                    dst = kb if part == 1 else vb
                    dst[2 * c, hrows, :] = y[:, :128]
                    dst[2 * c + 1, hrows, :] = y[:, 128:]
            return run
        return [item(part, c) for part in range(3) for c in range(4)]

    def next_x_items(seg, layer, ch, chunk=16):
        nxt = jnp.minimum(seg + 1, NSEG - 1) * L

        def item(r0):
            def run():
                cur = ch.link_first(x_f[r0:r0 + chunk, :])
                obuf[r0:r0 + chunk, :] = cur.astype(BF)
                new = xin[pl.ds(pl.multiple_of(nxt + r0, chunk), chunk), :].astype(F32)
                x = jnp.where(layer == 1, new, cur)
                x_f[r0:r0 + chunk, :] = x
                yf = _ln(x)
                y = yf.astype(BF)
                for b in range(G):
                    _st(xc, b, r0, y[:, b * 128:(b + 1) * 128])
                ch.done(yf)
            return run
        return [item(r0) for r0 in range(0, HL, chunk)]

    def step(t, carry):
        seg = t // 2
        layer = t % 2
        mt = mt_ref.at[layer]
        never = lax.broadcasted_iota(jnp.int32, (8, 128), 0) < -t
        pv = lambda g, p, l: _pv_stage(g, p, l, vt_ref, ot_ref, pq_ref, pk_ref, mt, gate_ref)

        @pl.when(t > 0)
        def _():
            with _scope("A_proj"):
                def a_half(hf, c):
                    d0 = hf * HL
                    items = ([q_item(xc, HL, d0, c) for c in range(4)]
                             + [k_item(xc, HL, d0, c) for c in range(4)]
                             + [v_item(xc, 0, 2 * hf, f0) for f0 in (0, 512)])
                    _interleave(items, _ln_items(x_f, xnx, HL, HL, 0, _Chain(never)), span=8)
                    xc.bitcast(U32)[...] = xnx.bitcast(U32)[...]
                    return c

                lax.fori_loop(0, 2, a_half, 0)

        with _scope("A_attn_pro"):
            _qk_stage(0, q_ref, k_ref, s_a, m_a)
            _qk_stage(1, q_ref, k_ref, s_b, m_b)
            _sm_stage(s_a, m_a, p_a, l_a)

        def pair(u, c):
            g = 2 * u + 1
            _qk_stage(g + 1, q_ref, k_ref, s_a, m_a)
            _sm_stage(s_b, m_b, p_b, l_b)
            pv(g - 1, p_a, l_a)
            _qk_stage(g + 2, q_ref, k_ref, s_b, m_b)
            _sm_stage(s_a, m_a, p_a, l_a)
            pv(g, p_b, l_b)
            return c

        with _scope("A_attn_loop"):
            lax.fori_loop(0, 3, pair, 0)

        @pl.when(t == 0)
        def _():
            wait(cp_xr)

        @pl.when(jnp.logical_and(layer == 0, seg > 0))
        def _():
            cp_out(seg - 1).wait()

        with _scope("A_attn_epi"):
            _sm_stage(s_b, m_b, p_b, l_b)
            pv(6, p_a, l_a)
            pv(7, p_b, l_b)
            for j in range(4):
                ot = _ld(ot_ref, j, 0, D).T
                for b in range(G):
                    _st(o_nat, b, j * 128, ot[:, b * 128:(b + 1) * 128])
            kb[:, 0:HALO, :] = halo[layer, 0]
            vb[:, 0:HALO, :] = halo[layer, 1]

        def out_half(hf, c):
            _run(_ln_items(x_f, xn, 0, HL, 0, _Chain(never, 2)))
            _run([out_item(o_nat, hf * HL, woa_cols, c) for c in range(4)])
            return c

        with _scope("A_out"):
            lax.fori_loop(0, 2, out_half, 0)

        with _scope("B"):
            _interleave(b_proj_items(0), _ln_items(x_f, xn, HL, HL, HL, _Chain(never)))
            _interleave(b_proj_items(1), _band_items(seg * L, 0, qb, kb, vb, ab, eb, ob, _Chain(never)))
            halo[layer, 0] = kb[:, L:L + HALO, :]
            halo[layer, 1] = vb[:, L:L + HALO, :]
            _interleave([out_item(ob, 0, wob_cols, c) for c in range(4)],
                        _band_items(seg * L, HL, qb, kb, vb, ab, eb, ob, _Chain(never, NCH_B1)))
            _run(next_x_items(seg, layer, _Chain(never, 2)))
            _run([out_item(ob, HL, wob_cols, c) for c in range(4)])

        @pl.when(layer == 1)
        def _():
            obuf[HL:L, :] = x_f[HL:L, :].astype(BF)
            cp_out(seg).start()
            x_f[HL:L, :] = xin[pl.ds(pl.multiple_of(jnp.minimum(seg + 1, NSEG - 1) * L + HL, HL), HL), :].astype(F32)

        return carry

    lax.fori_loop(0, 2 * NSEG, step, 0)
    cp_out(NSEG - 1).wait()


@jax.jit
def pallas_interleave_layers__memory_aug_infini_attn__sliding_local_dilated__prompt_kernel(
    A_x: jax.Array,
    A_wq: jax.Array,
    A_wk: jax.Array,
    A_wv: jax.Array,
    A_wo: jax.Array,
    A_beta: jax.Array,
    B_x: jax.Array,
    B_wqkv: jax.Array,
    B_wo: jax.Array,
):
    del B_x
    x = A_x.reshape(S, D)
    any_spec = pl.BlockSpec(memory_space=pl.ANY)
    blk = lambda rows, dt: pltpu.VMEM((G, rows, 128), dt)
    packed = lambda rows, n=G: pltpu.VMEM((n, rows, 128), BF)
    scratch = [
        pltpu.VMEM((S, D), BF),
        pltpu.VMEM((L, D), BF),
        pltpu.VMEM((L, D), F32),
        packed(L),
        packed(HL),
        packed(HL),
        blk(D, BF),
        blk(D, BF),
        blk(D, BF),
        pltpu.VMEM((D, D), BF),
        pltpu.VMEM((3, D, D), BF),
        packed(D),
        packed(3 * D),
        blk(D, BF),
        packed(D),
        pltpu.VMEM((H * PITCH, 128), F32),
        pltpu.VMEM((H * PITCH, 128), F32),
        pltpu.VMEM((H * PITCH, 128), F32),
        pltpu.VMEM((H * PITCH, 128), F32),
        packed(L),
        packed(L),
        packed(L),
        packed(L),
        packed(D, 4),
        packed(D, 4),
        packed(L),
        pltpu.VMEM((1280, 512), F32),
        pltpu.VMEM((1280, 512), F32),
        pltpu.VMEM((4, 8, 512), F32),
        pltpu.VMEM((4, 8, 512), F32),
        packed(1280, 4),
        packed(1280, 4),
        pltpu.VMEM((4, 8, 512), F32),
        pltpu.VMEM((4, 8, 512), F32),
        pltpu.VMEM((2, G, 144, 128), F32),
        pltpu.VMEM((H, 128), F32),
        blk(L, F32),
        blk(L + HALO, F32),
        blk(L + HALO, F32),
        pltpu.VMEM((2, 2, G, HALO, 128), F32),
        pltpu.VMEM((W, HL, 128), F32),
        pltpu.VMEM((W, HL, 128), F32),
        packed(L),
        pltpu.SemaphoreType.DMA((14,)),
    ]
    out = pl.pallas_call(
        _kernel,
        in_specs=[any_spec, any_spec, any_spec, any_spec, any_spec,
                  pl.BlockSpec(memory_space=pltpu.VMEM), any_spec, any_spec],
        out_specs=any_spec,
        out_shape=jax.ShapeDtypeStruct((S, D), BF),
        scratch_shapes=scratch,
        compiler_params=pltpu.CompilerParams(vmem_limit_bytes=100 * 1024 * 1024),
    )(x, A_wq, A_wk, A_wv, A_wo, A_beta, B_wqkv, B_wo)
    return out.reshape(1, S, D)
```

```python
import math

import jax
import jax.numpy as jnp
from jax import lax
import jax.experimental.pallas as pl
import jax.experimental.pallas.tpu as pltpu

S, D, H, DH = 2048, 1024, 32, 32
L, NSEG, G = 512, 4, 8
HL = L // 2
W, DIL = 8, 2
HALO = 16
BF, F32, U32 = jnp.bfloat16, jnp.float32, jnp.uint32
QSCALE = (DH ** -0.5) * math.log2(math.e)
NEG = -1e30
NT = (((1,), (1,)), ((), ()))
OFF = (0, 128, 384, 768)
SCOPES = False
NCH_B1 = 3
PITCH = 33


class _scope:
    def __init__(self, name):
        self.cm = jax.named_scope(name) if SCOPES else None

    def __enter__(self):
        if self.cm is not None:
            self.cm.__enter__()

    def __exit__(self, *a):
        if self.cm is not None:
            self.cm.__exit__(*a)


def _dot(a, b):
    return jnp.dot(a, b, preferred_element_type=F32)


def _dot_nt(a, b):
    return lax.dot_general(a, b, NT, preferred_element_type=F32)


def _rows(r0, n, align=16):
    return slice(r0, r0 + n) if isinstance(r0, int) else pl.ds(pl.multiple_of(r0, align), n)


def _ldu(ref, b, r0, n):
    idx = slice(r0 // 2, (r0 + n) // 2) if isinstance(r0, int) else pl.ds(pl.multiple_of(r0 // 2, 8), n // 2)
    return ref.bitcast(U32)[b, idx, :]


def _ld(ref, b, r0, n):
    return pltpu.bitcast(_ldu(ref, b, r0, n), BF)


def _st(ref, b, r0, val):
    ref[b, _rows(r0, val.shape[0]), :] = val


def _wide(ref, r0, n):
    return jnp.concatenate([_ld(ref, b, r0, n) for b in range(G)], axis=1)


class _Chain:
    def __init__(self, never, n=1):
        self.never, self.n, self.hist = never, n, []

    def link(self, x):
        if self.never is None or len(self.hist) < self.n:
            return x
        return jnp.where(self.never, self.hist[-self.n], x)

    def link_first(self, x):
        head = self.link(x[0:8, 0:128])
        if x.shape[1] > 128:
            head = jnp.concatenate([head, x[0:8, 128:]], axis=1)
        return head if x.shape[0] == 8 else jnp.concatenate([head, x[8:]], axis=0)

    def done(self, v):
        self.hist.append(v[v.shape[0] - 8:, v.shape[1] - 128:])


def _phi(t):
    return jnp.where(t > 0, t + 1.0, jnp.exp(t))


def _ln(x):
    d = x - jnp.mean(x, axis=-1, keepdims=True)
    v = jnp.mean(d * d, axis=-1, keepdims=True)
    return d * lax.rsqrt(v + 1e-5)


def _ln_items(x_ref, xn_ref, row0, nrows, dst0, ch, chunk=16):
    def item(r0):
        def run():
            yf = _ln(ch.link_first(x_ref[r0:r0 + chunk, :]))
            y = yf.astype(BF)
            for b in range(G):
                _st(xn_ref, b, r0 - row0 + dst0, y[:, b * 128:(b + 1) * 128])
            ch.done(yf)
        return run
    return [item(r0) for r0 in range(row0, row0 + nrows, chunk)]


def _interleave(main, side, span=None):
    span = len(main) if span is None else span
    done = 0
    for i, it in enumerate(main):
        upto = len(side) if i + 1 >= span else (len(side) * (i + 1)) // span
        for s_it in side[done:upto]:
            s_it()
        done = max(done, upto)
        it()


def _run(items):
    for it in items:
        it()


def _shuffle_rows(tf, tmp, store):
    for h in range(H):
        tmp[h * PITCH:h * PITCH + DH, :] = tf[h * DH:(h + 1) * DH]
    for d in range(DH):
        for th in range(2):
            rows = tmp[pl.ds(th * 16 * PITCH + d, 16, stride=PITCH), :]
            store(d * H + th * 16, rows.astype(BF))


def _qk_stage(g, q_ref, k_ref, s_ref, m_ref):
    lane = lax.broadcasted_iota(jnp.int32, (64, 128), 1)
    key = lax.broadcasted_iota(jnp.int32, (128, 512), 0)
    qry = lax.broadcasted_iota(jnp.int32, (128, 512), 1) & 127
    causal = key <= qry
    for j in range(4):
        nk = 128 * (j + 1)
        qt = _ldu(q_ref, g, j * 128, 128)
        wq = jnp.concatenate([jnp.where((lane >> 5) == h, qt, jnp.uint32(0)) for h in range(4)], axis=0)
        st = _dot_nt(_ld(k_ref, g, 0, nk), pltpu.bitcast(wq, BF))
        diag = jnp.where(causal, st[j * 128:], NEG)
        s_ref[OFF[j] + j * 128:OFF[j] + nk, :] = diag
        m = jnp.max(diag.reshape(16, 8, 512), axis=0)
        if j > 0:
            s_ref[OFF[j]:OFF[j] + j * 128, :] = st[:j * 128]
            m = jnp.maximum(m, jnp.max(st[:j * 128].reshape(16 * j, 8, 512), axis=0))
        m_ref[j] = jnp.broadcast_to(jnp.max(m, axis=0, keepdims=True), (8, 512))


def _sm_stage(s_ref, m_ref, p_ref, l_ref, sub=16):
    for j in range(4):
        nk = 128 * (j + 1)
        for h in range(4):
            m = m_ref[j, :, h * 128:(h + 1) * 128]
            l = None
            for r in range(0, nk, sub):
                s = s_ref[OFF[j] + r:OFF[j] + r + sub, h * 128:(h + 1) * 128]
                p = jnp.exp2(s.reshape(sub // 8, 8, 128) - m[None])
                ls = jnp.sum(p, axis=0)
                l = ls if l is None else l + ls
                _st(p_ref, h, OFF[j] + r, p.reshape(sub, 128).astype(BF))
            l_ref[j, :, h * 128:(h + 1) * 128] = l


def _pv_stage(g, p_ref, l_ref, vt_ref, ot_ref, pq_ref, pk_ref, mt_ref, gate_ref):
    mem = mt_ref[g].astype(BF)
    for j in range(4):
        nd = _dot_nt(mem, _ld(pq_ref, g, j * 128, 128))
        for h in range(4):
            r0 = (g * 4 + h) * DH
            gate = gate_ref[pl.ds(g * 4 + h, 1), :]
            acc = None
            for t in range(j + 1):
                o = _dot(_ld(vt_ref, t, r0, DH), _ld(p_ref, h, OFF[j] + t * 128, 128))
                acc = o if acc is None else acc + o
            l = jnp.sum(l_ref[j, :, h * 128:(h + 1) * 128], axis=0, keepdims=True)
            den = nd[128 + h:129 + h] + 1e-6
            res = nd[h * DH:(h + 1) * DH] * (gate / den) + acc * ((1.0 - gate) / l)
            _st(ot_ref, j, r0, res.astype(BF))
    row = lax.broadcasted_iota(jnp.int32, (144, 128), 0)
    lane = lax.broadcasted_iota(jnp.int32, (144, 128), 1)
    keep = jnp.where(row < 128, row >> 5, row - 128) == (lane >> 5)
    row16 = lax.broadcasted_iota(jnp.int32, (16, 128), 0)
    ones = jnp.where(row16 < 4, 1.0, 0.0).astype(BF)
    upd = None
    for t in range(4):
        lhs = jnp.concatenate([_ld(vt_ref, t, g * 128, 128), ones], axis=0)
        u = _dot(lhs, _ld(pk_ref, g, t * 128, 128))
        upd = u if upd is None else upd + u
    mt_ref[g] = mt_ref[g] + jnp.where(keep, upd, 0.0)


def _band_items(pos0, row0, q_ref, k_ref, v_ref, a_ref, e_ref, o_ref, ch, nrows=HL):
    def logits(r0):
        def run():
            q = [q_ref[b, r0:r0 + 8, :] for b in range(G)]
            for w in range(W):
                base = HALO + r0 - DIL * w
                acc = ch.link(q[0] * k_ref[0, base:base + 8, :])
                for b in range(1, G):
                    acc = acc + q[b] * k_ref[b, base:base + 8, :]
                a_ref[w, r0 - row0:r0 - row0 + 8, :] = acc
                ch.done(acc)
        return run

    def softmax(r0):
        def run():
            lg = []
            for w in range(W):
                t = a_ref[w, r0 - row0:r0 - row0 + 128, :].T
                t = ((t[0:32] + t[32:64]) + (t[64:96] + t[96:128])) * QSCALE
                if r0 == row0 and w > 0:
                    pos = pos0 - DIL * w + lax.broadcasted_iota(jnp.int32, (H, 128), 1)
                    t = jnp.where(pos >= 0, t, NEG)
                lg.append(t)
            m = lg[0]
            for w in range(1, W):
                m = jnp.maximum(m, lg[w])
            e = [jnp.exp2(x - m) for x in lg]
            l = e[0]
            for w in range(1, W):
                l = l + e[w]
            inv = 1.0 / l
            for w in range(W):
                p = e[w] * inv
                pt = jnp.concatenate([p, p, p, p], axis=0).T
                e_ref[w, r0 - row0:r0 - row0 + 128, :] = pt
        return run

    def pv(r0):
        e = [e_ref[w, r0 - row0:r0 - row0 + 8, :] for w in range(W)]
        outs = []
        for b in range(G):
            acc = ch.link(e[0] * v_ref[b, HALO + r0:HALO + r0 + 8, :])
            for w in range(1, W):
                base = HALO + r0 - DIL * w
                acc = acc + e[w] * v_ref[b, base:base + 8, :]
            outs.append(acc)
            ch.done(acc)
        return outs

    def pv16(r0):
        def run():
            lo = pv(r0)
            hi = pv(r0 + 8)
            for b in range(G):
                _st(o_ref, b, r0, jnp.concatenate([lo[b], hi[b]], axis=0).astype(BF))
        return run

    items = []
    for r0 in range(row0, row0 + nrows, 128):
        items += [logits(r) for r in range(r0, r0 + 128, 8)]
        items.append(softmax(r0))
        items += [pv16(r) for r in range(r0, r0 + 128, 16)]
    return items


def _kernel(x_hbm, wq_hbm, wk_hbm, wv_hbm, woa_hbm, beta_ref, wqkv_hbm, wob_hbm, out_hbm,
            xin, obuf, x_f, xn, xc, xnx, wq, wk, woa, wv, wqkv, wvt, wbt, wob, wobp, tmp_a, tmp_b, tmp_c, tmp_d,
            q_ref, pq_ref, k_ref, pk_ref, vt_ref, ot_ref, o_nat,
            s_a, s_b, m_a, m_b, p_a, p_b, l_a, l_b, mt_ref, gate_ref,
            qn, kn, vn, qo, ko, vo, halo, ab, eb, ob0, ob1, sems):

    def col_copies(src, dst, sem, c0=0, n=G):
        return [pltpu.make_async_copy(src.at[:, (c0 + i) * 128:(c0 + i + 1) * 128], dst.at[c0 + i], sem)
                for i in range(n)]

    cp_wq = [col_copies(wq_hbm, wq, sems.at[c], 2 * c, 2) for c in range(4)]
    cp_wk = col_copies(wk_hbm, wk, sems.at[4])
    cp_wv = [pltpu.make_async_copy(wv_hbm, wv, sems.at[5])]
    cp_wqkv = [[pltpu.make_async_copy(wqkv_hbm.at[:, part * D:(part + 1) * D], wqkv.at[part], sems.at[6 + part])]
               for part in range(3)]
    cp_wob = col_copies(wob_hbm, wob, sems.at[9])
    cp_woa = col_copies(woa_hbm, woa, sems.at[10])
    cp_x0 = [pltpu.make_async_copy(x_hbm.at[0:L], xin.at[0:L], sems.at[11])]
    cp_xr = [pltpu.make_async_copy(x_hbm.at[L:S], xin.at[L:S], sems.at[12])]

    def cp_out(seg):
        return pltpu.make_async_copy(obuf, out_hbm.at[pl.ds(pl.multiple_of(seg * L, L), L)], sems.at[13])

    def wait(cps):
        for c in cps:
            c.wait()

    def wcols(w_ref, c0):
        return jnp.concatenate([_ld(w_ref, c0, 0, D), _ld(w_ref, c0 + 1, 0, D)], axis=1)

    def q_item(src, n, d0, c):
        def run():
            y = _dot(_wide(src, 0, n), wcols(wq, 2 * c))
            for gg in range(2):
                yq = y[:, gg * 128:(gg + 1) * 128]
                _st(q_ref, 2 * c + gg, d0, (yq * QSCALE).astype(BF))
                _st(pq_ref, 2 * c + gg, d0, _phi(yq).astype(BF))
        return run

    def k_item(src, n, d0, c):
        def run():
            y = _dot(_wide(src, 0, n), wcols(wk, 2 * c))
            for gg in range(2):
                yk = y[:, gg * 128:(gg + 1) * 128]
                _st(k_ref, 2 * c + gg, d0, yk.astype(BF))
                _st(pk_ref, 2 * c + gg, d0, _phi(yk).astype(BF))
        return run

    def v_item(src, r0, tile0, f0):
        def run():
            y = _dot_nt(_wide(wvt, f0, 512), _wide(src, r0, HL))
            _st(vt_ref, tile0, f0, y[:, :128].astype(BF))
            _st(vt_ref, tile0 + 1, f0, y[:, 128:].astype(BF))
        return run

    def blk(i):
        return pl.ds(pl.multiple_of(i * 128, 128), 128)

    def qkv_shuffle(part, kbk, tmp):
        tf = wqkv[part, blk(kbk), :].T.astype(F32)
        _shuffle_rows(tf, tmp, lambda r, val: _st(wbt, kbk, part * D + r, val))

    with _scope("first_proj"):
        for cps in [cp_x0] + cp_wq + [cp_wv, cp_wk] + cp_wqkv + [cp_wob, cp_woa, cp_xr]:
            for c in cps:
                c.start()
        b = beta_ref[...].astype(F32).reshape(1, H)
        gt = jax.nn.sigmoid(b)
        row = lax.broadcasted_iota(jnp.int32, (H, H), 0)
        lane = lax.broadcasted_iota(jnp.int32, (H, H), 1)
        col = jnp.sum(jnp.where(row == lane, jnp.broadcast_to(gt, (H, H)), 0.0), axis=1, keepdims=True)
        gate_ref[...] = jnp.broadcast_to(col, (H, 128))
        halo[...] = jnp.zeros(halo.shape, F32)

        def zero_b(b, c):
            for r in (qn, kn, vn, ko, vo):
                r[b] = jnp.zeros(r.shape[1:], F32)
            return c
        lax.fori_loop(0, G, zero_b, 0)

        def zero_mem(i, c):
            mt_ref[i // G, i % G] = jnp.zeros((144, 128), F32)
            return c
        lax.fori_loop(0, 2 * G, zero_mem, 0)
        with _scope("p_wait_x"):
            wait(cp_x0)

        def ln0(i, c):
            for u in range(8):
                r0 = pl.multiple_of(i * 128 + u * 16, 16)
                x = xin[pl.ds(r0, 16), :].astype(F32)
                x_f[pl.ds(r0, 16), :] = x
                y = _ln(x).astype(BF)
                for b in range(G):
                    _st(xn, b, r0, y[:, b * 128:(b + 1) * 128])
            return c
        with _scope("p_ln"):
            lax.fori_loop(0, L // 128, ln0, 0)

        def q0(c, carry):
            for i in range(2):
                pltpu.make_async_copy(wq_hbm.at[:, 0:128], wq.at[0], sems.at[c]).wait()
            q_item(xn, L, 0, c)()
            return carry
        with _scope("p_q"):
            lax.fori_loop(0, 4, q0, 0)
        wait(cp_wv)

        def tr0(i, carry):
            for u in range(4):
                _st(wvt, 4 * i + u, 0, wv[blk(4 * i + u), :].T)
            return carry
        with _scope("p_tr"):
            lax.fori_loop(0, 2, tr0, 0)

        def v0(i, carry):
            hf = i // 2
            v_item(xn, hf * HL, 2 * hf, (i % 2) * 512)()
            return carry
        with _scope("p_v"):
            lax.fori_loop(0, 4, v0, 0)
        wait(cp_wk)
        wait(cp_wqkv[0])
        wait(cp_wqkv[1])
        tmps = (tmp_a, tmp_b, tmp_c, tmp_d)

        def k0(c, carry):
            k_item(xn, L, 0, c)()
            for u in range(4):
                qkv_shuffle(c // 2, 4 * (c % 2) + u, tmps[u])
            return carry
        with _scope("p_k"):
            lax.fori_loop(0, 4, k0, 0)
        wait(cp_wqkv[2])

        def sh0(i, carry):
            for u in range(4):
                qkv_shuffle(2, 4 * i + u, tmps[u])
            return carry
        with _scope("p_sh0"):
            lax.fori_loop(0, 2, sh0, 0)
        wait(cp_wob)

        def sh1(i, carry):
            for u in range(4):
                cb = 4 * i + u
                _shuffle_rows(wob[cb].astype(F32), tmps[u], lambda r, val, cb=cb: _st(wobp, cb, r, val))
            return carry
        with _scope("p_sh1"):
            lax.fori_loop(0, 2, sh1, 0)
        wait(cp_woa)

    def out_item(src, s0, r0, wcol, c):
        def run():
            x_f[r0:r0 + HL, c * 256:(c + 1) * 256] += _dot(_wide(src, s0, HL), wcol(c))
        return run

    woa_cols = lambda c: wcols(woa, 2 * c)
    wob_cols = lambda c: wcols(wobp, 2 * c)

    def b_proj_items():
        def item(part, c):
            def run():
                y = _dot_nt(_wide(xc, 0, HL), _wide(wbt, part * D + c * 256, 256))
                dst = (qn, kn, vn)[part]
                dst[2 * c] = y[:, :128]
                dst[2 * c + 1] = y[:, 128:]
            return run
        return [item(part, c) for part in range(3) for c in range(4)]

    def b_rotate():
        for b in range(G):
            qo[b] = qn[b]
            for new, old in ((kn, ko), (vn, vo)):
                old[b, 0:HALO, :] = old[b, HL:HL + HALO, :]
                old[b, HALO:, :] = new[b]

    def next_x_items(seg, layer, ch, chunk=16):
        nxt = jnp.minimum(seg + 1, NSEG - 1) * L

        def item(r0):
            def run():
                cur = ch.link_first(x_f[r0:r0 + chunk, :])
                obuf[r0:r0 + chunk, :] = cur.astype(BF)
                new = xin[pl.ds(pl.multiple_of(nxt + r0, chunk), chunk), :].astype(F32)
                x = jnp.where(layer == 1, new, cur)
                x_f[r0:r0 + chunk, :] = x
                yf = _ln(x)
                y = yf.astype(BF)
                for b in range(G):
                    _st(xc, b, r0, y[:, b * 128:(b + 1) * 128])
                ch.done(yf)
            return run
        return [item(r0) for r0 in range(0, HL, chunk)]

    def step(t, carry):
        seg = t // 2
        layer = t % 2
        mt = mt_ref.at[layer]
        never = lax.broadcasted_iota(jnp.int32, (8, 128), 0) < -t
        pv = lambda g, p, l: _pv_stage(g, p, l, vt_ref, ot_ref, pq_ref, pk_ref, mt, gate_ref)

        @pl.when(t > 0)
        def _():
            with _scope("A_proj"):
                def a_half(hf, c):
                    d0 = hf * HL
                    items = ([q_item(xc, HL, d0, c) for c in range(4)]
                             + [k_item(xc, HL, d0, c) for c in range(4)]
                             + [v_item(xc, 0, 2 * hf, f0) for f0 in (0, 512)])
                    _interleave(items, _ln_items(x_f, xnx, HL, HL, 0, _Chain(never)), span=8)
                    xc.bitcast(U32)[...] = xnx.bitcast(U32)[...]
                    return c

                lax.fori_loop(0, 2, a_half, 0)

        with _scope("A_attn_pro"):
            _qk_stage(0, q_ref, k_ref, s_a, m_a)
            _qk_stage(1, q_ref, k_ref, s_b, m_b)
            _sm_stage(s_a, m_a, p_a, l_a)

        def pair(u, c):
            g = 2 * u + 1
            _qk_stage(g + 1, q_ref, k_ref, s_a, m_a)
            _sm_stage(s_b, m_b, p_b, l_b)
            pv(g - 1, p_a, l_a)
            _qk_stage(g + 2, q_ref, k_ref, s_b, m_b)
            _sm_stage(s_a, m_a, p_a, l_a)
            pv(g, p_b, l_b)
            return c

        with _scope("A_attn_loop"):
            lax.fori_loop(0, 3, pair, 0)

        @pl.when(t == 0)
        def _():
            wait(cp_xr)

        @pl.when(jnp.logical_and(layer == 0, seg > 0))
        def _():
            cp_out(seg - 1).wait()

        with _scope("A_attn_epi"):
            _sm_stage(s_b, m_b, p_b, l_b)
            pv(6, p_a, l_a)
            pv(7, p_b, l_b)
            for j in range(4):
                ot = _ld(ot_ref, j, 0, D).T
                for b in range(G):
                    _st(o_nat, b, j * 128, ot[:, b * 128:(b + 1) * 128])

        with _scope("A_out"):
            kn[:, HL - HALO:HL, :] = halo[layer, 0]
            vn[:, HL - HALO:HL, :] = halo[layer, 1]
            _run([out_item(o_nat, 0, 0, woa_cols, c) for c in range(4)])
            _run(_ln_items(x_f, xc, 0, HL, 0, _Chain(never, 2)))
            _run([out_item(o_nat, HL, HL, woa_cols, c) for c in range(4)])

        def b_half(hf, c):
            b_rotate()
            band = _band_items(seg * L + (hf - 1) * HL, 0, qo, ko, vo, ab, eb, ob0, _Chain(never))
            _interleave(b_proj_items(), band + _ln_items(x_f, xnx, HL, HL, 0, _Chain(never)))
            xc.bitcast(U32)[...] = xnx.bitcast(U32)[...]
            return c

        with _scope("B_loop"):
            lax.fori_loop(0, 2, b_half, 0)

        with _scope("B_tail"):
            halo[layer, 0] = kn[:, HL - HALO:HL, :]
            halo[layer, 1] = vn[:, HL - HALO:HL, :]
            b_rotate()
            _interleave([out_item(ob0, 0, 0, wob_cols, c) for c in range(4)],
                        _band_items(seg * L + HL, 0, qo, ko, vo, ab, eb, ob1, _Chain(never, NCH_B1)))
            _run(next_x_items(seg, layer, _Chain(never, 2)))
            _run([out_item(ob1, 0, HL, wob_cols, c) for c in range(4)])

        @pl.when(layer == 1)
        def _():
            obuf[HL:L, :] = x_f[HL:L, :].astype(BF)
            cp_out(seg).start()
            x_f[HL:L, :] = xin[pl.ds(pl.multiple_of(jnp.minimum(seg + 1, NSEG - 1) * L + HL, HL), HL), :].astype(F32)

        return carry

    lax.fori_loop(0, 2 * NSEG, step, 0)
    cp_out(NSEG - 1).wait()


@jax.jit
def pallas_interleave_layers__memory_aug_infini_attn__sliding_local_dilated__prompt_kernel(
    A_x: jax.Array,
    A_wq: jax.Array,
    A_wk: jax.Array,
    A_wv: jax.Array,
    A_wo: jax.Array,
    A_beta: jax.Array,
    B_x: jax.Array,
    B_wqkv: jax.Array,
    B_wo: jax.Array,
):
    del B_x
    x = A_x.reshape(S, D)
    any_spec = pl.BlockSpec(memory_space=pl.ANY)
    blk = lambda rows, dt: pltpu.VMEM((G, rows, 128), dt)
    packed = lambda rows, n=G: pltpu.VMEM((n, rows, 128), BF)
    scratch = [
        pltpu.VMEM((S, D), BF),
        pltpu.VMEM((L, D), BF),
        pltpu.VMEM((L, D), F32),
        packed(L),
        packed(HL),
        packed(HL),
        blk(D, BF),
        blk(D, BF),
        blk(D, BF),
        pltpu.VMEM((D, D), BF),
        pltpu.VMEM((3, D, D), BF),
        packed(D),
        packed(3 * D),
        blk(D, BF),
        packed(D),
        pltpu.VMEM((H * PITCH, 128), F32),
        pltpu.VMEM((H * PITCH, 128), F32),
        pltpu.VMEM((H * PITCH, 128), F32),
        pltpu.VMEM((H * PITCH, 128), F32),
        packed(L),
        packed(L),
        packed(L),
        packed(L),
        packed(D, 4),
        packed(D, 4),
        packed(L),
        pltpu.VMEM((1280, 512), F32),
        pltpu.VMEM((1280, 512), F32),
        pltpu.VMEM((4, 8, 512), F32),
        pltpu.VMEM((4, 8, 512), F32),
        packed(1280, 4),
        packed(1280, 4),
        pltpu.VMEM((4, 8, 512), F32),
        pltpu.VMEM((4, 8, 512), F32),
        pltpu.VMEM((2, G, 144, 128), F32),
        pltpu.VMEM((H, 128), F32),
        blk(HL, F32),
        blk(HL, F32),
        blk(HL, F32),
        blk(HL, F32),
        blk(HL + HALO, F32),
        blk(HL + HALO, F32),
        pltpu.VMEM((2, 2, G, HALO, 128), F32),
        pltpu.VMEM((W, HL, 128), F32),
        pltpu.VMEM((W, HL, 128), F32),
        packed(HL),
        packed(HL),
        pltpu.SemaphoreType.DMA((14,)),
    ]
    out = pl.pallas_call(
        _kernel,
        in_specs=[any_spec, any_spec, any_spec, any_spec, any_spec,
                  pl.BlockSpec(memory_space=pltpu.VMEM), any_spec, any_spec],
        out_specs=any_spec,
        out_shape=jax.ShapeDtypeStruct((S, D), BF),
        scratch_shapes=scratch,
        compiler_params=pltpu.CompilerParams(vmem_limit_bytes=100 * 1024 * 1024),
    )(x, A_wq, A_wk, A_wv, A_wo, A_beta, B_wqkv, B_wo)
    return out.reshape(1, S, D)
```

```python
import math

import jax
import jax.numpy as jnp
from jax import lax
import jax.experimental.pallas as pl
import jax.experimental.pallas.tpu as pltpu

S, D, H, DH = 2048, 1024, 32, 32
L, NSEG, G = 512, 4, 8
HL = L // 2
W, DIL = 8, 2
HALO = 16
BF, F32, U32 = jnp.bfloat16, jnp.float32, jnp.uint32
QSCALE = (DH ** -0.5) * math.log2(math.e)
NEG = -1e30
NT = (((1,), (1,)), ((), ()))
OFF = (0, 128, 384, 768)
SCOPES = False
NCH_B1 = 3
PV_ONE_DOT = True
KSPLIT = 6
NCH_EPI = 2
PITCH = 33


class _scope:
    def __init__(self, name):
        self.cm = jax.named_scope(name) if SCOPES else None

    def __enter__(self):
        if self.cm is not None:
            self.cm.__enter__()

    def __exit__(self, *a):
        if self.cm is not None:
            self.cm.__exit__(*a)


def _dot(a, b):
    return jnp.dot(a, b, preferred_element_type=F32)


def _dot_nt(a, b):
    return lax.dot_general(a, b, NT, preferred_element_type=F32)


def _rows(r0, n, align=16):
    return slice(r0, r0 + n) if isinstance(r0, int) else pl.ds(pl.multiple_of(r0, align), n)


def _ldu(ref, b, r0, n):
    idx = slice(r0 // 2, (r0 + n) // 2) if isinstance(r0, int) else pl.ds(pl.multiple_of(r0 // 2, 8), n // 2)
    return ref.bitcast(U32)[b, idx, :]


def _ld(ref, b, r0, n):
    return pltpu.bitcast(_ldu(ref, b, r0, n), BF)


def _st(ref, b, r0, val):
    ref[b, _rows(r0, val.shape[0]), :] = val


def _wide(ref, r0, n):
    return jnp.concatenate([_ld(ref, b, r0, n) for b in range(G)], axis=1)


class _Chain:
    def __init__(self, never, n=1):
        self.never, self.n, self.hist = never, n, []

    def link(self, x):
        if self.never is None or len(self.hist) < self.n:
            return x
        return jnp.where(self.never, self.hist[-self.n], x)

    def link_first(self, x):
        head = self.link(x[0:8, 0:128])
        if x.shape[1] > 128:
            head = jnp.concatenate([head, x[0:8, 128:]], axis=1)
        return head if x.shape[0] == 8 else jnp.concatenate([head, x[8:]], axis=0)

    def done(self, v):
        self.hist.append(v[0:8, v.shape[1] - 128:])


def _phi(t):
    return jnp.where(t > 0, t + 1.0, jnp.exp(t))


def _ln(x):
    d = x - jnp.mean(x, axis=-1, keepdims=True)
    v = jnp.mean(d * d, axis=-1, keepdims=True)
    return d * lax.rsqrt(v + 1e-5)


def _ln_items(x_ref, xn_ref, row0, nrows, dst0, ch, chunk=16):
    def item(r0):
        def run():
            yf = _ln(ch.link_first(x_ref[r0:r0 + chunk, :]))
            y = yf.astype(BF)
            for b in range(G):
                _st(xn_ref, b, r0 - row0 + dst0, y[:, b * 128:(b + 1) * 128])
            ch.done(yf)
        return run
    return [item(r0) for r0 in range(row0, row0 + nrows, chunk)]


def _interleave(main, side, span=None):
    span = len(main) if span is None else span
    done = 0
    for i, it in enumerate(main):
        upto = len(side) if i + 1 >= span else (len(side) * (i + 1)) // span
        for s_it in side[done:upto]:
            s_it()
        done = max(done, upto)
        it()


def _run(items):
    for it in items:
        it()


def _shuffle_rows(tf, tmp, store):
    for h in range(H):
        tmp[h * PITCH:h * PITCH + DH, :] = tf[h * DH:(h + 1) * DH]
    for d in range(DH):
        for th in range(2):
            rows = tmp[pl.ds(th * 16 * PITCH + d, 16, stride=PITCH), :]
            store(d * H + th * 16, rows.astype(BF))


def _qk_stage(g, q_ref, k_ref, s_ref, m_ref):
    lane = lax.broadcasted_iota(jnp.int32, (64, 128), 1)
    key = lax.broadcasted_iota(jnp.int32, (128, 512), 0)
    qry = lax.broadcasted_iota(jnp.int32, (128, 512), 1) & 127
    causal = key <= qry
    for j in range(4):
        nk = 128 * (j + 1)
        qt = _ldu(q_ref, g, j * 128, 128)
        wq = jnp.concatenate([jnp.where((lane >> 5) == h, qt, jnp.uint32(0)) for h in range(4)], axis=0)
        st = _dot_nt(_ld(k_ref, g, 0, nk), pltpu.bitcast(wq, BF))
        diag = jnp.where(causal, st[j * 128:], NEG)
        s_ref[OFF[j] + j * 128:OFF[j] + nk, :] = diag
        m = jnp.max(diag.reshape(16, 8, 512), axis=0)
        if j > 0:
            s_ref[OFF[j]:OFF[j] + j * 128, :] = st[:j * 128]
            m = jnp.maximum(m, jnp.max(st[:j * 128].reshape(16 * j, 8, 512), axis=0))
        m_ref[j] = jnp.broadcast_to(jnp.max(m, axis=0, keepdims=True), (8, 512))


def _sm_stage(s_ref, m_ref, p_ref, l_ref, ch=None, sub=16):
    ch = _Chain(None) if ch is None else ch
    for j in range(4):
        nk = 128 * (j + 1)
        for h in range(4):
            m = m_ref[j, :, h * 128:(h + 1) * 128]
            l = None
            for r in range(0, nk, sub):
                s = ch.link_first(s_ref[OFF[j] + r:OFF[j] + r + sub, h * 128:(h + 1) * 128])
                p = jnp.exp2(s.reshape(sub // 8, 8, 128) - m[None])
                ls = jnp.sum(p, axis=0)
                l = ls if l is None else l + ls
                _st(p_ref, h, OFF[j] + r, p.reshape(sub, 128).astype(BF))
                ch.done(p[0])
            l_ref[j, :, h * 128:(h + 1) * 128] = l


def _pv_stage(g, p_ref, l_ref, vt_ref, ot_ref, pq_ref, pk_ref, mt_ref, gate_ref):
    mem = mt_ref[g].astype(BF)
    for j in range(4):
        nd = _dot_nt(mem, _ld(pq_ref, g, j * 128, 128))
        for h in range(4):
            r0 = (g * 4 + h) * DH
            gate = gate_ref[pl.ds(g * 4 + h, 1), :]
            if PV_ONE_DOT:
                vt = jnp.concatenate([_ld(vt_ref, t, r0, DH) for t in range(j + 1)], axis=1)
                acc = _dot(vt, _ld(p_ref, h, OFF[j], 128 * (j + 1)))
            else:
                acc = None
                for t in range(j + 1):
                    o = _dot(_ld(vt_ref, t, r0, DH), _ld(p_ref, h, OFF[j] + t * 128, 128))
                    acc = o if acc is None else acc + o
            l = jnp.sum(l_ref[j, :, h * 128:(h + 1) * 128], axis=0, keepdims=True)
            den = nd[128 + h:129 + h] + 1e-6
            res = nd[h * DH:(h + 1) * DH] * (gate / den) + acc * ((1.0 - gate) / l)
            _st(ot_ref, j, r0, res.astype(BF))
    row = lax.broadcasted_iota(jnp.int32, (144, 128), 0)
    lane = lax.broadcasted_iota(jnp.int32, (144, 128), 1)
    keep = jnp.where(row < 128, row >> 5, row - 128) == (lane >> 5)
    row16 = lax.broadcasted_iota(jnp.int32, (16, 128), 0)
    ones = jnp.where(row16 < 4, 1.0, 0.0).astype(BF)
    upd = None
    for t in range(4):
        lhs = jnp.concatenate([_ld(vt_ref, t, g * 128, 128), ones], axis=0)
        u = _dot(lhs, _ld(pk_ref, g, t * 128, 128))
        upd = u if upd is None else upd + u
    mt_ref[g] = mt_ref[g] + jnp.where(keep, upd, 0.0)


def _band_items(pos0, row0, q_ref, k_ref, v_ref, a_ref, e_ref, o_ref, ch, nrows=HL):
    def logits(r0):
        def run():
            q = [q_ref[b, r0:r0 + 8, :] for b in range(G)]
            for w in range(W):
                base = HALO + r0 - DIL * w
                acc = ch.link(q[0] * k_ref[0, base:base + 8, :])
                for b in range(1, G):
                    acc = acc + q[b] * k_ref[b, base:base + 8, :]
                a_ref[w, r0 - row0:r0 - row0 + 8, :] = acc
                ch.done(acc)
        return run

    def softmax(r0):
        def run():
            lg = []
            for w in range(W):
                t = a_ref[w, r0 - row0:r0 - row0 + 128, :].T
                t = ((t[0:32] + t[32:64]) + (t[64:96] + t[96:128])) * QSCALE
                if r0 == row0 and w > 0:
                    pos = pos0 - DIL * w + lax.broadcasted_iota(jnp.int32, (H, 128), 1)
                    t = jnp.where(pos >= 0, t, NEG)
                lg.append(t)
            m = lg[0]
            for w in range(1, W):
                m = jnp.maximum(m, lg[w])
            e = [jnp.exp2(x - m) for x in lg]
            l = e[0]
            for w in range(1, W):
                l = l + e[w]
            inv = 1.0 / l
            for w in range(W):
                p = e[w] * inv
                pt = jnp.concatenate([p, p, p, p], axis=0).T
                e_ref[w, r0 - row0:r0 - row0 + 128, :] = pt
        return run

    def pv(r0):
        e = [e_ref[w, r0 - row0:r0 - row0 + 8, :] for w in range(W)]
        outs = []
        for b in range(G):
            acc = ch.link(e[0] * v_ref[b, HALO + r0:HALO + r0 + 8, :])
            for w in range(1, W):
                base = HALO + r0 - DIL * w
                acc = acc + e[w] * v_ref[b, base:base + 8, :]
            outs.append(acc)
            ch.done(acc)
        return outs

    def pv16(r0):
        def run():
            lo = pv(r0)
            hi = pv(r0 + 8)
            for b in range(G):
                _st(o_ref, b, r0, jnp.concatenate([lo[b], hi[b]], axis=0).astype(BF))
        return run

    items = []
    for r0 in range(row0, row0 + nrows, 128):
        items += [logits(r) for r in range(r0, r0 + 128, 8)]
        items.append(softmax(r0))
        items += [pv16(r) for r in range(r0, r0 + 128, 16)]
    return items


def _kernel(x_hbm, wq_hbm, wk_hbm, wv_hbm, woa_hbm, beta_ref, wqkv_hbm, wob_hbm, out_hbm,
            xin, obuf, x_f, xn, xc, xnx, wq, wk, woa, wv, wqkv, wvt, wbt, wob, wobp, tmp_a, tmp_b, tmp_c, tmp_d,
            q_ref, pq_ref, k_ref, pk_ref, vt_ref, ot_ref, o_nat,
            s_a, s_b, m_a, m_b, p_a, p_b, l_a, l_b, mt_ref, gate_ref,
            qn, kn, vn, qo, ko, vo, halo, ab, eb, ob0, ob1, sems):

    def col_copies(src, dst, sem, c0=0, n=G):
        return [pltpu.make_async_copy(src.at[:, (c0 + i) * 128:(c0 + i + 1) * 128], dst.at[c0 + i], sem)
                for i in range(n)]

    cp_wq = [col_copies(wq_hbm, wq, sems.at[c], 2 * c, 2) for c in range(4)]
    cp_wk = col_copies(wk_hbm, wk, sems.at[4])
    cp_wv = [pltpu.make_async_copy(wv_hbm, wv, sems.at[5])]
    cp_wqkv = [[pltpu.make_async_copy(wqkv_hbm.at[:, part * D:(part + 1) * D], wqkv.at[part], sems.at[6 + part])]
               for part in range(3)]
    cp_wob = col_copies(wob_hbm, wob, sems.at[9])
    cp_woa = col_copies(woa_hbm, woa, sems.at[10])
    cp_x0 = [pltpu.make_async_copy(x_hbm.at[0:L], xin.at[0:L], sems.at[11])]
    cp_xr = [pltpu.make_async_copy(x_hbm.at[L:S], xin.at[L:S], sems.at[12])]

    def cp_out(seg):
        return pltpu.make_async_copy(obuf, out_hbm.at[pl.ds(pl.multiple_of(seg * L, L), L)], sems.at[13])

    def wait(cps):
        for c in cps:
            c.wait()

    def wcols(w_ref, c0):
        return jnp.concatenate([_ld(w_ref, c0, 0, D), _ld(w_ref, c0 + 1, 0, D)], axis=1)

    def q_item(src, n, d0, c):
        def run():
            y = _dot(_wide(src, 0, n), wcols(wq, 2 * c))
            for gg in range(2):
                yq = y[:, gg * 128:(gg + 1) * 128]
                _st(q_ref, 2 * c + gg, d0, (yq * QSCALE).astype(BF))
                _st(pq_ref, 2 * c + gg, d0, _phi(yq).astype(BF))
        return run

    def k_item(src, n, d0, c):
        def run():
            y = _dot(_wide(src, 0, n), wcols(wk, 2 * c))
            for gg in range(2):
                yk = y[:, gg * 128:(gg + 1) * 128]
                _st(k_ref, 2 * c + gg, d0, yk.astype(BF))
                _st(pk_ref, 2 * c + gg, d0, _phi(yk).astype(BF))
        return run

    def v_item(src, r0, tile0, f0):
        def run():
            y = _dot_nt(_wide(wvt, f0, 512), _wide(src, r0, HL))
            _st(vt_ref, tile0, f0, y[:, :128].astype(BF))
            _st(vt_ref, tile0 + 1, f0, y[:, 128:].astype(BF))
        return run

    def blk(i):
        return pl.ds(pl.multiple_of(i * 128, 128), 128)

    def qkv_shuffle(part, kbk, tmp):
        tf = wqkv[part, blk(kbk), :].T.astype(F32)
        _shuffle_rows(tf, tmp, lambda r, val: _st(wbt, kbk, part * D + r, val))

    with _scope("first_proj"):
        for cps in [cp_x0] + cp_wq + [cp_wv, cp_wk] + cp_wqkv + [cp_wob, cp_woa, cp_xr]:
            for c in cps:
                c.start()
        b = beta_ref[...].astype(F32).reshape(1, H)
        gt = jax.nn.sigmoid(b)
        row = lax.broadcasted_iota(jnp.int32, (H, H), 0)
        lane = lax.broadcasted_iota(jnp.int32, (H, H), 1)
        col = jnp.sum(jnp.where(row == lane, jnp.broadcast_to(gt, (H, H)), 0.0), axis=1, keepdims=True)
        gate_ref[...] = jnp.broadcast_to(col, (H, 128))
        halo[...] = jnp.zeros(halo.shape, F32)

        def zero_b(b, c):
            for r in (qn, kn, vn, ko, vo):
                r[b] = jnp.zeros(r.shape[1:], F32)
            return c
        lax.fori_loop(0, G, zero_b, 0)

        def zero_mem(i, c):
            mt_ref[i // G, i % G] = jnp.zeros((144, 128), F32)
            return c
        lax.fori_loop(0, 2 * G, zero_mem, 0)
        with _scope("p_wait_x"):
            wait(cp_x0)

        def ln0(i, c):
            for u in range(8):
                r0 = pl.multiple_of(i * 128 + u * 16, 16)
                x = xin[pl.ds(r0, 16), :].astype(F32)
                x_f[pl.ds(r0, 16), :] = x
                y = _ln(x).astype(BF)
                for b in range(G):
                    _st(xn, b, r0, y[:, b * 128:(b + 1) * 128])
            return c
        with _scope("p_ln"):
            lax.fori_loop(0, L // 128, ln0, 0)

        def q0(c, carry):
            for i in range(2):
                pltpu.make_async_copy(wq_hbm.at[:, 0:128], wq.at[0], sems.at[c]).wait()
            q_item(xn, L, 0, c)()
            return carry
        with _scope("p_q"):
            lax.fori_loop(0, 4, q0, 0)
        wait(cp_wv)

        def tr0(i, carry):
            for u in range(4):
                _st(wvt, 4 * i + u, 0, wv[blk(4 * i + u), :].T)
            return carry
        with _scope("p_tr"):
            lax.fori_loop(0, 2, tr0, 0)

        def v0(i, carry):
            hf = i // 2
            v_item(xn, hf * HL, 2 * hf, (i % 2) * 512)()
            return carry
        with _scope("p_v"):
            lax.fori_loop(0, 4, v0, 0)
        wait(cp_wk)
        wait(cp_wqkv[0])
        wait(cp_wqkv[1])
        tmps = (tmp_a, tmp_b, tmp_c, tmp_d)

        def k0(c, carry):
            k_item(xn, L, 0, c)()
            for u in range(4):
                qkv_shuffle(c // 2, 4 * (c % 2) + u, tmps[u])
            return carry
        with _scope("p_k"):
            lax.fori_loop(0, 4, k0, 0)
        wait(cp_wqkv[2])

        def sh0(i, carry):
            for u in range(4):
                qkv_shuffle(2, 4 * i + u, tmps[u])
            return carry
        with _scope("p_sh0"):
            lax.fori_loop(0, 2, sh0, 0)
        wait(cp_wob)

        def sh1(i, carry):
            for u in range(4):
                cb = 4 * i + u
                _shuffle_rows(wob[cb].astype(F32), tmps[u], lambda r, val, cb=cb: _st(wobp, cb, r, val))
            return carry
        with _scope("p_sh1"):
            lax.fori_loop(0, 2, sh1, 0)
        wait(cp_woa)

    def out_item(src, s0, r0, w_ref, c, b0=0, b1=G):
        def run():
            lhs = jnp.concatenate([_ld(src, b, s0, HL) for b in range(b0, b1)], axis=1)
            w = jnp.concatenate([_ld(w_ref, 2 * c + i, b0 * 128, (b1 - b0) * 128) for i in range(2)], axis=1)
            x_f[r0:r0 + HL, c * 256:(c + 1) * 256] += _dot(lhs, w)
        return run

    def b_proj_items():
        def item(part, c):
            def run():
                y = _dot_nt(_wide(xc, 0, HL), _wide(wbt, part * D + c * 256, 256))
                dst = (qn, kn, vn)[part]
                dst[2 * c] = y[:, :128]
                dst[2 * c + 1] = y[:, 128:]
            return run
        return [item(part, c) for part in range(3) for c in range(4)]

    def b_rotate():
        for b in range(G):
            qo[b] = qn[b]
            for new, old in ((kn, ko), (vn, vo)):
                old[b, 0:HALO, :] = old[b, HL:HL + HALO, :]
                old[b, HALO:, :] = new[b]

    def next_x_items(seg, layer, ch, chunk=16):
        nxt = jnp.minimum(seg + 1, NSEG - 1) * L

        def item(r0):
            def run():
                cur = ch.link_first(x_f[r0:r0 + chunk, :])
                obuf[r0:r0 + chunk, :] = cur.astype(BF)
                new = xin[pl.ds(pl.multiple_of(nxt + r0, chunk), chunk), :].astype(F32)
                x = jnp.where(layer == 1, new, cur)
                x_f[r0:r0 + chunk, :] = x
                yf = _ln(x)
                y = yf.astype(BF)
                for b in range(G):
                    _st(xc, b, r0, y[:, b * 128:(b + 1) * 128])
                ch.done(yf)
            return run
        return [item(r0) for r0 in range(0, HL, chunk)]

    def step(t, carry):
        seg = t // 2
        layer = t % 2
        mt = mt_ref.at[layer]
        never = lax.broadcasted_iota(jnp.int32, (8, 128), 0) < -t
        pv = lambda g, p, l: _pv_stage(g, p, l, vt_ref, ot_ref, pq_ref, pk_ref, mt, gate_ref)

        @pl.when(t > 0)
        def _():
            with _scope("A_proj"):
                def a_half(hf, c):
                    d0 = hf * HL
                    items = ([q_item(xc, HL, d0, c) for c in range(4)]
                             + [k_item(xc, HL, d0, c) for c in range(4)]
                             + [v_item(xc, 0, 2 * hf, f0) for f0 in (0, 512)])
                    _interleave(items, _ln_items(x_f, xnx, HL, HL, 0, _Chain(never)), span=8)
                    xc.bitcast(U32)[...] = xnx.bitcast(U32)[...]
                    return c

                lax.fori_loop(0, 2, a_half, 0)

        with _scope("A_attn_pro"):
            _qk_stage(0, q_ref, k_ref, s_a, m_a)
            _qk_stage(1, q_ref, k_ref, s_b, m_b)
            _sm_stage(s_a, m_a, p_a, l_a)

        def pair(u, c):
            g = 2 * u + 1
            _qk_stage(g + 1, q_ref, k_ref, s_a, m_a)
            _sm_stage(s_b, m_b, p_b, l_b)
            pv(g - 1, p_a, l_a)
            _qk_stage(g + 2, q_ref, k_ref, s_b, m_b)
            _sm_stage(s_a, m_a, p_a, l_a)
            pv(g, p_b, l_b)
            return c

        with _scope("A_attn_loop"):
            lax.fori_loop(0, 3, pair, 0)

        @pl.when(t == 0)
        def _():
            wait(cp_xr)

        @pl.when(jnp.logical_and(layer == 0, seg > 0))
        def _():
            cp_out(seg - 1).wait()

        def transpose_o(b0, b1):
            for j in range(4):
                ot = _ld(ot_ref, j, b0 * 128, (b1 - b0) * 128).T
                for b in range(b0, b1):
                    _st(o_nat, b, j * 128, ot[:, (b - b0) * 128:(b - b0 + 1) * 128])

        with _scope("A_out"):
            transpose_o(0, KSPLIT)
            _sm_stage(s_b, m_b, p_b, l_b, _Chain(never, NCH_EPI))
            pv(6, p_a, l_a)
            _run([out_item(o_nat, 0, 0, woa, c, 0, KSPLIT) for c in range(4)])
            pv(7, p_b, l_b)
            transpose_o(KSPLIT, G)
            kn[:, HL - HALO:HL, :] = halo[layer, 0]
            vn[:, HL - HALO:HL, :] = halo[layer, 1]
            _run([out_item(o_nat, 0, 0, woa, c, KSPLIT, G) for c in range(4)])
            _run(_ln_items(x_f, xc, 0, HL, 0, _Chain(never, 2)))
            _run([out_item(o_nat, HL, HL, woa, c) for c in range(4)])

        def b_half(hf, c):
            b_rotate()
            band = _band_items(seg * L + (hf - 1) * HL, 0, qo, ko, vo, ab, eb, ob0, _Chain(never))
            _interleave(b_proj_items(), band + _ln_items(x_f, xnx, HL, HL, 0, _Chain(never)))
            xc.bitcast(U32)[...] = xnx.bitcast(U32)[...]
            return c

        with _scope("B_loop"):
            lax.fori_loop(0, 2, b_half, 0)

        with _scope("B_tail"):
            halo[layer, 0] = kn[:, HL - HALO:HL, :]
            halo[layer, 1] = vn[:, HL - HALO:HL, :]
            b_rotate()
            _interleave([out_item(ob0, 0, 0, wobp, c) for c in range(4)],
                        _band_items(seg * L + HL, 0, qo, ko, vo, ab, eb, ob1, _Chain(never, NCH_B1)))
            _run(next_x_items(seg, layer, _Chain(never, 2)))
            _run([out_item(ob1, 0, HL, wobp, c) for c in range(4)])

        @pl.when(layer == 1)
        def _():
            obuf[HL:L, :] = x_f[HL:L, :].astype(BF)
            cp_out(seg).start()
            x_f[HL:L, :] = xin[pl.ds(pl.multiple_of(jnp.minimum(seg + 1, NSEG - 1) * L + HL, HL), HL), :].astype(F32)

        return carry

    lax.fori_loop(0, 2 * NSEG, step, 0)
    cp_out(NSEG - 1).wait()


@jax.jit
def pallas_interleave_layers__memory_aug_infini_attn__sliding_local_dilated__prompt_kernel(
    A_x: jax.Array,
    A_wq: jax.Array,
    A_wk: jax.Array,
    A_wv: jax.Array,
    A_wo: jax.Array,
    A_beta: jax.Array,
    B_x: jax.Array,
    B_wqkv: jax.Array,
    B_wo: jax.Array,
):
    del B_x
    x = A_x.reshape(S, D)
    any_spec = pl.BlockSpec(memory_space=pl.ANY)
    blk = lambda rows, dt: pltpu.VMEM((G, rows, 128), dt)
    packed = lambda rows, n=G: pltpu.VMEM((n, rows, 128), BF)
    scratch = [
        pltpu.VMEM((S, D), BF),
        pltpu.VMEM((L, D), BF),
        pltpu.VMEM((L, D), F32),
        packed(L),
        packed(HL),
        packed(HL),
        blk(D, BF),
        blk(D, BF),
        blk(D, BF),
        pltpu.VMEM((D, D), BF),
        pltpu.VMEM((3, D, D), BF),
        packed(D),
        packed(3 * D),
        blk(D, BF),
        packed(D),
        pltpu.VMEM((H * PITCH, 128), F32),
        pltpu.VMEM((H * PITCH, 128), F32),
        pltpu.VMEM((H * PITCH, 128), F32),
        pltpu.VMEM((H * PITCH, 128), F32),
        packed(L),
        packed(L),
        packed(L),
        packed(L),
        packed(D, 4),
        packed(D, 4),
        packed(L),
        pltpu.VMEM((1280, 512), F32),
        pltpu.VMEM((1280, 512), F32),
        pltpu.VMEM((4, 8, 512), F32),
        pltpu.VMEM((4, 8, 512), F32),
        packed(1280, 4),
        packed(1280, 4),
        pltpu.VMEM((4, 8, 512), F32),
        pltpu.VMEM((4, 8, 512), F32),
        pltpu.VMEM((2, G, 144, 128), F32),
        pltpu.VMEM((H, 128), F32),
        blk(HL, F32),
        blk(HL, F32),
        blk(HL, F32),
        blk(HL, F32),
        blk(HL + HALO, F32),
        blk(HL + HALO, F32),
        pltpu.VMEM((2, 2, G, HALO, 128), F32),
        pltpu.VMEM((W, HL, 128), F32),
        pltpu.VMEM((W, HL, 128), F32),
        packed(HL),
        packed(HL),
        pltpu.SemaphoreType.DMA((14,)),
    ]
    out = pl.pallas_call(
        _kernel,
        in_specs=[any_spec, any_spec, any_spec, any_spec, any_spec,
                  pl.BlockSpec(memory_space=pltpu.VMEM), any_spec, any_spec],
        out_specs=any_spec,
        out_shape=jax.ShapeDtypeStruct((S, D), BF),
        scratch_shapes=scratch,
        compiler_params=pltpu.CompilerParams(vmem_limit_bytes=100 * 1024 * 1024),
    )(x, A_wq, A_wk, A_wv, A_wo, A_beta, B_wqkv, B_wo)
    return out.reshape(1, S, D)
```

```python
import math

import jax
import jax.numpy as jnp
from jax import lax
import jax.experimental.pallas as pl
import jax.experimental.pallas.tpu as pltpu

S, D, H, DH = 2048, 1024, 32, 32
L, NSEG, G = 512, 4, 8
HL = L // 2
W, DIL = 8, 2
HALO = 16
BF, F32, U32 = jnp.bfloat16, jnp.float32, jnp.uint32
QSCALE = (DH ** -0.5) * math.log2(math.e)
NEG = -1e30
NT = (((1,), (1,)), ((), ()))
OFF = (0, 128, 384, 768)
SCOPES = False
NCH_B1 = 2
PV_ONE_DOT = True
KSPLIT = 6
NCH_EPI = 2
PITCH = 33


class _scope:
    def __init__(self, name):
        self.cm = jax.named_scope(name) if SCOPES else None

    def __enter__(self):
        if self.cm is not None:
            self.cm.__enter__()

    def __exit__(self, *a):
        if self.cm is not None:
            self.cm.__exit__(*a)


def _dot(a, b):
    return jnp.dot(a, b, preferred_element_type=F32)


def _dot_nt(a, b):
    return lax.dot_general(a, b, NT, preferred_element_type=F32)


def _rows(r0, n, align=16):
    return slice(r0, r0 + n) if isinstance(r0, int) else pl.ds(pl.multiple_of(r0, align), n)


def _ldu(ref, b, r0, n):
    idx = slice(r0 // 2, (r0 + n) // 2) if isinstance(r0, int) else pl.ds(pl.multiple_of(r0 // 2, 8), n // 2)
    return ref.bitcast(U32)[b, idx, :]


def _ld(ref, b, r0, n):
    return pltpu.bitcast(_ldu(ref, b, r0, n), BF)


def _st(ref, b, r0, val):
    ref[b, _rows(r0, val.shape[0]), :] = val


def _wide(ref, r0, n):
    return jnp.concatenate([_ld(ref, b, r0, n) for b in range(G)], axis=1)


class _Chain:
    def __init__(self, never, n=1):
        self.never, self.n, self.hist = never, n, []

    def link(self, x):
        if self.never is None or len(self.hist) < self.n:
            return x
        return jnp.where(self.never, self.hist[-self.n], x)

    def link_first(self, x):
        head = self.link(x[0:8, 0:128])
        if x.shape[1] > 128:
            head = jnp.concatenate([head, x[0:8, 128:]], axis=1)
        return head if x.shape[0] == 8 else jnp.concatenate([head, x[8:]], axis=0)

    def done(self, v):
        self.hist.append(v[0:8, v.shape[1] - 128:])


def _phi(t):
    return jnp.where(t > 0, t + 1.0, jnp.exp(t))


def _ln(x):
    d = x - jnp.mean(x, axis=-1, keepdims=True)
    v = jnp.mean(d * d, axis=-1, keepdims=True)
    return d * lax.rsqrt(v + 1e-5)


def _ln_items(x_ref, xn_ref, row0, nrows, dst0, ch, chunk=16):
    def item(r0):
        def run():
            yf = _ln(ch.link_first(x_ref[r0:r0 + chunk, :]))
            y = yf.astype(BF)
            for b in range(G):
                _st(xn_ref, b, r0 - row0 + dst0, y[:, b * 128:(b + 1) * 128])
            ch.done(yf)
        return run
    return [item(r0) for r0 in range(row0, row0 + nrows, chunk)]


def _interleave(main, side, span=None):
    span = len(main) if span is None else span
    done = 0
    for i, it in enumerate(main):
        upto = len(side) if i + 1 >= span else (len(side) * (i + 1)) // span
        for s_it in side[done:upto]:
            s_it()
        done = max(done, upto)
        it()


def _run(items):
    for it in items:
        it()


def _shuffle_rows(tf, tmp, store):
    for h in range(H):
        tmp[h * PITCH:h * PITCH + DH, :] = tf[h * DH:(h + 1) * DH]
    for d in range(DH):
        for th in range(2):
            rows = tmp[pl.ds(th * 16 * PITCH + d, 16, stride=PITCH), :]
            store(d * H + th * 16, rows.astype(BF))


def _qk_stage(g, q_ref, k_ref, s_ref, m_ref):
    lane = lax.broadcasted_iota(jnp.int32, (64, 128), 1)
    key = lax.broadcasted_iota(jnp.int32, (128, 512), 0)
    qry = lax.broadcasted_iota(jnp.int32, (128, 512), 1) & 127
    causal = key <= qry
    for j in range(4):
        nk = 128 * (j + 1)
        qt = _ldu(q_ref, g, j * 128, 128)
        wq = jnp.concatenate([jnp.where((lane >> 5) == h, qt, jnp.uint32(0)) for h in range(4)], axis=0)
        st = _dot_nt(_ld(k_ref, g, 0, nk), pltpu.bitcast(wq, BF))
        diag = jnp.where(causal, st[j * 128:], NEG)
        s_ref[OFF[j] + j * 128:OFF[j] + nk, :] = diag
        m = jnp.max(diag.reshape(16, 8, 512), axis=0)
        if j > 0:
            s_ref[OFF[j]:OFF[j] + j * 128, :] = st[:j * 128]
            m = jnp.maximum(m, jnp.max(st[:j * 128].reshape(16 * j, 8, 512), axis=0))
        m_ref[j] = jnp.broadcast_to(jnp.max(m, axis=0, keepdims=True), (8, 512))


def _sm_stage(s_ref, m_ref, p_ref, l_ref, ch=None, sub=16):
    ch = _Chain(None) if ch is None else ch
    for j in range(4):
        nk = 128 * (j + 1)
        for h in range(4):
            m = m_ref[j, :, h * 128:(h + 1) * 128]
            l = None
            for r in range(0, nk, sub):
                s = ch.link_first(s_ref[OFF[j] + r:OFF[j] + r + sub, h * 128:(h + 1) * 128])
                p = jnp.exp2(s.reshape(sub // 8, 8, 128) - m[None])
                ls = jnp.sum(p, axis=0)
                l = ls if l is None else l + ls
                _st(p_ref, h, OFF[j] + r, p.reshape(sub, 128).astype(BF))
                ch.done(p[0])
            l_ref[j, :, h * 128:(h + 1) * 128] = l


def _pv_stage(g, p_ref, l_ref, vt_ref, ot_ref, pq_ref, pk_ref, mt_ref, gate_ref):
    mem = mt_ref[g].astype(BF)
    for j in range(4):
        nd = _dot_nt(mem, _ld(pq_ref, g, j * 128, 128))
        for h in range(4):
            r0 = (g * 4 + h) * DH
            gate = gate_ref[pl.ds(g * 4 + h, 1), :]
            if PV_ONE_DOT:
                vt = jnp.concatenate([_ld(vt_ref, t, r0, DH) for t in range(j + 1)], axis=1)
                acc = _dot(vt, _ld(p_ref, h, OFF[j], 128 * (j + 1)))
            else:
                acc = None
                for t in range(j + 1):
                    o = _dot(_ld(vt_ref, t, r0, DH), _ld(p_ref, h, OFF[j] + t * 128, 128))
                    acc = o if acc is None else acc + o
            l = jnp.sum(l_ref[j, :, h * 128:(h + 1) * 128], axis=0, keepdims=True)
            den = nd[128 + h:129 + h] + 1e-6
            res = nd[h * DH:(h + 1) * DH] * (gate / den) + acc * ((1.0 - gate) / l)
            _st(ot_ref, j, r0, res.astype(BF))
    row = lax.broadcasted_iota(jnp.int32, (144, 128), 0)
    lane = lax.broadcasted_iota(jnp.int32, (144, 128), 1)
    keep = jnp.where(row < 128, row >> 5, row - 128) == (lane >> 5)
    row16 = lax.broadcasted_iota(jnp.int32, (16, 128), 0)
    ones = jnp.where(row16 < 4, 1.0, 0.0).astype(BF)
    upd = None
    for t in range(4):
        lhs = jnp.concatenate([_ld(vt_ref, t, g * 128, 128), ones], axis=0)
        u = _dot(lhs, _ld(pk_ref, g, t * 128, 128))
        upd = u if upd is None else upd + u
    mt_ref[g] = mt_ref[g] + jnp.where(keep, upd, 0.0)


def _band_items(pos0, row0, q_ref, k_ref, v_ref, a_ref, e_ref, o_ref, ch, nrows=HL):
    def logits(r0):
        def run():
            q = [q_ref[b, r0:r0 + 8, :] for b in range(G)]
            for w in range(W):
                base = HALO + r0 - DIL * w
                acc = ch.link(q[0] * k_ref[0, base:base + 8, :])
                for b in range(1, G):
                    acc = acc + q[b] * k_ref[b, base:base + 8, :]
                a_ref[w, r0 - row0:r0 - row0 + 8, :] = acc
                ch.done(acc)
        return run

    def softmax(r0):
        def run():
            lg = []
            for w in range(W):
                t = a_ref[w, r0 - row0:r0 - row0 + 128, :].T
                t = ((t[0:32] + t[32:64]) + (t[64:96] + t[96:128])) * QSCALE
                if r0 == row0 and w > 0:
                    pos = pos0 - DIL * w + lax.broadcasted_iota(jnp.int32, (H, 128), 1)
                    t = jnp.where(pos >= 0, t, NEG)
                lg.append(t)
            m = lg[0]
            for w in range(1, W):
                m = jnp.maximum(m, lg[w])
            e = [jnp.exp2(x - m) for x in lg]
            l = e[0]
            for w in range(1, W):
                l = l + e[w]
            inv = 1.0 / l
            for w in range(W):
                p = e[w] * inv
                pt = jnp.concatenate([p, p, p, p], axis=0).T
                e_ref[w, r0 - row0:r0 - row0 + 128, :] = pt
        return run

    def pv(r0):
        e = [e_ref[w, r0 - row0:r0 - row0 + 8, :] for w in range(W)]
        outs = []
        for b in range(G):
            acc = ch.link(e[0] * v_ref[b, HALO + r0:HALO + r0 + 8, :])
            for w in range(1, W):
                base = HALO + r0 - DIL * w
                acc = acc + e[w] * v_ref[b, base:base + 8, :]
            outs.append(acc)
            ch.done(acc)
        return outs

    def pv16(r0):
        def run():
            lo = pv(r0)
            hi = pv(r0 + 8)
            for b in range(G):
                _st(o_ref, b, r0, jnp.concatenate([lo[b], hi[b]], axis=0).astype(BF))
        return run

    items = []
    for r0 in range(row0, row0 + nrows, 128):
        items += [logits(r) for r in range(r0, r0 + 128, 8)]
        items.append(softmax(r0))
        items += [pv16(r) for r in range(r0, r0 + 128, 16)]
    return items


def _kernel(x_hbm, wq_hbm, wk_hbm, wv_hbm, woa_hbm, beta_ref, wqkv_hbm, wob_hbm, out_hbm,
            xin, obuf, x_f, xn, xc, xnx, wq, wk, woa, wv, wqkv, wvt, wbt, wob, wobp, tmp_a, tmp_b, tmp_c, tmp_d,
            q_ref, pq_ref, k_ref, pk_ref, vt_ref, ot_ref, o_nat,
            s_a, s_b, m_a, m_b, p_a, p_b, l_a, l_b, mt_ref, gate_ref,
            qn, kn, vn, qo, ko, vo, halo, ab, eb, ob0, ob1, sems):

    def col_copies(src, dst, sem, c0=0, n=G):
        return [pltpu.make_async_copy(src.at[:, (c0 + i) * 128:(c0 + i + 1) * 128], dst.at[c0 + i], sem)
                for i in range(n)]

    cp_wq = [col_copies(wq_hbm, wq, sems.at[c], 2 * c, 2) for c in range(4)]
    cp_wk = col_copies(wk_hbm, wk, sems.at[4])
    cp_wv = [pltpu.make_async_copy(wv_hbm, wv, sems.at[5])]
    cp_wqkv = [[pltpu.make_async_copy(wqkv_hbm.at[:, part * D:(part + 1) * D], wqkv.at[part], sems.at[6 + part])]
               for part in range(3)]
    cp_wob = col_copies(wob_hbm, wob, sems.at[9])
    cp_woa = col_copies(woa_hbm, woa, sems.at[10])
    cp_x0 = [pltpu.make_async_copy(x_hbm.at[0:L], xin.at[0:L], sems.at[11])]
    cp_xr = [pltpu.make_async_copy(x_hbm.at[L:S], xin.at[L:S], sems.at[12])]

    def cp_out(seg):
        return pltpu.make_async_copy(obuf, out_hbm.at[pl.ds(pl.multiple_of(seg * L, L), L)], sems.at[13])

    def wait(cps):
        for c in cps:
            c.wait()

    def wcols(w_ref, c0):
        return jnp.concatenate([_ld(w_ref, c0, 0, D), _ld(w_ref, c0 + 1, 0, D)], axis=1)

    def q_item(src, n, d0, c):
        def run():
            y = _dot(_wide(src, 0, n), wcols(wq, 2 * c))
            for gg in range(2):
                yq = y[:, gg * 128:(gg + 1) * 128]
                _st(q_ref, 2 * c + gg, d0, (yq * QSCALE).astype(BF))
                _st(pq_ref, 2 * c + gg, d0, _phi(yq).astype(BF))
        return run

    def k_item(src, n, d0, c):
        def run():
            y = _dot(_wide(src, 0, n), wcols(wk, 2 * c))
            for gg in range(2):
                yk = y[:, gg * 128:(gg + 1) * 128]
                _st(k_ref, 2 * c + gg, d0, yk.astype(BF))
                _st(pk_ref, 2 * c + gg, d0, _phi(yk).astype(BF))
        return run

    def v_item(src, r0, tile0, f0):
        def run():
            y = _dot_nt(_wide(wvt, f0, 512), _wide(src, r0, HL))
            _st(vt_ref, tile0, f0, y[:, :128].astype(BF))
            _st(vt_ref, tile0 + 1, f0, y[:, 128:].astype(BF))
        return run

    def blk(i):
        return pl.ds(pl.multiple_of(i * 128, 128), 128)

    def qkv_shuffle(part, kbk, tmp):
        tf = wqkv[part, blk(kbk), :].T.astype(F32)
        _shuffle_rows(tf, tmp, lambda r, val: _st(wbt, kbk, part * D + r, val))

    with _scope("first_proj"):
        for cps in [cp_x0] + cp_wq + [cp_wv, cp_wk] + cp_wqkv + [cp_wob, cp_woa, cp_xr]:
            for c in cps:
                c.start()
        b = beta_ref[...].astype(F32).reshape(1, H)
        gt = jax.nn.sigmoid(b)
        row = lax.broadcasted_iota(jnp.int32, (H, H), 0)
        lane = lax.broadcasted_iota(jnp.int32, (H, H), 1)
        col = jnp.sum(jnp.where(row == lane, jnp.broadcast_to(gt, (H, H)), 0.0), axis=1, keepdims=True)
        gate_ref[...] = jnp.broadcast_to(col, (H, 128))
        halo[...] = jnp.zeros(halo.shape, F32)

        def zero_b(b, c):
            for r in (qn, kn, vn, ko, vo):
                r[b] = jnp.zeros(r.shape[1:], F32)
            return c
        lax.fori_loop(0, G, zero_b, 0)

        def zero_mem(i, c):
            mt_ref[i // G, i % G] = jnp.zeros((144, 128), F32)
            return c
        lax.fori_loop(0, 2 * G, zero_mem, 0)
        with _scope("p_wait_x"):
            wait(cp_x0)

        def ln0(i, c):
            for u in range(8):
                r0 = pl.multiple_of(i * 128 + u * 16, 16)
                x = xin[pl.ds(r0, 16), :].astype(F32)
                x_f[pl.ds(r0, 16), :] = x
                y = _ln(x).astype(BF)
                for b in range(G):
                    _st(xn, b, r0, y[:, b * 128:(b + 1) * 128])
            return c
        with _scope("p_ln"):
            lax.fori_loop(0, L // 128, ln0, 0)

        def q0(c, carry):
            for i in range(2):
                pltpu.make_async_copy(wq_hbm.at[:, 0:128], wq.at[0], sems.at[c]).wait()
            q_item(xn, L, 0, c)()
            return carry
        with _scope("p_q"):
            lax.fori_loop(0, 4, q0, 0)
        wait(cp_wv)

        def tr0(i, carry):
            for u in range(4):
                _st(wvt, 4 * i + u, 0, wv[blk(4 * i + u), :].T)
            return carry
        with _scope("p_tr"):
            lax.fori_loop(0, 2, tr0, 0)

        def v0(i, carry):
            hf = i // 2
            v_item(xn, hf * HL, 2 * hf, (i % 2) * 512)()
            return carry
        with _scope("p_v"):
            lax.fori_loop(0, 4, v0, 0)
        wait(cp_wk)
        wait(cp_wqkv[0])
        wait(cp_wqkv[1])
        tmps = (tmp_a, tmp_b, tmp_c, tmp_d)

        def k0(c, carry):
            k_item(xn, L, 0, c)()
            for u in range(4):
                qkv_shuffle(c // 2, 4 * (c % 2) + u, tmps[u])
            return carry
        with _scope("p_k"):
            lax.fori_loop(0, 4, k0, 0)
        wait(cp_wqkv[2])

        def sh0(i, carry):
            for u in range(4):
                qkv_shuffle(2, 4 * i + u, tmps[u])
            return carry
        with _scope("p_sh0"):
            lax.fori_loop(0, 2, sh0, 0)
        wait(cp_wob)

        def sh1(i, carry):
            for u in range(4):
                cb = 4 * i + u
                _shuffle_rows(wob[cb].astype(F32), tmps[u], lambda r, val, cb=cb: _st(wobp, cb, r, val))
            return carry
        with _scope("p_sh1"):
            lax.fori_loop(0, 2, sh1, 0)
        wait(cp_woa)

    def out_item(src, s0, r0, w_ref, c, b0=0, b1=G, n=HL):
        def run():
            lhs = jnp.concatenate([_ld(src, b, s0, n) for b in range(b0, b1)], axis=1)
            w = jnp.concatenate([_ld(w_ref, 2 * c + i, b0 * 128, (b1 - b0) * 128) for i in range(2)], axis=1)
            x_f[r0:r0 + n, c * 256:(c + 1) * 256] += _dot(lhs, w)
        return run

    def b_proj_items():
        def item(part, c):
            def run():
                y = _dot_nt(_wide(xc, 0, HL), _wide(wbt, part * D + c * 256, 256))
                dst = (qn, kn, vn)[part]
                dst[2 * c] = y[:, :128]
                dst[2 * c + 1] = y[:, 128:]
            return run
        return [item(part, c) for part in range(3) for c in range(4)]

    def b_rotate():
        for b in range(G):
            qo[b] = qn[b]
            for new, old in ((kn, ko), (vn, vo)):
                old[b, 0:HALO, :] = old[b, HL:HL + HALO, :]
                old[b, HALO:, :] = new[b]

    def next_x_items(seg, layer, ch, chunk=16):
        nxt = jnp.minimum(seg + 1, NSEG - 1) * L

        def item(r0):
            def run():
                cur = ch.link_first(x_f[r0:r0 + chunk, :])
                obuf[r0:r0 + chunk, :] = cur.astype(BF)
                new = xin[pl.ds(pl.multiple_of(nxt + r0, chunk), chunk), :].astype(F32)
                x = jnp.where(layer == 1, new, cur)
                x_f[r0:r0 + chunk, :] = x
                yf = _ln(x)
                y = yf.astype(BF)
                for b in range(G):
                    _st(xc, b, r0, y[:, b * 128:(b + 1) * 128])
                ch.done(yf)
            return run
        return [item(r0) for r0 in range(0, HL, chunk)]

    def step(t, carry):
        seg = t // 2
        layer = t % 2
        mt = mt_ref.at[layer]
        never = lax.broadcasted_iota(jnp.int32, (8, 128), 0) < -t
        pv = lambda g, p, l: _pv_stage(g, p, l, vt_ref, ot_ref, pq_ref, pk_ref, mt, gate_ref)

        @pl.when(t > 0)
        def _():
            with _scope("A_proj"):
                def a_half(hf, c):
                    d0 = hf * HL
                    items = ([q_item(xc, HL, d0, c) for c in range(4)]
                             + [k_item(xc, HL, d0, c) for c in range(4)]
                             + [v_item(xc, 0, 2 * hf, f0) for f0 in (0, 512)])
                    _interleave(items, _ln_items(x_f, xnx, HL, HL, 0, _Chain(never)), span=8)
                    xc.bitcast(U32)[...] = xnx.bitcast(U32)[...]
                    return c

                lax.fori_loop(0, 2, a_half, 0)

        with _scope("A_attn_pro"):
            _qk_stage(0, q_ref, k_ref, s_a, m_a)
            _qk_stage(1, q_ref, k_ref, s_b, m_b)
            _sm_stage(s_a, m_a, p_a, l_a)

        def pair(u, c):
            g = 2 * u + 1
            _qk_stage(g + 1, q_ref, k_ref, s_a, m_a)
            _sm_stage(s_b, m_b, p_b, l_b)
            pv(g - 1, p_a, l_a)
            _qk_stage(g + 2, q_ref, k_ref, s_b, m_b)
            _sm_stage(s_a, m_a, p_a, l_a)
            pv(g, p_b, l_b)
            return c

        with _scope("A_attn_loop"):
            lax.fori_loop(0, 3, pair, 0)

        @pl.when(t == 0)
        def _():
            wait(cp_xr)

        @pl.when(jnp.logical_and(layer == 0, seg > 0))
        def _():
            cp_out(seg - 1).wait()

        def transpose_o(b0, b1):
            for j in range(4):
                ot = _ld(ot_ref, j, b0 * 128, (b1 - b0) * 128).T
                for b in range(b0, b1):
                    _st(o_nat, b, j * 128, ot[:, (b - b0) * 128:(b - b0 + 1) * 128])

        with _scope("A_out"):
            transpose_o(0, KSPLIT)
            _sm_stage(s_b, m_b, p_b, l_b, _Chain(never, NCH_EPI))
            pv(6, p_a, l_a)
            _run([out_item(o_nat, 0, 0, woa, c, 0, KSPLIT) for c in range(4)])
            pv(7, p_b, l_b)
            transpose_o(KSPLIT, G)
            kn[:, HL - HALO:HL, :] = halo[layer, 0]
            vn[:, HL - HALO:HL, :] = halo[layer, 1]
            _run([out_item(o_nat, 0, 0, woa, c, KSPLIT, G) for c in range(4)])
            _run(_ln_items(x_f, xc, 0, HL, 0, _Chain(never, 2)))
            _run([out_item(o_nat, HL, HL, woa, c) for c in range(4)])

        def b_half(hf, c):
            b_rotate()
            band = _band_items(seg * L + (hf - 1) * HL, 0, qo, ko, vo, ab, eb, ob0, _Chain(never))
            _interleave(b_proj_items(), band + _ln_items(x_f, xnx, HL, HL, 0, _Chain(never)))
            xc.bitcast(U32)[...] = xnx.bitcast(U32)[...]
            return c

        with _scope("B_loop"):
            lax.fori_loop(0, 2, b_half, 0)

        with _scope("B_tail"):
            halo[layer, 0] = kn[:, HL - HALO:HL, :]
            halo[layer, 1] = vn[:, HL - HALO:HL, :]
            b_rotate()
            _run(_band_items(seg * L + HL, 0, qo, ko, vo, ab, eb, ob1, _Chain(never, NCH_B1)))
            _run([out_item(ob0, 0, 0, wobp, c) for c in range(4)])
            _run(next_x_items(seg, layer, _Chain(never, 2)))
            _run([out_item(ob1, 0, HL, wobp, c, n=128) for c in range(4)])
            _run([out_item(ob1, 128, HL + 128, wobp, c, n=128) for c in range(4)])

        @pl.when(layer == 1)
        def _():
            obuf[HL:L, :] = x_f[HL:L, :].astype(BF)
            cp_out(seg).start()
            x_f[HL:L, :] = xin[pl.ds(pl.multiple_of(jnp.minimum(seg + 1, NSEG - 1) * L + HL, HL), HL), :].astype(F32)

        return carry

    lax.fori_loop(0, 2 * NSEG, step, 0)
    cp_out(NSEG - 1).wait()


@jax.jit
def pallas_interleave_layers__memory_aug_infini_attn__sliding_local_dilated__prompt_kernel(
    A_x: jax.Array,
    A_wq: jax.Array,
    A_wk: jax.Array,
    A_wv: jax.Array,
    A_wo: jax.Array,
    A_beta: jax.Array,
    B_x: jax.Array,
    B_wqkv: jax.Array,
    B_wo: jax.Array,
):
    del B_x
    x = A_x.reshape(S, D)
    any_spec = pl.BlockSpec(memory_space=pl.ANY)
    blk = lambda rows, dt: pltpu.VMEM((G, rows, 128), dt)
    packed = lambda rows, n=G: pltpu.VMEM((n, rows, 128), BF)
    scratch = [
        pltpu.VMEM((S, D), BF),
        pltpu.VMEM((L, D), BF),
        pltpu.VMEM((L, D), F32),
        packed(L),
        packed(HL),
        packed(HL),
        blk(D, BF),
        blk(D, BF),
        blk(D, BF),
        pltpu.VMEM((D, D), BF),
        pltpu.VMEM((3, D, D), BF),
        packed(D),
        packed(3 * D),
        blk(D, BF),
        packed(D),
        pltpu.VMEM((H * PITCH, 128), F32),
        pltpu.VMEM((H * PITCH, 128), F32),
        pltpu.VMEM((H * PITCH, 128), F32),
        pltpu.VMEM((H * PITCH, 128), F32),
        packed(L),
        packed(L),
        packed(L),
        packed(L),
        packed(D, 4),
        packed(D, 4),
        packed(L),
        pltpu.VMEM((1280, 512), F32),
        pltpu.VMEM((1280, 512), F32),
        pltpu.VMEM((4, 8, 512), F32),
        pltpu.VMEM((4, 8, 512), F32),
        packed(1280, 4),
        packed(1280, 4),
        pltpu.VMEM((4, 8, 512), F32),
        pltpu.VMEM((4, 8, 512), F32),
        pltpu.VMEM((2, G, 144, 128), F32),
        pltpu.VMEM((H, 128), F32),
        blk(HL, F32),
        blk(HL, F32),
        blk(HL, F32),
        blk(HL, F32),
        blk(HL + HALO, F32),
        blk(HL + HALO, F32),
        pltpu.VMEM((2, 2, G, HALO, 128), F32),
        pltpu.VMEM((W, HL, 128), F32),
        pltpu.VMEM((W, HL, 128), F32),
        packed(HL),
        packed(HL),
        pltpu.SemaphoreType.DMA((14,)),
    ]
    out = pl.pallas_call(
        _kernel,
        in_specs=[any_spec, any_spec, any_spec, any_spec, any_spec,
                  pl.BlockSpec(memory_space=pltpu.VMEM), any_spec, any_spec],
        out_specs=any_spec,
        out_shape=jax.ShapeDtypeStruct((S, D), BF),
        scratch_shapes=scratch,
        compiler_params=pltpu.CompilerParams(vmem_limit_bytes=100 * 1024 * 1024),
    )(x, A_wq, A_wk, A_wv, A_wo, A_beta, B_wqkv, B_wo)
    return out.reshape(1, S, D)
```

```python
import math

import jax
import jax.numpy as jnp
from jax import lax
import jax.experimental.pallas as pl
import jax.experimental.pallas.tpu as pltpu

S, D, H, DH = 2048, 1024, 32, 32
L, NSEG, G = 512, 4, 8
HL = L // 2
W, DIL = 8, 2
HALO = 16
BF, F32, U32 = jnp.bfloat16, jnp.float32, jnp.uint32
QSCALE = (DH ** -0.5) * math.log2(math.e)
NEG = -1e30
NT = (((1,), (1,)), ((), ()))
OFF = (0, 128, 384, 768)
SCOPES = False
NCH_B1 = 2
PV_ONE_DOT = True
KSPLIT = 6
NCH_EPI = 2
PITCH = 33


class _scope:
    def __init__(self, name):
        self.cm = jax.named_scope(name) if SCOPES else None

    def __enter__(self):
        if self.cm is not None:
            self.cm.__enter__()

    def __exit__(self, *a):
        if self.cm is not None:
            self.cm.__exit__(*a)


def _dot(a, b):
    return jnp.dot(a, b, preferred_element_type=F32)


def _dot_nt(a, b):
    return lax.dot_general(a, b, NT, preferred_element_type=F32)


def _rows(r0, n, align=16):
    return slice(r0, r0 + n) if isinstance(r0, int) else pl.ds(pl.multiple_of(r0, align), n)


def _ldu(ref, b, r0, n):
    idx = slice(r0 // 2, (r0 + n) // 2) if isinstance(r0, int) else pl.ds(pl.multiple_of(r0 // 2, 8), n // 2)
    return ref.bitcast(U32)[b, idx, :]


def _ld(ref, b, r0, n):
    return pltpu.bitcast(_ldu(ref, b, r0, n), BF)


def _st(ref, b, r0, val):
    ref[b, _rows(r0, val.shape[0]), :] = val


def _wide(ref, r0, n):
    return jnp.concatenate([_ld(ref, b, r0, n) for b in range(G)], axis=1)


class _Chain:
    def __init__(self, never, n=1):
        self.never, self.n, self.hist = never, n, []

    def link(self, x):
        if self.never is None or len(self.hist) < self.n:
            return x
        return jnp.where(self.never, self.hist[-self.n], x)

    def link_first(self, x):
        head = self.link(x[0:8, 0:128])
        if x.shape[1] > 128:
            head = jnp.concatenate([head, x[0:8, 128:]], axis=1)
        return head if x.shape[0] == 8 else jnp.concatenate([head, x[8:]], axis=0)

    def done(self, v):
        self.hist.append(v[0:8, v.shape[1] - 128:])


def _phi(t):
    return jnp.where(t > 0, t + 1.0, jnp.exp(t))


def _ln(x):
    d = x - jnp.mean(x, axis=-1, keepdims=True)
    v = jnp.mean(d * d, axis=-1, keepdims=True)
    return d * lax.rsqrt(v + 1e-5)


def _ln_items(x_ref, xn_ref, row0, nrows, dst0, ch, chunk=16):
    def item(r0):
        def run():
            yf = _ln(ch.link_first(x_ref[r0:r0 + chunk, :]))
            y = yf.astype(BF)
            for b in range(G):
                _st(xn_ref, b, r0 - row0 + dst0, y[:, b * 128:(b + 1) * 128])
            ch.done(yf)
        return run
    return [item(r0) for r0 in range(row0, row0 + nrows, chunk)]


def _interleave(main, side, span=None):
    span = len(main) if span is None else span
    done = 0
    for i, it in enumerate(main):
        upto = len(side) if i + 1 >= span else (len(side) * (i + 1)) // span
        for s_it in side[done:upto]:
            s_it()
        done = max(done, upto)
        it()


def _run(items):
    for it in items:
        it()


def _shuffle_rows(tf, tmp, store):
    for h in range(H):
        tmp[h * PITCH:h * PITCH + DH, :] = tf[h * DH:(h + 1) * DH]
    for d in range(DH):
        for th in range(2):
            rows = tmp[pl.ds(th * 16 * PITCH + d, 16, stride=PITCH), :]
            store(d * H + th * 16, rows.astype(BF))


def _qk_stage(g, q_ref, k_ref, s_ref, m_ref):
    lane = lax.broadcasted_iota(jnp.int32, (64, 128), 1)
    key = lax.broadcasted_iota(jnp.int32, (128, 512), 0)
    qry = lax.broadcasted_iota(jnp.int32, (128, 512), 1) & 127
    causal = key <= qry
    for j in range(4):
        nk = 128 * (j + 1)
        qt = _ldu(q_ref, g, j * 128, 128)
        wq = jnp.concatenate([jnp.where((lane >> 5) == h, qt, jnp.uint32(0)) for h in range(4)], axis=0)
        st = _dot_nt(_ld(k_ref, g, 0, nk), pltpu.bitcast(wq, BF))
        diag = jnp.where(causal, st[j * 128:], NEG)
        s_ref[OFF[j] + j * 128:OFF[j] + nk, :] = diag
        m = jnp.max(diag.reshape(16, 8, 512), axis=0)
        if j > 0:
            s_ref[OFF[j]:OFF[j] + j * 128, :] = st[:j * 128]
            m = jnp.maximum(m, jnp.max(st[:j * 128].reshape(16 * j, 8, 512), axis=0))
        m_ref[j] = jnp.broadcast_to(jnp.max(m, axis=0, keepdims=True), (8, 512))


def _sm_stage(s_ref, m_ref, p_ref, l_ref, ch=None, sub=16):
    ch = _Chain(None) if ch is None else ch
    for j in range(4):
        nk = 128 * (j + 1)
        for h in range(4):
            m = m_ref[j, :, h * 128:(h + 1) * 128]
            l = None
            for r in range(0, nk, sub):
                s = ch.link_first(s_ref[OFF[j] + r:OFF[j] + r + sub, h * 128:(h + 1) * 128])
                p = jnp.exp2(s.reshape(sub // 8, 8, 128) - m[None])
                ls = jnp.sum(p, axis=0)
                l = ls if l is None else l + ls
                _st(p_ref, h, OFF[j] + r, p.reshape(sub, 128).astype(BF))
                ch.done(p[0])
            l_ref[j, :, h * 128:(h + 1) * 128] = l


def _pv_stage(g, p_ref, l_ref, vt_ref, ot_ref, pq_ref, pk_ref, mt_ref, gate_ref):
    mem = mt_ref[g].astype(BF)
    for j in range(4):
        nd = _dot_nt(mem, _ld(pq_ref, g, j * 128, 128))
        for h in range(4):
            r0 = (g * 4 + h) * DH
            gate = gate_ref[pl.ds(g * 4 + h, 1), :]
            if PV_ONE_DOT:
                vt = jnp.concatenate([_ld(vt_ref, t, r0, DH) for t in range(j + 1)], axis=1)
                acc = _dot(vt, _ld(p_ref, h, OFF[j], 128 * (j + 1)))
            else:
                acc = None
                for t in range(j + 1):
                    o = _dot(_ld(vt_ref, t, r0, DH), _ld(p_ref, h, OFF[j] + t * 128, 128))
                    acc = o if acc is None else acc + o
            l = jnp.sum(l_ref[j, :, h * 128:(h + 1) * 128], axis=0, keepdims=True)
            den = nd[128 + h:129 + h] + 1e-6
            res = nd[h * DH:(h + 1) * DH] * (gate / den) + acc * ((1.0 - gate) / l)
            _st(ot_ref, j, r0, res.astype(BF))
    row = lax.broadcasted_iota(jnp.int32, (144, 128), 0)
    lane = lax.broadcasted_iota(jnp.int32, (144, 128), 1)
    keep = jnp.where(row < 128, row >> 5, row - 128) == (lane >> 5)
    row16 = lax.broadcasted_iota(jnp.int32, (16, 128), 0)
    ones = jnp.where(row16 < 4, 1.0, 0.0).astype(BF)
    upd = None
    for t in range(4):
        lhs = jnp.concatenate([_ld(vt_ref, t, g * 128, 128), ones], axis=0)
        u = _dot(lhs, _ld(pk_ref, g, t * 128, 128))
        upd = u if upd is None else upd + u
    mt_ref[g] = mt_ref[g] + jnp.where(keep, upd, 0.0)


def _band_items(pos0, row0, q_ref, k_ref, v_ref, a_ref, e_ref, o_ref, ch, nrows=HL):
    def logits(r0):
        def run():
            q = [q_ref[b, r0:r0 + 8, :] for b in range(G)]
            for w in range(W):
                base = HALO + r0 - DIL * w
                acc = ch.link(q[0] * k_ref[0, base:base + 8, :])
                for b in range(1, G):
                    acc = acc + q[b] * k_ref[b, base:base + 8, :]
                a_ref[w, r0 - row0:r0 - row0 + 8, :] = acc
                ch.done(acc)
        return run

    def softmax(r0):
        def run():
            lg = []
            for w in range(W):
                t = a_ref[w, r0 - row0:r0 - row0 + 128, :].T
                t = ((t[0:32] + t[32:64]) + (t[64:96] + t[96:128])) * QSCALE
                if r0 == row0 and w > 0:
                    pos = pos0 - DIL * w + lax.broadcasted_iota(jnp.int32, (H, 128), 1)
                    t = jnp.where(pos >= 0, t, NEG)
                lg.append(t)
            m = lg[0]
            for w in range(1, W):
                m = jnp.maximum(m, lg[w])
            e = [jnp.exp2(x - m) for x in lg]
            l = e[0]
            for w in range(1, W):
                l = l + e[w]
            inv = 1.0 / l
            for w in range(W):
                p = e[w] * inv
                pt = jnp.concatenate([p, p, p, p], axis=0).T
                e_ref[w, r0 - row0:r0 - row0 + 128, :] = pt
        return run

    def pv(r0):
        e = [e_ref[w, r0 - row0:r0 - row0 + 8, :] for w in range(W)]
        outs = []
        for b in range(G):
            acc = ch.link(e[0] * v_ref[b, HALO + r0:HALO + r0 + 8, :])
            for w in range(1, W):
                base = HALO + r0 - DIL * w
                acc = acc + e[w] * v_ref[b, base:base + 8, :]
            outs.append(acc)
            ch.done(acc)
        return outs

    def pv16(r0):
        def run():
            lo = pv(r0)
            hi = pv(r0 + 8)
            for b in range(G):
                _st(o_ref, b, r0, jnp.concatenate([lo[b], hi[b]], axis=0).astype(BF))
        return run

    items = []
    for r0 in range(row0, row0 + nrows, 128):
        items += [logits(r) for r in range(r0, r0 + 128, 8)]
        items.append(softmax(r0))
        items += [pv16(r) for r in range(r0, r0 + 128, 16)]
    return items


def _kernel(x_hbm, wq_hbm, wk_hbm, wv_hbm, woa_hbm, beta_ref, wqkv_hbm, wob_hbm, out_hbm,
            xin, obuf, x_f, xn, xc, xnx, wq, wk, woa, wv, wqkv, wvt, wbt, wob, wobp, tmp_a, tmp_b, tmp_c, tmp_d,
            q_ref, pq_ref, k_ref, pk_ref, vt_ref, ot_ref, o_nat,
            s_a, s_b, m_a, m_b, p_a, p_b, l_a, l_b, mt_ref, gate_ref,
            qn, kn, vn, qo, ko, vo, halo, ab, eb, ob0, ob1, sems):

    def col_copies(src, dst, sem, c0=0, n=G):
        return [pltpu.make_async_copy(src.at[:, (c0 + i) * 128:(c0 + i + 1) * 128], dst.at[c0 + i], sem)
                for i in range(n)]

    cp_wq = [col_copies(wq_hbm, wq, sems.at[c], 2 * c, 2) for c in range(4)]
    cp_wk = col_copies(wk_hbm, wk, sems.at[4])
    cp_wv = [pltpu.make_async_copy(wv_hbm, wv, sems.at[5])]
    cp_wqkv = [[pltpu.make_async_copy(wqkv_hbm.at[:, part * D:(part + 1) * D], wqkv.at[part], sems.at[6 + part])]
               for part in range(3)]
    cp_wob = col_copies(wob_hbm, wob, sems.at[9])
    cp_woa = col_copies(woa_hbm, woa, sems.at[10])
    cp_x0 = [pltpu.make_async_copy(x_hbm.at[0:L], xin.at[0:L], sems.at[11])]
    cp_xr = [pltpu.make_async_copy(x_hbm.at[L:S], xin.at[L:S], sems.at[12])]

    def cp_out(seg):
        return pltpu.make_async_copy(obuf, out_hbm.at[pl.ds(pl.multiple_of(seg * L, L), L)], sems.at[13])

    def wait(cps):
        for c in cps:
            c.wait()

    def wcols(w_ref, c0):
        return jnp.concatenate([_ld(w_ref, c0, 0, D), _ld(w_ref, c0 + 1, 0, D)], axis=1)

    def q_item(src, n, d0, c):
        def run():
            y = _dot(_wide(src, 0, n), wcols(wq, 2 * c))
            for gg in range(2):
                yq = y[:, gg * 128:(gg + 1) * 128]
                _st(q_ref, 2 * c + gg, d0, (yq * QSCALE).astype(BF))
                _st(pq_ref, 2 * c + gg, d0, _phi(yq).astype(BF))
        return run

    def k_item(src, n, d0, c):
        def run():
            y = _dot(_wide(src, 0, n), wcols(wk, 2 * c))
            for gg in range(2):
                yk = y[:, gg * 128:(gg + 1) * 128]
                _st(k_ref, 2 * c + gg, d0, yk.astype(BF))
                _st(pk_ref, 2 * c + gg, d0, _phi(yk).astype(BF))
        return run

    def v_item(src, r0, tile0, f0):
        def run():
            y = _dot_nt(_wide(wvt, f0, 512), _wide(src, r0, HL))
            _st(vt_ref, tile0, f0, y[:, :128].astype(BF))
            _st(vt_ref, tile0 + 1, f0, y[:, 128:].astype(BF))
        return run

    def attn_prologue():
        _qk_stage(0, q_ref, k_ref, s_a, m_a)
        _qk_stage(1, q_ref, k_ref, s_b, m_b)
        _sm_stage(s_a, m_a, p_a, l_a)

    def blk(i):
        return pl.ds(pl.multiple_of(i * 128, 128), 128)

    def qkv_shuffle(part, kbk, tmp):
        tf = wqkv[part, blk(kbk), :].T.astype(F32)
        _shuffle_rows(tf, tmp, lambda r, val: _st(wbt, kbk, part * D + r, val))

    with _scope("first_proj"):
        for cps in [cp_x0] + cp_wq + [cp_wv, cp_wk] + cp_wqkv + [cp_wob, cp_woa, cp_xr]:
            for c in cps:
                c.start()
        b = beta_ref[...].astype(F32).reshape(1, H)
        gt = jax.nn.sigmoid(b)
        row = lax.broadcasted_iota(jnp.int32, (H, H), 0)
        lane = lax.broadcasted_iota(jnp.int32, (H, H), 1)
        col = jnp.sum(jnp.where(row == lane, jnp.broadcast_to(gt, (H, H)), 0.0), axis=1, keepdims=True)
        gate_ref[...] = jnp.broadcast_to(col, (H, 128))
        halo[...] = jnp.zeros(halo.shape, F32)

        def zero_b(b, c):
            for r in (qn, kn, vn, ko, vo):
                r[b] = jnp.zeros(r.shape[1:], F32)
            return c
        lax.fori_loop(0, G, zero_b, 0)

        def zero_mem(i, c):
            mt_ref[i // G, i % G] = jnp.zeros((144, 128), F32)
            return c
        lax.fori_loop(0, 2 * G, zero_mem, 0)
        with _scope("p_wait_x"):
            wait(cp_x0)

        def ln0(i, c):
            for u in range(16):
                r0 = pl.multiple_of(i * HL + u * 16, 16)
                x = xin[pl.ds(r0, 16), :].astype(F32)
                x_f[pl.ds(r0, 16), :] = x
                y = _ln(x).astype(BF)
                for b in range(G):
                    _st(xn, b, r0, y[:, b * 128:(b + 1) * 128])
            return c
        with _scope("p_ln"):
            lax.fori_loop(0, 2, ln0, 0)

        def q0(c, carry):
            for i in range(2):
                pltpu.make_async_copy(wq_hbm.at[:, 0:128], wq.at[0], sems.at[c]).wait()
            q_item(xn, L, 0, c)()
            return carry
        with _scope("p_q"):
            lax.fori_loop(0, 4, q0, 0)
        wait(cp_wv)

        def tr0(i, carry):
            for u in range(4):
                _st(wvt, 4 * i + u, 0, wv[blk(4 * i + u), :].T)
            return carry
        with _scope("p_tr"):
            lax.fori_loop(0, 2, tr0, 0)

        def v0(i, carry):
            hf = i // 2
            v_item(xn, hf * HL, 2 * hf, (i % 2) * 512)()
            return carry
        with _scope("p_v"):
            lax.fori_loop(0, 4, v0, 0)
        wait(cp_wk)
        wait(cp_wqkv[0])
        wait(cp_wqkv[1])
        tmps = (tmp_a, tmp_b, tmp_c, tmp_d)

        def k0(c, carry):
            k_item(xn, L, 0, c)()
            for u in range(4):
                qkv_shuffle(c // 2, 4 * (c % 2) + u, tmps[u])
            return carry
        with _scope("p_k"):
            lax.fori_loop(0, 4, k0, 0)
        wait(cp_wqkv[2])
        wait(cp_wob)
        with _scope("p_attn"):
            attn_prologue()
            for u in range(G):
                qkv_shuffle(2, u, tmps[u % 4])
            for cb in range(G):
                _shuffle_rows(wob[cb].astype(F32), tmps[cb % 4], lambda r, val, cb=cb: _st(wobp, cb, r, val))
        wait(cp_woa)

    def out_item(src, s0, r0, w_ref, c, b0=0, b1=G, n=HL):
        def run():
            lhs = jnp.concatenate([_ld(src, b, s0, n) for b in range(b0, b1)], axis=1)
            w = jnp.concatenate([_ld(w_ref, 2 * c + i, b0 * 128, (b1 - b0) * 128) for i in range(2)], axis=1)
            x_f[r0:r0 + n, c * 256:(c + 1) * 256] += _dot(lhs, w)
        return run

    def b_proj_items():
        def item(part, c):
            def run():
                y = _dot_nt(_wide(xc, 0, HL), _wide(wbt, part * D + c * 256, 256))
                dst = (qn, kn, vn)[part]
                dst[2 * c] = y[:, :128]
                dst[2 * c + 1] = y[:, 128:]
            return run
        return [item(part, c) for part in range(3) for c in range(4)]

    def b_rotate():
        for b in range(G):
            qo[b] = qn[b]
            for new, old in ((kn, ko), (vn, vo)):
                old[b, 0:HALO, :] = old[b, HL:HL + HALO, :]
                old[b, HALO:, :] = new[b]

    def next_x_items(seg, layer, ch, chunk=16):
        nxt = jnp.minimum(seg + 1, NSEG - 1) * L

        def item(r0):
            def run():
                cur = ch.link_first(x_f[r0:r0 + chunk, :])
                obuf[r0:r0 + chunk, :] = cur.astype(BF)
                new = xin[pl.ds(pl.multiple_of(nxt + r0, chunk), chunk), :].astype(F32)
                x = jnp.where(layer == 1, new, cur)
                x_f[r0:r0 + chunk, :] = x
                yf = _ln(x)
                y = yf.astype(BF)
                for b in range(G):
                    _st(xc, b, r0, y[:, b * 128:(b + 1) * 128])
                ch.done(yf)
            return run
        return [item(r0) for r0 in range(0, HL, chunk)]

    def step(t, carry):
        seg = t // 2
        layer = t % 2
        mt = mt_ref.at[layer]
        never = lax.broadcasted_iota(jnp.int32, (8, 128), 0) < -t
        pv = lambda g, p, l: _pv_stage(g, p, l, vt_ref, ot_ref, pq_ref, pk_ref, mt, gate_ref)

        @pl.when(t > 0)
        def _():
            with _scope("A_proj"):
                def a_half(hf, c):
                    d0 = hf * HL
                    items = ([q_item(xc, HL, d0, c) for c in range(4)]
                             + [k_item(xc, HL, d0, c) for c in range(4)]
                             + [v_item(xc, 0, 2 * hf, f0) for f0 in (0, 512)])
                    _interleave(items, _ln_items(x_f, xnx, HL, HL, 0, _Chain(never)), span=8)
                    xc.bitcast(U32)[...] = xnx.bitcast(U32)[...]
                    return c

                lax.fori_loop(0, 2, a_half, 0)
            with _scope("A_attn_pro"):
                attn_prologue()

        def pair(u, c):
            g = 2 * u + 1
            _qk_stage(g + 1, q_ref, k_ref, s_a, m_a)
            _sm_stage(s_b, m_b, p_b, l_b)
            pv(g - 1, p_a, l_a)
            _qk_stage(g + 2, q_ref, k_ref, s_b, m_b)
            _sm_stage(s_a, m_a, p_a, l_a)
            pv(g, p_b, l_b)
            return c

        with _scope("A_attn_loop"):
            lax.fori_loop(0, 3, pair, 0)

        @pl.when(t == 0)
        def _():
            wait(cp_xr)

        @pl.when(jnp.logical_and(layer == 0, seg > 0))
        def _():
            cp_out(seg - 1).wait()

        def transpose_o(b0, b1):
            for j in range(4):
                ot = _ld(ot_ref, j, b0 * 128, (b1 - b0) * 128).T
                for b in range(b0, b1):
                    _st(o_nat, b, j * 128, ot[:, (b - b0) * 128:(b - b0 + 1) * 128])

        with _scope("A_out"):
            transpose_o(0, KSPLIT)
            _sm_stage(s_b, m_b, p_b, l_b, _Chain(never, NCH_EPI))
            pv(6, p_a, l_a)
            _run([out_item(o_nat, 0, 0, woa, c, 0, KSPLIT) for c in range(4)])
            pv(7, p_b, l_b)
            transpose_o(KSPLIT, G)
            kn[:, HL - HALO:HL, :] = halo[layer, 0]
            vn[:, HL - HALO:HL, :] = halo[layer, 1]
            _run([out_item(o_nat, 0, 0, woa, c, KSPLIT, G) for c in range(4)])
            _run(_ln_items(x_f, xc, 0, HL, 0, _Chain(never, 2)))
            _run([out_item(o_nat, HL, HL, woa, c) for c in range(4)])

        def b_half(hf, c):
            b_rotate()
            band = _band_items(seg * L + (hf - 1) * HL, 0, qo, ko, vo, ab, eb, ob0, _Chain(never))
            _interleave(b_proj_items(), band + _ln_items(x_f, xnx, HL, HL, 0, _Chain(never)))
            xc.bitcast(U32)[...] = xnx.bitcast(U32)[...]
            return c

        with _scope("B_loop"):
            lax.fori_loop(0, 2, b_half, 0)

        with _scope("B_tail"):
            halo[layer, 0] = kn[:, HL - HALO:HL, :]
            halo[layer, 1] = vn[:, HL - HALO:HL, :]
            b_rotate()
            _run(_band_items(seg * L + HL, 0, qo, ko, vo, ab, eb, ob1, _Chain(never, NCH_B1)))
            _run([out_item(ob0, 0, 0, wobp, c) for c in range(4)])
            _run(next_x_items(seg, layer, _Chain(never, 2)))
            _run([out_item(ob1, 0, HL, wobp, c, n=128) for c in range(4)])
            _run([out_item(ob1, 128, HL + 128, wobp, c, n=128) for c in range(4)])

        @pl.when(layer == 1)
        def _():
            obuf[HL:L, :] = x_f[HL:L, :].astype(BF)
            cp_out(seg).start()
            x_f[HL:L, :] = xin[pl.ds(pl.multiple_of(jnp.minimum(seg + 1, NSEG - 1) * L + HL, HL), HL), :].astype(F32)

        return carry

    lax.fori_loop(0, 2 * NSEG, step, 0)
    cp_out(NSEG - 1).wait()


@jax.jit
def pallas_interleave_layers__memory_aug_infini_attn__sliding_local_dilated__prompt_kernel(
    A_x: jax.Array,
    A_wq: jax.Array,
    A_wk: jax.Array,
    A_wv: jax.Array,
    A_wo: jax.Array,
    A_beta: jax.Array,
    B_x: jax.Array,
    B_wqkv: jax.Array,
    B_wo: jax.Array,
):
    del B_x
    x = A_x.reshape(S, D)
    any_spec = pl.BlockSpec(memory_space=pl.ANY)
    blk = lambda rows, dt: pltpu.VMEM((G, rows, 128), dt)
    packed = lambda rows, n=G: pltpu.VMEM((n, rows, 128), BF)
    scratch = [
        pltpu.VMEM((S, D), BF),
        pltpu.VMEM((L, D), BF),
        pltpu.VMEM((L, D), F32),
        packed(L),
        packed(HL),
        packed(HL),
        blk(D, BF),
        blk(D, BF),
        blk(D, BF),
        pltpu.VMEM((D, D), BF),
        pltpu.VMEM((3, D, D), BF),
        packed(D),
        packed(3 * D),
        blk(D, BF),
        packed(D),
        pltpu.VMEM((H * PITCH, 128), F32),
        pltpu.VMEM((H * PITCH, 128), F32),
        pltpu.VMEM((H * PITCH, 128), F32),
        pltpu.VMEM((H * PITCH, 128), F32),
        packed(L),
        packed(L),
        packed(L),
        packed(L),
        packed(D, 4),
        packed(D, 4),
        packed(L),
        pltpu.VMEM((1280, 512), F32),
        pltpu.VMEM((1280, 512), F32),
        pltpu.VMEM((4, 8, 512), F32),
        pltpu.VMEM((4, 8, 512), F32),
        packed(1280, 4),
        packed(1280, 4),
        pltpu.VMEM((4, 8, 512), F32),
        pltpu.VMEM((4, 8, 512), F32),
        pltpu.VMEM((2, G, 144, 128), F32),
        pltpu.VMEM((H, 128), F32),
        blk(HL, F32),
        blk(HL, F32),
        blk(HL, F32),
        blk(HL, F32),
        blk(HL + HALO, F32),
        blk(HL + HALO, F32),
        pltpu.VMEM((2, 2, G, HALO, 128), F32),
        pltpu.VMEM((W, HL, 128), F32),
        pltpu.VMEM((W, HL, 128), F32),
        packed(HL),
        packed(HL),
        pltpu.SemaphoreType.DMA((14,)),
    ]
    out = pl.pallas_call(
        _kernel,
        in_specs=[any_spec, any_spec, any_spec, any_spec, any_spec,
                  pl.BlockSpec(memory_space=pltpu.VMEM), any_spec, any_spec],
        out_specs=any_spec,
        out_shape=jax.ShapeDtypeStruct((S, D), BF),
        scratch_shapes=scratch,
        compiler_params=pltpu.CompilerParams(vmem_limit_bytes=100 * 1024 * 1024),
    )(x, A_wq, A_wk, A_wv, A_wo, A_beta, B_wqkv, B_wo)
    return out.reshape(1, S, D)
```

```python
import math

import jax
import jax.numpy as jnp
from jax import lax
import jax.experimental.pallas as pl
import jax.experimental.pallas.tpu as pltpu

S, D, H, DH = 2048, 1024, 32, 32
L, NSEG, G = 512, 4, 8
HL = L // 2
W, DIL = 8, 2
HALO = 16
BF, F32, U32 = jnp.bfloat16, jnp.float32, jnp.uint32
QSCALE = (DH ** -0.5) * math.log2(math.e)
NEG = -1e30
NT = (((1,), (1,)), ((), ()))
OFF = (0, 128, 384, 768)
SCOPES = False
NCH_B1 = 2
PV_ONE_DOT = True
KSPLIT = 6
NCH_EPI = 2
PITCH = 33


class _scope:
    def __init__(self, name):
        self.cm = jax.named_scope(name) if SCOPES else None

    def __enter__(self):
        if self.cm is not None:
            self.cm.__enter__()

    def __exit__(self, *a):
        if self.cm is not None:
            self.cm.__exit__(*a)


def _dot(a, b):
    return jnp.dot(a, b, preferred_element_type=F32)


def _dot_nt(a, b):
    return lax.dot_general(a, b, NT, preferred_element_type=F32)


def _rows(r0, n, align=16):
    return slice(r0, r0 + n) if isinstance(r0, int) else pl.ds(pl.multiple_of(r0, align), n)


def _ldu(ref, b, r0, n):
    idx = slice(r0 // 2, (r0 + n) // 2) if isinstance(r0, int) else pl.ds(pl.multiple_of(r0 // 2, 8), n // 2)
    return ref.bitcast(U32)[b, idx, :]


def _ld(ref, b, r0, n):
    return pltpu.bitcast(_ldu(ref, b, r0, n), BF)


def _st(ref, b, r0, val):
    ref[b, _rows(r0, val.shape[0]), :] = val


def _wide(ref, r0, n):
    return jnp.concatenate([_ld(ref, b, r0, n) for b in range(G)], axis=1)


class _Chain:
    def __init__(self, never, n=1):
        self.never, self.n, self.hist = never, n, []

    def link(self, x):
        if self.never is None or len(self.hist) < self.n:
            return x
        return jnp.where(self.never, self.hist[-self.n], x)

    def link_first(self, x):
        head = self.link(x[0:8, 0:128])
        if x.shape[1] > 128:
            head = jnp.concatenate([head, x[0:8, 128:]], axis=1)
        return head if x.shape[0] == 8 else jnp.concatenate([head, x[8:]], axis=0)

    def done(self, v):
        self.hist.append(v[0:8, v.shape[1] - 128:])


def _phi(t):
    return jnp.where(t > 0, t + 1.0, jnp.exp(t))


def _ln(x):
    d = x - jnp.mean(x, axis=-1, keepdims=True)
    v = jnp.mean(d * d, axis=-1, keepdims=True)
    return d * lax.rsqrt(v + 1e-5)


def _ln_items(x_ref, xn_ref, row0, nrows, dst0, ch, chunk=16):
    def item(r0):
        def run():
            yf = _ln(ch.link_first(x_ref[r0:r0 + chunk, :]))
            y = yf.astype(BF)
            for b in range(G):
                _st(xn_ref, b, r0 - row0 + dst0, y[:, b * 128:(b + 1) * 128])
            ch.done(yf)
        return run
    return [item(r0) for r0 in range(row0, row0 + nrows, chunk)]


def _interleave(main, side, span=None):
    span = len(main) if span is None else span
    done = 0
    for i, it in enumerate(main):
        upto = len(side) if i + 1 >= span else (len(side) * (i + 1)) // span
        for s_it in side[done:upto]:
            s_it()
        done = max(done, upto)
        it()


def _run(items):
    for it in items:
        it()


def _shuffle_rows(tf, tmp, store):
    for h in range(H):
        tmp[h * PITCH:h * PITCH + DH, :] = tf[h * DH:(h + 1) * DH]
    for d in range(DH):
        for th in range(2):
            rows = tmp[pl.ds(th * 16 * PITCH + d, 16, stride=PITCH), :]
            store(d * H + th * 16, rows.astype(BF))


def _qk_stage(g, q_ref, k_ref, s_ref, m_ref):
    lane = lax.broadcasted_iota(jnp.int32, (64, 128), 1)
    key = lax.broadcasted_iota(jnp.int32, (128, 512), 0)
    qry = lax.broadcasted_iota(jnp.int32, (128, 512), 1) & 127
    causal = key <= qry
    for j in range(4):
        nk = 128 * (j + 1)
        qt = _ldu(q_ref, g, j * 128, 128)
        wq = jnp.concatenate([jnp.where((lane >> 5) == h, qt, jnp.uint32(0)) for h in range(4)], axis=0)
        st = _dot_nt(_ld(k_ref, g, 0, nk), pltpu.bitcast(wq, BF))
        diag = jnp.where(causal, st[j * 128:], NEG)
        s_ref[OFF[j] + j * 128:OFF[j] + nk, :] = diag
        m = jnp.max(diag.reshape(16, 8, 512), axis=0)
        if j > 0:
            s_ref[OFF[j]:OFF[j] + j * 128, :] = st[:j * 128]
            m = jnp.maximum(m, jnp.max(st[:j * 128].reshape(16 * j, 8, 512), axis=0))
        m_ref[j] = jnp.broadcast_to(jnp.max(m, axis=0, keepdims=True), (8, 512))


def _sm_stage(s_ref, m_ref, p_ref, l_ref, ch=None, sub=16):
    ch = _Chain(None) if ch is None else ch
    for j in range(4):
        nk = 128 * (j + 1)
        for h in range(4):
            m = m_ref[j, :, h * 128:(h + 1) * 128]
            l = None
            for r in range(0, nk, sub):
                s = ch.link_first(s_ref[OFF[j] + r:OFF[j] + r + sub, h * 128:(h + 1) * 128])
                p = jnp.exp2(s.reshape(sub // 8, 8, 128) - m[None])
                ls = jnp.sum(p, axis=0)
                l = ls if l is None else l + ls
                _st(p_ref, h, OFF[j] + r, p.reshape(sub, 128).astype(BF))
                ch.done(p[0])
            l_ref[j, :, h * 128:(h + 1) * 128] = l


def _pv_stage(g, p_ref, l_ref, vt_ref, ot_ref, pq_ref, pk_ref, mt_ref, gate_ref):
    mem = mt_ref[g].astype(BF)
    for j in range(4):
        nd = _dot_nt(mem, _ld(pq_ref, g, j * 128, 128))
        for h in range(4):
            r0 = (g * 4 + h) * DH
            gate = gate_ref[pl.ds(g * 4 + h, 1), :]
            if PV_ONE_DOT:
                vt = jnp.concatenate([_ld(vt_ref, t, r0, DH) for t in range(j + 1)], axis=1)
                acc = _dot(vt, _ld(p_ref, h, OFF[j], 128 * (j + 1)))
            else:
                acc = None
                for t in range(j + 1):
                    o = _dot(_ld(vt_ref, t, r0, DH), _ld(p_ref, h, OFF[j] + t * 128, 128))
                    acc = o if acc is None else acc + o
            l = jnp.sum(l_ref[j, :, h * 128:(h + 1) * 128], axis=0, keepdims=True)
            den = nd[128 + h:129 + h] + 1e-6
            res = nd[h * DH:(h + 1) * DH] * (gate / den) + acc * ((1.0 - gate) / l)
            _st(ot_ref, j, r0, res.astype(BF))
    row = lax.broadcasted_iota(jnp.int32, (144, 128), 0)
    lane = lax.broadcasted_iota(jnp.int32, (144, 128), 1)
    keep = jnp.where(row < 128, row >> 5, row - 128) == (lane >> 5)
    row16 = lax.broadcasted_iota(jnp.int32, (16, 128), 0)
    ones = jnp.where(row16 < 4, 1.0, 0.0).astype(BF)
    upd = None
    for t in range(4):
        lhs = jnp.concatenate([_ld(vt_ref, t, g * 128, 128), ones], axis=0)
        u = _dot(lhs, _ld(pk_ref, g, t * 128, 128))
        upd = u if upd is None else upd + u
    mt_ref[g] = mt_ref[g] + jnp.where(keep, upd, 0.0)


def _band_items(pos0, row0, q_ref, k_ref, v_ref, a_ref, e_ref, o_ref, ch, nrows=HL):
    def logits(r0):
        def run():
            q = [q_ref[b, r0:r0 + 8, :] for b in range(G)]
            for w in range(W):
                base = HALO + r0 - DIL * w
                acc = ch.link(q[0] * k_ref[0, base:base + 8, :])
                for b in range(1, G):
                    acc = acc + q[b] * k_ref[b, base:base + 8, :]
                a_ref[w, r0 - row0:r0 - row0 + 8, :] = acc
                ch.done(acc)
        return run

    def softmax(r0):
        def run():
            lg = []
            for w in range(W):
                t = a_ref[w, r0 - row0:r0 - row0 + 128, :].T
                t = ((t[0:32] + t[32:64]) + (t[64:96] + t[96:128])) * QSCALE
                if r0 == row0 and w > 0:
                    pos = pos0 - DIL * w + lax.broadcasted_iota(jnp.int32, (H, 128), 1)
                    t = jnp.where(pos >= 0, t, NEG)
                lg.append(t)
            m = lg[0]
            for w in range(1, W):
                m = jnp.maximum(m, lg[w])
            e = [jnp.exp2(x - m) for x in lg]
            l = e[0]
            for w in range(1, W):
                l = l + e[w]
            inv = 1.0 / l
            for w in range(W):
                p = e[w] * inv
                pt = jnp.concatenate([p, p, p, p], axis=0).T
                e_ref[w, r0 - row0:r0 - row0 + 128, :] = pt
        return run

    def pv(r0):
        e = [e_ref[w, r0 - row0:r0 - row0 + 8, :] for w in range(W)]
        outs = []
        for b in range(G):
            acc = ch.link(e[0] * v_ref[b, HALO + r0:HALO + r0 + 8, :])
            for w in range(1, W):
                base = HALO + r0 - DIL * w
                acc = acc + e[w] * v_ref[b, base:base + 8, :]
            outs.append(acc)
            ch.done(acc)
        return outs

    def pv16(r0):
        def run():
            lo = pv(r0)
            hi = pv(r0 + 8)
            for b in range(G):
                _st(o_ref, b, r0, jnp.concatenate([lo[b], hi[b]], axis=0).astype(BF))
        return run

    items = []
    for r0 in range(row0, row0 + nrows, 128):
        items += [logits(r) for r in range(r0, r0 + 128, 8)]
        items.append(softmax(r0))
        items += [pv16(r) for r in range(r0, r0 + 128, 16)]
    return items


def _kernel(x_hbm, wq_hbm, wk_hbm, wv_hbm, woa_hbm, beta_ref, wqkv_hbm, wob_hbm, out_hbm,
            xin, obuf, x_f, xn, xc, xnx, wq, wk, woa, wv, wqkv, wvt, wbt, wob, wobp, tmp_a, tmp_b, tmp_c, tmp_d,
            q_ref, pq_ref, k_ref, pk_ref, vt_ref, ot_ref, o_nat,
            s_a, s_b, m_a, m_b, p_a, p_b, l_a, l_b, mt_ref, gate_ref,
            qn, kn, vn, qo, ko, vo, halo, ab, eb, ob0, ob1, sems):

    def col_copies(src, dst, sem, c0=0, n=G):
        return [pltpu.make_async_copy(src.at[:, (c0 + i) * 128:(c0 + i + 1) * 128], dst.at[c0 + i], sem)
                for i in range(n)]

    cp_wq = [col_copies(wq_hbm, wq, sems.at[c], 2 * c, 2) for c in range(4)]
    cp_wk = col_copies(wk_hbm, wk, sems.at[4])
    cp_wv = [pltpu.make_async_copy(wv_hbm, wv, sems.at[5])]
    cp_wqkv = [[pltpu.make_async_copy(wqkv_hbm.at[:, part * D:(part + 1) * D], wqkv.at[part], sems.at[6 + part])]
               for part in range(3)]
    cp_wob = col_copies(wob_hbm, wob, sems.at[9])
    cp_woa = col_copies(woa_hbm, woa, sems.at[10])
    cp_x0 = [pltpu.make_async_copy(x_hbm.at[0:L], xin.at[0:L], sems.at[11])]
    cp_xr = [pltpu.make_async_copy(x_hbm.at[L:S], xin.at[L:S], sems.at[12])]

    def cp_out(seg):
        return pltpu.make_async_copy(obuf, out_hbm.at[pl.ds(pl.multiple_of(seg * L, L), L)], sems.at[13])

    def wait(cps):
        for c in cps:
            c.wait()

    def wcols(w_ref, c0):
        return jnp.concatenate([_ld(w_ref, c0, 0, D), _ld(w_ref, c0 + 1, 0, D)], axis=1)

    def q_item(src, n, d0, c):
        def run():
            y = _dot(_wide(src, 0, n), wcols(wq, 2 * c))
            for gg in range(2):
                yq = y[:, gg * 128:(gg + 1) * 128]
                _st(q_ref, 2 * c + gg, d0, (yq * QSCALE).astype(BF))
                _st(pq_ref, 2 * c + gg, d0, _phi(yq).astype(BF))
        return run

    def k_item(src, n, d0, c):
        def run():
            y = _dot(_wide(src, 0, n), wcols(wk, 2 * c))
            for gg in range(2):
                yk = y[:, gg * 128:(gg + 1) * 128]
                _st(k_ref, 2 * c + gg, d0, yk.astype(BF))
                _st(pk_ref, 2 * c + gg, d0, _phi(yk).astype(BF))
        return run

    def v_item(src, r0, tile0, f0):
        def run():
            y = _dot_nt(_wide(wvt, f0, 512), _wide(src, r0, HL))
            _st(vt_ref, tile0, f0, y[:, :128].astype(BF))
            _st(vt_ref, tile0 + 1, f0, y[:, 128:].astype(BF))
        return run

    def attn_prologue():
        _qk_stage(0, q_ref, k_ref, s_a, m_a)
        _qk_stage(1, q_ref, k_ref, s_b, m_b)
        _sm_stage(s_a, m_a, p_a, l_a)

    def blk(i):
        return pl.ds(pl.multiple_of(i * 128, 128), 128)

    def qkv_shuffle(part, kbk, tmp):
        tf = wqkv[part, blk(kbk), :].T.astype(F32)
        _shuffle_rows(tf, tmp, lambda r, val: _st(wbt, kbk, part * D + r, val))

    with _scope("first_proj"):
        for cps in [cp_x0] + cp_wq + [cp_wv, cp_wk] + cp_wqkv + [cp_wob, cp_woa, cp_xr]:
            for c in cps:
                c.start()
        b = beta_ref[...].astype(F32).reshape(1, H)
        gt = jax.nn.sigmoid(b)
        row = lax.broadcasted_iota(jnp.int32, (H, H), 0)
        lane = lax.broadcasted_iota(jnp.int32, (H, H), 1)
        col = jnp.sum(jnp.where(row == lane, jnp.broadcast_to(gt, (H, H)), 0.0), axis=1, keepdims=True)
        gate_ref[...] = jnp.broadcast_to(col, (H, 128))
        halo[...] = jnp.zeros(halo.shape, F32)

        def zero_b(b, c):
            for r in (qn, kn, vn, ko, vo):
                r[b] = jnp.zeros(r.shape[1:], F32)
            return c
        lax.fori_loop(0, G, zero_b, 0)

        def zero_mem(i, c):
            mt_ref[i // G, i % G] = jnp.zeros((144, 128), F32)
            return c
        lax.fori_loop(0, 2 * G, zero_mem, 0)
        with _scope("p_wait_x"):
            wait(cp_x0)

        def ln0(i, c):
            for u in range(16):
                r0 = pl.multiple_of(i * HL + u * 16, 16)
                x = xin[pl.ds(r0, 16), :].astype(F32)
                x_f[pl.ds(r0, 16), :] = x
                y = _ln(x).astype(BF)
                for b in range(G):
                    _st(xn, b, r0, y[:, b * 128:(b + 1) * 128])
            return c
        with _scope("p_ln"):
            lax.fori_loop(0, 2, ln0, 0)

        def q0(c, carry):
            for i in range(2):
                pltpu.make_async_copy(wq_hbm.at[:, 0:128], wq.at[0], sems.at[c]).wait()
            q_item(xn, L, 0, c)()
            return carry
        with _scope("p_q"):
            lax.fori_loop(0, 3, q0, 0)
        wait(cp_wq[3])
        wait(cp_wv)
        with _scope("p_tr"):
            q_item(xn, L, 0, 3)()
            for kbk in range(G):
                _st(wvt, kbk, 0, wv[kbk * 128:(kbk + 1) * 128, :].T)

        def v0(i, carry):
            hf = i // 2
            v_item(xn, hf * HL, 2 * hf, (i % 2) * 512)()
            return carry
        with _scope("p_v"):
            lax.fori_loop(0, 4, v0, 0)
        wait(cp_wk)
        wait(cp_wqkv[0])
        tmps = (tmp_a, tmp_b, tmp_c, tmp_d)

        def k0(c, carry):
            k_item(xn, L, 0, c)()
            for u in range(2):
                qkv_shuffle(0, 2 * c + u, tmps[u])
            return carry
        with _scope("p_k"):
            lax.fori_loop(0, 4, k0, 0)
        wait(cp_wqkv[1])
        wait(cp_wqkv[2])
        with _scope("p_attn"):
            attn_prologue()
            for u in range(2 * G):
                qkv_shuffle(1 + u // G, u % G, tmps[u % 4])
        wait(cp_wob)

        def sh1(i, carry):
            for u in range(4):
                cb = 4 * i + u
                _shuffle_rows(wob[cb].astype(F32), tmps[u], lambda r, val, cb=cb: _st(wobp, cb, r, val))
            return carry
        with _scope("p_sh1"):
            lax.fori_loop(0, 2, sh1, 0)
        wait(cp_woa)

    def out_item(src, s0, r0, w_ref, c, b0=0, b1=G, n=HL):
        def run():
            lhs = jnp.concatenate([_ld(src, b, s0, n) for b in range(b0, b1)], axis=1)
            w = jnp.concatenate([_ld(w_ref, 2 * c + i, b0 * 128, (b1 - b0) * 128) for i in range(2)], axis=1)
            x_f[r0:r0 + n, c * 256:(c + 1) * 256] += _dot(lhs, w)
        return run

    def b_proj_items():
        def item(part, c):
            def run():
                y = _dot_nt(_wide(xc, 0, HL), _wide(wbt, part * D + c * 256, 256))
                dst = (qn, kn, vn)[part]
                dst[2 * c] = y[:, :128]
                dst[2 * c + 1] = y[:, 128:]
            return run
        return [item(part, c) for part in range(3) for c in range(4)]

    def b_rotate():
        for b in range(G):
            qo[b] = qn[b]
            for new, old in ((kn, ko), (vn, vo)):
                old[b, 0:HALO, :] = old[b, HL:HL + HALO, :]
                old[b, HALO:, :] = new[b]

    def next_x_items(seg, layer, ch, chunk=16):
        nxt = jnp.minimum(seg + 1, NSEG - 1) * L

        def item(r0):
            def run():
                cur = ch.link_first(x_f[r0:r0 + chunk, :])
                obuf[r0:r0 + chunk, :] = cur.astype(BF)
                new = xin[pl.ds(pl.multiple_of(nxt + r0, chunk), chunk), :].astype(F32)
                x = jnp.where(layer == 1, new, cur)
                x_f[r0:r0 + chunk, :] = x
                yf = _ln(x)
                y = yf.astype(BF)
                for b in range(G):
                    _st(xc, b, r0, y[:, b * 128:(b + 1) * 128])
                ch.done(yf)
            return run
        return [item(r0) for r0 in range(0, HL, chunk)]

    def step(t, carry):
        seg = t // 2
        layer = t % 2
        mt = mt_ref.at[layer]
        never = lax.broadcasted_iota(jnp.int32, (8, 128), 0) < -t
        pv = lambda g, p, l: _pv_stage(g, p, l, vt_ref, ot_ref, pq_ref, pk_ref, mt, gate_ref)

        @pl.when(t > 0)
        def _():
            with _scope("A_proj"):
                def a_half(hf, c):
                    d0 = hf * HL
                    items = ([q_item(xc, HL, d0, c) for c in range(4)]
                             + [k_item(xc, HL, d0, c) for c in range(4)]
                             + [v_item(xc, 0, 2 * hf, f0) for f0 in (0, 512)])
                    _interleave(items, _ln_items(x_f, xnx, HL, HL, 0, _Chain(never)), span=8)
                    xc.bitcast(U32)[...] = xnx.bitcast(U32)[...]
                    return c

                lax.fori_loop(0, 2, a_half, 0)
            with _scope("A_attn_pro"):
                attn_prologue()

        def pair(u, c):
            g = 2 * u + 1
            _qk_stage(g + 1, q_ref, k_ref, s_a, m_a)
            _sm_stage(s_b, m_b, p_b, l_b)
            pv(g - 1, p_a, l_a)
            _qk_stage(g + 2, q_ref, k_ref, s_b, m_b)
            _sm_stage(s_a, m_a, p_a, l_a)
            pv(g, p_b, l_b)
            return c

        with _scope("A_attn_loop"):
            lax.fori_loop(0, 3, pair, 0)

        @pl.when(t == 0)
        def _():
            wait(cp_xr)

        @pl.when(jnp.logical_and(layer == 0, seg > 0))
        def _():
            cp_out(seg - 1).wait()

        def transpose_o(b0, b1):
            for j in range(4):
                ot = _ld(ot_ref, j, b0 * 128, (b1 - b0) * 128).T
                for b in range(b0, b1):
                    _st(o_nat, b, j * 128, ot[:, (b - b0) * 128:(b - b0 + 1) * 128])

        with _scope("A_out"):
            transpose_o(0, KSPLIT)
            _sm_stage(s_b, m_b, p_b, l_b, _Chain(never, NCH_EPI))
            pv(6, p_a, l_a)
            _run([out_item(o_nat, 0, 0, woa, c, 0, KSPLIT) for c in range(4)])
            pv(7, p_b, l_b)
            transpose_o(KSPLIT, G)
            kn[:, HL - HALO:HL, :] = halo[layer, 0]
            vn[:, HL - HALO:HL, :] = halo[layer, 1]
            _run([out_item(o_nat, 0, 0, woa, c, KSPLIT, G) for c in range(4)])
            _run(_ln_items(x_f, xc, 0, HL, 0, _Chain(never, 2)))
            _run([out_item(o_nat, HL, HL, woa, c) for c in range(4)])

        def b_half(hf, c):
            b_rotate()
            band = _band_items(seg * L + (hf - 1) * HL, 0, qo, ko, vo, ab, eb, ob0, _Chain(never))
            _interleave(b_proj_items(), band + _ln_items(x_f, xnx, HL, HL, 0, _Chain(never)))
            xc.bitcast(U32)[...] = xnx.bitcast(U32)[...]
            return c

        with _scope("B_loop"):
            lax.fori_loop(0, 2, b_half, 0)

        with _scope("B_tail"):
            halo[layer, 0] = kn[:, HL - HALO:HL, :]
            halo[layer, 1] = vn[:, HL - HALO:HL, :]
            b_rotate()
            _run(_band_items(seg * L + HL, 0, qo, ko, vo, ab, eb, ob1, _Chain(never, NCH_B1)))
            _run([out_item(ob0, 0, 0, wobp, c) for c in range(4)])
            _run(next_x_items(seg, layer, _Chain(never, 2)))
            _run([out_item(ob1, 0, HL, wobp, c, n=128) for c in range(4)])
            _run([out_item(ob1, 128, HL + 128, wobp, c, n=128) for c in range(4)])

        @pl.when(layer == 1)
        def _():
            obuf[HL:L, :] = x_f[HL:L, :].astype(BF)
            cp_out(seg).start()
            x_f[HL:L, :] = xin[pl.ds(pl.multiple_of(jnp.minimum(seg + 1, NSEG - 1) * L + HL, HL), HL), :].astype(F32)

        return carry

    lax.fori_loop(0, 2 * NSEG, step, 0)
    cp_out(NSEG - 1).wait()


@jax.jit
def pallas_interleave_layers__memory_aug_infini_attn__sliding_local_dilated__prompt_kernel(
    A_x: jax.Array,
    A_wq: jax.Array,
    A_wk: jax.Array,
    A_wv: jax.Array,
    A_wo: jax.Array,
    A_beta: jax.Array,
    B_x: jax.Array,
    B_wqkv: jax.Array,
    B_wo: jax.Array,
):
    del B_x
    x = A_x.reshape(S, D)
    any_spec = pl.BlockSpec(memory_space=pl.ANY)
    blk = lambda rows, dt: pltpu.VMEM((G, rows, 128), dt)
    packed = lambda rows, n=G: pltpu.VMEM((n, rows, 128), BF)
    scratch = [
        pltpu.VMEM((S, D), BF),
        pltpu.VMEM((L, D), BF),
        pltpu.VMEM((L, D), F32),
        packed(L),
        packed(HL),
        packed(HL),
        blk(D, BF),
        blk(D, BF),
        blk(D, BF),
        pltpu.VMEM((D, D), BF),
        pltpu.VMEM((3, D, D), BF),
        packed(D),
        packed(3 * D),
        blk(D, BF),
        packed(D),
        pltpu.VMEM((H * PITCH, 128), F32),
        pltpu.VMEM((H * PITCH, 128), F32),
        pltpu.VMEM((H * PITCH, 128), F32),
        pltpu.VMEM((H * PITCH, 128), F32),
        packed(L),
        packed(L),
        packed(L),
        packed(L),
        packed(D, 4),
        packed(D, 4),
        packed(L),
        pltpu.VMEM((1280, 512), F32),
        pltpu.VMEM((1280, 512), F32),
        pltpu.VMEM((4, 8, 512), F32),
        pltpu.VMEM((4, 8, 512), F32),
        packed(1280, 4),
        packed(1280, 4),
        pltpu.VMEM((4, 8, 512), F32),
        pltpu.VMEM((4, 8, 512), F32),
        pltpu.VMEM((2, G, 144, 128), F32),
        pltpu.VMEM((H, 128), F32),
        blk(HL, F32),
        blk(HL, F32),
        blk(HL, F32),
        blk(HL, F32),
        blk(HL + HALO, F32),
        blk(HL + HALO, F32),
        pltpu.VMEM((2, 2, G, HALO, 128), F32),
        pltpu.VMEM((W, HL, 128), F32),
        pltpu.VMEM((W, HL, 128), F32),
        packed(HL),
        packed(HL),
        pltpu.SemaphoreType.DMA((14,)),
    ]
    out = pl.pallas_call(
        _kernel,
        in_specs=[any_spec, any_spec, any_spec, any_spec, any_spec,
                  pl.BlockSpec(memory_space=pltpu.VMEM), any_spec, any_spec],
        out_specs=any_spec,
        out_shape=jax.ShapeDtypeStruct((S, D), BF),
        scratch_shapes=scratch,
        compiler_params=pltpu.CompilerParams(vmem_limit_bytes=100 * 1024 * 1024),
    )(x, A_wq, A_wk, A_wv, A_wo, A_beta, B_wqkv, B_wo)
    return out.reshape(1, S, D)
```

```python
import math

import jax
import jax.numpy as jnp
from jax import lax
import jax.experimental.pallas as pl
import jax.experimental.pallas.tpu as pltpu

S, D, H, DH = 2048, 1024, 32, 32
L, NSEG, G = 512, 4, 8
HL = L // 2
W, DIL = 8, 2
HALO = 16
BF, F32, U32 = jnp.bfloat16, jnp.float32, jnp.uint32
QSCALE = (DH ** -0.5) * math.log2(math.e)
NEG = -1e30
NT = (((1,), (1,)), ((), ()))
OFF = (0, 128, 384, 768)
SCOPES = False
NCH_B1 = 2
PV_ONE_DOT = True
KSPLIT = 6
NCH_EPI = 2
PITCH = 33


class _scope:
    def __init__(self, name):
        self.cm = jax.named_scope(name) if SCOPES else None

    def __enter__(self):
        if self.cm is not None:
            self.cm.__enter__()

    def __exit__(self, *a):
        if self.cm is not None:
            self.cm.__exit__(*a)


def _dot(a, b):
    return jnp.dot(a, b, preferred_element_type=F32)


def _dot_nt(a, b):
    return lax.dot_general(a, b, NT, preferred_element_type=F32)


def _rows(r0, n, align=16):
    return slice(r0, r0 + n) if isinstance(r0, int) else pl.ds(pl.multiple_of(r0, align), n)


def _ldu(ref, b, r0, n):
    idx = slice(r0 // 2, (r0 + n) // 2) if isinstance(r0, int) else pl.ds(pl.multiple_of(r0 // 2, 8), n // 2)
    return ref.bitcast(U32)[b, idx, :]


def _ld(ref, b, r0, n):
    return pltpu.bitcast(_ldu(ref, b, r0, n), BF)


def _st(ref, b, r0, val):
    ref[b, _rows(r0, val.shape[0]), :] = val


def _wide(ref, r0, n):
    return jnp.concatenate([_ld(ref, b, r0, n) for b in range(G)], axis=1)


class _Chain:
    def __init__(self, never, n=1):
        self.never, self.n, self.hist = never, n, []

    def link(self, x):
        if self.never is None or len(self.hist) < self.n:
            return x
        return jnp.where(self.never, self.hist[-self.n], x)

    def link_first(self, x):
        head = self.link(x[0:8, 0:128])
        if x.shape[1] > 128:
            head = jnp.concatenate([head, x[0:8, 128:]], axis=1)
        return head if x.shape[0] == 8 else jnp.concatenate([head, x[8:]], axis=0)

    def done(self, v):
        self.hist.append(v[0:8, v.shape[1] - 128:])


def _phi(t):
    return jnp.where(t > 0, t + 1.0, jnp.exp(t))


def _ln(x):
    d = x - jnp.mean(x, axis=-1, keepdims=True)
    v = jnp.mean(d * d, axis=-1, keepdims=True)
    return d * lax.rsqrt(v + 1e-5)


def _ln_items(x_ref, xn_ref, row0, nrows, dst0, ch, chunk=16):
    def item(r0):
        def run():
            yf = _ln(ch.link_first(x_ref[r0:r0 + chunk, :]))
            y = yf.astype(BF)
            for b in range(G):
                _st(xn_ref, b, r0 - row0 + dst0, y[:, b * 128:(b + 1) * 128])
            ch.done(yf)
        return run
    return [item(r0) for r0 in range(row0, row0 + nrows, chunk)]


def _interleave(main, side, span=None):
    span = len(main) if span is None else span
    done = 0
    for i, it in enumerate(main):
        upto = len(side) if i + 1 >= span else (len(side) * (i + 1)) // span
        for s_it in side[done:upto]:
            s_it()
        done = max(done, upto)
        it()


def _run(items):
    for it in items:
        it()


def _shuffle_rows(tf, tmp, store):
    for h in range(H):
        tmp[h * PITCH:h * PITCH + DH, :] = tf[h * DH:(h + 1) * DH]
    for d in range(DH):
        for th in range(2):
            rows = tmp[pl.ds(th * 16 * PITCH + d, 16, stride=PITCH), :]
            store(d * H + th * 16, rows.astype(BF))


def _qk_stage(g, q_ref, k_ref, s_ref, m_ref, bias_ref):
    lane = lax.broadcasted_iota(jnp.int32, (64, 128), 1)
    for j in range(4):
        nk = 128 * (j + 1)
        qt = _ldu(q_ref, g, j * 128, 128)
        wq = jnp.concatenate([jnp.where((lane >> 5) == h, qt, jnp.uint32(0)) for h in range(4)], axis=0)
        st = _dot_nt(_ld(k_ref, g, 0, nk), pltpu.bitcast(wq, BF))
        bias = bias_ref[...]
        diag = st[j * 128:] + jnp.concatenate([bias] * 4, axis=1)
        s_ref[OFF[j] + j * 128:OFF[j] + nk, :] = diag
        m = jnp.max(diag.reshape(16, 8, 512), axis=0)
        if j > 0:
            s_ref[OFF[j]:OFF[j] + j * 128, :] = st[:j * 128]
            m = jnp.maximum(m, jnp.max(st[:j * 128].reshape(16 * j, 8, 512), axis=0))
        m_ref[j] = jnp.broadcast_to(jnp.max(m, axis=0, keepdims=True), (8, 512))


def _sm_stage(s_ref, m_ref, p_ref, l_ref, ch=None, sub=16):
    ch = _Chain(None) if ch is None else ch
    for j in range(4):
        nk = 128 * (j + 1)
        sums = []
        for h in range(4):
            m = m_ref[j, :, h * 128:(h + 1) * 128]
            l = None
            for r in range(0, nk, sub):
                s = ch.link_first(s_ref[OFF[j] + r:OFF[j] + r + sub, h * 128:(h + 1) * 128])
                p = jnp.exp2(s.reshape(sub // 8, 8, 128) - m[None])
                ls = jnp.sum(p, axis=0)
                l = ls if l is None else l + ls
                _st(p_ref, h, OFF[j] + r, p.reshape(sub, 128).astype(BF))
                ch.done(p[0])
            sums.append(jnp.sum(l, axis=0, keepdims=True))
        l_ref[j] = jnp.concatenate(sums + sums, axis=0)


def _pv_stage(g, p_ref, l_ref, vt_ref, ot_ref, pq_ref, pk_ref, mt_ref, gate_ref):
    mem = mt_ref[g].astype(BF)
    gate = gate_ref[g]
    for j in range(4):
        nd = _dot_nt(mem, _ld(pq_ref, g, j * 128, 128))
        c_mem = gate / (nd[128:136] + 1e-6)
        c_att = (1.0 - gate) / l_ref[j]
        for h in range(4):
            r0 = (g * 4 + h) * DH
            vt = jnp.concatenate([_ld(vt_ref, t, r0, DH) for t in range(j + 1)], axis=1)
            acc = _dot(vt, _ld(p_ref, h, OFF[j], 128 * (j + 1)))
            res = nd[h * DH:(h + 1) * DH] * c_mem[h:h + 1] + acc * c_att[h:h + 1]
            _st(ot_ref, j, r0, res.astype(BF))
    row = lax.broadcasted_iota(jnp.int32, (144, 128), 0)
    lane = lax.broadcasted_iota(jnp.int32, (144, 128), 1)
    keep = jnp.where(row < 128, row >> 5, row - 128) == (lane >> 5)
    row16 = lax.broadcasted_iota(jnp.int32, (16, 128), 0)
    ones = jnp.where(row16 < 4, 1.0, 0.0).astype(BF)
    upd = None
    for t in range(4):
        lhs = jnp.concatenate([_ld(vt_ref, t, g * 128, 128), ones], axis=0)
        u = _dot(lhs, _ld(pk_ref, g, t * 128, 128))
        upd = u if upd is None else upd + u
    mt_ref[g] = mt_ref[g] + jnp.where(keep, upd, 0.0)


def _band_items(pos0, row0, q_ref, k_ref, v_ref, a_ref, e_ref, o_ref, ch, nrows=HL):
    def logits(r0):
        def run():
            q = [q_ref[b, r0:r0 + 8, :] for b in range(G)]
            for w in range(W):
                base = HALO + r0 - DIL * w
                acc = ch.link(q[0] * k_ref[0, base:base + 8, :])
                for b in range(1, G):
                    acc = acc + q[b] * k_ref[b, base:base + 8, :]
                a_ref[w, r0 - row0:r0 - row0 + 8, :] = acc
                ch.done(acc)
        return run

    def softmax(r0):
        def run():
            lg = []
            for w in range(W):
                t = a_ref[w, r0 - row0:r0 - row0 + 128, :].T
                t = ((t[0:32] + t[32:64]) + (t[64:96] + t[96:128])) * QSCALE
                if r0 == row0 and w > 0:
                    pos = pos0 - DIL * w + lax.broadcasted_iota(jnp.int32, (H, 128), 1)
                    t = jnp.where(pos >= 0, t, NEG)
                lg.append(t)
            m = lg[0]
            for w in range(1, W):
                m = jnp.maximum(m, lg[w])
            e = [jnp.exp2(x - m) for x in lg]
            l = e[0]
            for w in range(1, W):
                l = l + e[w]
            inv = 1.0 / l
            for w in range(W):
                p = e[w] * inv
                pt = jnp.concatenate([p, p, p, p], axis=0).T
                e_ref[w, r0 - row0:r0 - row0 + 128, :] = pt
        return run

    def pv(r0):
        e = [e_ref[w, r0 - row0:r0 - row0 + 8, :] for w in range(W)]
        outs = []
        for b in range(G):
            acc = ch.link(e[0] * v_ref[b, HALO + r0:HALO + r0 + 8, :])
            for w in range(1, W):
                base = HALO + r0 - DIL * w
                acc = acc + e[w] * v_ref[b, base:base + 8, :]
            outs.append(acc)
            ch.done(acc)
        return outs

    def pv16(r0):
        def run():
            lo = pv(r0)
            hi = pv(r0 + 8)
            for b in range(G):
                _st(o_ref, b, r0, jnp.concatenate([lo[b], hi[b]], axis=0).astype(BF))
        return run

    items = []
    for r0 in range(row0, row0 + nrows, 128):
        items += [logits(r) for r in range(r0, r0 + 128, 8)]
        items.append(softmax(r0))
        items += [pv16(r) for r in range(r0, r0 + 128, 16)]
    return items


def _kernel(x_hbm, wq_hbm, wk_hbm, wv_hbm, woa_hbm, beta_ref, wqkv_hbm, wob_hbm, out_hbm,
            xin, obuf, x_f, xn, xc, xnx, wq, wk, woa, wv, wqkv, wvt, wbt, wob, wobp, tmp_a, tmp_b, tmp_c, tmp_d,
            q_ref, pq_ref, k_ref, pk_ref, vt_ref, ot_ref, o_nat,
            s_a, s_b, m_a, m_b, p_a, p_b, l_a, l_b, mt_ref, gate_ref, bias_ref,
            qn, kn, vn, qo, ko, vo, halo, ab, eb, ob0, ob1, sems):

    def col_copies(src, dst, sem, c0=0, n=G):
        return [pltpu.make_async_copy(src.at[:, (c0 + i) * 128:(c0 + i + 1) * 128], dst.at[c0 + i], sem)
                for i in range(n)]

    cp_wq = [col_copies(wq_hbm, wq, sems.at[c], 2 * c, 2) for c in range(4)]
    cp_wk = col_copies(wk_hbm, wk, sems.at[4])
    cp_wv = [pltpu.make_async_copy(wv_hbm, wv, sems.at[5])]
    cp_wqkv = [[pltpu.make_async_copy(wqkv_hbm.at[:, part * D:(part + 1) * D], wqkv.at[part], sems.at[6 + part])]
               for part in range(3)]
    cp_wob = col_copies(wob_hbm, wob, sems.at[9])
    cp_woa = col_copies(woa_hbm, woa, sems.at[10])
    cp_x0 = [pltpu.make_async_copy(x_hbm.at[0:L], xin.at[0:L], sems.at[11])]
    cp_xr = [pltpu.make_async_copy(x_hbm.at[L:S], xin.at[L:S], sems.at[12])]

    def cp_out(seg):
        return pltpu.make_async_copy(obuf, out_hbm.at[pl.ds(pl.multiple_of(seg * L, L), L)], sems.at[13])

    def wait(cps):
        for c in cps:
            c.wait()

    def wcols(w_ref, c0):
        return jnp.concatenate([_ld(w_ref, c0, 0, D), _ld(w_ref, c0 + 1, 0, D)], axis=1)

    def q_item(src, n, d0, c):
        def run():
            y = _dot(_wide(src, 0, n), wcols(wq, 2 * c))
            for gg in range(2):
                yq = y[:, gg * 128:(gg + 1) * 128]
                _st(q_ref, 2 * c + gg, d0, (yq * QSCALE).astype(BF))
                _st(pq_ref, 2 * c + gg, d0, _phi(yq).astype(BF))
        return run

    def k_item(src, n, d0, c):
        def run():
            y = _dot(_wide(src, 0, n), wcols(wk, 2 * c))
            for gg in range(2):
                yk = y[:, gg * 128:(gg + 1) * 128]
                _st(k_ref, 2 * c + gg, d0, yk.astype(BF))
                _st(pk_ref, 2 * c + gg, d0, _phi(yk).astype(BF))
        return run

    def v_item(src, r0, tile0, f0):
        def run():
            y = _dot_nt(_wide(wvt, f0, 512), _wide(src, r0, HL))
            _st(vt_ref, tile0, f0, y[:, :128].astype(BF))
            _st(vt_ref, tile0 + 1, f0, y[:, 128:].astype(BF))
        return run

    def attn_prologue():
        _qk_stage(0, q_ref, k_ref, s_a, m_a, bias_ref)
        _qk_stage(1, q_ref, k_ref, s_b, m_b, bias_ref)
        _sm_stage(s_a, m_a, p_a, l_a)

    def blk(i):
        return pl.ds(pl.multiple_of(i * 128, 128), 128)

    def qkv_shuffle(part, kbk, tmp):
        tf = wqkv[part, blk(kbk), :].T.astype(F32)
        _shuffle_rows(tf, tmp, lambda r, val: _st(wbt, kbk, part * D + r, val))

    with _scope("first_proj"):
        for cps in [cp_x0] + cp_wq + [cp_wv, cp_wk] + cp_wqkv + [cp_wob, cp_woa, cp_xr]:
            for c in cps:
                c.start()
        b = beta_ref[...].astype(F32).reshape(1, H)
        gt = jax.nn.sigmoid(b)
        row = lax.broadcasted_iota(jnp.int32, (H, H), 0)
        lane = lax.broadcasted_iota(jnp.int32, (H, H), 1)
        col = jnp.sum(jnp.where(row == lane, jnp.broadcast_to(gt, (H, H)), 0.0), axis=1, keepdims=True)
        col = jnp.broadcast_to(col, (H, 128))
        for g in range(G):
            gate_ref[g] = jnp.concatenate([col[4 * g:4 * g + 4], col[4 * g:4 * g + 4]], axis=0)
        key = lax.broadcasted_iota(jnp.int32, (128, 128), 0)
        qry = lax.broadcasted_iota(jnp.int32, (128, 128), 1)
        bias_ref[...] = jnp.where(key <= qry, 0.0, NEG)
        halo[...] = jnp.zeros(halo.shape, F32)

        def zero_b(b, c):
            for r in (qn, kn, vn, ko, vo):
                r[b] = jnp.zeros(r.shape[1:], F32)
            return c
        lax.fori_loop(0, G, zero_b, 0)

        def zero_mem(i, c):
            mt_ref[i // G, i % G] = jnp.zeros((144, 128), F32)
            return c
        lax.fori_loop(0, 2 * G, zero_mem, 0)
        with _scope("p_wait_x"):
            wait(cp_x0)

        def ln0(i, c):
            for u in range(16):
                r0 = pl.multiple_of(i * HL + u * 16, 16)
                x = xin[pl.ds(r0, 16), :].astype(F32)
                x_f[pl.ds(r0, 16), :] = x
                y = _ln(x).astype(BF)
                for b in range(G):
                    _st(xn, b, r0, y[:, b * 128:(b + 1) * 128])
            return c
        with _scope("p_ln"):
            lax.fori_loop(0, 2, ln0, 0)

        def q0(c, carry):
            for i in range(2):
                pltpu.make_async_copy(wq_hbm.at[:, 0:128], wq.at[0], sems.at[c]).wait()
            q_item(xn, L, 0, c)()
            return carry
        with _scope("p_q"):
            lax.fori_loop(0, 3, q0, 0)
        wait(cp_wq[3])
        wait(cp_wv)
        with _scope("p_tr"):
            q_item(xn, L, 0, 3)()
            for kbk in range(G):
                _st(wvt, kbk, 0, wv[kbk * 128:(kbk + 1) * 128, :].T)

        def v0(i, carry):
            hf = i // 2
            v_item(xn, hf * HL, 2 * hf, (i % 2) * 512)()
            return carry
        with _scope("p_v"):
            lax.fori_loop(0, 4, v0, 0)
        wait(cp_wk)
        wait(cp_wqkv[0])
        tmps = (tmp_a, tmp_b, tmp_c, tmp_d)

        def k0(c, carry):
            k_item(xn, L, 0, c)()
            for u in range(2):
                qkv_shuffle(0, 2 * c + u, tmps[u])
            return carry
        with _scope("p_k"):
            lax.fori_loop(0, 4, k0, 0)
        wait(cp_wqkv[1])
        wait(cp_wqkv[2])
        with _scope("p_attn"):
            attn_prologue()
            for u in range(2 * G):
                qkv_shuffle(1 + u // G, u % G, tmps[u % 4])
        wait(cp_wob)

        def sh1(i, carry):
            for u in range(4):
                cb = 4 * i + u
                _shuffle_rows(wob[cb].astype(F32), tmps[u], lambda r, val, cb=cb: _st(wobp, cb, r, val))
            return carry
        with _scope("p_sh1"):
            lax.fori_loop(0, 2, sh1, 0)
        wait(cp_woa)

    def out_item(src, s0, r0, w_ref, c, b0=0, b1=G, n=HL):
        def run():
            lhs = jnp.concatenate([_ld(src, b, s0, n) for b in range(b0, b1)], axis=1)
            w = jnp.concatenate([_ld(w_ref, 2 * c + i, b0 * 128, (b1 - b0) * 128) for i in range(2)], axis=1)
            x_f[r0:r0 + n, c * 256:(c + 1) * 256] += _dot(lhs, w)
        return run

    def b_proj_items():
        def item(part, c):
            def run():
                y = _dot_nt(_wide(xc, 0, HL), _wide(wbt, part * D + c * 256, 256))
                dst = (qn, kn, vn)[part]
                dst[2 * c] = y[:, :128]
                dst[2 * c + 1] = y[:, 128:]
            return run
        return [item(part, c) for part in range(3) for c in range(4)]

    def b_rotate():
        for b in range(G):
            qo[b] = qn[b]
            for new, old in ((kn, ko), (vn, vo)):
                old[b, 0:HALO, :] = old[b, HL:HL + HALO, :]
                old[b, HALO:, :] = new[b]

    def next_x_items(seg, layer, ch, chunk=16):
        nxt = jnp.minimum(seg + 1, NSEG - 1) * L

        def item(r0):
            def run():
                cur = ch.link_first(x_f[r0:r0 + chunk, :])
                obuf[r0:r0 + chunk, :] = cur.astype(BF)
                new = xin[pl.ds(pl.multiple_of(nxt + r0, chunk), chunk), :].astype(F32)
                x = jnp.where(layer == 1, new, cur)
                x_f[r0:r0 + chunk, :] = x
                yf = _ln(x)
                y = yf.astype(BF)
                for b in range(G):
                    _st(xc, b, r0, y[:, b * 128:(b + 1) * 128])
                ch.done(yf)
            return run
        return [item(r0) for r0 in range(0, HL, chunk)]

    def step(t, carry):
        seg = t // 2
        layer = t % 2
        mt = mt_ref.at[layer]
        never = lax.broadcasted_iota(jnp.int32, (8, 128), 0) < -t
        pv = lambda g, p, l: _pv_stage(g, p, l, vt_ref, ot_ref, pq_ref, pk_ref, mt, gate_ref)

        @pl.when(t > 0)
        def _():
            with _scope("A_proj"):
                def a_half(hf, c):
                    d0 = hf * HL
                    items = ([q_item(xc, HL, d0, c) for c in range(4)]
                             + [k_item(xc, HL, d0, c) for c in range(4)]
                             + [v_item(xc, 0, 2 * hf, f0) for f0 in (0, 512)])
                    _interleave(items, _ln_items(x_f, xnx, HL, HL, 0, _Chain(never)), span=8)
                    xc.bitcast(U32)[...] = xnx.bitcast(U32)[...]
                    return c

                lax.fori_loop(0, 2, a_half, 0)
            with _scope("A_attn_pro"):
                attn_prologue()

        def pair(u, c):
            g = 2 * u + 1
            _qk_stage(g + 1, q_ref, k_ref, s_a, m_a, bias_ref)
            _sm_stage(s_b, m_b, p_b, l_b)
            pv(g - 1, p_a, l_a)
            _qk_stage(g + 2, q_ref, k_ref, s_b, m_b, bias_ref)
            _sm_stage(s_a, m_a, p_a, l_a)
            pv(g, p_b, l_b)
            return c

        with _scope("A_attn_loop"):
            lax.fori_loop(0, 3, pair, 0)

        @pl.when(t == 0)
        def _():
            wait(cp_xr)

        @pl.when(jnp.logical_and(layer == 0, seg > 0))
        def _():
            cp_out(seg - 1).wait()

        def transpose_o(b0, b1):
            for j in range(4):
                ot = _ld(ot_ref, j, b0 * 128, (b1 - b0) * 128).T
                for b in range(b0, b1):
                    _st(o_nat, b, j * 128, ot[:, (b - b0) * 128:(b - b0 + 1) * 128])

        with _scope("A_out"):
            transpose_o(0, KSPLIT)
            _sm_stage(s_b, m_b, p_b, l_b, _Chain(never, NCH_EPI))
            pv(6, p_a, l_a)
            _run([out_item(o_nat, 0, 0, woa, c, 0, KSPLIT) for c in range(4)])
            pv(7, p_b, l_b)
            transpose_o(KSPLIT, G)
            kn[:, HL - HALO:HL, :] = halo[layer, 0]
            vn[:, HL - HALO:HL, :] = halo[layer, 1]
            _run([out_item(o_nat, 0, 0, woa, c, KSPLIT, G) for c in range(4)])
            _run(_ln_items(x_f, xc, 0, HL, 0, _Chain(never, 2)))
            _run([out_item(o_nat, HL, HL, woa, c) for c in range(4)])

        def b_half(hf, c):
            b_rotate()
            band = _band_items(seg * L + (hf - 1) * HL, 0, qo, ko, vo, ab, eb, ob0, _Chain(never))
            _interleave(b_proj_items(), band + _ln_items(x_f, xnx, HL, HL, 0, _Chain(never)))
            xc.bitcast(U32)[...] = xnx.bitcast(U32)[...]
            return c

        with _scope("B_loop"):
            lax.fori_loop(0, 2, b_half, 0)

        with _scope("B_tail"):
            halo[layer, 0] = kn[:, HL - HALO:HL, :]
            halo[layer, 1] = vn[:, HL - HALO:HL, :]
            b_rotate()
            _run(_band_items(seg * L + HL, 0, qo, ko, vo, ab, eb, ob1, _Chain(never, NCH_B1)))
            _run([out_item(ob0, 0, 0, wobp, c) for c in range(4)])
            _run(next_x_items(seg, layer, _Chain(never, 2)))
            _run([out_item(ob1, 0, HL, wobp, c, n=128) for c in range(4)])
            _run([out_item(ob1, 128, HL + 128, wobp, c, n=128) for c in range(4)])

        @pl.when(layer == 1)
        def _():
            obuf[HL:L, :] = x_f[HL:L, :].astype(BF)
            cp_out(seg).start()
            x_f[HL:L, :] = xin[pl.ds(pl.multiple_of(jnp.minimum(seg + 1, NSEG - 1) * L + HL, HL), HL), :].astype(F32)

        return carry

    lax.fori_loop(0, 2 * NSEG, step, 0)
    cp_out(NSEG - 1).wait()


@jax.jit
def pallas_interleave_layers__memory_aug_infini_attn__sliding_local_dilated__prompt_kernel(
    A_x: jax.Array,
    A_wq: jax.Array,
    A_wk: jax.Array,
    A_wv: jax.Array,
    A_wo: jax.Array,
    A_beta: jax.Array,
    B_x: jax.Array,
    B_wqkv: jax.Array,
    B_wo: jax.Array,
):
    del B_x
    x = A_x.reshape(S, D)
    any_spec = pl.BlockSpec(memory_space=pl.ANY)
    blk = lambda rows, dt: pltpu.VMEM((G, rows, 128), dt)
    packed = lambda rows, n=G: pltpu.VMEM((n, rows, 128), BF)
    scratch = [
        pltpu.VMEM((S, D), BF),
        pltpu.VMEM((L, D), BF),
        pltpu.VMEM((L, D), F32),
        packed(L),
        packed(HL),
        packed(HL),
        blk(D, BF),
        blk(D, BF),
        blk(D, BF),
        pltpu.VMEM((D, D), BF),
        pltpu.VMEM((3, D, D), BF),
        packed(D),
        packed(3 * D),
        blk(D, BF),
        packed(D),
        pltpu.VMEM((H * PITCH, 128), F32),
        pltpu.VMEM((H * PITCH, 128), F32),
        pltpu.VMEM((H * PITCH, 128), F32),
        pltpu.VMEM((H * PITCH, 128), F32),
        packed(L),
        packed(L),
        packed(L),
        packed(L),
        packed(D, 4),
        packed(D, 4),
        packed(L),
        pltpu.VMEM((1280, 512), F32),
        pltpu.VMEM((1280, 512), F32),
        pltpu.VMEM((4, 8, 512), F32),
        pltpu.VMEM((4, 8, 512), F32),
        packed(1280, 4),
        packed(1280, 4),
        pltpu.VMEM((4, 8, 128), F32),
        pltpu.VMEM((4, 8, 128), F32),
        pltpu.VMEM((2, G, 144, 128), F32),
        pltpu.VMEM((G, 8, 128), F32),
        pltpu.VMEM((128, 128), F32),
        blk(HL, F32),
        blk(HL, F32),
        blk(HL, F32),
        blk(HL, F32),
        blk(HL + HALO, F32),
        blk(HL + HALO, F32),
        pltpu.VMEM((2, 2, G, HALO, 128), F32),
        pltpu.VMEM((W, HL, 128), F32),
        pltpu.VMEM((W, HL, 128), F32),
        packed(HL),
        packed(HL),
        pltpu.SemaphoreType.DMA((14,)),
    ]
    out = pl.pallas_call(
        _kernel,
        in_specs=[any_spec, any_spec, any_spec, any_spec, any_spec,
                  pl.BlockSpec(memory_space=pltpu.VMEM), any_spec, any_spec],
        out_specs=any_spec,
        out_shape=jax.ShapeDtypeStruct((S, D), BF),
        scratch_shapes=scratch,
        compiler_params=pltpu.CompilerParams(vmem_limit_bytes=100 * 1024 * 1024),
    )(x, A_wq, A_wk, A_wv, A_wo, A_beta, B_wqkv, B_wo)
    return out.reshape(1, S, D)
```

```python
import math

import jax
import jax.numpy as jnp
from jax import lax
import jax.experimental.pallas as pl
import jax.experimental.pallas.tpu as pltpu

S, D, H, DH = 2048, 1024, 32, 32
L, NSEG, G = 512, 4, 8
HL = L // 2
W, DIL = 8, 2
HALO = 16
BF, F32, U32 = jnp.bfloat16, jnp.float32, jnp.uint32
QSCALE = (DH ** -0.5) * math.log2(math.e)
NEG = -1e30
NT = (((1,), (1,)), ((), ()))
OFF = (0, 128, 384, 768)
SCOPES = False
NCH_B1 = 2
PV_ONE_DOT = True
KSPLIT = 6
NCH_EPI = 2
PITCH = 33


class _scope:
    def __init__(self, name):
        self.cm = jax.named_scope(name) if SCOPES else None

    def __enter__(self):
        if self.cm is not None:
            self.cm.__enter__()

    def __exit__(self, *a):
        if self.cm is not None:
            self.cm.__exit__(*a)


def _dot(a, b):
    return jnp.dot(a, b, preferred_element_type=F32)


def _dot_nt(a, b):
    return lax.dot_general(a, b, NT, preferred_element_type=F32)


def _rows(r0, n, align=16):
    return slice(r0, r0 + n) if isinstance(r0, int) else pl.ds(pl.multiple_of(r0, align), n)


def _ldu(ref, b, r0, n):
    idx = slice(r0 // 2, (r0 + n) // 2) if isinstance(r0, int) else pl.ds(pl.multiple_of(r0 // 2, 8), n // 2)
    return ref.bitcast(U32)[b, idx, :]


def _ld(ref, b, r0, n):
    return pltpu.bitcast(_ldu(ref, b, r0, n), BF)


def _st(ref, b, r0, val):
    ref[b, _rows(r0, val.shape[0]), :] = val


def _wide(ref, r0, n):
    return jnp.concatenate([_ld(ref, b, r0, n) for b in range(G)], axis=1)


class _Chain:
    def __init__(self, never, n=1):
        self.never, self.n, self.hist = never, n, []

    def link(self, x):
        if self.never is None or len(self.hist) < self.n:
            return x
        return jnp.where(self.never, self.hist[-self.n], x)

    def link_first(self, x):
        head = self.link(x[0:8, 0:128])
        if x.shape[1] > 128:
            head = jnp.concatenate([head, x[0:8, 128:]], axis=1)
        return head if x.shape[0] == 8 else jnp.concatenate([head, x[8:]], axis=0)

    def done(self, v):
        self.hist.append(v[0:8, v.shape[1] - 128:])


def _phi(t):
    return jnp.where(t > 0, t + 1.0, jnp.exp(t))


def _ln(x):
    d = x - jnp.mean(x, axis=-1, keepdims=True)
    v = jnp.mean(d * d, axis=-1, keepdims=True)
    return d * lax.rsqrt(v + 1e-5)


def _ln_items(x_ref, xn_ref, row0, nrows, dst0, ch, chunk=16):
    def item(r0):
        def run():
            yf = _ln(ch.link_first(x_ref[r0:r0 + chunk, :]))
            y = yf.astype(BF)
            for b in range(G):
                _st(xn_ref, b, r0 - row0 + dst0, y[:, b * 128:(b + 1) * 128])
            ch.done(yf)
        return run
    return [item(r0) for r0 in range(row0, row0 + nrows, chunk)]


def _interleave(main, side, span=None):
    span = len(main) if span is None else span
    done = 0
    for i, it in enumerate(main):
        upto = len(side) if i + 1 >= span else (len(side) * (i + 1)) // span
        for s_it in side[done:upto]:
            s_it()
        done = max(done, upto)
        it()


def _run(items):
    for it in items:
        it()


def _shuffle_rows(tf, tmp, store):
    for h in range(H):
        tmp[h * PITCH:h * PITCH + DH, :] = tf[h * DH:(h + 1) * DH]
    for d in range(DH):
        for th in range(2):
            rows = tmp[pl.ds(th * 16 * PITCH + d, 16, stride=PITCH), :]
            store(d * H + th * 16, rows.astype(BF))


def _qk_stage(g, q_ref, k_ref, s_ref, m_ref, bias_ref):
    lane = lax.broadcasted_iota(jnp.int32, (64, 128), 1)
    for j in range(4):
        nk = 128 * (j + 1)
        qt = _ldu(q_ref, g, j * 128, 128)
        wq = jnp.concatenate([jnp.where((lane >> 5) == h, qt, jnp.uint32(0)) for h in range(4)], axis=0)
        st = _dot_nt(_ld(k_ref, g, 0, nk), pltpu.bitcast(wq, BF))
        bias = bias_ref[...]
        diag = st[j * 128:] + jnp.concatenate([bias] * 4, axis=1)
        s_ref[OFF[j] + j * 128:OFF[j] + nk, :] = diag
        m = jnp.max(diag.reshape(16, 8, 512), axis=0)
        if j > 0:
            s_ref[OFF[j]:OFF[j] + j * 128, :] = st[:j * 128]
            m = jnp.maximum(m, jnp.max(st[:j * 128].reshape(16 * j, 8, 512), axis=0))
        m_ref[j] = jnp.broadcast_to(jnp.max(m, axis=0, keepdims=True), (8, 512))


def _sm_stage(s_ref, m_ref, p_ref, l_ref, ch=None, sub=16):
    ch = _Chain(None) if ch is None else ch
    for j in range(4):
        nk = 128 * (j + 1)
        sums = []
        for h in range(4):
            m = m_ref[j, :, h * 128:(h + 1) * 128]
            l = None
            for r in range(0, nk, sub):
                s = ch.link_first(s_ref[OFF[j] + r:OFF[j] + r + sub, h * 128:(h + 1) * 128])
                p = jnp.exp2(s.reshape(sub // 8, 8, 128) - m[None])
                ls = jnp.sum(p, axis=0)
                l = ls if l is None else l + ls
                _st(p_ref, h, OFF[j] + r, p.reshape(sub, 128).astype(BF))
                ch.done(p[0])
            sums.append(jnp.sum(l, axis=0, keepdims=True))
        l_ref[j] = jnp.concatenate(sums + sums, axis=0)


def _pv_stage(g, p_ref, l_ref, vt_ref, ot_ref, pq_ref, pk_ref, mt_ref, gate_ref):
    mem = mt_ref[g].astype(BF)
    gate = gate_ref[g]
    for j in range(4):
        nd = _dot_nt(mem, _ld(pq_ref, g, j * 128, 128))
        c_mem = gate / (nd[128:136] + 1e-6)
        c_att = (1.0 - gate) / l_ref[j]
        for h in range(4):
            r0 = (g * 4 + h) * DH
            vt = jnp.concatenate([_ld(vt_ref, t, r0, DH) for t in range(j + 1)], axis=1)
            acc = _dot(vt, _ld(p_ref, h, OFF[j], 128 * (j + 1)))
            res = nd[h * DH:(h + 1) * DH] * c_mem[h:h + 1] + acc * c_att[h:h + 1]
            _st(ot_ref, j, r0, res.astype(BF))
    row = lax.broadcasted_iota(jnp.int32, (144, 128), 0)
    lane = lax.broadcasted_iota(jnp.int32, (144, 128), 1)
    keep = jnp.where(row < 128, row >> 5, row - 128) == (lane >> 5)
    row16 = lax.broadcasted_iota(jnp.int32, (16, 128), 0)
    ones = jnp.where(row16 < 4, 1.0, 0.0).astype(BF)
    upd = None
    for t in range(4):
        lhs = jnp.concatenate([_ld(vt_ref, t, g * 128, 128), ones], axis=0)
        u = _dot(lhs, _ld(pk_ref, g, t * 128, 128))
        upd = u if upd is None else upd + u
    mt_ref[g] = mt_ref[g] + jnp.where(keep, upd, 0.0)


def _band_items(pos0, row0, q_ref, k_ref, v_ref, a_ref, e_ref, o_ref, ch, nrows=HL):
    def logits(r0):
        def run():
            q = [q_ref[b, r0:r0 + 8, :] for b in range(G)]
            for w in range(W):
                base = HALO + r0 - DIL * w
                acc = ch.link(q[0] * k_ref[0, base:base + 8, :])
                for b in range(1, G):
                    acc = acc + q[b] * k_ref[b, base:base + 8, :]
                a_ref[w, r0 - row0:r0 - row0 + 8, :] = acc
                ch.done(acc)
        return run

    def softmax(r0):
        def run():
            lg = []
            for w in range(W):
                t = a_ref[w, r0 - row0:r0 - row0 + 128, :].T
                t = ((t[0:32] + t[32:64]) + (t[64:96] + t[96:128])) * QSCALE
                if r0 == row0 and w > 0:
                    pos = pos0 - DIL * w + lax.broadcasted_iota(jnp.int32, (H, 128), 1)
                    t = jnp.where(pos >= 0, t, NEG)
                lg.append(t)
            m = lg[0]
            for w in range(1, W):
                m = jnp.maximum(m, lg[w])
            e = [jnp.exp2(x - m) for x in lg]
            l = e[0]
            for w in range(1, W):
                l = l + e[w]
            inv = 1.0 / l
            for w in range(W):
                p = e[w] * inv
                pt = jnp.concatenate([p, p, p, p], axis=0).T
                e_ref[w, r0 - row0:r0 - row0 + 128, :] = pt
        return run

    def pv(r0):
        e = [e_ref[w, r0 - row0:r0 - row0 + 8, :] for w in range(W)]
        outs = []
        for b in range(G):
            acc = ch.link(e[0] * v_ref[b, HALO + r0:HALO + r0 + 8, :])
            for w in range(1, W):
                base = HALO + r0 - DIL * w
                acc = acc + e[w] * v_ref[b, base:base + 8, :]
            outs.append(acc)
            ch.done(acc)
        return outs

    def pv16(r0):
        def run():
            lo = pv(r0)
            hi = pv(r0 + 8)
            for b in range(G):
                _st(o_ref, b, r0, jnp.concatenate([lo[b], hi[b]], axis=0).astype(BF))
        return run

    items = []
    for r0 in range(row0, row0 + nrows, 128):
        items += [logits(r) for r in range(r0, r0 + 128, 8)]
        items.append(softmax(r0))
        items += [pv16(r) for r in range(r0, r0 + 128, 16)]
    return items


def _kernel(x_hbm, wq_hbm, wk_hbm, wv_hbm, woa_hbm, beta_ref, wqkv_hbm, wob_hbm, out_hbm,
            xin, obuf, x_f, xn, xc, xnx, wq, wk, woa, wv, wqkv, wvt, wbt, wob, wobp, tmp_a, tmp_b, tmp_c, tmp_d,
            q_ref, pq_ref, k_ref, pk_ref, vt_ref, ot_ref, o_nat,
            s_a, s_b, m_a, m_b, p_a, p_b, l_a, l_b, mt_ref, gate_ref, bias_ref,
            qn, kn, vn, qo, ko, vo, halo, ab, eb, ob0, ob1, sems):

    def col_copies(src, dst, sem, c0=0, n=G):
        return [pltpu.make_async_copy(src.at[:, (c0 + i) * 128:(c0 + i + 1) * 128], dst.at[c0 + i], sem)
                for i in range(n)]

    cp_wq = [col_copies(wq_hbm, wq, sems.at[c], 2 * c, 2) for c in range(4)]
    cp_wk = col_copies(wk_hbm, wk, sems.at[4])
    cp_wv = [pltpu.make_async_copy(wv_hbm, wv, sems.at[5])]
    cp_wqkv = [[pltpu.make_async_copy(wqkv_hbm.at[:, part * D:(part + 1) * D], wqkv.at[part], sems.at[6 + part])]
               for part in range(3)]
    cp_wob = col_copies(wob_hbm, wob, sems.at[9])
    cp_woa = col_copies(woa_hbm, woa, sems.at[10])
    cp_x0 = [pltpu.make_async_copy(x_hbm.at[0:L], xin.at[0:L], sems.at[11])]
    cp_xr = [pltpu.make_async_copy(x_hbm.at[L:S], xin.at[L:S], sems.at[12])]

    def cp_out(seg, hf):
        return pltpu.make_async_copy(obuf.at[hf * HL:(hf + 1) * HL],
                                     out_hbm.at[pl.ds(pl.multiple_of(seg * L + hf * HL, HL), HL)], sems.at[13 + hf])

    def wait(cps):
        for c in cps:
            c.wait()

    def wcols(w_ref, c0):
        return jnp.concatenate([_ld(w_ref, c0, 0, D), _ld(w_ref, c0 + 1, 0, D)], axis=1)

    def q_item(src, n, d0, c):
        def run():
            y = _dot(_wide(src, 0, n), wcols(wq, 2 * c))
            for gg in range(2):
                yq = y[:, gg * 128:(gg + 1) * 128]
                _st(q_ref, 2 * c + gg, d0, (yq * QSCALE).astype(BF))
                _st(pq_ref, 2 * c + gg, d0, _phi(yq).astype(BF))
        return run

    def k_item(src, n, d0, c):
        def run():
            y = _dot(_wide(src, 0, n), wcols(wk, 2 * c))
            for gg in range(2):
                yk = y[:, gg * 128:(gg + 1) * 128]
                _st(k_ref, 2 * c + gg, d0, yk.astype(BF))
                _st(pk_ref, 2 * c + gg, d0, _phi(yk).astype(BF))
        return run

    def v_item(src, r0, tile0, f0):
        def run():
            y = _dot_nt(_wide(wvt, f0, 512), _wide(src, r0, HL))
            _st(vt_ref, tile0, f0, y[:, :128].astype(BF))
            _st(vt_ref, tile0 + 1, f0, y[:, 128:].astype(BF))
        return run

    def attn_prologue():
        _qk_stage(0, q_ref, k_ref, s_a, m_a, bias_ref)
        _qk_stage(1, q_ref, k_ref, s_b, m_b, bias_ref)
        _sm_stage(s_a, m_a, p_a, l_a)

    def blk(i):
        return pl.ds(pl.multiple_of(i * 128, 128), 128)

    def qkv_shuffle(part, kbk, tmp):
        tf = wqkv[part, blk(kbk), :].T.astype(F32)
        _shuffle_rows(tf, tmp, lambda r, val: _st(wbt, kbk, part * D + r, val))

    with _scope("first_proj"):
        for cps in [cp_x0] + cp_wq + [cp_wv, cp_wk] + cp_wqkv + [cp_wob, cp_woa, cp_xr]:
            for c in cps:
                c.start()
        b = beta_ref[...].astype(F32).reshape(1, H)
        gt = jax.nn.sigmoid(b)
        row = lax.broadcasted_iota(jnp.int32, (H, H), 0)
        lane = lax.broadcasted_iota(jnp.int32, (H, H), 1)
        col = jnp.sum(jnp.where(row == lane, jnp.broadcast_to(gt, (H, H)), 0.0), axis=1, keepdims=True)
        col = jnp.broadcast_to(col, (H, 128))
        for g in range(G):
            gate_ref[g] = jnp.concatenate([col[4 * g:4 * g + 4], col[4 * g:4 * g + 4]], axis=0)
        key = lax.broadcasted_iota(jnp.int32, (128, 128), 0)
        qry = lax.broadcasted_iota(jnp.int32, (128, 128), 1)
        bias_ref[...] = jnp.where(key <= qry, 0.0, NEG)
        halo[...] = jnp.zeros(halo.shape, F32)

        def zero_b(b, c):
            for r in (qn, kn, vn, ko, vo):
                r[b] = jnp.zeros(r.shape[1:], F32)
            return c
        lax.fori_loop(0, G, zero_b, 0)

        def zero_mem(i, c):
            mt_ref[i // G, i % G] = jnp.zeros((144, 128), F32)
            return c
        lax.fori_loop(0, 2 * G, zero_mem, 0)
        with _scope("p_wait_x"):
            wait(cp_x0)

        def ln0(i, c):
            for u in range(16):
                r0 = pl.multiple_of(i * HL + u * 16, 16)
                x = xin[pl.ds(r0, 16), :].astype(F32)
                x_f[pl.ds(r0, 16), :] = x
                y = _ln(x).astype(BF)
                for b in range(G):
                    _st(xn, b, r0, y[:, b * 128:(b + 1) * 128])
            return c
        with _scope("p_ln"):
            lax.fori_loop(0, 2, ln0, 0)

        def q0(c, carry):
            for i in range(2):
                pltpu.make_async_copy(wq_hbm.at[:, 0:128], wq.at[0], sems.at[c]).wait()
            q_item(xn, L, 0, c)()
            return carry
        with _scope("p_q"):
            lax.fori_loop(0, 3, q0, 0)
        wait(cp_wq[3])
        wait(cp_wv)
        with _scope("p_tr"):
            q_item(xn, L, 0, 3)()
            for kbk in range(G):
                _st(wvt, kbk, 0, wv[kbk * 128:(kbk + 1) * 128, :].T)

        def v0(i, carry):
            hf = i // 2
            v_item(xn, hf * HL, 2 * hf, (i % 2) * 512)()
            return carry
        with _scope("p_v"):
            lax.fori_loop(0, 4, v0, 0)
        wait(cp_wk)
        wait(cp_wqkv[0])
        tmps = (tmp_a, tmp_b, tmp_c, tmp_d)

        def k0(c, carry):
            k_item(xn, L, 0, c)()
            for u in range(2):
                qkv_shuffle(0, 2 * c + u, tmps[u])
            return carry
        with _scope("p_k"):
            lax.fori_loop(0, 4, k0, 0)
        wait(cp_wqkv[1])
        wait(cp_wqkv[2])
        with _scope("p_attn"):
            attn_prologue()
            for u in range(2 * G):
                qkv_shuffle(1 + u // G, u % G, tmps[u % 4])
        wait(cp_wob)

        def sh1(i, carry):
            for u in range(4):
                cb = 4 * i + u
                _shuffle_rows(wob[cb].astype(F32), tmps[u], lambda r, val, cb=cb: _st(wobp, cb, r, val))
            return carry
        with _scope("p_sh1"):
            lax.fori_loop(0, 2, sh1, 0)
        wait(cp_woa)

    def out_item(src, s0, r0, w_ref, c, b0=0, b1=G, n=HL):
        def run():
            lhs = jnp.concatenate([_ld(src, b, s0, n) for b in range(b0, b1)], axis=1)
            w = jnp.concatenate([_ld(w_ref, 2 * c + i, b0 * 128, (b1 - b0) * 128) for i in range(2)], axis=1)
            x_f[r0:r0 + n, c * 256:(c + 1) * 256] += _dot(lhs, w)
        return run

    def b_proj_items():
        def item(part, c):
            def run():
                y = _dot_nt(_wide(xc, 0, HL), _wide(wbt, part * D + c * 256, 256))
                dst = (qn, kn, vn)[part]
                dst[2 * c] = y[:, :128]
                dst[2 * c + 1] = y[:, 128:]
            return run
        return [item(part, c) for part in range(3) for c in range(4)]

    def b_rotate():
        for b in range(G):
            qo[b] = qn[b]
            for new, old in ((kn, ko), (vn, vo)):
                old[b, 0:HALO, :] = old[b, HL:HL + HALO, :]
                old[b, HALO:, :] = new[b]

    def next_x_items(seg, layer, ch, chunk=16):
        nxt = jnp.minimum(seg + 1, NSEG - 1) * L

        def item(r0):
            def run():
                cur = ch.link_first(x_f[r0:r0 + chunk, :])
                obuf[r0:r0 + chunk, :] = cur.astype(BF)
                new = xin[pl.ds(pl.multiple_of(nxt + r0, chunk), chunk), :].astype(F32)
                x = jnp.where(layer == 1, new, cur)
                x_f[r0:r0 + chunk, :] = x
                yf = _ln(x)
                y = yf.astype(BF)
                for b in range(G):
                    _st(xc, b, r0, y[:, b * 128:(b + 1) * 128])
                ch.done(yf)
            return run
        return [item(r0) for r0 in range(0, HL, chunk)]

    def step(t, carry):
        seg = t // 2
        layer = t % 2
        mt = mt_ref.at[layer]
        never = lax.broadcasted_iota(jnp.int32, (8, 128), 0) < -t
        pv = lambda g, p, l: _pv_stage(g, p, l, vt_ref, ot_ref, pq_ref, pk_ref, mt, gate_ref)

        @pl.when(t > 0)
        def _():
            with _scope("A_proj"):
                def a_half(hf, c):
                    d0 = hf * HL
                    items = ([q_item(xc, HL, d0, c) for c in range(4)]
                             + [k_item(xc, HL, d0, c) for c in range(4)]
                             + [v_item(xc, 0, 2 * hf, f0) for f0 in (0, 512)])
                    _interleave(items, _ln_items(x_f, xnx, HL, HL, 0, _Chain(never)), span=8)
                    xc.bitcast(U32)[...] = xnx.bitcast(U32)[...]
                    return c

                lax.fori_loop(0, 2, a_half, 0)
            with _scope("A_attn_pro"):
                attn_prologue()

        def pair(u, c):
            g = 2 * u + 1
            _qk_stage(g + 1, q_ref, k_ref, s_a, m_a, bias_ref)
            _sm_stage(s_b, m_b, p_b, l_b)
            pv(g - 1, p_a, l_a)
            _qk_stage(g + 2, q_ref, k_ref, s_b, m_b, bias_ref)
            _sm_stage(s_a, m_a, p_a, l_a)
            pv(g, p_b, l_b)
            return c

        with _scope("A_attn_loop"):
            lax.fori_loop(0, 3, pair, 0)

        @pl.when(t == 0)
        def _():
            wait(cp_xr)

        @pl.when(jnp.logical_and(layer == 0, seg > 0))
        def _():
            cp_out(seg - 1, 0).wait()
            cp_out(seg - 1, 1).wait()

        def transpose_o(b0, b1):
            for j in range(4):
                ot = _ld(ot_ref, j, b0 * 128, (b1 - b0) * 128).T
                for b in range(b0, b1):
                    _st(o_nat, b, j * 128, ot[:, (b - b0) * 128:(b - b0 + 1) * 128])

        with _scope("A_out"):
            transpose_o(0, KSPLIT)
            _sm_stage(s_b, m_b, p_b, l_b, _Chain(never, NCH_EPI))
            pv(6, p_a, l_a)
            _run([out_item(o_nat, 0, 0, woa, c, 0, KSPLIT) for c in range(4)])
            pv(7, p_b, l_b)
            transpose_o(KSPLIT, G)
            kn[:, HL - HALO:HL, :] = halo[layer, 0]
            vn[:, HL - HALO:HL, :] = halo[layer, 1]
            _run([out_item(o_nat, 0, 0, woa, c, KSPLIT, G) for c in range(4)])
            _run(_ln_items(x_f, xc, 0, HL, 0, _Chain(never, 2)))
            _run([out_item(o_nat, HL, HL, woa, c) for c in range(4)])

        def b_half(hf, c):
            b_rotate()
            band = _band_items(seg * L + (hf - 1) * HL, 0, qo, ko, vo, ab, eb, ob0, _Chain(never))
            _interleave(b_proj_items(), band + _ln_items(x_f, xnx, HL, HL, 0, _Chain(never)))
            xc.bitcast(U32)[...] = xnx.bitcast(U32)[...]
            return c

        with _scope("B_loop"):
            lax.fori_loop(0, 2, b_half, 0)

        with _scope("B_tail"):
            halo[layer, 0] = kn[:, HL - HALO:HL, :]
            halo[layer, 1] = vn[:, HL - HALO:HL, :]
            b_rotate()
            _run(_band_items(seg * L + HL, 0, qo, ko, vo, ab, eb, ob1, _Chain(never, NCH_B1)))
            _run([out_item(ob0, 0, 0, wobp, c) for c in range(4)])
            _run(next_x_items(seg, layer, _Chain(never, 2)))
            _run([out_item(ob1, 0, HL, wobp, c, n=128) for c in range(4)])
            _run([out_item(ob1, 128, HL + 128, wobp, c, n=128) for c in range(4)])

        @pl.when(layer == 1)
        def _():
            cp_out(seg, 0).start()
            obuf[HL:L, :] = x_f[HL:L, :].astype(BF)
            cp_out(seg, 1).start()

            @pl.when(seg < NSEG - 1)
            def _():
                x_f[HL:L, :] = xin[pl.ds(pl.multiple_of((seg + 1) * L + HL, HL), HL), :].astype(F32)

        return carry

    lax.fori_loop(0, 2 * NSEG, step, 0)
    cp_out(NSEG - 1, 0).wait()
    cp_out(NSEG - 1, 1).wait()


@jax.jit
def pallas_interleave_layers__memory_aug_infini_attn__sliding_local_dilated__prompt_kernel(
    A_x: jax.Array,
    A_wq: jax.Array,
    A_wk: jax.Array,
    A_wv: jax.Array,
    A_wo: jax.Array,
    A_beta: jax.Array,
    B_x: jax.Array,
    B_wqkv: jax.Array,
    B_wo: jax.Array,
):
    del B_x
    x = A_x.reshape(S, D)
    any_spec = pl.BlockSpec(memory_space=pl.ANY)
    blk = lambda rows, dt: pltpu.VMEM((G, rows, 128), dt)
    packed = lambda rows, n=G: pltpu.VMEM((n, rows, 128), BF)
    scratch = [
        pltpu.VMEM((S, D), BF),
        pltpu.VMEM((L, D), BF),
        pltpu.VMEM((L, D), F32),
        packed(L),
        packed(HL),
        packed(HL),
        blk(D, BF),
        blk(D, BF),
        blk(D, BF),
        pltpu.VMEM((D, D), BF),
        pltpu.VMEM((3, D, D), BF),
        packed(D),
        packed(3 * D),
        blk(D, BF),
        packed(D),
        pltpu.VMEM((H * PITCH, 128), F32),
        pltpu.VMEM((H * PITCH, 128), F32),
        pltpu.VMEM((H * PITCH, 128), F32),
        pltpu.VMEM((H * PITCH, 128), F32),
        packed(L),
        packed(L),
        packed(L),
        packed(L),
        packed(D, 4),
        packed(D, 4),
        packed(L),
        pltpu.VMEM((1280, 512), F32),
        pltpu.VMEM((1280, 512), F32),
        pltpu.VMEM((4, 8, 512), F32),
        pltpu.VMEM((4, 8, 512), F32),
        packed(1280, 4),
        packed(1280, 4),
        pltpu.VMEM((4, 8, 128), F32),
        pltpu.VMEM((4, 8, 128), F32),
        pltpu.VMEM((2, G, 144, 128), F32),
        pltpu.VMEM((G, 8, 128), F32),
        pltpu.VMEM((128, 128), F32),
        blk(HL, F32),
        blk(HL, F32),
        blk(HL, F32),
        blk(HL, F32),
        blk(HL + HALO, F32),
        blk(HL + HALO, F32),
        pltpu.VMEM((2, 2, G, HALO, 128), F32),
        pltpu.VMEM((W, HL, 128), F32),
        pltpu.VMEM((W, HL, 128), F32),
        packed(HL),
        packed(HL),
        pltpu.SemaphoreType.DMA((15,)),
    ]
    out = pl.pallas_call(
        _kernel,
        in_specs=[any_spec, any_spec, any_spec, any_spec, any_spec,
                  pl.BlockSpec(memory_space=pltpu.VMEM), any_spec, any_spec],
        out_specs=any_spec,
        out_shape=jax.ShapeDtypeStruct((S, D), BF),
        scratch_shapes=scratch,
        compiler_params=pltpu.CompilerParams(vmem_limit_bytes=100 * 1024 * 1024),
    )(x, A_wq, A_wk, A_wv, A_wo, A_beta, B_wqkv, B_wo)
    return out.reshape(1, S, D)
```

```python
import math

import jax
import jax.numpy as jnp
from jax import lax
import jax.experimental.pallas as pl
import jax.experimental.pallas.tpu as pltpu

S, D, H, DH = 2048, 1024, 32, 32
L, NSEG, G = 512, 4, 8
HL = L // 2
W, DIL = 8, 2
HALO = 16
BF, F32, U32 = jnp.bfloat16, jnp.float32, jnp.uint32
QSCALE = (DH ** -0.5) * math.log2(math.e)
NEG = -1e30
NT = (((1,), (1,)), ((), ()))
OFF = (0, 128, 384, 768)
SCOPES = False
NCH_B1 = 2
PV_ONE_DOT = True
KSPLIT = 7
NCH_EPI = 0
SM_SUB = 32
NCH_LN_A, NCH_LN_OUT, NCH_LN_B, NCH_B0, NCH_NEXT = 1, 3, 2, 1, 2
QK_ORDER, SM_ORDER, PV_ORDER = (0, 1, 2, 3), (0, 1, 2, 3), (0, 1, 2, 3)
PV_ONE_DOT, QK_SPLIT, SPAN_A, A_ORDER = True, False, 8, 'qkv'
BODY_ORDER = 'qsp'
LN_FIRST_B, SPAN_B = False, 12
PITCH = 33


class _scope:
    def __init__(self, name):
        self.cm = jax.named_scope(name) if SCOPES else None

    def __enter__(self):
        if self.cm is not None:
            self.cm.__enter__()

    def __exit__(self, *a):
        if self.cm is not None:
            self.cm.__exit__(*a)


def _dot(a, b):
    return jnp.dot(a, b, preferred_element_type=F32)


def _dot_nt(a, b):
    return lax.dot_general(a, b, NT, preferred_element_type=F32)


def _rows(r0, n, align=16):
    return slice(r0, r0 + n) if isinstance(r0, int) else pl.ds(pl.multiple_of(r0, align), n)


def _ldu(ref, b, r0, n):
    idx = slice(r0 // 2, (r0 + n) // 2) if isinstance(r0, int) else pl.ds(pl.multiple_of(r0 // 2, 8), n // 2)
    return ref.bitcast(U32)[b, idx, :]


def _ld(ref, b, r0, n):
    return pltpu.bitcast(_ldu(ref, b, r0, n), BF)


def _st(ref, b, r0, val):
    ref[b, _rows(r0, val.shape[0]), :] = val


def _wide(ref, r0, n):
    return jnp.concatenate([_ld(ref, b, r0, n) for b in range(G)], axis=1)


class _Chain:
    def __init__(self, never, n=1):
        self.never, self.n, self.hist = never, n, []

    def link(self, x):
        if self.never is None or len(self.hist) < self.n:
            return x
        return jnp.where(self.never, self.hist[-self.n], x)

    def link_first(self, x):
        head = self.link(x[0:8, 0:128])
        if x.shape[1] > 128:
            head = jnp.concatenate([head, x[0:8, 128:]], axis=1)
        return head if x.shape[0] == 8 else jnp.concatenate([head, x[8:]], axis=0)

    def done(self, v):
        self.hist.append(v[0:8, v.shape[1] - 128:])


def _phi(t):
    return jnp.where(t > 0, t + 1.0, jnp.exp(t))


def _ln(x):
    d = x - jnp.mean(x, axis=-1, keepdims=True)
    v = jnp.mean(d * d, axis=-1, keepdims=True)
    return d * lax.rsqrt(v + 1e-5)


def _ln_items(x_ref, xn_ref, row0, nrows, dst0, ch, chunk=16):
    def item(r0):
        def run():
            yf = _ln(ch.link_first(x_ref[r0:r0 + chunk, :]))
            y = yf.astype(BF)
            for b in range(G):
                _st(xn_ref, b, r0 - row0 + dst0, y[:, b * 128:(b + 1) * 128])
            ch.done(yf)
        return run
    return [item(r0) for r0 in range(row0, row0 + nrows, chunk)]


def _interleave(main, side, span=None):
    span = len(main) if span is None else span
    done = 0
    for i, it in enumerate(main):
        upto = len(side) if i + 1 >= span else (len(side) * (i + 1)) // span
        for s_it in side[done:upto]:
            s_it()
        done = max(done, upto)
        it()


def _run(items):
    for it in items:
        it()


def _shuffle_rows(tf, tmp, store):
    for h in range(H):
        tmp[h * PITCH:h * PITCH + DH, :] = tf[h * DH:(h + 1) * DH]
    for d in range(DH):
        for th in range(2):
            rows = tmp[pl.ds(th * 16 * PITCH + d, 16, stride=PITCH), :]
            store(d * H + th * 16, rows.astype(BF))


def _qk_stage(g, q_ref, k_ref, s_ref, m_ref, bias_ref):
    lane = lax.broadcasted_iota(jnp.int32, (64, 128), 1)
    for j in QK_ORDER:
        nk = 128 * (j + 1)
        qt = _ldu(q_ref, g, j * 128, 128)
        wq = jnp.concatenate([jnp.where((lane >> 5) == h, qt, jnp.uint32(0)) for h in range(4)], axis=0)
        if QK_SPLIT:
            st = jnp.concatenate([_dot_nt(_ld(k_ref, g, t * 128, 128), pltpu.bitcast(wq, BF)) for t in range(j + 1)], axis=0)
        else:
            st = _dot_nt(_ld(k_ref, g, 0, nk), pltpu.bitcast(wq, BF))
        bias = bias_ref[...]
        diag = st[j * 128:] + jnp.concatenate([bias] * 4, axis=1)
        s_ref[OFF[j] + j * 128:OFF[j] + nk, :] = diag
        m = jnp.max(diag.reshape(16, 8, 512), axis=0)
        if j > 0:
            s_ref[OFF[j]:OFF[j] + j * 128, :] = st[:j * 128]
            m = jnp.maximum(m, jnp.max(st[:j * 128].reshape(16 * j, 8, 512), axis=0))
        m_ref[j] = jnp.broadcast_to(jnp.max(m, axis=0, keepdims=True), (8, 512))


def _sm_stage(s_ref, m_ref, p_ref, l_ref, ch=None):
    ch = _Chain(None) if ch is None else ch
    sub = SM_SUB
    for j in SM_ORDER:
        nk = 128 * (j + 1)
        sums = []
        for h in range(4):
            m = m_ref[j, :, h * 128:(h + 1) * 128]
            l = None
            for r in range(0, nk, sub):
                s = ch.link_first(s_ref[OFF[j] + r:OFF[j] + r + sub, h * 128:(h + 1) * 128])
                p = jnp.exp2(s.reshape(sub // 8, 8, 128) - m[None])
                ls = jnp.sum(p, axis=0)
                l = ls if l is None else l + ls
                _st(p_ref, h, OFF[j] + r, p.reshape(sub, 128).astype(BF))
                ch.done(p[0])
            sums.append(jnp.sum(l, axis=0, keepdims=True))
        l_ref[j] = jnp.concatenate(sums + sums, axis=0)


def _pv_stage(g, p_ref, l_ref, vt_ref, ot_ref, pq_ref, pk_ref, mt_ref, gate_ref):
    mem = mt_ref[g].astype(BF)
    gate = gate_ref[g]
    for j in PV_ORDER:
        nd = _dot_nt(mem, _ld(pq_ref, g, j * 128, 128))
        c_mem = gate / (nd[128:136] + 1e-6)
        c_att = (1.0 - gate) / l_ref[j]
        for h in range(4):
            r0 = (g * 4 + h) * DH
            if PV_ONE_DOT:
                vt = jnp.concatenate([_ld(vt_ref, t, r0, DH) for t in range(j + 1)], axis=1)
                acc = _dot(vt, _ld(p_ref, h, OFF[j], 128 * (j + 1)))
            else:
                acc = None
                for t in range(j + 1):
                    o = _dot(_ld(vt_ref, t, r0, DH), _ld(p_ref, h, OFF[j] + t * 128, 128))
                    acc = o if acc is None else acc + o
            res = nd[h * DH:(h + 1) * DH] * c_mem[h:h + 1] + acc * c_att[h:h + 1]
            _st(ot_ref, j, r0, res.astype(BF))
    row = lax.broadcasted_iota(jnp.int32, (144, 128), 0)
    lane = lax.broadcasted_iota(jnp.int32, (144, 128), 1)
    keep = jnp.where(row < 128, row >> 5, row - 128) == (lane >> 5)
    row16 = lax.broadcasted_iota(jnp.int32, (16, 128), 0)
    ones = jnp.where(row16 < 4, 1.0, 0.0).astype(BF)
    upd = None
    for t in range(4):
        lhs = jnp.concatenate([_ld(vt_ref, t, g * 128, 128), ones], axis=0)
        u = _dot(lhs, _ld(pk_ref, g, t * 128, 128))
        upd = u if upd is None else upd + u
    mt_ref[g] = mt_ref[g] + jnp.where(keep, upd, 0.0)


def _band_items(pos0, row0, q_ref, k_ref, v_ref, a_ref, e_ref, o_ref, ch, nrows=HL):
    def logits(r0):
        def run():
            q = [q_ref[b, r0:r0 + 8, :] for b in range(G)]
            for w in range(W):
                base = HALO + r0 - DIL * w
                acc = ch.link(q[0] * k_ref[0, base:base + 8, :])
                for b in range(1, G):
                    acc = acc + q[b] * k_ref[b, base:base + 8, :]
                a_ref[w, r0 - row0:r0 - row0 + 8, :] = acc
                ch.done(acc)
        return run

    def softmax(r0):
        def run():
            lg = []
            for w in range(W):
                t = a_ref[w, r0 - row0:r0 - row0 + 128, :].T
                t = ((t[0:32] + t[32:64]) + (t[64:96] + t[96:128])) * QSCALE
                if r0 == row0 and w > 0:
                    pos = pos0 - DIL * w + lax.broadcasted_iota(jnp.int32, (H, 128), 1)
                    t = jnp.where(pos >= 0, t, NEG)
                lg.append(t)
            m = lg[0]
            for w in range(1, W):
                m = jnp.maximum(m, lg[w])
            e = [jnp.exp2(x - m) for x in lg]
            l = e[0]
            for w in range(1, W):
                l = l + e[w]
            inv = 1.0 / l
            for w in range(W):
                p = e[w] * inv
                pt = jnp.concatenate([p, p, p, p], axis=0).T
                e_ref[w, r0 - row0:r0 - row0 + 128, :] = pt
        return run

    def pv(r0):
        e = [e_ref[w, r0 - row0:r0 - row0 + 8, :] for w in range(W)]
        outs = []
        for b in range(G):
            acc = ch.link(e[0] * v_ref[b, HALO + r0:HALO + r0 + 8, :])
            for w in range(1, W):
                base = HALO + r0 - DIL * w
                acc = acc + e[w] * v_ref[b, base:base + 8, :]
            outs.append(acc)
            ch.done(acc)
        return outs

    def pv16(r0):
        def run():
            lo = pv(r0)
            hi = pv(r0 + 8)
            for b in range(G):
                _st(o_ref, b, r0, jnp.concatenate([lo[b], hi[b]], axis=0).astype(BF))
        return run

    items = []
    for r0 in range(row0, row0 + nrows, 128):
        items += [logits(r) for r in range(r0, r0 + 128, 8)]
        items.append(softmax(r0))
        items += [pv16(r) for r in range(r0, r0 + 128, 16)]
    return items


def _kernel(x_hbm, wq_hbm, wk_hbm, wv_hbm, woa_hbm, beta_ref, wqkv_hbm, wob_hbm, out_hbm,
            xin, obuf, x_f, xn, xc, xnx, wq, wk, woa, wv, wqkv, wvt, wbt, wob, wobp, tmp_a, tmp_b, tmp_c, tmp_d,
            q_ref, pq_ref, k_ref, pk_ref, vt_ref, ot_ref, o_nat,
            s_a, s_b, m_a, m_b, p_a, p_b, l_a, l_b, mt_ref, gate_ref, bias_ref,
            qn, kn, vn, qo, ko, vo, halo, ab, eb, ob0, ob1, sems):

    def col_copies(src, dst, sem, c0=0, n=G):
        return [pltpu.make_async_copy(src.at[:, (c0 + i) * 128:(c0 + i + 1) * 128], dst.at[c0 + i], sem)
                for i in range(n)]

    cp_wq = [col_copies(wq_hbm, wq, sems.at[c], 2 * c, 2) for c in range(4)]
    cp_wk = col_copies(wk_hbm, wk, sems.at[4])
    cp_wv = [pltpu.make_async_copy(wv_hbm, wv, sems.at[5])]
    cp_wqkv = [[pltpu.make_async_copy(wqkv_hbm.at[:, part * D:(part + 1) * D], wqkv.at[part], sems.at[6 + part])]
               for part in range(3)]
    cp_wob = col_copies(wob_hbm, wob, sems.at[9])
    cp_woa = col_copies(woa_hbm, woa, sems.at[10])
    cp_x0 = [pltpu.make_async_copy(x_hbm.at[0:L], xin.at[0:L], sems.at[11])]
    cp_xr = [pltpu.make_async_copy(x_hbm.at[L:S], xin.at[L:S], sems.at[12])]

    def cp_out(seg, hf):
        return pltpu.make_async_copy(obuf.at[hf * HL:(hf + 1) * HL],
                                     out_hbm.at[pl.ds(pl.multiple_of(seg * L + hf * HL, HL), HL)], sems.at[13 + hf])

    def wait(cps):
        for c in cps:
            c.wait()

    def wcols(w_ref, c0):
        return jnp.concatenate([_ld(w_ref, c0, 0, D), _ld(w_ref, c0 + 1, 0, D)], axis=1)

    def q_item(src, n, d0, c):
        def run():
            y = _dot(_wide(src, 0, n), wcols(wq, 2 * c))
            for gg in range(2):
                yq = y[:, gg * 128:(gg + 1) * 128]
                _st(q_ref, 2 * c + gg, d0, (yq * QSCALE).astype(BF))
                _st(pq_ref, 2 * c + gg, d0, _phi(yq).astype(BF))
        return run

    def k_item(src, n, d0, c):
        def run():
            y = _dot(_wide(src, 0, n), wcols(wk, 2 * c))
            for gg in range(2):
                yk = y[:, gg * 128:(gg + 1) * 128]
                _st(k_ref, 2 * c + gg, d0, yk.astype(BF))
                _st(pk_ref, 2 * c + gg, d0, _phi(yk).astype(BF))
        return run

    def v_item(src, r0, tile0, f0):
        def run():
            y = _dot_nt(_wide(wvt, f0, 512), _wide(src, r0, HL))
            _st(vt_ref, tile0, f0, y[:, :128].astype(BF))
            _st(vt_ref, tile0 + 1, f0, y[:, 128:].astype(BF))
        return run

    def attn_prologue():
        _qk_stage(0, q_ref, k_ref, s_a, m_a, bias_ref)
        _qk_stage(1, q_ref, k_ref, s_b, m_b, bias_ref)
        _sm_stage(s_a, m_a, p_a, l_a)

    def blk(i):
        return pl.ds(pl.multiple_of(i * 128, 128), 128)

    def qkv_shuffle(part, kbk, tmp):
        tf = wqkv[part, blk(kbk), :].T.astype(F32)
        _shuffle_rows(tf, tmp, lambda r, val: _st(wbt, kbk, part * D + r, val))

    with _scope("first_proj"):
        for cps in [cp_x0] + cp_wq + [cp_wv, cp_wk] + cp_wqkv + [cp_wob, cp_woa, cp_xr]:
            for c in cps:
                c.start()
        b = beta_ref[...].astype(F32).reshape(1, H)
        gt = jax.nn.sigmoid(b)
        row = lax.broadcasted_iota(jnp.int32, (H, H), 0)
        lane = lax.broadcasted_iota(jnp.int32, (H, H), 1)
        col = jnp.sum(jnp.where(row == lane, jnp.broadcast_to(gt, (H, H)), 0.0), axis=1, keepdims=True)
        col = jnp.broadcast_to(col, (H, 128))
        for g in range(G):
            gate_ref[g] = jnp.concatenate([col[4 * g:4 * g + 4], col[4 * g:4 * g + 4]], axis=0)
        key = lax.broadcasted_iota(jnp.int32, (128, 128), 0)
        qry = lax.broadcasted_iota(jnp.int32, (128, 128), 1)
        bias_ref[...] = jnp.where(key <= qry, 0.0, NEG)
        halo[...] = jnp.zeros(halo.shape, F32)

        def zero_b(b, c):
            for r in (qn, kn, vn, ko, vo):
                r[b] = jnp.zeros(r.shape[1:], F32)
            return c
        lax.fori_loop(0, G, zero_b, 0)

        def zero_mem(i, c):
            mt_ref[i // G, i % G] = jnp.zeros((144, 128), F32)
            return c
        lax.fori_loop(0, 2 * G, zero_mem, 0)
        with _scope("p_wait_x"):
            wait(cp_x0)

        def ln0(i, c):
            for u in range(16):
                r0 = pl.multiple_of(i * HL + u * 16, 16)
                x = xin[pl.ds(r0, 16), :].astype(F32)
                x_f[pl.ds(r0, 16), :] = x
                y = _ln(x).astype(BF)
                for b in range(G):
                    _st(xn, b, r0, y[:, b * 128:(b + 1) * 128])
            return c
        with _scope("p_ln"):
            lax.fori_loop(0, 2, ln0, 0)

        def q0(c, carry):
            for i in range(2):
                pltpu.make_async_copy(wq_hbm.at[:, 0:128], wq.at[0], sems.at[c]).wait()
            q_item(xn, L, 0, c)()
            return carry
        with _scope("p_q"):
            lax.fori_loop(0, 3, q0, 0)
        wait(cp_wq[3])
        wait(cp_wv)
        with _scope("p_tr"):
            q_item(xn, L, 0, 3)()
            for kbk in range(G):
                _st(wvt, kbk, 0, wv[kbk * 128:(kbk + 1) * 128, :].T)

        def v0(i, carry):
            hf = i // 2
            v_item(xn, hf * HL, 2 * hf, (i % 2) * 512)()
            return carry
        with _scope("p_v"):
            lax.fori_loop(0, 4, v0, 0)
        wait(cp_wk)
        wait(cp_wqkv[0])
        tmps = (tmp_a, tmp_b, tmp_c, tmp_d)

        def k0(c, carry):
            k_item(xn, L, 0, c)()
            for u in range(2):
                qkv_shuffle(0, 2 * c + u, tmps[u])
            return carry
        with _scope("p_k"):
            lax.fori_loop(0, 4, k0, 0)
        wait(cp_wqkv[1])
        wait(cp_wqkv[2])
        with _scope("p_attn"):
            attn_prologue()
            for u in range(2 * G):
                qkv_shuffle(1 + u // G, u % G, tmps[u % 4])
        wait(cp_wob)

        def sh1(i, carry):
            for u in range(4):
                cb = 4 * i + u
                _shuffle_rows(wob[cb].astype(F32), tmps[u], lambda r, val, cb=cb: _st(wobp, cb, r, val))
            return carry
        with _scope("p_sh1"):
            lax.fori_loop(0, 2, sh1, 0)
        wait(cp_woa)

    def out_item(src, s0, r0, w_ref, c, b0=0, b1=G, n=HL):
        def run():
            lhs = jnp.concatenate([_ld(src, b, s0, n) for b in range(b0, b1)], axis=1)
            w = jnp.concatenate([_ld(w_ref, 2 * c + i, b0 * 128, (b1 - b0) * 128) for i in range(2)], axis=1)
            x_f[r0:r0 + n, c * 256:(c + 1) * 256] += _dot(lhs, w)
        return run

    def b_proj_items():
        def item(part, c):
            def run():
                y = _dot_nt(_wide(xc, 0, HL), _wide(wbt, part * D + c * 256, 256))
                dst = (qn, kn, vn)[part]
                dst[2 * c] = y[:, :128]
                dst[2 * c + 1] = y[:, 128:]
            return run
        return [item(part, c) for part in range(3) for c in range(4)]

    def b_rotate():
        for b in range(G):
            qo[b] = qn[b]
            for new, old in ((kn, ko), (vn, vo)):
                old[b, 0:HALO, :] = old[b, HL:HL + HALO, :]
                old[b, HALO:, :] = new[b]

    def next_x_items(seg, layer, ch, chunk=16):
        nxt = jnp.minimum(seg + 1, NSEG - 1) * L

        def item(r0):
            def run():
                cur = ch.link_first(x_f[r0:r0 + chunk, :])
                obuf[r0:r0 + chunk, :] = cur.astype(BF)
                new = xin[pl.ds(pl.multiple_of(nxt + r0, chunk), chunk), :].astype(F32)
                x = jnp.where(layer == 1, new, cur)
                x_f[r0:r0 + chunk, :] = x
                yf = _ln(x)
                y = yf.astype(BF)
                for b in range(G):
                    _st(xc, b, r0, y[:, b * 128:(b + 1) * 128])
                ch.done(yf)
            return run
        return [item(r0) for r0 in range(0, HL, chunk)]

    def step(t, carry):
        seg = t // 2
        layer = t % 2
        mt = mt_ref.at[layer]
        never = lax.broadcasted_iota(jnp.int32, (8, 128), 0) < -t
        pv = lambda g, p, l: _pv_stage(g, p, l, vt_ref, ot_ref, pq_ref, pk_ref, mt, gate_ref)

        @pl.when(t > 0)
        def _():
            with _scope("A_proj"):
                def a_half(hf, c):
                    d0 = hf * HL
                    parts = {'q': [q_item(xc, HL, d0, c) for c in range(4)],
                             'k': [k_item(xc, HL, d0, c) for c in range(4)],
                             'v': [v_item(xc, 0, 2 * hf, f0) for f0 in (0, 512)]}
                    items = [it for ch in A_ORDER for it in parts[ch]]
                    _interleave(items, _ln_items(x_f, xnx, HL, HL, 0, _Chain(never, NCH_LN_A)), span=SPAN_A)
                    xc.bitcast(U32)[...] = xnx.bitcast(U32)[...]
                    return c

                lax.fori_loop(0, 2, a_half, 0)
            with _scope("A_attn_pro"):
                attn_prologue()

        def pair(u, c):
            g = 2 * u + 1
            halves = ({'q': lambda: _qk_stage(g + 1, q_ref, k_ref, s_a, m_a, bias_ref),
                       's': lambda: _sm_stage(s_b, m_b, p_b, l_b), 'p': lambda: pv(g - 1, p_a, l_a)},
                      {'q': lambda: _qk_stage(g + 2, q_ref, k_ref, s_b, m_b, bias_ref),
                       's': lambda: _sm_stage(s_a, m_a, p_a, l_a), 'p': lambda: pv(g, p_b, l_b)})
            for half in halves:
                for st in BODY_ORDER:
                    half[st]()
            return c

        with _scope("A_attn_loop"):
            lax.fori_loop(0, 3, pair, 0)

        @pl.when(t == 0)
        def _():
            wait(cp_xr)

        @pl.when(jnp.logical_and(layer == 0, seg > 0))
        def _():
            cp_out(seg - 1, 0).wait()
            cp_out(seg - 1, 1).wait()

        def transpose_o(b0, b1):
            for j in range(4):
                ot = _ld(ot_ref, j, b0 * 128, (b1 - b0) * 128).T
                for b in range(b0, b1):
                    _st(o_nat, b, j * 128, ot[:, (b - b0) * 128:(b - b0 + 1) * 128])

        with _scope("A_out"):
            transpose_o(0, G - 2)
            _sm_stage(s_b, m_b, p_b, l_b, _Chain(never if NCH_EPI else None, max(NCH_EPI, 1)))
            pv(G - 2, p_a, l_a)
            if KSPLIT == G - 1:
                transpose_o(G - 2, G - 1)
            _run([out_item(o_nat, 0, 0, woa, c, 0, KSPLIT) for c in range(4)])
            pv(G - 1, p_b, l_b)
            transpose_o(KSPLIT, G)
            kn[:, HL - HALO:HL, :] = halo[layer, 0]
            vn[:, HL - HALO:HL, :] = halo[layer, 1]
            _run([out_item(o_nat, 0, 0, woa, c, KSPLIT, G) for c in range(4)])
            _run(_ln_items(x_f, xc, 0, HL, 0, _Chain(never, NCH_LN_OUT)))
            _run([out_item(o_nat, HL, HL, woa, c) for c in range(4)])

        def b_half(hf, c):
            b_rotate()
            band = _band_items(seg * L + (hf - 1) * HL, 0, qo, ko, vo, ab, eb, ob0, _Chain(never, NCH_B0))
            ln = _ln_items(x_f, xnx, HL, HL, 0, _Chain(never, NCH_LN_B))
            _interleave(b_proj_items(), ln + band if LN_FIRST_B else band + ln, span=SPAN_B)
            xc.bitcast(U32)[...] = xnx.bitcast(U32)[...]
            return c

        with _scope("B_loop"):
            lax.fori_loop(0, 2, b_half, 0)

        with _scope("B_tail"):
            halo[layer, 0] = kn[:, HL - HALO:HL, :]
            halo[layer, 1] = vn[:, HL - HALO:HL, :]
            b_rotate()
            _run(_band_items(seg * L + HL, 0, qo, ko, vo, ab, eb, ob1, _Chain(never, NCH_B1)))
            _run([out_item(ob0, 0, 0, wobp, c) for c in range(4)])
            _run(next_x_items(seg, layer, _Chain(never, NCH_NEXT)))
            _run([out_item(ob1, 0, HL, wobp, c, n=128) for c in range(4)])
            _run([out_item(ob1, 128, HL + 128, wobp, c, n=128) for c in range(4)])

        @pl.when(layer == 1)
        def _():
            cp_out(seg, 0).start()
            obuf[HL:L, :] = x_f[HL:L, :].astype(BF)
            cp_out(seg, 1).start()

            @pl.when(seg < NSEG - 1)
            def _():
                x_f[HL:L, :] = xin[pl.ds(pl.multiple_of((seg + 1) * L + HL, HL), HL), :].astype(F32)

        return carry

    lax.fori_loop(0, 2 * NSEG, step, 0)
    cp_out(NSEG - 1, 0).wait()
    cp_out(NSEG - 1, 1).wait()


@jax.jit
def pallas_interleave_layers__memory_aug_infini_attn__sliding_local_dilated__prompt_kernel(
    A_x: jax.Array,
    A_wq: jax.Array,
    A_wk: jax.Array,
    A_wv: jax.Array,
    A_wo: jax.Array,
    A_beta: jax.Array,
    B_x: jax.Array,
    B_wqkv: jax.Array,
    B_wo: jax.Array,
):
    del B_x
    x = A_x.reshape(S, D)
    any_spec = pl.BlockSpec(memory_space=pl.ANY)
    blk = lambda rows, dt: pltpu.VMEM((G, rows, 128), dt)
    packed = lambda rows, n=G: pltpu.VMEM((n, rows, 128), BF)
    scratch = [
        pltpu.VMEM((S, D), BF),
        pltpu.VMEM((L, D), BF),
        pltpu.VMEM((L, D), F32),
        packed(L),
        packed(HL),
        packed(HL),
        blk(D, BF),
        blk(D, BF),
        blk(D, BF),
        pltpu.VMEM((D, D), BF),
        pltpu.VMEM((3, D, D), BF),
        packed(D),
        packed(3 * D),
        blk(D, BF),
        packed(D),
        pltpu.VMEM((H * PITCH, 128), F32),
        pltpu.VMEM((H * PITCH, 128), F32),
        pltpu.VMEM((H * PITCH, 128), F32),
        pltpu.VMEM((H * PITCH, 128), F32),
        packed(L),
        packed(L),
        packed(L),
        packed(L),
        packed(D, 4),
        packed(D, 4),
        packed(L),
        pltpu.VMEM((1280, 512), F32),
        pltpu.VMEM((1280, 512), F32),
        pltpu.VMEM((4, 8, 512), F32),
        pltpu.VMEM((4, 8, 512), F32),
        packed(1280, 4),
        packed(1280, 4),
        pltpu.VMEM((4, 8, 128), F32),
        pltpu.VMEM((4, 8, 128), F32),
        pltpu.VMEM((2, G, 144, 128), F32),
        pltpu.VMEM((G, 8, 128), F32),
        pltpu.VMEM((128, 128), F32),
        blk(HL, F32),
        blk(HL, F32),
        blk(HL, F32),
        blk(HL, F32),
        blk(HL + HALO, F32),
        blk(HL + HALO, F32),
        pltpu.VMEM((2, 2, G, HALO, 128), F32),
        pltpu.VMEM((W, HL, 128), F32),
        pltpu.VMEM((W, HL, 128), F32),
        packed(HL),
        packed(HL),
        pltpu.SemaphoreType.DMA((15,)),
    ]
    out = pl.pallas_call(
        _kernel,
        in_specs=[any_spec, any_spec, any_spec, any_spec, any_spec,
                  pl.BlockSpec(memory_space=pltpu.VMEM), any_spec, any_spec],
        out_specs=any_spec,
        out_shape=jax.ShapeDtypeStruct((S, D), BF),
        scratch_shapes=scratch,
        compiler_params=pltpu.CompilerParams(vmem_limit_bytes=100 * 1024 * 1024),
    )(x, A_wq, A_wk, A_wv, A_wo, A_beta, B_wqkv, B_wo)
    return out.reshape(1, S, D)
```

```python
import math

import jax
import jax.numpy as jnp
from jax import lax
import jax.experimental.pallas as pl
import jax.experimental.pallas.tpu as pltpu

S, D, H, DH = 2048, 1024, 32, 32
L, NSEG, G = 512, 4, 8
HL = L // 2
W, DIL = 8, 2
HALO = 16
BF, F32, U32 = jnp.bfloat16, jnp.float32, jnp.uint32
QSCALE = (DH ** -0.5) * math.log2(math.e)
NEG = -1e30
NT = (((1,), (1,)), ((), ()))
OFF = (0, 128, 384, 768)
SCOPES = False
NCH_B1 = 2
PV_ONE_DOT = True
KSPLIT = 7
NCH_EPI = 0
SM_SUB = 32
NCH_LN_A, NCH_LN_OUT, NCH_LN_B, NCH_B0, NCH_NEXT = 1, 3, 2, 1, 2
QK_ORDER, SM_ORDER, PV_ORDER = (0, 1, 2, 3), (0, 1, 2, 3), (0, 1, 2, 3)
PV_ONE_DOT, QK_SPLIT, SPAN_A, A_ORDER = True, False, 8, 'qkv'
UPD_SHIFT = False
QK_LINK, SM1_DONE = False, False
LN_FIRST_B, SPAN_B = False, 12
PITCH = 33


class _scope:
    def __init__(self, name):
        self.cm = jax.named_scope(name) if SCOPES else None

    def __enter__(self):
        if self.cm is not None:
            self.cm.__enter__()

    def __exit__(self, *a):
        if self.cm is not None:
            self.cm.__exit__(*a)


def _dot(a, b):
    return jnp.dot(a, b, preferred_element_type=F32)


def _dot_nt(a, b):
    return lax.dot_general(a, b, NT, preferred_element_type=F32)


def _rows(r0, n, align=16):
    return slice(r0, r0 + n) if isinstance(r0, int) else pl.ds(pl.multiple_of(r0, align), n)


def _ldu(ref, b, r0, n):
    idx = slice(r0 // 2, (r0 + n) // 2) if isinstance(r0, int) else pl.ds(pl.multiple_of(r0 // 2, 8), n // 2)
    return ref.bitcast(U32)[b, idx, :]


def _ld(ref, b, r0, n):
    return pltpu.bitcast(_ldu(ref, b, r0, n), BF)


def _st(ref, b, r0, val):
    ref[b, _rows(r0, val.shape[0]), :] = val


def _wide(ref, r0, n):
    return jnp.concatenate([_ld(ref, b, r0, n) for b in range(G)], axis=1)


class _Chain:
    def __init__(self, never, n=1):
        self.never, self.n, self.hist = never, n, []

    def link(self, x):
        if self.never is None or len(self.hist) < self.n:
            return x
        return jnp.where(self.never, self.hist[-self.n], x)

    def link_first(self, x):
        head = self.link(x[0:8, 0:128])
        if x.shape[1] > 128:
            head = jnp.concatenate([head, x[0:8, 128:]], axis=1)
        return head if x.shape[0] == 8 else jnp.concatenate([head, x[8:]], axis=0)

    def link_packed(self, u):
        if self.never is None or len(self.hist) < self.n:
            return u
        head = jnp.where(self.never, pltpu.bitcast(self.hist[-self.n], U32), u[0:8])
        return head if u.shape[0] == 8 else jnp.concatenate([head, u[8:]], axis=0)

    def done(self, v):
        self.hist.append(v[0:8, v.shape[1] - 128:])


def _phi(t):
    return jnp.where(t > 0, t + 1.0, jnp.exp(t))


def _ln(x):
    d = x - jnp.mean(x, axis=-1, keepdims=True)
    v = jnp.mean(d * d, axis=-1, keepdims=True)
    return d * lax.rsqrt(v + 1e-5)


def _ln_items(x_ref, xn_ref, row0, nrows, dst0, ch, chunk=16):
    def item(r0):
        def run():
            yf = _ln(ch.link_first(x_ref[r0:r0 + chunk, :]))
            y = yf.astype(BF)
            for b in range(G):
                _st(xn_ref, b, r0 - row0 + dst0, y[:, b * 128:(b + 1) * 128])
            ch.done(yf)
        return run
    return [item(r0) for r0 in range(row0, row0 + nrows, chunk)]


def _interleave(main, side, span=None):
    span = len(main) if span is None else span
    done = 0
    for i, it in enumerate(main):
        upto = len(side) if i + 1 >= span else (len(side) * (i + 1)) // span
        for s_it in side[done:upto]:
            s_it()
        done = max(done, upto)
        it()


def _run(items):
    for it in items:
        it()


def _shuffle_rows(tf, tmp, store):
    for h in range(H):
        tmp[h * PITCH:h * PITCH + DH, :] = tf[h * DH:(h + 1) * DH]
    for d in range(DH):
        for th in range(2):
            rows = tmp[pl.ds(th * 16 * PITCH + d, 16, stride=PITCH), :]
            store(d * H + th * 16, rows.astype(BF))


def _qk_stage(g, q_ref, k_ref, s_ref, m_ref, bias_ref, after=None):
    lane = lax.broadcasted_iota(jnp.int32, (64, 128), 1)
    for j in QK_ORDER:
        nk = 128 * (j + 1)
        qt = _ldu(q_ref, g, j * 128, 128)
        if after is not None:
            qt = after.link_packed(qt)
        wq = jnp.concatenate([jnp.where((lane >> 5) == h, qt, jnp.uint32(0)) for h in range(4)], axis=0)
        if QK_SPLIT:
            st = jnp.concatenate([_dot_nt(_ld(k_ref, g, t * 128, 128), pltpu.bitcast(wq, BF)) for t in range(j + 1)], axis=0)
        else:
            st = _dot_nt(_ld(k_ref, g, 0, nk), pltpu.bitcast(wq, BF))
        bias = bias_ref[...]
        diag = st[j * 128:] + jnp.concatenate([bias] * 4, axis=1)
        s_ref[OFF[j] + j * 128:OFF[j] + nk, :] = diag
        m = jnp.max(diag.reshape(16, 8, 512), axis=0)
        if j > 0:
            s_ref[OFF[j]:OFF[j] + j * 128, :] = st[:j * 128]
            m = jnp.maximum(m, jnp.max(st[:j * 128].reshape(16 * j, 8, 512), axis=0))
        m_ref[j] = jnp.broadcast_to(jnp.max(m, axis=0, keepdims=True), (8, 512))


def _sm_stage(s_ref, m_ref, p_ref, l_ref, ch=None, after=None, fin=None):
    ch = _Chain(None) if ch is None else ch
    sub = SM_SUB
    for j in SM_ORDER:
        nk = 128 * (j + 1)
        sums = []
        for h in range(4):
            m = m_ref[j, :, h * 128:(h + 1) * 128]
            if after is not None:
                m = after.link(m)
            l = None
            for r in range(0, nk, sub):
                s = ch.link_first(s_ref[OFF[j] + r:OFF[j] + r + sub, h * 128:(h + 1) * 128])
                p = jnp.exp2(s.reshape(sub // 8, 8, 128) - m[None])
                ls = jnp.sum(p, axis=0)
                l = ls if l is None else l + ls
                _st(p_ref, h, OFF[j] + r, p.reshape(sub, 128).astype(BF))
                ch.done(p[0])
            sums.append(jnp.sum(l, axis=0, keepdims=True))
        lsum = jnp.concatenate(sums + sums, axis=0)
        l_ref[j] = lsum
    if fin is not None:
        fin.done(lsum)


def _pv_stage(g, p_ref, l_ref, vt_ref, ot_ref, pq_ref, mt_ref, gate_ref):
    mem = mt_ref[g].astype(BF)
    gate = gate_ref[g]
    for j in PV_ORDER:
        nd = _dot_nt(mem, _ld(pq_ref, g, j * 128, 128))
        c_mem = gate / (nd[128:136] + 1e-6)
        c_att = (1.0 - gate) / l_ref[j]
        for h in range(4):
            r0 = (g * 4 + h) * DH
            if PV_ONE_DOT:
                vt = jnp.concatenate([_ld(vt_ref, t, r0, DH) for t in range(j + 1)], axis=1)
                acc = _dot(vt, _ld(p_ref, h, OFF[j], 128 * (j + 1)))
            else:
                acc = None
                for t in range(j + 1):
                    o = _dot(_ld(vt_ref, t, r0, DH), _ld(p_ref, h, OFF[j] + t * 128, 128))
                    acc = o if acc is None else acc + o
            res = nd[h * DH:(h + 1) * DH] * c_mem[h:h + 1] + acc * c_att[h:h + 1]
            _st(ot_ref, j, r0, res.astype(BF))


def _mem_update(g, vt_ref, pk_ref, mt_ref, ch=None, slot=None):
    row = lax.broadcasted_iota(jnp.int32, (144, 128), 0)
    lane = lax.broadcasted_iota(jnp.int32, (144, 128), 1)
    keep = jnp.where(row < 128, row >> 5, row - 128) == (lane >> 5)
    row16 = lax.broadcasted_iota(jnp.int32, (16, 128), 0)
    ones = jnp.where(row16 < 4, 1.0, 0.0).astype(BF)
    upd = None
    for t in range(4):
        lhs = jnp.concatenate([_ld(vt_ref, t, g * 128, 128), ones], axis=0)
        u = _dot(lhs, _ld(pk_ref, g, t * 128, 128))
        upd = u if upd is None else upd + u
    slot = g if slot is None else slot
    new = mt_ref[slot] + jnp.where(keep, upd, 0.0)
    mt_ref[slot] = new
    if ch is not None:
        ch.done(new)


def _band_items(pos0, row0, q_ref, k_ref, v_ref, a_ref, e_ref, o_ref, ch, nrows=HL):
    def logits(r0):
        def run():
            q = [q_ref[b, r0:r0 + 8, :] for b in range(G)]
            for w in range(W):
                base = HALO + r0 - DIL * w
                acc = ch.link(q[0] * k_ref[0, base:base + 8, :])
                for b in range(1, G):
                    acc = acc + q[b] * k_ref[b, base:base + 8, :]
                a_ref[w, r0 - row0:r0 - row0 + 8, :] = acc
                ch.done(acc)
        return run

    def softmax(r0):
        def run():
            lg = []
            for w in range(W):
                t = a_ref[w, r0 - row0:r0 - row0 + 128, :].T
                t = ((t[0:32] + t[32:64]) + (t[64:96] + t[96:128])) * QSCALE
                if r0 == row0 and w > 0:
                    pos = pos0 - DIL * w + lax.broadcasted_iota(jnp.int32, (H, 128), 1)
                    t = jnp.where(pos >= 0, t, NEG)
                lg.append(t)
            m = lg[0]
            for w in range(1, W):
                m = jnp.maximum(m, lg[w])
            e = [jnp.exp2(x - m) for x in lg]
            l = e[0]
            for w in range(1, W):
                l = l + e[w]
            inv = 1.0 / l
            for w in range(W):
                p = e[w] * inv
                pt = jnp.concatenate([p, p, p, p], axis=0).T
                e_ref[w, r0 - row0:r0 - row0 + 128, :] = pt
        return run

    def pv(r0):
        e = [e_ref[w, r0 - row0:r0 - row0 + 8, :] for w in range(W)]
        outs = []
        for b in range(G):
            acc = ch.link(e[0] * v_ref[b, HALO + r0:HALO + r0 + 8, :])
            for w in range(1, W):
                base = HALO + r0 - DIL * w
                acc = acc + e[w] * v_ref[b, base:base + 8, :]
            outs.append(acc)
            ch.done(acc)
        return outs

    def pv16(r0):
        def run():
            lo = pv(r0)
            hi = pv(r0 + 8)
            for b in range(G):
                _st(o_ref, b, r0, jnp.concatenate([lo[b], hi[b]], axis=0).astype(BF))
        return run

    items = []
    for r0 in range(row0, row0 + nrows, 128):
        items += [logits(r) for r in range(r0, r0 + 128, 8)]
        items.append(softmax(r0))
        items += [pv16(r) for r in range(r0, r0 + 128, 16)]
    return items


def _kernel(x_hbm, wq_hbm, wk_hbm, wv_hbm, woa_hbm, beta_ref, wqkv_hbm, wob_hbm, out_hbm,
            xin, obuf, x_f, xn, xc, xnx, wq, wk, woa, wv, wqkv, wvt, wbt, wob, wobp, tmp_a, tmp_b, tmp_c, tmp_d,
            q_ref, pq_ref, k_ref, pk_ref, vt_ref, ot_ref, o_nat,
            s_a, s_b, m_a, m_b, p_a, p_b, l_a, l_b, mt_ref, gate_ref, bias_ref,
            qn, kn, vn, qo, ko, vo, halo, ab, eb, ob0, ob1, sems):

    def col_copies(src, dst, sem, c0=0, n=G):
        return [pltpu.make_async_copy(src.at[:, (c0 + i) * 128:(c0 + i + 1) * 128], dst.at[c0 + i], sem)
                for i in range(n)]

    cp_wq = [col_copies(wq_hbm, wq, sems.at[c], 2 * c, 2) for c in range(4)]
    cp_wk = col_copies(wk_hbm, wk, sems.at[4])
    cp_wv = [pltpu.make_async_copy(wv_hbm, wv, sems.at[5])]
    cp_wqkv = [[pltpu.make_async_copy(wqkv_hbm.at[:, part * D:(part + 1) * D], wqkv.at[part], sems.at[6 + part])]
               for part in range(3)]
    cp_wob = col_copies(wob_hbm, wob, sems.at[9])
    cp_woa = col_copies(woa_hbm, woa, sems.at[10])
    cp_x0 = [pltpu.make_async_copy(x_hbm.at[0:L], xin.at[0:L], sems.at[11])]
    cp_xr = [pltpu.make_async_copy(x_hbm.at[L:S], xin.at[L:S], sems.at[12])]

    def cp_out(seg, hf):
        return pltpu.make_async_copy(obuf.at[hf * HL:(hf + 1) * HL],
                                     out_hbm.at[pl.ds(pl.multiple_of(seg * L + hf * HL, HL), HL)], sems.at[13 + hf])

    def wait(cps):
        for c in cps:
            c.wait()

    def wcols(w_ref, c0):
        return jnp.concatenate([_ld(w_ref, c0, 0, D), _ld(w_ref, c0 + 1, 0, D)], axis=1)

    def q_item(src, n, d0, c):
        def run():
            y = _dot(_wide(src, 0, n), wcols(wq, 2 * c))
            for gg in range(2):
                yq = y[:, gg * 128:(gg + 1) * 128]
                _st(q_ref, 2 * c + gg, d0, (yq * QSCALE).astype(BF))
                _st(pq_ref, 2 * c + gg, d0, _phi(yq).astype(BF))
        return run

    def k_item(src, n, d0, c):
        def run():
            y = _dot(_wide(src, 0, n), wcols(wk, 2 * c))
            for gg in range(2):
                yk = y[:, gg * 128:(gg + 1) * 128]
                _st(k_ref, 2 * c + gg, d0, yk.astype(BF))
                _st(pk_ref, 2 * c + gg, d0, _phi(yk).astype(BF))
        return run

    def v_item(src, r0, tile0, f0):
        def run():
            y = _dot_nt(_wide(wvt, f0, 512), _wide(src, r0, HL))
            _st(vt_ref, tile0, f0, y[:, :128].astype(BF))
            _st(vt_ref, tile0 + 1, f0, y[:, 128:].astype(BF))
        return run

    def attn_prologue():
        _qk_stage(0, q_ref, k_ref, s_a, m_a, bias_ref)
        _qk_stage(1, q_ref, k_ref, s_b, m_b, bias_ref)
        _sm_stage(s_a, m_a, p_a, l_a)

    def blk(i):
        return pl.ds(pl.multiple_of(i * 128, 128), 128)

    def qkv_shuffle(part, kbk, tmp):
        tf = wqkv[part, blk(kbk), :].T.astype(F32)
        _shuffle_rows(tf, tmp, lambda r, val: _st(wbt, kbk, part * D + r, val))

    with _scope("first_proj"):
        for cps in [cp_x0] + cp_wq + [cp_wv, cp_wk] + cp_wqkv + [cp_wob, cp_woa, cp_xr]:
            for c in cps:
                c.start()
        b = beta_ref[...].astype(F32).reshape(1, H)
        gt = jax.nn.sigmoid(b)
        row = lax.broadcasted_iota(jnp.int32, (H, H), 0)
        lane = lax.broadcasted_iota(jnp.int32, (H, H), 1)
        col = jnp.sum(jnp.where(row == lane, jnp.broadcast_to(gt, (H, H)), 0.0), axis=1, keepdims=True)
        col = jnp.broadcast_to(col, (H, 128))
        for g in range(G):
            gate_ref[g] = jnp.concatenate([col[4 * g:4 * g + 4], col[4 * g:4 * g + 4]], axis=0)
        key = lax.broadcasted_iota(jnp.int32, (128, 128), 0)
        qry = lax.broadcasted_iota(jnp.int32, (128, 128), 1)
        bias_ref[...] = jnp.where(key <= qry, 0.0, NEG)
        halo[...] = jnp.zeros(halo.shape, F32)

        def zero_b(b, c):
            for r in (qn, kn, vn, ko, vo):
                r[b] = jnp.zeros(r.shape[1:], F32)
            return c
        lax.fori_loop(0, G, zero_b, 0)

        def zero_mem(i, c):
            mt_ref[i // (G + 1), i % (G + 1)] = jnp.zeros((144, 128), F32)
            return c
        lax.fori_loop(0, 2 * (G + 1), zero_mem, 0)
        with _scope("p_wait_x"):
            wait(cp_x0)

        def ln0(i, c):
            for u in range(16):
                r0 = pl.multiple_of(i * HL + u * 16, 16)
                x = xin[pl.ds(r0, 16), :].astype(F32)
                x_f[pl.ds(r0, 16), :] = x
                y = _ln(x).astype(BF)
                for b in range(G):
                    _st(xn, b, r0, y[:, b * 128:(b + 1) * 128])
            return c
        with _scope("p_ln"):
            lax.fori_loop(0, 2, ln0, 0)

        def q0(c, carry):
            for i in range(2):
                pltpu.make_async_copy(wq_hbm.at[:, 0:128], wq.at[0], sems.at[c]).wait()
            q_item(xn, L, 0, c)()
            return carry
        with _scope("p_q"):
            lax.fori_loop(0, 3, q0, 0)
        wait(cp_wq[3])
        wait(cp_wv)
        with _scope("p_tr"):
            q_item(xn, L, 0, 3)()
            for kbk in range(G):
                _st(wvt, kbk, 0, wv[kbk * 128:(kbk + 1) * 128, :].T)

        def v0(i, carry):
            hf = i // 2
            v_item(xn, hf * HL, 2 * hf, (i % 2) * 512)()
            return carry
        with _scope("p_v"):
            lax.fori_loop(0, 4, v0, 0)
        wait(cp_wk)
        wait(cp_wqkv[0])
        tmps = (tmp_a, tmp_b, tmp_c, tmp_d)

        def k0(c, carry):
            k_item(xn, L, 0, c)()
            for u in range(2):
                qkv_shuffle(0, 2 * c + u, tmps[u])
            return carry
        with _scope("p_k"):
            lax.fori_loop(0, 4, k0, 0)
        wait(cp_wqkv[1])
        wait(cp_wqkv[2])
        with _scope("p_attn"):
            attn_prologue()
            for u in range(2 * G):
                qkv_shuffle(1 + u // G, u % G, tmps[u % 4])
        wait(cp_wob)

        def sh1(i, carry):
            for u in range(4):
                cb = 4 * i + u
                _shuffle_rows(wob[cb].astype(F32), tmps[u], lambda r, val, cb=cb: _st(wobp, cb, r, val))
            return carry
        with _scope("p_sh1"):
            lax.fori_loop(0, 2, sh1, 0)
        wait(cp_woa)

    def out_item(src, s0, r0, w_ref, c, b0=0, b1=G, n=HL):
        def run():
            lhs = jnp.concatenate([_ld(src, b, s0, n) for b in range(b0, b1)], axis=1)
            w = jnp.concatenate([_ld(w_ref, 2 * c + i, b0 * 128, (b1 - b0) * 128) for i in range(2)], axis=1)
            x_f[r0:r0 + n, c * 256:(c + 1) * 256] += _dot(lhs, w)
        return run

    def b_proj_items():
        def item(part, c):
            def run():
                y = _dot_nt(_wide(xc, 0, HL), _wide(wbt, part * D + c * 256, 256))
                dst = (qn, kn, vn)[part]
                dst[2 * c] = y[:, :128]
                dst[2 * c + 1] = y[:, 128:]
            return run
        return [item(part, c) for part in range(3) for c in range(4)]

    def b_rotate():
        for b in range(G):
            qo[b] = qn[b]
            for new, old in ((kn, ko), (vn, vo)):
                old[b, 0:HALO, :] = old[b, HL:HL + HALO, :]
                old[b, HALO:, :] = new[b]

    def next_x_items(seg, layer, ch, chunk=16):
        nxt = jnp.minimum(seg + 1, NSEG - 1) * L

        def item(r0):
            def run():
                cur = ch.link_first(x_f[r0:r0 + chunk, :])
                obuf[r0:r0 + chunk, :] = cur.astype(BF)
                new = xin[pl.ds(pl.multiple_of(nxt + r0, chunk), chunk), :].astype(F32)
                x = jnp.where(layer == 1, new, cur)
                x_f[r0:r0 + chunk, :] = x
                yf = _ln(x)
                y = yf.astype(BF)
                for b in range(G):
                    _st(xc, b, r0, y[:, b * 128:(b + 1) * 128])
                ch.done(yf)
            return run
        return [item(r0) for r0 in range(0, HL, chunk)]

    def step(t, carry):
        seg = t // 2
        layer = t % 2
        mt = mt_ref.at[layer]
        never = lax.broadcasted_iota(jnp.int32, (8, 128), 0) < -t
        pv0 = lambda g, p, l: _pv_stage(g, p, l, vt_ref, ot_ref, pq_ref, mt, gate_ref)

        def pv(g, p, l):
            pv0(g, p, l)
            _mem_update(g, vt_ref, pk_ref, mt)

        @pl.when(t > 0)
        def _():
            with _scope("A_proj"):
                def a_half(hf, c):
                    d0 = hf * HL
                    parts = {'q': [q_item(xc, HL, d0, c) for c in range(4)],
                             'k': [k_item(xc, HL, d0, c) for c in range(4)],
                             'v': [v_item(xc, 0, 2 * hf, f0) for f0 in (0, 512)]}
                    items = [it for ch in A_ORDER for it in parts[ch]]
                    _interleave(items, _ln_items(x_f, xnx, HL, HL, 0, _Chain(never, NCH_LN_A)), span=SPAN_A)
                    xc.bitcast(U32)[...] = xnx.bitcast(U32)[...]
                    return c

                lax.fori_loop(0, 2, a_half, 0)
            with _scope("A_attn_pro"):
                attn_prologue()

        def pair(u, c):
            g = 2 * u + 1
            if UPD_SHIFT:
                for gq, gp, sq, mq, ss, ms, ps, ls, pp, lp in ((g + 1, g - 1, s_a, m_a, s_b, m_b, p_b, l_b, p_a, l_a),
                                                               (g + 2, g, s_b, m_b, s_a, m_a, p_a, l_a, p_b, l_b)):
                    ch = _Chain(never)
                    gu = jnp.maximum(gp - 1, 0)
                    _mem_update(gu, vt_ref, pk_ref, mt, ch, slot=jnp.where(gp > 0, gu, G))
                    _qk_stage(gq, q_ref, k_ref, sq, mq, bias_ref)
                    _sm_stage(ss, ms, ps, ls, after=ch)
                    pv0(gp, pp, lp)
            else:
                _qk_stage(g + 1, q_ref, k_ref, s_a, m_a, bias_ref)
                c1 = _Chain(never if QK_LINK else None)
                _sm_stage(s_b, m_b, p_b, l_b, fin=c1)
                pv0(g - 1, p_a, l_a)
                ch = _Chain(never)
                _mem_update(g - 1, vt_ref, pk_ref, mt, ch)
                _qk_stage(g + 2, q_ref, k_ref, s_b, m_b, bias_ref, after=c1)
                _sm_stage(s_a, m_a, p_a, l_a, after=ch)
                pv(g, p_b, l_b)
            return c

        with _scope("A_attn_loop"):
            lax.fori_loop(0, 3, pair, 0)

        @pl.when(t == 0)
        def _():
            wait(cp_xr)

        @pl.when(jnp.logical_and(layer == 0, seg > 0))
        def _():
            cp_out(seg - 1, 0).wait()
            cp_out(seg - 1, 1).wait()

        def transpose_o(b0, b1):
            for j in range(4):
                ot = _ld(ot_ref, j, b0 * 128, (b1 - b0) * 128).T
                for b in range(b0, b1):
                    _st(o_nat, b, j * 128, ot[:, (b - b0) * 128:(b - b0 + 1) * 128])

        with _scope("A_out"):
            transpose_o(0, G - 2)
            _sm_stage(s_b, m_b, p_b, l_b, _Chain(never if NCH_EPI else None, max(NCH_EPI, 1)))
            if UPD_SHIFT:
                _mem_update(G - 3, vt_ref, pk_ref, mt)
            pv(G - 2, p_a, l_a)
            if KSPLIT == G - 1:
                transpose_o(G - 2, G - 1)
            _run([out_item(o_nat, 0, 0, woa, c, 0, KSPLIT) for c in range(4)])
            pv(G - 1, p_b, l_b)
            transpose_o(KSPLIT, G)
            kn[:, HL - HALO:HL, :] = halo[layer, 0]
            vn[:, HL - HALO:HL, :] = halo[layer, 1]
            _run([out_item(o_nat, 0, 0, woa, c, KSPLIT, G) for c in range(4)])
            _run(_ln_items(x_f, xc, 0, HL, 0, _Chain(never, NCH_LN_OUT)))
            _run([out_item(o_nat, HL, HL, woa, c) for c in range(4)])

        def b_half(hf, c):
            b_rotate()
            band = _band_items(seg * L + (hf - 1) * HL, 0, qo, ko, vo, ab, eb, ob0, _Chain(never, NCH_B0))
            ln = _ln_items(x_f, xnx, HL, HL, 0, _Chain(never, NCH_LN_B))
            _interleave(b_proj_items(), ln + band if LN_FIRST_B else band + ln, span=SPAN_B)
            xc.bitcast(U32)[...] = xnx.bitcast(U32)[...]
            return c

        with _scope("B_loop"):
            lax.fori_loop(0, 2, b_half, 0)

        with _scope("B_tail"):
            halo[layer, 0] = kn[:, HL - HALO:HL, :]
            halo[layer, 1] = vn[:, HL - HALO:HL, :]
            b_rotate()
            _run(_band_items(seg * L + HL, 0, qo, ko, vo, ab, eb, ob1, _Chain(never, NCH_B1)))
            _run([out_item(ob0, 0, 0, wobp, c) for c in range(4)])
            _run(next_x_items(seg, layer, _Chain(never, NCH_NEXT)))
            _run([out_item(ob1, 0, HL, wobp, c, n=128) for c in range(4)])
            _run([out_item(ob1, 128, HL + 128, wobp, c, n=128) for c in range(4)])

        @pl.when(layer == 1)
        def _():
            cp_out(seg, 0).start()
            obuf[HL:L, :] = x_f[HL:L, :].astype(BF)
            cp_out(seg, 1).start()

            @pl.when(seg < NSEG - 1)
            def _():
                x_f[HL:L, :] = xin[pl.ds(pl.multiple_of((seg + 1) * L + HL, HL), HL), :].astype(F32)

        return carry

    lax.fori_loop(0, 2 * NSEG, step, 0)
    cp_out(NSEG - 1, 0).wait()
    cp_out(NSEG - 1, 1).wait()


@jax.jit
def pallas_interleave_layers__memory_aug_infini_attn__sliding_local_dilated__prompt_kernel(
    A_x: jax.Array,
    A_wq: jax.Array,
    A_wk: jax.Array,
    A_wv: jax.Array,
    A_wo: jax.Array,
    A_beta: jax.Array,
    B_x: jax.Array,
    B_wqkv: jax.Array,
    B_wo: jax.Array,
):
    del B_x
    x = A_x.reshape(S, D)
    any_spec = pl.BlockSpec(memory_space=pl.ANY)
    blk = lambda rows, dt: pltpu.VMEM((G, rows, 128), dt)
    packed = lambda rows, n=G: pltpu.VMEM((n, rows, 128), BF)
    scratch = [
        pltpu.VMEM((S, D), BF),
        pltpu.VMEM((L, D), BF),
        pltpu.VMEM((L, D), F32),
        packed(L),
        packed(HL),
        packed(HL),
        blk(D, BF),
        blk(D, BF),
        blk(D, BF),
        pltpu.VMEM((D, D), BF),
        pltpu.VMEM((3, D, D), BF),
        packed(D),
        packed(3 * D),
        blk(D, BF),
        packed(D),
        pltpu.VMEM((H * PITCH, 128), F32),
        pltpu.VMEM((H * PITCH, 128), F32),
        pltpu.VMEM((H * PITCH, 128), F32),
        pltpu.VMEM((H * PITCH, 128), F32),
        packed(L),
        packed(L),
        packed(L),
        packed(L),
        packed(D, 4),
        packed(D, 4),
        packed(L),
        pltpu.VMEM((1280, 512), F32),
        pltpu.VMEM((1280, 512), F32),
        pltpu.VMEM((4, 8, 512), F32),
        pltpu.VMEM((4, 8, 512), F32),
        packed(1280, 4),
        packed(1280, 4),
        pltpu.VMEM((4, 8, 128), F32),
        pltpu.VMEM((4, 8, 128), F32),
        pltpu.VMEM((2, G + 1, 144, 128), F32),
        pltpu.VMEM((G, 8, 128), F32),
        pltpu.VMEM((128, 128), F32),
        blk(HL, F32),
        blk(HL, F32),
        blk(HL, F32),
        blk(HL, F32),
        blk(HL + HALO, F32),
        blk(HL + HALO, F32),
        pltpu.VMEM((2, 2, G, HALO, 128), F32),
        pltpu.VMEM((W, HL, 128), F32),
        pltpu.VMEM((W, HL, 128), F32),
        packed(HL),
        packed(HL),
        pltpu.SemaphoreType.DMA((15,)),
    ]
    out = pl.pallas_call(
        _kernel,
        in_specs=[any_spec, any_spec, any_spec, any_spec, any_spec,
                  pl.BlockSpec(memory_space=pltpu.VMEM), any_spec, any_spec],
        out_specs=any_spec,
        out_shape=jax.ShapeDtypeStruct((S, D), BF),
        scratch_shapes=scratch,
        compiler_params=pltpu.CompilerParams(vmem_limit_bytes=100 * 1024 * 1024),
    )(x, A_wq, A_wk, A_wv, A_wo, A_beta, B_wqkv, B_wo)
    return out.reshape(1, S, D)
```

```python
import math

import jax
import jax.numpy as jnp
from jax import lax
import jax.experimental.pallas as pl
import jax.experimental.pallas.tpu as pltpu

S, D, H, DH = 2048, 1024, 32, 32
L, NSEG, G = 512, 4, 8
HL = L // 2
W, DIL = 8, 2
HALO = 16
BF, F32, U32 = jnp.bfloat16, jnp.float32, jnp.uint32
QSCALE = (DH ** -0.5) * math.log2(math.e)
NEG = -1e30
NT = (((1,), (1,)), ((), ()))
OFF = (0, 128, 384, 768)
SCOPES = False
NCH_B1 = 2
PV_ONE_DOT = True
KSPLIT = 7
NCH_EPI = 0
SM_SUB = 32
NCH_LN_A, NCH_LN_OUT, NCH_LN_B, NCH_B0, NCH_NEXT = 1, 3, 2, 1, 2
QK_ORDER, SM_ORDER, PV_ORDER = (0, 1, 2, 3), (0, 1, 2, 3), (0, 1, 2, 3)
PV_ONE_DOT, QK_SPLIT, SPAN_A, A_ORDER = True, False, 8, 'qkv'
UPD_SHIFT = False
QK_LINK = False
ATT_UNROLL = False
EPI_UPD_LINK = True
LN_FIRST_B, SPAN_B = False, 12
PITCH = 33


class _scope:
    def __init__(self, name):
        self.cm = jax.named_scope(name) if SCOPES else None

    def __enter__(self):
        if self.cm is not None:
            self.cm.__enter__()

    def __exit__(self, *a):
        if self.cm is not None:
            self.cm.__exit__(*a)


def _dot(a, b):
    return jnp.dot(a, b, preferred_element_type=F32)


def _dot_nt(a, b):
    return lax.dot_general(a, b, NT, preferred_element_type=F32)


def _rows(r0, n, align=16):
    return slice(r0, r0 + n) if isinstance(r0, int) else pl.ds(pl.multiple_of(r0, align), n)


def _ldu(ref, b, r0, n):
    idx = slice(r0 // 2, (r0 + n) // 2) if isinstance(r0, int) else pl.ds(pl.multiple_of(r0 // 2, 8), n // 2)
    return ref.bitcast(U32)[b, idx, :]


def _ld(ref, b, r0, n):
    return pltpu.bitcast(_ldu(ref, b, r0, n), BF)


def _st(ref, b, r0, val):
    ref[b, _rows(r0, val.shape[0]), :] = val


def _wide(ref, r0, n):
    return jnp.concatenate([_ld(ref, b, r0, n) for b in range(G)], axis=1)


class _Chain:
    def __init__(self, never, n=1):
        self.never, self.n, self.hist = never, n, []

    def link(self, x):
        if self.never is None or len(self.hist) < self.n:
            return x
        return jnp.where(self.never, self.hist[-self.n], x)

    def link_first(self, x):
        head = self.link(x[0:8, 0:128])
        if x.shape[1] > 128:
            head = jnp.concatenate([head, x[0:8, 128:]], axis=1)
        return head if x.shape[0] == 8 else jnp.concatenate([head, x[8:]], axis=0)

    def link_packed(self, u):
        if self.never is None or len(self.hist) < self.n:
            return u
        head = jnp.where(self.never, pltpu.bitcast(self.hist[-self.n], U32), u[0:8])
        return head if u.shape[0] == 8 else jnp.concatenate([head, u[8:]], axis=0)

    def done(self, v):
        self.hist.append(v[0:8, v.shape[1] - 128:])


def _phi(t):
    return jnp.where(t > 0, t + 1.0, jnp.exp(t))


def _ln(x):
    d = x - jnp.mean(x, axis=-1, keepdims=True)
    v = jnp.mean(d * d, axis=-1, keepdims=True)
    return d * lax.rsqrt(v + 1e-5)


def _ln_items(x_ref, xn_ref, row0, nrows, dst0, ch, chunk=16):
    def item(r0):
        def run():
            yf = _ln(ch.link_first(x_ref[r0:r0 + chunk, :]))
            y = yf.astype(BF)
            for b in range(G):
                _st(xn_ref, b, r0 - row0 + dst0, y[:, b * 128:(b + 1) * 128])
            ch.done(yf)
        return run
    return [item(r0) for r0 in range(row0, row0 + nrows, chunk)]


def _interleave(main, side, span=None):
    span = len(main) if span is None else span
    done = 0
    for i, it in enumerate(main):
        upto = len(side) if i + 1 >= span else (len(side) * (i + 1)) // span
        for s_it in side[done:upto]:
            s_it()
        done = max(done, upto)
        it()


def _run(items):
    for it in items:
        it()


def _shuffle_rows(tf, tmp, store):
    for h in range(H):
        tmp[h * PITCH:h * PITCH + DH, :] = tf[h * DH:(h + 1) * DH]
    for d in range(DH):
        for th in range(2):
            rows = tmp[pl.ds(th * 16 * PITCH + d, 16, stride=PITCH), :]
            store(d * H + th * 16, rows.astype(BF))


def _qk_stage(g, q_ref, k_ref, s_ref, m_ref, bias_ref, after=None):
    lane = lax.broadcasted_iota(jnp.int32, (64, 128), 1)
    for j in QK_ORDER:
        nk = 128 * (j + 1)
        qt = _ldu(q_ref, g, j * 128, 128)
        if after is not None:
            qt = after.link_packed(qt)
        wq = jnp.concatenate([jnp.where((lane >> 5) == h, qt, jnp.uint32(0)) for h in range(4)], axis=0)
        if QK_SPLIT:
            st = jnp.concatenate([_dot_nt(_ld(k_ref, g, t * 128, 128), pltpu.bitcast(wq, BF)) for t in range(j + 1)], axis=0)
        else:
            st = _dot_nt(_ld(k_ref, g, 0, nk), pltpu.bitcast(wq, BF))
        bias = bias_ref[...]
        diag = st[j * 128:] + jnp.concatenate([bias] * 4, axis=1)
        s_ref[OFF[j] + j * 128:OFF[j] + nk, :] = diag
        m = jnp.max(diag.reshape(16, 8, 512), axis=0)
        if j > 0:
            s_ref[OFF[j]:OFF[j] + j * 128, :] = st[:j * 128]
            m = jnp.maximum(m, jnp.max(st[:j * 128].reshape(16 * j, 8, 512), axis=0))
        m_ref[j] = jnp.broadcast_to(jnp.max(m, axis=0, keepdims=True), (8, 512))


def _sm_stage(s_ref, m_ref, p_ref, l_ref, ch=None, after=None, fin=None):
    ch = _Chain(None) if ch is None else ch
    sub = SM_SUB
    for j in SM_ORDER:
        nk = 128 * (j + 1)
        sums = []
        for h in range(4):
            m = m_ref[j, :, h * 128:(h + 1) * 128]
            if after is not None:
                m = after.link(m)
            l = None
            for r in range(0, nk, sub):
                s = ch.link_first(s_ref[OFF[j] + r:OFF[j] + r + sub, h * 128:(h + 1) * 128])
                p = jnp.exp2(s.reshape(sub // 8, 8, 128) - m[None])
                ls = jnp.sum(p, axis=0)
                l = ls if l is None else l + ls
                _st(p_ref, h, OFF[j] + r, p.reshape(sub, 128).astype(BF))
                ch.done(p[0])
            sums.append(jnp.sum(l, axis=0, keepdims=True))
        lsum = jnp.concatenate(sums + sums, axis=0)
        l_ref[j] = lsum
    if fin is not None:
        fin.done(lsum)


def _pv_stage(g, p_ref, l_ref, vt_ref, ot_ref, pq_ref, mt_ref, gate_ref):
    mem = mt_ref[g].astype(BF)
    gate = gate_ref[g]
    for j in PV_ORDER:
        nd = _dot_nt(mem, _ld(pq_ref, g, j * 128, 128))
        c_mem = gate / (nd[128:136] + 1e-6)
        c_att = (1.0 - gate) / l_ref[j]
        for h in range(4):
            r0 = (g * 4 + h) * DH
            if PV_ONE_DOT:
                vt = jnp.concatenate([_ld(vt_ref, t, r0, DH) for t in range(j + 1)], axis=1)
                acc = _dot(vt, _ld(p_ref, h, OFF[j], 128 * (j + 1)))
            else:
                acc = None
                for t in range(j + 1):
                    o = _dot(_ld(vt_ref, t, r0, DH), _ld(p_ref, h, OFF[j] + t * 128, 128))
                    acc = o if acc is None else acc + o
            res = nd[h * DH:(h + 1) * DH] * c_mem[h:h + 1] + acc * c_att[h:h + 1]
            _st(ot_ref, j, r0, res.astype(BF))


def _mem_update(g, vt_ref, pk_ref, mt_ref, ch=None, slot=None):
    row = lax.broadcasted_iota(jnp.int32, (144, 128), 0)
    lane = lax.broadcasted_iota(jnp.int32, (144, 128), 1)
    keep = jnp.where(row < 128, row >> 5, row - 128) == (lane >> 5)
    row16 = lax.broadcasted_iota(jnp.int32, (16, 128), 0)
    ones = jnp.where(row16 < 4, 1.0, 0.0).astype(BF)
    upd = None
    for t in range(4):
        lhs = jnp.concatenate([_ld(vt_ref, t, g * 128, 128), ones], axis=0)
        u = _dot(lhs, _ld(pk_ref, g, t * 128, 128))
        upd = u if upd is None else upd + u
    slot = g if slot is None else slot
    new = mt_ref[slot] + jnp.where(keep, upd, 0.0)
    mt_ref[slot] = new
    if ch is not None:
        ch.done(new)


def _band_items(pos0, row0, q_ref, k_ref, v_ref, a_ref, e_ref, o_ref, ch, nrows=HL):
    def logits(r0):
        def run():
            q = [q_ref[b, r0:r0 + 8, :] for b in range(G)]
            for w in range(W):
                base = HALO + r0 - DIL * w
                acc = ch.link(q[0] * k_ref[0, base:base + 8, :])
                for b in range(1, G):
                    acc = acc + q[b] * k_ref[b, base:base + 8, :]
                a_ref[w, r0 - row0:r0 - row0 + 8, :] = acc
                ch.done(acc)
        return run

    def softmax(r0):
        def run():
            lg = []
            for w in range(W):
                t = a_ref[w, r0 - row0:r0 - row0 + 128, :].T
                t = ((t[0:32] + t[32:64]) + (t[64:96] + t[96:128])) * QSCALE
                if r0 == row0 and w > 0:
                    pos = pos0 - DIL * w + lax.broadcasted_iota(jnp.int32, (H, 128), 1)
                    t = jnp.where(pos >= 0, t, NEG)
                lg.append(t)
            m = lg[0]
            for w in range(1, W):
                m = jnp.maximum(m, lg[w])
            e = [jnp.exp2(x - m) for x in lg]
            l = e[0]
            for w in range(1, W):
                l = l + e[w]
            inv = 1.0 / l
            for w in range(W):
                p = e[w] * inv
                pt = jnp.concatenate([p, p, p, p], axis=0).T
                e_ref[w, r0 - row0:r0 - row0 + 128, :] = pt
        return run

    def pv(r0):
        e = [e_ref[w, r0 - row0:r0 - row0 + 8, :] for w in range(W)]
        outs = []
        for b in range(G):
            acc = ch.link(e[0] * v_ref[b, HALO + r0:HALO + r0 + 8, :])
            for w in range(1, W):
                base = HALO + r0 - DIL * w
                acc = acc + e[w] * v_ref[b, base:base + 8, :]
            outs.append(acc)
            ch.done(acc)
        return outs

    def pv16(r0):
        def run():
            lo = pv(r0)
            hi = pv(r0 + 8)
            for b in range(G):
                _st(o_ref, b, r0, jnp.concatenate([lo[b], hi[b]], axis=0).astype(BF))
        return run

    items = []
    for r0 in range(row0, row0 + nrows, 128):
        items += [logits(r) for r in range(r0, r0 + 128, 8)]
        items.append(softmax(r0))
        items += [pv16(r) for r in range(r0, r0 + 128, 16)]
    return items


def _kernel(x_hbm, wq_hbm, wk_hbm, wv_hbm, woa_hbm, beta_ref, wqkv_hbm, wob_hbm, out_hbm,
            xin, obuf, x_f, xn, xc, xnx, wq, wk, woa, wv, wqkv, wvt, wbt, wob, wobp, tmp_a, tmp_b, tmp_c, tmp_d,
            q_ref, pq_ref, k_ref, pk_ref, vt_ref, ot_ref, o_nat,
            s_a, s_b, m_a, m_b, p_a, p_b, l_a, l_b, mt_ref, gate_ref, bias_ref,
            qn, kn, vn, qo, ko, vo, halo, ab, eb, ob0, ob1, sems):

    def col_copies(src, dst, sem, c0=0, n=G):
        return [pltpu.make_async_copy(src.at[:, (c0 + i) * 128:(c0 + i + 1) * 128], dst.at[c0 + i], sem)
                for i in range(n)]

    cp_wq = [col_copies(wq_hbm, wq, sems.at[c], 2 * c, 2) for c in range(4)]
    cp_wk = col_copies(wk_hbm, wk, sems.at[4])
    cp_wv = [pltpu.make_async_copy(wv_hbm, wv, sems.at[5])]
    cp_wqkv = [[pltpu.make_async_copy(wqkv_hbm.at[:, part * D:(part + 1) * D], wqkv.at[part], sems.at[6 + part])]
               for part in range(3)]
    cp_wob = col_copies(wob_hbm, wob, sems.at[9])
    cp_woa = col_copies(woa_hbm, woa, sems.at[10])
    cp_x0 = [pltpu.make_async_copy(x_hbm.at[0:L], xin.at[0:L], sems.at[11])]
    cp_xr = [pltpu.make_async_copy(x_hbm.at[L:S], xin.at[L:S], sems.at[12])]

    def cp_out(seg, hf):
        return pltpu.make_async_copy(obuf.at[hf * HL:(hf + 1) * HL],
                                     out_hbm.at[pl.ds(pl.multiple_of(seg * L + hf * HL, HL), HL)], sems.at[13 + hf])

    def wait(cps):
        for c in cps:
            c.wait()

    def wcols(w_ref, c0):
        return jnp.concatenate([_ld(w_ref, c0, 0, D), _ld(w_ref, c0 + 1, 0, D)], axis=1)

    def q_item(src, n, d0, c):
        def run():
            y = _dot(_wide(src, 0, n), wcols(wq, 2 * c))
            for gg in range(2):
                yq = y[:, gg * 128:(gg + 1) * 128]
                _st(q_ref, 2 * c + gg, d0, (yq * QSCALE).astype(BF))
                _st(pq_ref, 2 * c + gg, d0, _phi(yq).astype(BF))
        return run

    def k_item(src, n, d0, c):
        def run():
            y = _dot(_wide(src, 0, n), wcols(wk, 2 * c))
            for gg in range(2):
                yk = y[:, gg * 128:(gg + 1) * 128]
                _st(k_ref, 2 * c + gg, d0, yk.astype(BF))
                _st(pk_ref, 2 * c + gg, d0, _phi(yk).astype(BF))
        return run

    def v_item(src, r0, tile0, f0):
        def run():
            y = _dot_nt(_wide(wvt, f0, 512), _wide(src, r0, HL))
            _st(vt_ref, tile0, f0, y[:, :128].astype(BF))
            _st(vt_ref, tile0 + 1, f0, y[:, 128:].astype(BF))
        return run

    def attn_prologue():
        _qk_stage(0, q_ref, k_ref, s_a, m_a, bias_ref)
        _qk_stage(1, q_ref, k_ref, s_b, m_b, bias_ref)
        _sm_stage(s_a, m_a, p_a, l_a)

    def blk(i):
        return pl.ds(pl.multiple_of(i * 128, 128), 128)

    def qkv_shuffle(part, kbk, tmp):
        tf = wqkv[part, blk(kbk), :].T.astype(F32)
        _shuffle_rows(tf, tmp, lambda r, val: _st(wbt, kbk, part * D + r, val))

    with _scope("first_proj"):
        for cps in [cp_x0] + cp_wq + [cp_wv, cp_wk] + cp_wqkv + [cp_wob, cp_woa, cp_xr]:
            for c in cps:
                c.start()
        b = beta_ref[...].astype(F32).reshape(1, H)
        gt = jax.nn.sigmoid(b)
        row = lax.broadcasted_iota(jnp.int32, (H, H), 0)
        lane = lax.broadcasted_iota(jnp.int32, (H, H), 1)
        col = jnp.sum(jnp.where(row == lane, jnp.broadcast_to(gt, (H, H)), 0.0), axis=1, keepdims=True)
        col = jnp.broadcast_to(col, (H, 128))
        for g in range(G):
            gate_ref[g] = jnp.concatenate([col[4 * g:4 * g + 4], col[4 * g:4 * g + 4]], axis=0)
        key = lax.broadcasted_iota(jnp.int32, (128, 128), 0)
        qry = lax.broadcasted_iota(jnp.int32, (128, 128), 1)
        bias_ref[...] = jnp.where(key <= qry, 0.0, NEG)
        halo[...] = jnp.zeros(halo.shape, F32)

        def zero_b(b, c):
            for r in (qn, kn, vn, ko, vo):
                r[b] = jnp.zeros(r.shape[1:], F32)
            return c
        lax.fori_loop(0, G, zero_b, 0)

        def zero_mem(i, c):
            mt_ref[i // (G + 1), i % (G + 1)] = jnp.zeros((144, 128), F32)
            return c
        lax.fori_loop(0, 2 * (G + 1), zero_mem, 0)
        with _scope("p_wait_x"):
            wait(cp_x0)

        def ln0(i, c):
            for u in range(16):
                r0 = pl.multiple_of(i * HL + u * 16, 16)
                x = xin[pl.ds(r0, 16), :].astype(F32)
                x_f[pl.ds(r0, 16), :] = x
                y = _ln(x).astype(BF)
                for b in range(G):
                    _st(xn, b, r0, y[:, b * 128:(b + 1) * 128])
            return c
        with _scope("p_ln"):
            lax.fori_loop(0, 2, ln0, 0)

        def q0(c, carry):
            for i in range(2):
                pltpu.make_async_copy(wq_hbm.at[:, 0:128], wq.at[0], sems.at[c]).wait()
            q_item(xn, L, 0, c)()
            return carry
        with _scope("p_q"):
            lax.fori_loop(0, 3, q0, 0)
        wait(cp_wq[3])
        wait(cp_wv)
        with _scope("p_tr"):
            q_item(xn, L, 0, 3)()
            for kbk in range(G):
                _st(wvt, kbk, 0, wv[kbk * 128:(kbk + 1) * 128, :].T)

        def v0(i, carry):
            hf = i // 2
            v_item(xn, hf * HL, 2 * hf, (i % 2) * 512)()
            return carry
        with _scope("p_v"):
            lax.fori_loop(0, 4, v0, 0)
        wait(cp_wk)
        wait(cp_wqkv[0])
        tmps = (tmp_a, tmp_b, tmp_c, tmp_d)

        def k0(c, carry):
            k_item(xn, L, 0, c)()
            for u in range(2):
                qkv_shuffle(0, 2 * c + u, tmps[u])
            return carry
        with _scope("p_k"):
            lax.fori_loop(0, 4, k0, 0)
        wait(cp_wqkv[1])
        wait(cp_wqkv[2])
        with _scope("p_attn"):
            attn_prologue()
            for u in range(2 * G):
                qkv_shuffle(1 + u // G, u % G, tmps[u % 4])
        wait(cp_wob)

        def sh1(i, carry):
            for u in range(4):
                cb = 4 * i + u
                _shuffle_rows(wob[cb].astype(F32), tmps[u], lambda r, val, cb=cb: _st(wobp, cb, r, val))
            return carry
        with _scope("p_sh1"):
            lax.fori_loop(0, 2, sh1, 0)
        wait(cp_woa)

    def out_item(src, s0, r0, w_ref, c, b0=0, b1=G, n=HL):
        def run():
            lhs = jnp.concatenate([_ld(src, b, s0, n) for b in range(b0, b1)], axis=1)
            w = jnp.concatenate([_ld(w_ref, 2 * c + i, b0 * 128, (b1 - b0) * 128) for i in range(2)], axis=1)
            x_f[r0:r0 + n, c * 256:(c + 1) * 256] += _dot(lhs, w)
        return run

    def b_proj_items():
        def item(part, c):
            def run():
                y = _dot_nt(_wide(xc, 0, HL), _wide(wbt, part * D + c * 256, 256))
                dst = (qn, kn, vn)[part]
                dst[2 * c] = y[:, :128]
                dst[2 * c + 1] = y[:, 128:]
            return run
        return [item(part, c) for part in range(3) for c in range(4)]

    def b_rotate():
        for b in range(G):
            qo[b] = qn[b]
            for new, old in ((kn, ko), (vn, vo)):
                old[b, 0:HALO, :] = old[b, HL:HL + HALO, :]
                old[b, HALO:, :] = new[b]

    def next_x_items(seg, layer, ch, chunk=16):
        nxt = jnp.minimum(seg + 1, NSEG - 1) * L

        def item(r0):
            def run():
                cur = ch.link_first(x_f[r0:r0 + chunk, :])
                obuf[r0:r0 + chunk, :] = cur.astype(BF)
                new = xin[pl.ds(pl.multiple_of(nxt + r0, chunk), chunk), :].astype(F32)
                x = jnp.where(layer == 1, new, cur)
                x_f[r0:r0 + chunk, :] = x
                yf = _ln(x)
                y = yf.astype(BF)
                for b in range(G):
                    _st(xc, b, r0, y[:, b * 128:(b + 1) * 128])
                ch.done(yf)
            return run
        return [item(r0) for r0 in range(0, HL, chunk)]

    def step(t, carry):
        seg = t // 2
        layer = t % 2
        mt = mt_ref.at[layer]
        never = lax.broadcasted_iota(jnp.int32, (8, 128), 0) < -t
        pv0 = lambda g, p, l: _pv_stage(g, p, l, vt_ref, ot_ref, pq_ref, mt, gate_ref)

        def pv(g, p, l):
            pv0(g, p, l)
            _mem_update(g, vt_ref, pk_ref, mt)

        @pl.when(t > 0)
        def _():
            with _scope("A_proj"):
                def a_half(hf, c):
                    d0 = hf * HL
                    parts = {'q': [q_item(xc, HL, d0, c) for c in range(4)],
                             'k': [k_item(xc, HL, d0, c) for c in range(4)],
                             'v': [v_item(xc, 0, 2 * hf, f0) for f0 in (0, 512)]}
                    items = [it for ch in A_ORDER for it in parts[ch]]
                    _interleave(items, _ln_items(x_f, xnx, HL, HL, 0, _Chain(never, NCH_LN_A)), span=SPAN_A)
                    xc.bitcast(U32)[...] = xnx.bitcast(U32)[...]
                    return c

                lax.fori_loop(0, 2, a_half, 0)
            with _scope("A_attn_pro"):
                attn_prologue()

        def pair(u, c):
            g = 2 * u + 1
            if UPD_SHIFT:
                for gq, gp, sq, mq, ss, ms, ps, ls, pp, lp in ((g + 1, g - 1, s_a, m_a, s_b, m_b, p_b, l_b, p_a, l_a),
                                                               (g + 2, g, s_b, m_b, s_a, m_a, p_a, l_a, p_b, l_b)):
                    ch = _Chain(never)
                    gu = jnp.maximum(gp - 1, 0)
                    _mem_update(gu, vt_ref, pk_ref, mt, ch, slot=jnp.where(gp > 0, gu, G))
                    _qk_stage(gq, q_ref, k_ref, sq, mq, bias_ref)
                    _sm_stage(ss, ms, ps, ls, after=ch)
                    pv0(gp, pp, lp)
            else:
                _qk_stage(g + 1, q_ref, k_ref, s_a, m_a, bias_ref)
                c1 = _Chain(never if QK_LINK else None)
                _sm_stage(s_b, m_b, p_b, l_b, fin=c1)
                pv0(g - 1, p_a, l_a)
                ch = _Chain(never)
                _mem_update(g - 1, vt_ref, pk_ref, mt, ch)
                _qk_stage(g + 2, q_ref, k_ref, s_b, m_b, bias_ref, after=c1)
                _sm_stage(s_a, m_a, p_a, l_a, after=ch)
                pv(g, p_b, l_b)
            return c

        with _scope("A_attn_loop"):
            if ATT_UNROLL:
                for u in range(3):
                    pair(u, 0)
            else:
                lax.fori_loop(0, 3, pair, 0)

        @pl.when(t == 0)
        def _():
            wait(cp_xr)

        @pl.when(jnp.logical_and(layer == 0, seg > 0))
        def _():
            cp_out(seg - 1, 0).wait()
            cp_out(seg - 1, 1).wait()

        def transpose_o(b0, b1):
            for j in range(4):
                ot = _ld(ot_ref, j, b0 * 128, (b1 - b0) * 128).T
                for b in range(b0, b1):
                    _st(o_nat, b, j * 128, ot[:, (b - b0) * 128:(b - b0 + 1) * 128])

        with _scope("A_out"):
            transpose_o(0, G - 2)
            _sm_stage(s_b, m_b, p_b, l_b, _Chain(never if NCH_EPI else None, max(NCH_EPI, 1)))
            ch_ln = _Chain(never, NCH_LN_OUT)
            u6, u7 = _Chain(None), _Chain(None)
            pv0(G - 2, p_a, l_a)
            _mem_update(G - 2, vt_ref, pk_ref, mt, u6)
            if KSPLIT == G - 1:
                transpose_o(G - 2, G - 1)
            _run([out_item(o_nat, 0, 0, woa, c, 0, KSPLIT) for c in range(4)])
            pv0(G - 1, p_b, l_b)
            _mem_update(G - 1, vt_ref, pk_ref, mt, u7)
            transpose_o(KSPLIT, G)
            kn[:, HL - HALO:HL, :] = halo[layer, 0]
            vn[:, HL - HALO:HL, :] = halo[layer, 1]
            _run([out_item(o_nat, 0, 0, woa, c, KSPLIT, G) for c in range(4)])
            if EPI_UPD_LINK:
                ch_ln.hist = [u6.hist[0], u7.hist[0]][-NCH_LN_OUT:] + [u7.hist[0]] * max(NCH_LN_OUT - 2, 0)
            _run(_ln_items(x_f, xc, 0, HL, 0, ch_ln))
            _run([out_item(o_nat, HL, HL, woa, c) for c in range(4)])

        def b_half(hf, c):
            b_rotate()
            band = _band_items(seg * L + (hf - 1) * HL, 0, qo, ko, vo, ab, eb, ob0, _Chain(never, NCH_B0))
            ln = _ln_items(x_f, xnx, HL, HL, 0, _Chain(never, NCH_LN_B))
            _interleave(b_proj_items(), ln + band if LN_FIRST_B else band + ln, span=SPAN_B)
            xc.bitcast(U32)[...] = xnx.bitcast(U32)[...]
            return c

        with _scope("B_loop"):
            lax.fori_loop(0, 2, b_half, 0)

        with _scope("B_tail"):
            halo[layer, 0] = kn[:, HL - HALO:HL, :]
            halo[layer, 1] = vn[:, HL - HALO:HL, :]
            b_rotate()
            _run(_band_items(seg * L + HL, 0, qo, ko, vo, ab, eb, ob1, _Chain(never, NCH_B1)))
            _run([out_item(ob0, 0, 0, wobp, c) for c in range(4)])
            _run(next_x_items(seg, layer, _Chain(never, NCH_NEXT)))
            _run([out_item(ob1, 0, HL, wobp, c, n=128) for c in range(4)])
            _run([out_item(ob1, 128, HL + 128, wobp, c, n=128) for c in range(4)])

        @pl.when(layer == 1)
        def _():
            cp_out(seg, 0).start()
            obuf[HL:L, :] = x_f[HL:L, :].astype(BF)
            cp_out(seg, 1).start()

            @pl.when(seg < NSEG - 1)
            def _():
                x_f[HL:L, :] = xin[pl.ds(pl.multiple_of((seg + 1) * L + HL, HL), HL), :].astype(F32)

        return carry

    lax.fori_loop(0, 2 * NSEG, step, 0)
    cp_out(NSEG - 1, 0).wait()
    cp_out(NSEG - 1, 1).wait()


@jax.jit
def pallas_interleave_layers__memory_aug_infini_attn__sliding_local_dilated__prompt_kernel(
    A_x: jax.Array,
    A_wq: jax.Array,
    A_wk: jax.Array,
    A_wv: jax.Array,
    A_wo: jax.Array,
    A_beta: jax.Array,
    B_x: jax.Array,
    B_wqkv: jax.Array,
    B_wo: jax.Array,
):
    del B_x
    x = A_x.reshape(S, D)
    any_spec = pl.BlockSpec(memory_space=pl.ANY)
    blk = lambda rows, dt: pltpu.VMEM((G, rows, 128), dt)
    packed = lambda rows, n=G: pltpu.VMEM((n, rows, 128), BF)
    scratch = [
        pltpu.VMEM((S, D), BF),
        pltpu.VMEM((L, D), BF),
        pltpu.VMEM((L, D), F32),
        packed(L),
        packed(HL),
        packed(HL),
        blk(D, BF),
        blk(D, BF),
        blk(D, BF),
        pltpu.VMEM((D, D), BF),
        pltpu.VMEM((3, D, D), BF),
        packed(D),
        packed(3 * D),
        blk(D, BF),
        packed(D),
        pltpu.VMEM((H * PITCH, 128), F32),
        pltpu.VMEM((H * PITCH, 128), F32),
        pltpu.VMEM((H * PITCH, 128), F32),
        pltpu.VMEM((H * PITCH, 128), F32),
        packed(L),
        packed(L),
        packed(L),
        packed(L),
        packed(D, 4),
        packed(D, 4),
        packed(L),
        pltpu.VMEM((1280, 512), F32),
        pltpu.VMEM((1280, 512), F32),
        pltpu.VMEM((4, 8, 512), F32),
        pltpu.VMEM((4, 8, 512), F32),
        packed(1280, 4),
        packed(1280, 4),
        pltpu.VMEM((4, 8, 128), F32),
        pltpu.VMEM((4, 8, 128), F32),
        pltpu.VMEM((2, G + 1, 144, 128), F32),
        pltpu.VMEM((G, 8, 128), F32),
        pltpu.VMEM((128, 128), F32),
        blk(HL, F32),
        blk(HL, F32),
        blk(HL, F32),
        blk(HL, F32),
        blk(HL + HALO, F32),
        blk(HL + HALO, F32),
        pltpu.VMEM((2, 2, G, HALO, 128), F32),
        pltpu.VMEM((W, HL, 128), F32),
        pltpu.VMEM((W, HL, 128), F32),
        packed(HL),
        packed(HL),
        pltpu.SemaphoreType.DMA((15,)),
    ]
    out = pl.pallas_call(
        _kernel,
        in_specs=[any_spec, any_spec, any_spec, any_spec, any_spec,
                  pl.BlockSpec(memory_space=pltpu.VMEM), any_spec, any_spec],
        out_specs=any_spec,
        out_shape=jax.ShapeDtypeStruct((S, D), BF),
        scratch_shapes=scratch,
        compiler_params=pltpu.CompilerParams(vmem_limit_bytes=100 * 1024 * 1024),
    )(x, A_wq, A_wk, A_wv, A_wo, A_beta, B_wqkv, B_wo)
    return out.reshape(1, S, D)
```

```python
import math

import jax
import jax.numpy as jnp
from jax import lax
import jax.experimental.pallas as pl
import jax.experimental.pallas.tpu as pltpu

S, D, H, DH = 2048, 1024, 32, 32
L, NSEG, G = 512, 4, 8
HL = L // 2
W, DIL = 8, 2
HALO = 16
BF, F32, U32 = jnp.bfloat16, jnp.float32, jnp.uint32
QSCALE = (DH ** -0.5) * math.log2(math.e)
NEG = -1e30
NT = (((1,), (1,)), ((), ()))
OFF = (0, 128, 384, 768)
SCOPES = False
NCH_LN_A, NCH_LN_OUT, NCH_LN_B, NCH_NEXT = 1, 3, 2, 2
NCH_B0, NCH_B1 = 1, 2
KSPLIT = 7
SM_SUB = 32
PITCH = 33


class _scope:
    def __init__(self, name):
        self.cm = jax.named_scope(name) if SCOPES else None

    def __enter__(self):
        if self.cm is not None:
            self.cm.__enter__()

    def __exit__(self, *a):
        if self.cm is not None:
            self.cm.__exit__(*a)


def _dot(a, b):
    return jnp.dot(a, b, preferred_element_type=F32)


def _dot_nt(a, b):
    return lax.dot_general(a, b, NT, preferred_element_type=F32)


def _rows(r0, n, align=16):
    return slice(r0, r0 + n) if isinstance(r0, int) else pl.ds(pl.multiple_of(r0, align), n)


def _ldu(ref, b, r0, n):
    idx = slice(r0 // 2, (r0 + n) // 2) if isinstance(r0, int) else pl.ds(pl.multiple_of(r0 // 2, 8), n // 2)
    return ref.bitcast(U32)[b, idx, :]


def _ld(ref, b, r0, n):
    return pltpu.bitcast(_ldu(ref, b, r0, n), BF)


def _st(ref, b, r0, val):
    ref[b, _rows(r0, val.shape[0]), :] = val


def _wide(ref, r0, n):
    return jnp.concatenate([_ld(ref, b, r0, n) for b in range(G)], axis=1)


class _Chain:
    def __init__(self, never, n=1):
        self.never, self.n, self.hist = never, n, []

    def link(self, x):
        if self.never is None or len(self.hist) < self.n:
            return x
        return jnp.where(self.never, self.hist[-self.n], x)

    def link_first(self, x):
        head = self.link(x[0:8, 0:128])
        if x.shape[1] > 128:
            head = jnp.concatenate([head, x[0:8, 128:]], axis=1)
        return head if x.shape[0] == 8 else jnp.concatenate([head, x[8:]], axis=0)

    def done(self, v):
        self.hist.append(v[0:8, v.shape[1] - 128:])


def _phi(t):
    return jnp.where(t > 0, t + 1.0, jnp.exp(t))


def _ln(x):
    d = x - jnp.mean(x, axis=-1, keepdims=True)
    v = jnp.mean(d * d, axis=-1, keepdims=True)
    return d * lax.rsqrt(v + 1e-5)


def _ln_items(x_ref, xn_ref, row0, nrows, dst0, ch, chunk=16):
    def item(r0):
        def run():
            yf = _ln(ch.link_first(x_ref[r0:r0 + chunk, :]))
            y = yf.astype(BF)
            for b in range(G):
                _st(xn_ref, b, r0 - row0 + dst0, y[:, b * 128:(b + 1) * 128])
            ch.done(yf)
        return run
    return [item(r0) for r0 in range(row0, row0 + nrows, chunk)]


def _interleave(main, side, span=None):
    span = len(main) if span is None else span
    done = 0
    for i, it in enumerate(main):
        upto = len(side) if i + 1 >= span else (len(side) * (i + 1)) // span
        for s_it in side[done:upto]:
            s_it()
        done = max(done, upto)
        it()


def _run(items):
    for it in items:
        it()


def _shuffle_rows(tf, tmp, store):
    for h in range(H):
        tmp[h * PITCH:h * PITCH + DH, :] = tf[h * DH:(h + 1) * DH]
    for d in range(DH):
        for th in range(2):
            rows = tmp[pl.ds(th * 16 * PITCH + d, 16, stride=PITCH), :]
            store(d * H + th * 16, rows.astype(BF))


def _qk_stage(g, q_ref, k_ref, s_ref, m_ref, bias_ref):
    lane = lax.broadcasted_iota(jnp.int32, (64, 128), 1)
    for j in range(4):
        nk = 128 * (j + 1)
        qt = _ldu(q_ref, g, j * 128, 128)
        wq = jnp.concatenate([jnp.where((lane >> 5) == h, qt, jnp.uint32(0)) for h in range(4)], axis=0)
        st = _dot_nt(_ld(k_ref, g, 0, nk), pltpu.bitcast(wq, BF))
        bias = bias_ref[...]
        diag = st[j * 128:] + jnp.concatenate([bias] * 4, axis=1)
        s_ref[OFF[j] + j * 128:OFF[j] + nk, :] = diag
        m = jnp.max(diag.reshape(16, 8, 512), axis=0)
        if j > 0:
            s_ref[OFF[j]:OFF[j] + j * 128, :] = st[:j * 128]
            m = jnp.maximum(m, jnp.max(st[:j * 128].reshape(16 * j, 8, 512), axis=0))
        m_ref[j] = jnp.broadcast_to(jnp.max(m, axis=0, keepdims=True), (8, 512))


def _sm_stage(s_ref, m_ref, p_ref, l_ref, after=None):
    for j in range(4):
        nk = 128 * (j + 1)
        sums = []
        for h in range(4):
            m = m_ref[j, :, h * 128:(h + 1) * 128]
            if after is not None:
                m = after.link(m)
            l = None
            for r in range(0, nk, SM_SUB):
                s = s_ref[OFF[j] + r:OFF[j] + r + SM_SUB, h * 128:(h + 1) * 128]
                p = jnp.exp2(s.reshape(SM_SUB // 8, 8, 128) - m[None])
                ls = jnp.sum(p, axis=0)
                l = ls if l is None else l + ls
                _st(p_ref, h, OFF[j] + r, p.reshape(SM_SUB, 128).astype(BF))
            sums.append(jnp.sum(l, axis=0, keepdims=True))
        l_ref[j] = jnp.concatenate(sums + sums, axis=0)


def _pv_stage(g, p_ref, l_ref, vt_ref, ot_ref, pq_ref, mt_ref, gate_ref):
    mem = mt_ref[g].astype(BF)
    gate = gate_ref[g]
    for j in range(4):
        nd = _dot_nt(mem, _ld(pq_ref, g, j * 128, 128))
        c_mem = gate / (nd[128:136] + 1e-6)
        c_att = (1.0 - gate) / l_ref[j]
        for h in range(4):
            r0 = (g * 4 + h) * DH
            vt = jnp.concatenate([_ld(vt_ref, t, r0, DH) for t in range(j + 1)], axis=1)
            acc = _dot(vt, _ld(p_ref, h, OFF[j], 128 * (j + 1)))
            res = nd[h * DH:(h + 1) * DH] * c_mem[h:h + 1] + acc * c_att[h:h + 1]
            _st(ot_ref, j, r0, res.astype(BF))


def _mem_update(g, vt_ref, pk_ref, mt_ref, ch=None):
    row = lax.broadcasted_iota(jnp.int32, (144, 128), 0)
    lane = lax.broadcasted_iota(jnp.int32, (144, 128), 1)
    keep = jnp.where(row < 128, row >> 5, row - 128) == (lane >> 5)
    row16 = lax.broadcasted_iota(jnp.int32, (16, 128), 0)
    ones = jnp.where(row16 < 4, 1.0, 0.0).astype(BF)
    upd = None
    for t in range(4):
        lhs = jnp.concatenate([_ld(vt_ref, t, g * 128, 128), ones], axis=0)
        u = _dot(lhs, _ld(pk_ref, g, t * 128, 128))
        upd = u if upd is None else upd + u
    new = mt_ref[g] + jnp.where(keep, upd, 0.0)
    mt_ref[g] = new
    if ch is not None:
        ch.done(new)


def _band_items(pos0, row0, q_ref, k_ref, v_ref, a_ref, e_ref, o_ref, ch, nrows=HL):
    def logits(r0):
        def run():
            q = [q_ref[b, r0:r0 + 8, :] for b in range(G)]
            for w in range(W):
                base = HALO + r0 - DIL * w
                acc = ch.link(q[0] * k_ref[0, base:base + 8, :])
                for b in range(1, G):
                    acc = acc + q[b] * k_ref[b, base:base + 8, :]
                a_ref[w, r0 - row0:r0 - row0 + 8, :] = acc
                ch.done(acc)
        return run

    def softmax(r0):
        def run():
            lg = []
            for w in range(W):
                t = a_ref[w, r0 - row0:r0 - row0 + 128, :].T
                t = ((t[0:32] + t[32:64]) + (t[64:96] + t[96:128])) * QSCALE
                if r0 == row0 and w > 0:
                    pos = pos0 - DIL * w + lax.broadcasted_iota(jnp.int32, (H, 128), 1)
                    t = jnp.where(pos >= 0, t, NEG)
                lg.append(t)
            m = lg[0]
            for w in range(1, W):
                m = jnp.maximum(m, lg[w])
            e = [jnp.exp2(x - m) for x in lg]
            l = e[0]
            for w in range(1, W):
                l = l + e[w]
            inv = 1.0 / l
            for w in range(W):
                p = e[w] * inv
                pt = jnp.concatenate([p, p, p, p], axis=0).T
                e_ref[w, r0 - row0:r0 - row0 + 128, :] = pt
        return run

    def pv(r0):
        e = [e_ref[w, r0 - row0:r0 - row0 + 8, :] for w in range(W)]
        outs = []
        for b in range(G):
            acc = ch.link(e[0] * v_ref[b, HALO + r0:HALO + r0 + 8, :])
            for w in range(1, W):
                base = HALO + r0 - DIL * w
                acc = acc + e[w] * v_ref[b, base:base + 8, :]
            outs.append(acc)
            ch.done(acc)
        return outs

    def pv16(r0):
        def run():
            lo = pv(r0)
            hi = pv(r0 + 8)
            for b in range(G):
                _st(o_ref, b, r0, jnp.concatenate([lo[b], hi[b]], axis=0).astype(BF))
        return run

    items = []
    for r0 in range(row0, row0 + nrows, 128):
        items += [logits(r) for r in range(r0, r0 + 128, 8)]
        items.append(softmax(r0))
        items += [pv16(r) for r in range(r0, r0 + 128, 16)]
    return items


def _kernel(x_hbm, wq_hbm, wk_hbm, wv_hbm, woa_hbm, beta_ref, wqkv_hbm, wob_hbm, out_hbm,
            xin, obuf, x_f, xn, xc, xnx, wq, wk, woa, wv, wqkv, wvt, wbt, wob, wobp, tmp_a, tmp_b, tmp_c, tmp_d,
            q_ref, pq_ref, k_ref, pk_ref, vt_ref, ot_ref, o_nat,
            s_a, s_b, m_a, m_b, p_a, p_b, l_a, l_b, mt_ref, gate_ref, bias_ref,
            qn, kn, vn, qo, ko, vo, halo, ab, eb, ob0, ob1, sems):

    def col_copies(src, dst, sem, c0=0, n=G):
        return [pltpu.make_async_copy(src.at[:, (c0 + i) * 128:(c0 + i + 1) * 128], dst.at[c0 + i], sem)
                for i in range(n)]

    cp_wq = [col_copies(wq_hbm, wq, sems.at[c], 2 * c, 2) for c in range(4)]
    cp_wk = col_copies(wk_hbm, wk, sems.at[4])
    cp_wv = [pltpu.make_async_copy(wv_hbm, wv, sems.at[5])]
    cp_wqkv = [[pltpu.make_async_copy(wqkv_hbm.at[:, part * D:(part + 1) * D], wqkv.at[part], sems.at[6 + part])]
               for part in range(3)]
    cp_wob = col_copies(wob_hbm, wob, sems.at[9])
    cp_woa = col_copies(woa_hbm, woa, sems.at[10])
    cp_x0 = [pltpu.make_async_copy(x_hbm.at[0:L], xin.at[0:L], sems.at[11])]
    cp_xr = [pltpu.make_async_copy(x_hbm.at[L:S], xin.at[L:S], sems.at[12])]

    def cp_out(seg, hf):
        return pltpu.make_async_copy(obuf.at[hf * HL:(hf + 1) * HL],
                                     out_hbm.at[pl.ds(pl.multiple_of(seg * L + hf * HL, HL), HL)], sems.at[13 + hf])

    def wait(cps):
        for c in cps:
            c.wait()

    def wcols(w_ref, c0):
        return jnp.concatenate([_ld(w_ref, c0, 0, D), _ld(w_ref, c0 + 1, 0, D)], axis=1)

    def q_item(src, n, d0, c):
        def run():
            y = _dot(_wide(src, 0, n), wcols(wq, 2 * c))
            for gg in range(2):
                yq = y[:, gg * 128:(gg + 1) * 128]
                _st(q_ref, 2 * c + gg, d0, (yq * QSCALE).astype(BF))
                _st(pq_ref, 2 * c + gg, d0, _phi(yq).astype(BF))
        return run

    def k_item(src, n, d0, c):
        def run():
            y = _dot(_wide(src, 0, n), wcols(wk, 2 * c))
            for gg in range(2):
                yk = y[:, gg * 128:(gg + 1) * 128]
                _st(k_ref, 2 * c + gg, d0, yk.astype(BF))
                _st(pk_ref, 2 * c + gg, d0, _phi(yk).astype(BF))
        return run

    def v_item(src, r0, tile0, f0):
        def run():
            y = _dot_nt(_wide(wvt, f0, 512), _wide(src, r0, HL))
            _st(vt_ref, tile0, f0, y[:, :128].astype(BF))
            _st(vt_ref, tile0 + 1, f0, y[:, 128:].astype(BF))
        return run

    def attn_prologue():
        _qk_stage(0, q_ref, k_ref, s_a, m_a, bias_ref)
        _qk_stage(1, q_ref, k_ref, s_b, m_b, bias_ref)
        _sm_stage(s_a, m_a, p_a, l_a)

    def blk(i):
        return pl.ds(pl.multiple_of(i * 128, 128), 128)

    def qkv_shuffle(part, kbk, tmp):
        tf = wqkv[part, blk(kbk), :].T.astype(F32)
        _shuffle_rows(tf, tmp, lambda r, val: _st(wbt, kbk, part * D + r, val))

    with _scope("first_proj"):
        for cps in [cp_x0] + cp_wq + [cp_wv, cp_wk] + cp_wqkv + [cp_wob, cp_woa, cp_xr]:
            for c in cps:
                c.start()
        b = beta_ref[...].astype(F32).reshape(1, H)
        gt = jax.nn.sigmoid(b)
        row = lax.broadcasted_iota(jnp.int32, (H, H), 0)
        lane = lax.broadcasted_iota(jnp.int32, (H, H), 1)
        col = jnp.sum(jnp.where(row == lane, jnp.broadcast_to(gt, (H, H)), 0.0), axis=1, keepdims=True)
        col = jnp.broadcast_to(col, (H, 128))
        for g in range(G):
            gate_ref[g] = jnp.concatenate([col[4 * g:4 * g + 4], col[4 * g:4 * g + 4]], axis=0)
        key = lax.broadcasted_iota(jnp.int32, (128, 128), 0)
        qry = lax.broadcasted_iota(jnp.int32, (128, 128), 1)
        bias_ref[...] = jnp.where(key <= qry, 0.0, NEG)
        halo[...] = jnp.zeros(halo.shape, F32)

        def zero_b(b, c):
            for r in (qn, kn, vn, ko, vo):
                r[b] = jnp.zeros(r.shape[1:], F32)
            return c
        lax.fori_loop(0, G, zero_b, 0)

        def zero_mem(i, c):
            mt_ref[i // G, i % G] = jnp.zeros((144, 128), F32)
            return c
        lax.fori_loop(0, 2 * G, zero_mem, 0)
        with _scope("p_wait_x"):
            wait(cp_x0)

        def ln0(i, c):
            for u in range(16):
                r0 = pl.multiple_of(i * HL + u * 16, 16)
                x = xin[pl.ds(r0, 16), :].astype(F32)
                x_f[pl.ds(r0, 16), :] = x
                y = _ln(x).astype(BF)
                for b in range(G):
                    _st(xn, b, r0, y[:, b * 128:(b + 1) * 128])
            return c
        with _scope("p_ln"):
            lax.fori_loop(0, 2, ln0, 0)

        def q0(c, carry):
            for i in range(2):
                pltpu.make_async_copy(wq_hbm.at[:, 0:128], wq.at[0], sems.at[c]).wait()
            q_item(xn, L, 0, c)()
            return carry
        with _scope("p_q"):
            lax.fori_loop(0, 3, q0, 0)
        wait(cp_wq[3])
        wait(cp_wv)
        with _scope("p_tr"):
            q_item(xn, L, 0, 3)()
            for kbk in range(G):
                _st(wvt, kbk, 0, wv[kbk * 128:(kbk + 1) * 128, :].T)

        def v0(i, carry):
            hf = i // 2
            v_item(xn, hf * HL, 2 * hf, (i % 2) * 512)()
            return carry
        with _scope("p_v"):
            lax.fori_loop(0, 4, v0, 0)
        wait(cp_wk)
        wait(cp_wqkv[0])
        tmps = (tmp_a, tmp_b, tmp_c, tmp_d)

        def k0(c, carry):
            k_item(xn, L, 0, c)()
            for u in range(2):
                qkv_shuffle(0, 2 * c + u, tmps[u])
            return carry
        with _scope("p_k"):
            lax.fori_loop(0, 4, k0, 0)
        wait(cp_wqkv[1])
        wait(cp_wqkv[2])
        with _scope("p_attn"):
            attn_prologue()
            for u in range(2 * G):
                qkv_shuffle(1 + u // G, u % G, tmps[u % 4])
        wait(cp_wob)

        def sh1(i, carry):
            for u in range(4):
                cb = 4 * i + u
                _shuffle_rows(wob[cb].astype(F32), tmps[u], lambda r, val, cb=cb: _st(wobp, cb, r, val))
            return carry
        with _scope("p_sh1"):
            lax.fori_loop(0, 2, sh1, 0)
        wait(cp_woa)

    def out_item(src, s0, r0, w_ref, c, b0=0, b1=G, n=HL):
        def run():
            lhs = jnp.concatenate([_ld(src, b, s0, n) for b in range(b0, b1)], axis=1)
            w = jnp.concatenate([_ld(w_ref, 2 * c + i, b0 * 128, (b1 - b0) * 128) for i in range(2)], axis=1)
            x_f[r0:r0 + n, c * 256:(c + 1) * 256] += _dot(lhs, w)
        return run

    def b_proj_items():
        def item(part, c):
            def run():
                y = _dot_nt(_wide(xc, 0, HL), _wide(wbt, part * D + c * 256, 256))
                dst = (qn, kn, vn)[part]
                dst[2 * c] = y[:, :128]
                dst[2 * c + 1] = y[:, 128:]
            return run
        return [item(part, c) for part in range(3) for c in range(4)]

    def b_rotate():
        for b in range(G):
            qo[b] = qn[b]
            for new, old in ((kn, ko), (vn, vo)):
                old[b, 0:HALO, :] = old[b, HL:HL + HALO, :]
                old[b, HALO:, :] = new[b]

    def next_x_items(seg, layer, ch, chunk=16):
        nxt = jnp.minimum(seg + 1, NSEG - 1) * L

        def item(r0):
            def run():
                cur = ch.link_first(x_f[r0:r0 + chunk, :])
                obuf[r0:r0 + chunk, :] = cur.astype(BF)
                new = xin[pl.ds(pl.multiple_of(nxt + r0, chunk), chunk), :].astype(F32)
                x = jnp.where(layer == 1, new, cur)
                x_f[r0:r0 + chunk, :] = x
                yf = _ln(x)
                y = yf.astype(BF)
                for b in range(G):
                    _st(xc, b, r0, y[:, b * 128:(b + 1) * 128])
                ch.done(yf)
            return run
        return [item(r0) for r0 in range(0, HL, chunk)]

    def step(t, carry):
        seg = t // 2
        layer = t % 2
        mt = mt_ref.at[layer]
        never = lax.broadcasted_iota(jnp.int32, (8, 128), 0) < -t
        pv0 = lambda g, p, l: _pv_stage(g, p, l, vt_ref, ot_ref, pq_ref, mt, gate_ref)

        def pv(g, p, l):
            pv0(g, p, l)
            _mem_update(g, vt_ref, pk_ref, mt)

        @pl.when(t > 0)
        def _():
            with _scope("A_proj"):
                def a_half(hf, c):
                    d0 = hf * HL
                    items = ([q_item(xc, HL, d0, c) for c in range(4)]
                             + [k_item(xc, HL, d0, c) for c in range(4)]
                             + [v_item(xc, 0, 2 * hf, f0) for f0 in (0, 512)])
                    _interleave(items, _ln_items(x_f, xnx, HL, HL, 0, _Chain(never, NCH_LN_A)), span=8)
                    xc.bitcast(U32)[...] = xnx.bitcast(U32)[...]
                    return c

                lax.fori_loop(0, 2, a_half, 0)
            with _scope("A_attn_pro"):
                attn_prologue()

        def pair(u, c):
            g = 2 * u + 1
            _qk_stage(g + 1, q_ref, k_ref, s_a, m_a, bias_ref)
            _sm_stage(s_b, m_b, p_b, l_b)
            pv0(g - 1, p_a, l_a)
            ch = _Chain(never)
            _mem_update(g - 1, vt_ref, pk_ref, mt, ch)
            _qk_stage(g + 2, q_ref, k_ref, s_b, m_b, bias_ref)
            _sm_stage(s_a, m_a, p_a, l_a, after=ch)
            pv(g, p_b, l_b)
            return c

        with _scope("A_attn_loop"):
            lax.fori_loop(0, 3, pair, 0)

        @pl.when(t == 0)
        def _():
            wait(cp_xr)

        @pl.when(jnp.logical_and(layer == 0, seg > 0))
        def _():
            cp_out(seg - 1, 0).wait()
            cp_out(seg - 1, 1).wait()

        def transpose_o(b0, b1):
            for j in range(4):
                ot = _ld(ot_ref, j, b0 * 128, (b1 - b0) * 128).T
                for b in range(b0, b1):
                    _st(o_nat, b, j * 128, ot[:, (b - b0) * 128:(b - b0 + 1) * 128])

        with _scope("A_out"):
            transpose_o(0, G - 2)
            _sm_stage(s_b, m_b, p_b, l_b)
            ch_ln = _Chain(never, NCH_LN_OUT)
            u6, u7 = _Chain(None), _Chain(None)
            pv0(G - 2, p_a, l_a)
            _mem_update(G - 2, vt_ref, pk_ref, mt, u6)
            transpose_o(G - 2, KSPLIT)
            _run([out_item(o_nat, 0, 0, woa, c, 0, KSPLIT) for c in range(4)])
            pv0(G - 1, p_b, l_b)
            _mem_update(G - 1, vt_ref, pk_ref, mt, u7)
            transpose_o(KSPLIT, G)
            kn[:, HL - HALO:HL, :] = halo[layer, 0]
            vn[:, HL - HALO:HL, :] = halo[layer, 1]
            _run([out_item(o_nat, 0, 0, woa, c, KSPLIT, G) for c in range(4)])
            ch_ln.hist = [u6.hist[0]] + [u7.hist[0]] * (NCH_LN_OUT - 1)
            _run(_ln_items(x_f, xc, 0, HL, 0, ch_ln))
            _run([out_item(o_nat, HL, HL, woa, c) for c in range(4)])

        def b_half(hf, c):
            b_rotate()
            band = _band_items(seg * L + (hf - 1) * HL, 0, qo, ko, vo, ab, eb, ob0, _Chain(never, NCH_B0))
            ln = _ln_items(x_f, xnx, HL, HL, 0, _Chain(never, NCH_LN_B))
            _interleave(b_proj_items(), band + ln)
            xc.bitcast(U32)[...] = xnx.bitcast(U32)[...]
            return c

        with _scope("B_loop"):
            lax.fori_loop(0, 2, b_half, 0)

        with _scope("B_tail"):
            halo[layer, 0] = kn[:, HL - HALO:HL, :]
            halo[layer, 1] = vn[:, HL - HALO:HL, :]
            b_rotate()
            _run(_band_items(seg * L + HL, 0, qo, ko, vo, ab, eb, ob1, _Chain(never, NCH_B1)))
            _run([out_item(ob0, 0, 0, wobp, c) for c in range(4)])
            _run(next_x_items(seg, layer, _Chain(never, NCH_NEXT)))
            _run([out_item(ob1, 0, HL, wobp, c, n=128) for c in range(4)])
            _run([out_item(ob1, 128, HL + 128, wobp, c, n=128) for c in range(4)])

        @pl.when(layer == 1)
        def _():
            cp_out(seg, 0).start()
            obuf[HL:L, :] = x_f[HL:L, :].astype(BF)
            cp_out(seg, 1).start()

            @pl.when(seg < NSEG - 1)
            def _():
                x_f[HL:L, :] = xin[pl.ds(pl.multiple_of((seg + 1) * L + HL, HL), HL), :].astype(F32)

        return carry

    lax.fori_loop(0, 2 * NSEG, step, 0)
    cp_out(NSEG - 1, 0).wait()
    cp_out(NSEG - 1, 1).wait()


@jax.jit
def pallas_interleave_layers__memory_aug_infini_attn__sliding_local_dilated__prompt_kernel(
    A_x: jax.Array,
    A_wq: jax.Array,
    A_wk: jax.Array,
    A_wv: jax.Array,
    A_wo: jax.Array,
    A_beta: jax.Array,
    B_x: jax.Array,
    B_wqkv: jax.Array,
    B_wo: jax.Array,
):
    del B_x
    x = A_x.reshape(S, D)
    any_spec = pl.BlockSpec(memory_space=pl.ANY)
    blk = lambda rows, dt: pltpu.VMEM((G, rows, 128), dt)
    packed = lambda rows, n=G: pltpu.VMEM((n, rows, 128), BF)
    scratch = [
        pltpu.VMEM((S, D), BF),
        pltpu.VMEM((L, D), BF),
        pltpu.VMEM((L, D), F32),
        packed(L),
        packed(HL),
        packed(HL),
        blk(D, BF),
        blk(D, BF),
        blk(D, BF),
        pltpu.VMEM((D, D), BF),
        pltpu.VMEM((3, D, D), BF),
        packed(D),
        packed(3 * D),
        blk(D, BF),
        packed(D),
        pltpu.VMEM((H * PITCH, 128), F32),
        pltpu.VMEM((H * PITCH, 128), F32),
        pltpu.VMEM((H * PITCH, 128), F32),
        pltpu.VMEM((H * PITCH, 128), F32),
        packed(L),
        packed(L),
        packed(L),
        packed(L),
        packed(D, 4),
        packed(D, 4),
        packed(L),
        pltpu.VMEM((1280, 512), F32),
        pltpu.VMEM((1280, 512), F32),
        pltpu.VMEM((4, 8, 512), F32),
        pltpu.VMEM((4, 8, 512), F32),
        packed(1280, 4),
        packed(1280, 4),
        pltpu.VMEM((4, 8, 128), F32),
        pltpu.VMEM((4, 8, 128), F32),
        pltpu.VMEM((2, G, 144, 128), F32),
        pltpu.VMEM((G, 8, 128), F32),
        pltpu.VMEM((128, 128), F32),
        blk(HL, F32),
        blk(HL, F32),
        blk(HL, F32),
        blk(HL, F32),
        blk(HL + HALO, F32),
        blk(HL + HALO, F32),
        pltpu.VMEM((2, 2, G, HALO, 128), F32),
        pltpu.VMEM((W, HL, 128), F32),
        pltpu.VMEM((W, HL, 128), F32),
        packed(HL),
        packed(HL),
        pltpu.SemaphoreType.DMA((15,)),
    ]
    out = pl.pallas_call(
        _kernel,
        in_specs=[any_spec, any_spec, any_spec, any_spec, any_spec,
                  pl.BlockSpec(memory_space=pltpu.VMEM), any_spec, any_spec],
        out_specs=any_spec,
        out_shape=jax.ShapeDtypeStruct((S, D), BF),
        scratch_shapes=scratch,
        compiler_params=pltpu.CompilerParams(vmem_limit_bytes=100 * 1024 * 1024),
    )(x, A_wq, A_wk, A_wv, A_wo, A_beta, B_wqkv, B_wo)
    return out.reshape(1, S, D)
```
